```python
import jax
import jax.numpy as jnp

def _softmax(x, axis=-1):
    return jax.nn.softmax(x, axis=axis)
def _gelu(x):
    return jax.nn.gelu(x, approximate=True)
def _silu(x):
    return jax.nn.silu(x)
def _sigmoid(x):
    return jax.nn.sigmoid(x)
def _layernorm(x, axis=-1, eps=1e-5):
    m = jnp.mean(x, axis=axis, keepdims=True)
    v = jnp.var(x, axis=axis, keepdims=True)
    return (x - m) / jnp.sqrt(v + eps)
def _scatter_add(tgt, idx, src, axis=0):
    return tgt.at[idx].add(src)
def _segment_sum(src, seg, n):
    return jax.ops.segment_sum(src, seg, n)
class _Rng:
    def __init__(self, key):
        self._k = key
    def _next(self):
        self._k, sub = jax.random.split(self._k)
        return sub
    def normal(self, shape):
        return jax.random.normal(self._next(), shape, dtype=jnp.bfloat16)
    def randint(self, lo, hi, shape):
        return jax.random.randint(self._next(), shape, lo, hi, dtype=jnp.int32)
    def uniform(self, shape, lo=0.0, hi=1.0):
        return jax.random.uniform(self._next(), shape, jnp.bfloat16, lo, hi)
    def permutation(self, n):
        return jax.random.permutation(self._next(), n)


kernel_name = 'interleave_layers__linear_kernel_hedgehog__sliding_local_dilated__prompt'

def setup_inputs():
    _rng = _Rng(jax.random.key(int.from_bytes(__import__("os").urandom(4), "little")))
    _w = (lambda a: (lambda t: t.astype(jnp.bfloat16) if jnp.issubdtype(t.dtype, jnp.floating) else t)(jnp.asarray(a)))
    def _A_setup():
        B, S, D, H = 1, 2048, 1024, 32
        Dh = D // H
        return {
            "x": _w((lambda *s: _rng.normal(s) * 0.05)(B, S, D)),
            "wqkv": _w((lambda *s: _rng.normal(s) * 0.05)(D, 3 * D)),
            "w_phi": _w((lambda *s: _rng.normal(s) * 0.05)(H, Dh, Dh) * (Dh ** -0.5)),
            "wo": _w((lambda *s: _rng.normal(s) * 0.05)(D, D)),
        }
    _A_in = _A_setup()

    def _B_setup():
        B, S, D = 1, 2048, 1024
        return {
            "x": _w((lambda *s: _rng.normal(s) * 0.05)(B, S, D)),
            "wqkv": _w((lambda *s: _rng.normal(s) * 0.05)(D, 3 * D)),
            "wo": _w((lambda *s: _rng.normal(s) * 0.05)(D, D)),
        }
    _B_in = _B_setup()

    return {
        "A_x": _A_in["x"],
        "A_wqkv": _A_in["wqkv"],
        "A_w_phi": _A_in["w_phi"],
        "A_wo": _A_in["wo"],
        "B_x": _B_in["x"],
        "B_wqkv": _B_in["wqkv"],
        "B_wo": _B_in["wo"],
    }

def reference(A_x, A_wqkv, A_w_phi, A_wo, B_x, B_wqkv, B_wo):
    def _A_ref(x, wqkv, w_phi, wo):
        B, S, D = x.shape
        H = 32; Dh = D // H
        qkv = (lambda x, *d: x.transpose(*d))((x @ wqkv).reshape(B, S, 3, H, Dh), 2, 0, 3, 1, 4)
        q, k, v = qkv[0], qkv[1], qkv[2]
        pq = jnp.einsum("bhsd,hdf->bhsf", q, w_phi)
        pk = jnp.einsum("bhsd,hdf->bhsf", k, w_phi)
        phi_q = jnp.concatenate([_softmax(pq, axis=-1), _softmax(-pq, axis=-1)], axis=-1)
        phi_k = jnp.concatenate([_softmax(pk, axis=-1), _softmax(-pk, axis=-1)], axis=-1)
        kv = jnp.einsum("bhsf,bhsd->bhfd", phi_k, v)
        z  = jnp.einsum("bhsf->bhf", phi_k)
        num = jnp.einsum("bhqf,bhfd->bhqd", phi_q, kv)
        den = jnp.einsum("bhqf,bhf->bhq", phi_q, z)[..., None] + 1e-6
        o = num / den
        return (lambda x, *d: x.transpose(*d))(o, 0, 2, 1, 3).reshape(B, S, D) @ wo

    def _B_ref(x, wqkv, wo):
        B, S, D = x.shape
        H = 32; Dh = D // H
        W, dil = 8, 2
        qkv = (lambda x, *d: x.transpose(*d))((x @ wqkv).reshape(B, S, 3, H, Dh), 2, 0, 3, 1, 4)
        q, k, v = qkv[0], qkv[1], qkv[2]
        scale = Dh ** -0.5
        pos = jnp.arange(S)
        off = jnp.arange(W) * dil
        idx = pos[:, None] - off[None, :]
        mask = idx >= 0
        idx_c = jnp.where(mask, idx, 0).reshape(-1)
        kg = k[:, :, idx_c, :].reshape(B, H, S, W, Dh)
        vg = v[:, :, idx_c, :].reshape(B, H, S, W, Dh)
        logits = jnp.einsum("bhsd,bhswd->bhsw", q, kg) * scale
        logits = jnp.where(mask[None, None, :, :], logits, -1e9)
        attn = _softmax(logits, axis=-1)
        o = jnp.einsum("bhsw,bhswd->bhsd", attn, vg)
        return (lambda x, *d: x.transpose(*d))(o, 0, 2, 1, 3).reshape(B, S, D) @ wo

    x = A_x
    x = x + _A_ref(_layernorm(x, axis=-1), A_wqkv, A_w_phi, A_wo)
    x = x + _B_ref(_layernorm(x, axis=-1), B_wqkv, B_wo)
    x = x + _A_ref(_layernorm(x, axis=-1), A_wqkv, A_w_phi, A_wo)
    x = x + _B_ref(_layernorm(x, axis=-1), B_wqkv, B_wo)
    return x
```

```python
import math

import jax
import jax.numpy as jnp
from jax import lax
import jax.experimental.pallas as pl
import jax.experimental.pallas.tpu as pltpu

S = 2048
D = 1024
H = 32
DH = 32
NBLK = 16
L = 128
WIN = 8
HALO = WIN - 1
LOG2E = math.log2(math.e)
F32 = jnp.float32
BF16 = jnp.bfloat16
NT = (((1,), (1,)), ((), ()))

NB = 2


def _mm(a, b):
    return jnp.dot(a, b, preferred_element_type=F32)


def _mm_nt(a, b):
    return lax.dot_general(a, b, NT, preferred_element_type=F32)


def _tree(op, xs):
    xs = list(xs)
    while len(xs) > 1:
        nxt = [op(xs[i], xs[i + 1]) for i in range(0, len(xs) - 1, 2)]
        if len(xs) % 2:
            nxt.append(xs[-1])
        xs = nxt
    return xs[0]


def _rows(a, n=8):
    return [a[i * n:(i + 1) * n, :] for i in range(a.shape[0] // n)]


def _layernorm_t(xt):
    s = _tree(jnp.add, _rows(xt))
    m = jnp.sum(s, axis=0, keepdims=True) * (1.0 / D)
    xc = xt - m
    s2 = _tree(jnp.add, _rows(xc * xc))
    v = jnp.sum(s2, axis=0, keepdims=True) * (1.0 / D)
    return (xc * lax.rsqrt(v + 1e-5)).astype(BF16)


def _fold4(op, xs):
    r = _tree(op, xs)
    return op(r, pltpu.roll(r, 4, 0))


def _phi_parts(p):
    ps = _rows(p)
    mx = _fold4(jnp.maximum, ps)
    mn = _fold4(jnp.minimum, ps)
    ep = [jnp.exp2(x - mx) for x in ps]
    en = [jnp.exp2(mn - x) for x in ps]
    sp = _fold4(jnp.add, ep)
    sn = _fold4(jnp.add, en)
    return ep, en, sp, sn


def _kernel(x_hbm, wa_hbm, wphi_hbm, woa_hbm, wb_hbm, wob_hbm, out_hbm,
            xio, wa_raw, woa_raw, wb_raw, wob_raw, wphi,
            waT, woaT, wbT, wobT, xT, xn, kb, vb, kv_acc, kvm, zacc, zb, att, sems):
    T = NB * L
    NIT = NBLK // NB

    cp_x = [pltpu.make_async_copy(x_hbm.at[:, pl.ds(c * L, L)], xio.at[c], sems.at[8 + c]) for c in range(8)]
    cp_phi = pltpu.make_async_copy(wphi_hbm, wphi, sems.at[1])
    cp_wa = pltpu.make_async_copy(wa_hbm, wa_raw, sems.at[2])
    cp_woa = pltpu.make_async_copy(woa_hbm, woa_raw, sems.at[3])
    cp_wb = pltpu.make_async_copy(wb_hbm, wb_raw, sems.at[4])
    cp_wob = pltpu.make_async_copy(wob_hbm, wob_raw, sems.at[5])
    for c in cp_x + [cp_phi, cp_wa, cp_woa, cp_wb, cp_wob]:
        c.start()

    xio32 = xio.bitcast(jnp.uint32)

    def wload(ref, r0, n):
        return jnp.concatenate([ref[c, r0:r0 + n, :] for c in range(8)], axis=1)

    def wstore(ref, off, val):
        for c in range(8):
            ref[c, pl.ds(off, 128), :] = val[:, c * L:(c + 1) * L]

    for c in cp_x:
        c.wait()

    def quad(a):
        return xio32.at[:, pl.ds(pl.multiple_of(a * 4, 4), 1012), :]

    def prep_x(a, c):
        xq = quad(a)
        for b in range(4):
            blk = jnp.concatenate(
                [pltpu.bitcast(xq[cc, pl.ds(b, 64, stride=16), :], BF16) for cc in range(8)], axis=1)
            xt = blk.T.astype(F32)
            xT[a * 4 + b] = xt
            xn[a * 4 + b] = _layernorm_t(xt)
        return c
    lax.fori_loop(0, 4, prep_x, 0)

    r128 = lax.broadcasted_iota(jnp.int32, (128, 128), 0)
    c128 = lax.broadcasted_iota(jnp.int32, (128, 128), 1)
    same_head = (r128 % 4) == (c128 // 32)
    perm = jnp.where(jnp.logical_and(same_head, (r128 // 4) == (c128 % 32)), 1.0, 0.0).astype(BF16)
    er = lax.broadcasted_iota(jnp.int32, (128, 32), 0)
    ec = lax.broadcasted_iota(jnp.int32, (128, 32), 1)
    expand = jnp.where((er // 4) == ec, 1.0, 0.0).astype(BF16)

    cp_phi.wait()
    cp_wa.wait()

    def prep_a(g, c):
        off = pl.multiple_of(g * 128, 128)
        pg = _mm_nt(expand, wphi[pl.ds(off, 128), :])
        pg = jnp.where(same_head, pg, 0.0).astype(BF16)
        wstore(waT, off, (_mm_nt(pg, wa_raw[:, pl.ds(off, 128)]) * LOG2E).astype(BF16))
        off2 = pl.multiple_of(D + g * 128, 128)
        wstore(waT, off2, (_mm_nt(pg, wa_raw[:, pl.ds(off2, 128)]) * LOG2E).astype(BF16))
        off3 = pl.multiple_of(2 * D + g * 128, 128)
        wstore(waT, off3, wa_raw[:, pl.ds(off3, 128)].T)
        return c
    lax.fori_loop(0, 8, prep_a, 0)

    cp_woa.wait()
    cp_wb.wait()
    cp_wob.wait()

    def prep_b(g, c):
        off = pl.multiple_of(g * 128, 128)
        wstore(wbT, off, _mm_nt(perm, wb_raw[:, pl.ds(off, 128)]).astype(BF16))
        off2 = pl.multiple_of(D + g * 128, 128)
        wstore(wbT, off2, _mm_nt(perm, wb_raw[:, pl.ds(off2, 128)]).astype(BF16))
        off3 = pl.multiple_of(2 * D + g * 128, 128)
        wstore(wbT, off3, wb_raw[:, pl.ds(off3, 128)].T)
        wstore(woaT, off, woa_raw[:, pl.ds(off, 128)].T)
        wstore(wobT, off, wob_raw[:, pl.ds(off, 128)].T)
        return c
    lax.fori_loop(0, 8, prep_b, 0)

    def load_blocks(ref, j0):
        return jnp.concatenate([ref[j0 + b] for b in range(NB)], axis=1)

    def store_blocks(ref, j0, val):
        for b in range(NB):
            ref[j0 + b] = val[:, b * L:(b + 1) * L]

    def a_kv(xnt):
        kvp = _mm(wload(waT, D, 2 * D), xnt)
        for g in range(8):
            ep, en, sp, sn = _phi_parts(kvp[g * 128:(g + 1) * 128, :])
            rp = 1.0 / sp
            rn = 1.0 / sn
            phi = jnp.concatenate([e * rp for e in ep] + [e * rn for e in en], axis=0)
            zs = _tree(jnp.add, [phi[:, b * L:(b + 1) * L] for b in range(NB)])
            zacc[g * 256:(g + 1) * 256, :] += zs
            vg = kvp[D + g * 128:D + (g + 1) * 128, :].astype(BF16)
            kv_acc[g] += _mm_nt(vg, phi.astype(BF16))

    def a_init():
        kv_acc[...] = jnp.zeros(kv_acc.shape, F32)
        zacc[...] = jnp.zeros(zacc.shape, F32)

    def a_finish():
        r = lax.broadcasted_iota(jnp.int32, (128, 256), 0)
        c = lax.broadcasted_iota(jnp.int32, (128, 256), 1)
        keep = (r // 32) == (c % 4)
        for g in range(8):
            kvm[g] = jnp.where(keep, kv_acc[g], 0.0).astype(BF16)
        zb[...] = jnp.broadcast_to(jnp.sum(zacc[...], axis=1, keepdims=True), zb.shape)

    def a_q(xnt):
        qp = _mm(wload(waT, 0, D), xnt)
        outs = []
        for g in range(8):
            ep, en, sp, sn = _phi_parts(qp[g * 128:(g + 1) * 128, :])
            z = zb[g * 256:(g + 1) * 256, :]
            z = jnp.concatenate([z] * NB, axis=1)
            zr = _rows(z)
            dp = _fold4(jnp.add, [e * zz for e, zz in zip(ep, zr[:16])])
            dn = _fold4(jnp.add, [e * zz for e, zz in zip(en, zr[16:])])
            rp = 1.0 / sp
            rn = 1.0 / sn
            rden = 1.0 / (dp * rp + dn * rn + 1e-6)
            rp = rp * rden
            rn = rn * rden
            phi = jnp.concatenate([e * rp for e in ep] + [e * rn for e in en], axis=0)
            outs.append(_mm(kvm[g], phi.astype(BF16)).astype(BF16))
        return jnp.concatenate(outs, axis=0)

    def b_kv(xnt, j0):
        kvp = _mm(wload(wbT, D, 2 * D), xnt)
        for b in range(NB):
            j = j0 + b
            kk = kvp[0:D, b * L:(b + 1) * L]
            vv = kvp[D:2 * D, b * L:(b + 1) * L]
            kb[HALO + j] = kk
            vb[HALO + j] = vv
            slot = jnp.where(j >= NBLK - HALO, j - (NBLK - HALO), HALO + NBLK)
            kb[slot] = pltpu.roll(kk, 2, 1)
            vb[slot] = pltpu.roll(vv, 2, 1)

    def b_q(xnt, j0):
        qp = _mm(wload(wbT, 0, D), xnt)
        lo = lax.broadcasted_iota(jnp.int32, (8, L), 0) < 4
        first = lax.broadcasted_iota(jnp.int32, (8, L), 1) < 2
        cs = DH ** -0.5
        outs = []
        for b in range(NB):
            j = j0 + b
            q = qp[:, b * L:(b + 1) * L]
            for G in range(4):
                lg = []
                for w in range(WIN):
                    halves = []
                    for g in (2 * G, 2 * G + 1):
                        kk = kb[HALO + j - w, g * 128:(g + 1) * 128, :]
                        halves.append(_tree(jnp.add, _rows(q[g * 128:(g + 1) * 128, :] * kk)))
                    la, lb = halves
                    l = jnp.where(lo, la, lb) + pltpu.roll(jnp.where(lo, lb, la), 4, 0)
                    l = l * cs
                    if w > 0:
                        l = jnp.where(jnp.logical_and(first, j < w), -1e9, l)
                    lg.append(l)
                mx = _tree(jnp.maximum, lg)
                ex = [jnp.exp(l - mx) for l in lg]
                r = 1.0 / _tree(jnp.add, ex)
                for w in range(WIN):
                    att[b, w, G * 8:(G + 1) * 8, :] = ex[w] * r
            oh = []
            for h in range(H):
                terms = []
                for w in range(WIN):
                    a = att[b, w, h:h + 1, :]
                    terms.append(a * vb[HALO + j - w, h * DH:(h + 1) * DH, :])
                oh.append(_tree(jnp.add, terms).astype(BF16))
            outs.append(jnp.concatenate(oh, axis=0))
        return jnp.concatenate(outs, axis=1)

    a_init()

    def s1(i, c):
        a_kv(load_blocks(xn, i * NB))
        return c
    lax.fori_loop(0, NIT, s1, 0)

    def s2(i, c):
        j0 = i * NB
        o = a_q(load_blocks(xn, j0))
        xt = load_blocks(xT, j0) + _mm(wload(woaT, 0, D), o)
        store_blocks(xT, j0, xt)
        xnt = _layernorm_t(xt)
        store_blocks(xn, j0, xnt)
        b_kv(xnt, j0)
        return c

    def s3(i, c):
        j0 = i * NB
        o = b_q(load_blocks(xn, j0), j0)
        xt = load_blocks(xT, j0) + _mm(wload(wobT, 0, D), o)
        store_blocks(xT, j0, xt)
        xnt = _layernorm_t(xt)
        store_blocks(xn, j0, xnt)
        a_kv(xnt)
        return c

    def s5(a, c):
        xq = quad(a)
        for u in range(4 // NB):
            j0 = a * 4 + u * NB
            o = b_q(load_blocks(xn, j0), j0)
            xt = load_blocks(xT, j0) + _mm(wload(wobT, 0, D), o)
            for b in range(NB):
                y = xt[:, b * L:(b + 1) * L].astype(BF16).T
                y = pltpu.bitcast(y, jnp.uint32)
                for cc in range(8):
                    xq[cc, pl.ds(u * NB + b, 64, stride=16), :] = y[:, cc * L:(cc + 1) * L]
        return c

    a_finish()
    lax.fori_loop(0, NIT, s2, 0)
    a_init()
    lax.fori_loop(0, NIT, s3, 0)
    a_finish()
    lax.fori_loop(0, NIT, s2, 0)
    lax.fori_loop(0, 4, s5, 0)

    cp_out = [pltpu.make_async_copy(xio.at[c], out_hbm.at[:, pl.ds(c * L, L)], sems.at[8 + c]) for c in range(8)]
    for c in cp_out:
        c.start()
    for c in cp_out:
        c.wait()


@jax.jit
def pallas_interleave_layers__linear_kernel_hedgehog__sliding_local_dilated__prompt_kernel(
    A_x: jax.Array,
    A_wqkv: jax.Array,
    A_w_phi: jax.Array,
    A_wo: jax.Array,
    B_x: jax.Array,
    B_wqkv: jax.Array,
    B_wo: jax.Array,
):
    del B_x
    x2 = A_x.reshape(S, D)
    wphi2 = A_w_phi.reshape(H * DH, DH)
    any_spec = pl.BlockSpec(memory_space=pl.ANY)
    scratch = [
        pltpu.VMEM((8, S, L), BF16),
        pltpu.VMEM((D, 3 * D), BF16),
        pltpu.VMEM((D, D), BF16),
        pltpu.VMEM((D, 3 * D), BF16),
        pltpu.VMEM((D, D), BF16),
        pltpu.VMEM((H * DH, DH), BF16),
        pltpu.VMEM((8, 3 * D, L), BF16),
        pltpu.VMEM((8, D, L), BF16),
        pltpu.VMEM((8, 3 * D, L), BF16),
        pltpu.VMEM((8, D, L), BF16),
        pltpu.VMEM((NBLK, D, L), F32),
        pltpu.VMEM((NBLK, D, L), BF16),
        pltpu.VMEM((HALO + NBLK + 1, D, L), F32),
        pltpu.VMEM((HALO + NBLK + 1, D, L), F32),
        pltpu.VMEM((8, 128, 256), F32),
        pltpu.VMEM((8, 128, 256), BF16),
        pltpu.VMEM((2 * D, L), F32),
        pltpu.VMEM((2 * D, L), F32),
        pltpu.VMEM((NB, WIN, H, L), F32),
        pltpu.SemaphoreType.DMA((16,)),
    ]
    out = pl.pallas_call(
        _kernel,
        out_shape=jax.ShapeDtypeStruct((S, D), BF16),
        in_specs=[any_spec] * 6,
        out_specs=any_spec,
        scratch_shapes=scratch,
        compiler_params=pltpu.CompilerParams(vmem_limit_bytes=120 * 1024 * 1024),
        name="hedgehog_dilated",
    )(x2, A_wqkv, wphi2, A_wo, B_wqkv, B_wo)
    return out.reshape(1, S, D)
```

```python
import math

import jax
import jax.numpy as jnp
from jax import lax
import jax.experimental.pallas as pl
import jax.experimental.pallas.tpu as pltpu

S = 2048
D = 1024
H = 32
DH = 32
NBLK = 16
L = 128
WIN = 8
HALO = WIN - 1
LOG2E = math.log2(math.e)
F32 = jnp.float32
BF16 = jnp.bfloat16
U32 = jnp.uint32
NT = (((1,), (1,)), ((), ()))

NB = 2
MC = 256
LAG_Q = 1
LAG_KV = 2


def _mm(a, b):
    return jnp.dot(a, b, preferred_element_type=F32)


def _mm_nt(a, b):
    return lax.dot_general(a, b, NT, preferred_element_type=F32)


def _tree(op, xs):
    xs = list(xs)
    while len(xs) > 1:
        nxt = [op(xs[i], xs[i + 1]) for i in range(0, len(xs) - 1, 2)]
        if len(xs) % 2:
            nxt.append(xs[-1])
        xs = nxt
    return xs[0]


def _chain(op, xs, ways=4):
    acc = list(xs[:ways])
    for i, x in enumerate(xs[ways:]):
        acc[i % ways] = op(acc[i % ways], x)
    return _tree(op, acc)


def _rows(a, n=8):
    return [a[i * n:(i + 1) * n, :] for i in range(a.shape[0] // n)]


def _pack(a):
    return pltpu.bitcast(a.astype(BF16), U32)


def _unpk(a):
    return pltpu.bitcast(a, BF16)


def _fold4(op, xs):
    r = _tree(op, xs)
    return op(r, pltpu.roll(r, 4, 0))


def _phi_parts(p):
    ps = _rows(p)
    mx = _fold4(jnp.maximum, ps)
    mn = _fold4(jnp.minimum, ps)
    ep = [jnp.exp2(x - mx) for x in ps]
    en = [jnp.exp2(mn - x) for x in ps]
    sp = _fold4(jnp.add, ep)
    sn = _fold4(jnp.add, en)
    return ep, en, sp, sn


def _kernel(x_hbm, wa_hbm, wphi_hbm, woa_hbm, wb_hbm, wob_hbm, out_hbm,
            xio, wa_raw, woa_raw, wb_raw, wob_raw, wphi,
            waT, woaT, wbT, wobT, xT, xn, kb, vb, kv_acc, kvm, zacc, zb, sems):
    NIT = NBLK // NB

    cp_x = [pltpu.make_async_copy(x_hbm.at[:, pl.ds(c * L, L)], xio.at[c], sems.at[8 + c]) for c in range(8)]
    cp_phi = pltpu.make_async_copy(wphi_hbm, wphi, sems.at[1])
    cp_wa = pltpu.make_async_copy(wa_hbm, wa_raw, sems.at[2])
    cp_woa = pltpu.make_async_copy(woa_hbm, woa_raw, sems.at[3])
    cp_wb = pltpu.make_async_copy(wb_hbm, wb_raw, sems.at[4])
    cp_wob = pltpu.make_async_copy(wob_hbm, wob_raw, sems.at[5])
    for c in cp_x + [cp_phi, cp_wa, cp_woa, cp_wb, cp_wob]:
        c.start()

    xio32 = xio.bitcast(U32)

    def wload(ref, r0, n):
        return jnp.concatenate([_unpk(ref[c, r0 // 2:(r0 + n) // 2, :]) for c in range(8)], axis=1)

    def wstore(ref, g, val):
        off = pl.multiple_of(g * 64, 64)
        for c in range(8):
            ref[c, pl.ds(off, 64), :] = _pack(val[:, c * L:(c + 1) * L])

    class LN:
        def __init__(self, j):
            self.j = j
            self.piv = None
            self.s1 = []
            self.s2 = []

        def add(self, xt):
            if self.piv is None:
                self.piv = jnp.broadcast_to(xt[0:1, :], (8, L))
            d = [r - self.piv for r in _rows(xt)]
            self.s1.append(_chain(jnp.add, d, 2))
            self.s2.append(_chain(jnp.add, [x * x for x in d], 2))

        def finish(self):
            j = self.j
            m1 = jnp.sum(_tree(jnp.add, self.s1), axis=0, keepdims=True) * (1.0 / D)
            m2 = jnp.sum(_tree(jnp.add, self.s2), axis=0, keepdims=True) * (1.0 / D)
            var = jnp.maximum(m2 - m1 * m1, 0.0)
            mean = jnp.broadcast_to(self.piv[0:1, :] + m1, (16, L))
            rs = jnp.broadcast_to(lax.rsqrt(var + 1e-5), (16, L))
            for r in range(D // 16):
                xn[j, r * 8:(r + 1) * 8, :] = _pack((xT[j, r * 16:(r + 1) * 16, :] - mean) * rs)

    for c in cp_x:
        c.wait()

    def quad(a):
        return xio32.at[:, pl.ds(pl.multiple_of(a * 4, 4), 1012), :]

    def prep_x(a, c):
        xq = quad(a)
        for b in range(4):
            j = a * 4 + b
            ln = LN(j)
            for cc in range(8):
                xt = _unpk(xq[cc, pl.ds(b, 64, stride=16), :]).T.astype(F32)
                xT[j, cc * 128:(cc + 1) * 128, :] = xt
                ln.add(xt)
            ln.finish()
        return c
    lax.fori_loop(0, 4, prep_x, 0)

    r128 = lax.broadcasted_iota(jnp.int32, (128, 128), 0)
    c128 = lax.broadcasted_iota(jnp.int32, (128, 128), 1)
    same_head = (r128 % 4) == (c128 // 32)
    perm = jnp.where(jnp.logical_and(same_head, (r128 // 4) == (c128 % 32)), 1.0, 0.0).astype(BF16)
    er = lax.broadcasted_iota(jnp.int32, (128, 32), 0)
    ec = lax.broadcasted_iota(jnp.int32, (128, 32), 1)
    expand = jnp.where((er // 4) == ec, 1.0, 0.0).astype(BF16)

    def cols(ref, g):
        return ref[:, pl.ds(pl.multiple_of(g * 128, 128), 128)]

    cp_phi.wait()
    cp_wa.wait()

    def prep_a(g, c):
        pg = _mm_nt(expand, wphi[pl.ds(pl.multiple_of(g * 128, 128), 128), :])
        pg = jnp.where(same_head, pg, 0.0).astype(BF16)
        wstore(waT, g, _mm_nt(pg, cols(wa_raw, g)) * LOG2E)
        wstore(waT, 8 + g, _mm_nt(pg, cols(wa_raw, 8 + g)) * LOG2E)
        wstore(waT, 16 + g, cols(wa_raw, 16 + g).T)
        return c
    lax.fori_loop(0, 8, prep_a, 0)

    cp_woa.wait()
    cp_wb.wait()
    cp_wob.wait()

    def prep_b(g, c):
        wstore(wbT, g, _mm_nt(perm, cols(wb_raw, g)))
        wstore(wbT, 8 + g, _mm_nt(perm, cols(wb_raw, 8 + g)))
        wstore(wbT, 16 + g, cols(wb_raw, 16 + g).T)
        wstore(woaT, g, cols(woa_raw, g).T)
        wstore(wobT, g, cols(wob_raw, g).T)
        return c
    lax.fori_loop(0, 8, prep_b, 0)

    def proj(ref, r0, n, j):
        return _mm(wload(ref, r0, n), _unpk(xn[j]))

    NCH = D // MC
    GPC = MC // 128

    def emit(steps, lag):
        pend = []
        for main, late in steps:
            main()
            pend.append(late)
            if len(pend) > lag:
                f = pend.pop(0)
                if f is not None:
                    f()
        for f in pend:
            if f is not None:
                f()

    def a_kv(j):
        steps = []
        for ch in range(NCH):
            st = {}

            def kstep(ch=ch, st=st):
                kp = proj(waT, D + ch * MC, MC, j)
                st["phi"] = []
                for u in range(GPC):
                    g = ch * GPC + u
                    ep, en, sp, sn = _phi_parts(kp[u * 128:(u + 1) * 128, :])
                    rp = 1.0 / sp
                    rn = 1.0 / sn
                    phi = jnp.concatenate([e * rp for e in ep] + [e * rn for e in en], axis=0)
                    zacc[g * 256:(g + 1) * 256, :] += phi
                    st["phi"].append(phi.astype(BF16))

            def vstep(ch=ch, st=st):
                st["v"] = proj(waT, 2 * D + ch * MC, MC, j)

            def mstep(ch=ch, st=st):
                for u in range(GPC):
                    g = ch * GPC + u
                    vg = st["v"][u * 128:(u + 1) * 128, :].astype(BF16)
                    kv_acc[g] += _mm_nt(vg, st["phi"][u])

            steps.append((kstep, None))
            steps.append((vstep, mstep))
        return steps

    def a_init():
        kv_acc[...] = jnp.zeros(kv_acc.shape, F32)
        zacc[...] = jnp.zeros(zacc.shape, F32)

    def a_finish():
        r = lax.broadcasted_iota(jnp.int32, (128, 128), 0)
        c = lax.broadcasted_iota(jnp.int32, (128, 128), 1)
        keep = (r // 32) == (c % 4)
        for g in range(8):
            for hf in range(2):
                kvm[g, hf] = _pack(jnp.where(keep, kv_acc[g, :, hf * 128:(hf + 1) * 128], 0.0))
        zb[...] = jnp.broadcast_to(jnp.sum(zacc[...], axis=1, keepdims=True), zb.shape)

    def a_q(j, outs):
        steps = []
        for ch in range(NCH):
            st = {}

            def qstep(ch=ch, st=st):
                qp = proj(waT, ch * MC, MC, j)
                st["phi"] = []
                for u in range(GPC):
                    g = ch * GPC + u
                    ep, en, sp, sn = _phi_parts(qp[u * 128:(u + 1) * 128, :])
                    zr = _rows(zb[g * 256:(g + 1) * 256, :])
                    dp = _fold4(jnp.add, [e * zz for e, zz in zip(ep, zr[:16])])
                    dn = _fold4(jnp.add, [e * zz for e, zz in zip(en, zr[16:])])
                    rp = 1.0 / sp
                    rn = 1.0 / sn
                    rden = 1.0 / (dp * rp + dn * rn + 1e-6)
                    rp = rp * rden
                    rn = rn * rden
                    phi = jnp.concatenate([e * rp for e in ep] + [e * rn for e in en], axis=0)
                    st["phi"].append(phi.astype(BF16))

            def nstep(ch=ch, st=st):
                for u in range(GPC):
                    g = ch * GPC + u
                    kvg = jnp.concatenate([_unpk(kvm[g, 0]), _unpk(kvm[g, 1])], axis=1)
                    outs.append(_mm(kvg, st["phi"][u]))

            steps.append((qstep, nstep))
        return steps

    def out_proj(wo, outs, j):
        steps = []
        ln = LN(j)
        st = {}
        for ch in range(NCH):
            def ostep(ch=ch):
                if ch == 0:
                    st["o"] = jnp.concatenate(outs, axis=0).astype(BF16)
                m0 = ch * MC
                xt = xT[j, m0:m0 + MC, :] + _mm(wload(wo, m0, MC), st["o"])
                xT[j, m0:m0 + MC, :] = xt
                ln.add(xt)
                if ch == NCH - 1:
                    ln.finish()
            steps.append((ostep, None))
        return steps

    def b_kv(j):
        slot = jnp.where(j >= NBLK - HALO, j - (NBLK - HALO), HALO + NBLK)
        steps = []
        for base, ref in ((D, kb), (2 * D, vb)):
            for m0 in range(0, D, MC):
                def step(base=base, ref=ref, m0=m0):
                    p = proj(wbT, base + m0, MC, j)
                    ref[HALO + j, m0:m0 + MC, :] = p
                    ref[slot, m0:m0 + MC, :] = pltpu.roll(p, 2, 1)
                steps.append((step, None))
        return steps

    def b_q(j, outs):
        lo = lax.broadcasted_iota(jnp.int32, (8, L), 0) < 4
        first = lax.broadcasted_iota(jnp.int32, (8, L), 1) < 2
        cs = DH ** -0.5
        steps = []
        for G in range(4):
            def step(G=G):
                q = proj(wbT, G * 256, 256, j)
                halves = []
                for u in range(2):
                    acc = [None] * WIN
                    for r in range(16):
                        r0 = u * 128 + r * 8
                        qv = q[r0:r0 + 8, :]
                        for w in range(WIN):
                            t = qv * kb[HALO + j - w, G * 256 + r0:G * 256 + r0 + 8, :]
                            acc[w] = t if acc[w] is None else acc[w] + t
                    halves.append(acc)
                lg = []
                for w in range(WIN):
                    la, lb = halves[0][w], halves[1][w]
                    l = jnp.where(lo, la, lb) + pltpu.roll(jnp.where(lo, lb, la), 4, 0)
                    l = l * cs
                    if w > 0:
                        l = jnp.where(jnp.logical_and(first, j < w), -1e9, l)
                    lg.append(l)
                mx = _tree(jnp.maximum, lg)
                ex = [jnp.exp(l - mx) for l in lg]
                rs = 1.0 / _tree(jnp.add, ex)
                at = [e * rs for e in ex]
                for s in range(8):
                    h = G * 8 + s
                    o = None
                    for w in range(WIN):
                        a = jnp.broadcast_to(at[w][s:s + 1, :], (DH, L))
                        t = a * vb[HALO + j - w, h * DH:(h + 1) * DH, :]
                        o = t if o is None else o + t
                    outs.append(o)
            steps.append((step, None))
        return steps

    def final_proj(outs, j, xq, b):
        steps = []
        st = {}
        for ch in range(NCH):
            def ostep(ch=ch):
                if ch == 0:
                    st["o"] = jnp.concatenate(outs, axis=0).astype(BF16)
                m0 = ch * MC
                xt = xT[j, m0:m0 + MC, :] + _mm(wload(wobT, m0, MC), st["o"])
                for u in range(GPC):
                    y = xt[u * 128:(u + 1) * 128, :].astype(BF16).T
                    xq[ch * GPC + u, pl.ds(b, 64, stride=16), :] = pltpu.bitcast(y, U32)
            steps.append((ostep, None))
        return steps

    a_init()

    def s1(i, c):
        steps = []
        for b in range(NB):
            steps += a_kv(i * NB + b)
        emit(steps, LAG_KV)
        return c
    lax.fori_loop(0, NIT, s1, 0)

    def s2(i, c):
        js = [i * NB + b for b in range(NB)]
        outs = [[] for _ in js]
        steps = []
        for j, o in zip(js, outs):
            steps += a_q(j, o)
        for j, o in zip(js, outs):
            steps += out_proj(woaT, o, j)
        for j in js:
            steps += b_kv(j)
        emit(steps, LAG_Q)
        return c

    def s3(i, c):
        js = [i * NB + b for b in range(NB)]
        outs = [[] for _ in js]
        steps = []
        for j, o in zip(js, outs):
            steps += b_q(j, o)
        for j, o in zip(js, outs):
            steps += out_proj(wobT, o, j)
        for j in js:
            steps += a_kv(j)
        emit(steps, LAG_KV)
        return c

    def s5(a, c):
        xq = quad(a)
        outs = [[] for _ in range(4)]
        steps = b_q(a * 4, outs[0]) + b_q(a * 4 + 1, outs[1])
        for b in range(4):
            steps += final_proj(outs[b], a * 4 + b, xq, b)
            if b + 2 < 4:
                steps += b_q(a * 4 + b + 2, outs[b + 2])
        emit(steps, 0)
        return c

    a_finish()
    lax.fori_loop(0, NIT, s2, 0)
    a_init()
    lax.fori_loop(0, NIT, s3, 0)
    a_finish()
    lax.fori_loop(0, NIT, s2, 0)
    lax.fori_loop(0, 4, s5, 0)

    cp_out = [pltpu.make_async_copy(xio.at[c], out_hbm.at[:, pl.ds(c * L, L)], sems.at[8 + c]) for c in range(8)]
    for c in cp_out:
        c.start()
    for c in cp_out:
        c.wait()


@jax.jit
def pallas_interleave_layers__linear_kernel_hedgehog__sliding_local_dilated__prompt_kernel(
    A_x: jax.Array,
    A_wqkv: jax.Array,
    A_w_phi: jax.Array,
    A_wo: jax.Array,
    B_x: jax.Array,
    B_wqkv: jax.Array,
    B_wo: jax.Array,
):
    del B_x
    x2 = A_x.reshape(S, D)
    wphi2 = A_w_phi.reshape(H * DH, DH)
    any_spec = pl.BlockSpec(memory_space=pl.ANY)
    scratch = [
        pltpu.VMEM((8, S, L), BF16),
        pltpu.VMEM((D, 3 * D), BF16),
        pltpu.VMEM((D, D), BF16),
        pltpu.VMEM((D, 3 * D), BF16),
        pltpu.VMEM((D, D), BF16),
        pltpu.VMEM((H * DH, DH), BF16),
        pltpu.VMEM((8, 3 * D // 2, L), U32),
        pltpu.VMEM((8, D // 2, L), U32),
        pltpu.VMEM((8, 3 * D // 2, L), U32),
        pltpu.VMEM((8, D // 2, L), U32),
        pltpu.VMEM((NBLK, D, L), F32),
        pltpu.VMEM((NBLK, D // 2, L), U32),
        pltpu.VMEM((HALO + NBLK + 1, D, L), F32),
        pltpu.VMEM((HALO + NBLK + 1, D, L), F32),
        pltpu.VMEM((8, 128, 256), F32),
        pltpu.VMEM((8, 2, 64, 128), U32),
        pltpu.VMEM((2 * D, L), F32),
        pltpu.VMEM((2 * D, L), F32),
        pltpu.SemaphoreType.DMA((16,)),
    ]
    out = pl.pallas_call(
        _kernel,
        out_shape=jax.ShapeDtypeStruct((S, D), BF16),
        in_specs=[any_spec] * 6,
        out_specs=any_spec,
        scratch_shapes=scratch,
        compiler_params=pltpu.CompilerParams(vmem_limit_bytes=120 * 1024 * 1024),
        name="hedgehog_dilated",
    )(x2, A_wqkv, wphi2, A_wo, B_wqkv, B_wo)
    return out.reshape(1, S, D)
```

```python
import math

import jax
import jax.numpy as jnp
from jax import lax
import jax.experimental.pallas as pl
import jax.experimental.pallas.tpu as pltpu

S = 2048
D = 1024
H = 32
DH = 32
NBLK = 16
L = 128
WIN = 8
HALO = WIN - 1
LOG2E = math.log2(math.e)
F32 = jnp.float32
BF16 = jnp.bfloat16
U32 = jnp.uint32
NT = (((1,), (1,)), ((), ()))

MC = 256
NCH = D // MC
GPC = MC // 128
LAG_Q = 1
LAG_KV = 2

SEM_X = 0
SEM_PHI = 4
SEM_KV = 5
SEM_SET = 13
SEM_LATE = 21
NSEM = 22


def _mm(a, b):
    return jnp.dot(a, b, preferred_element_type=F32)


def _mm_nt(a, b):
    return lax.dot_general(a, b, NT, preferred_element_type=F32)


def _tree(op, xs):
    xs = list(xs)
    while len(xs) > 1:
        nxt = [op(xs[i], xs[i + 1]) for i in range(0, len(xs) - 1, 2)]
        if len(xs) % 2:
            nxt.append(xs[-1])
        xs = nxt
    return xs[0]


def _chain(op, xs, ways=4):
    acc = list(xs[:ways])
    for i, x in enumerate(xs[ways:]):
        acc[i % ways] = op(acc[i % ways], x)
    return _tree(op, acc)


def _rows(a, n=8):
    return [a[i * n:(i + 1) * n, :] for i in range(a.shape[0] // n)]


def _pack(a):
    return pltpu.bitcast(a.astype(BF16), U32)


def _unpk(a):
    return pltpu.bitcast(a, BF16)


def _fold4(op, xs):
    r = _tree(op, xs)
    return op(r, pltpu.roll(r, 4, 0))


def _phi_parts(p):
    ps = _rows(p)
    mx = _fold4(jnp.maximum, ps)
    mn = _fold4(jnp.minimum, ps)
    ep = [jnp.exp2(x - mx) for x in ps]
    en = [jnp.exp2(mn - x) for x in ps]
    sp = _fold4(jnp.add, ep)
    sn = _fold4(jnp.add, en)
    return ep, en, sp, sn


def _mult(x, m):
    return x if isinstance(x, int) else pl.multiple_of(x, m)


def _kernel(x_hbm, wa_hbm, wphi_hbm, woa_hbm, wb_hbm, wob_hbm, out_hbm,
            xio, wa_raw, woa_raw, wb_raw, wob_raw, wphi, pmat,
            waT, woaT, wbT, wobT, xT, xn, kb, vb, kv_acc, kvm, zacc, zb, sems):

    def x_in(a):
        return [pltpu.make_async_copy(x_hbm.at[:, pl.ds(8 * a, 8), pl.ds(c * L, L)],
                                      xio.at[c, :, pl.ds(8 * a, 8), :], sems.at[SEM_X + a]) for c in range(8)]

    def x_out(a):
        r = _mult(8 * a, 8)
        return [pltpu.make_async_copy(xio.at[c, :, pl.ds(r, 8), :],
                                      out_hbm.at[:, pl.ds(r, 8), pl.ds(c * L, L)], sems.at[SEM_X + a])
                for c in range(8)]

    def colcopy(src, dst, c0, n, sem):
        c0 = _mult(c0, 128)
        return pltpu.make_async_copy(src.at[:, pl.ds(c0, n)], dst.at[:, pl.ds(c0, n)], sems.at[sem])

    cp_phi = pltpu.make_async_copy(wphi_hbm, wphi, sems.at[SEM_PHI])
    cp_k = [colcopy(wa_hbm, wa_raw, D + ch * MC, MC, SEM_KV + 2 * ch) for ch in range(NCH)]
    cp_v = [colcopy(wa_hbm, wa_raw, 2 * D + ch * MC, MC, SEM_KV + 2 * ch + 1) for ch in range(NCH)]

    def w_set(g):
        return [colcopy(wa_hbm, wa_raw, g * 128, 128, SEM_SET + g),
                colcopy(woa_hbm, woa_raw, g * 128, 128, SEM_SET + g),
                colcopy(wb_hbm, wb_raw, D + g * 128, 128, SEM_SET + g),
                colcopy(wb_hbm, wb_raw, 2 * D + g * 128, 128, SEM_SET + g)]

    cp_late = [colcopy(wb_hbm, wb_raw, 0, D, SEM_LATE), colcopy(wob_hbm, wob_raw, 0, D, SEM_LATE)]

    order = [cp_phi, cp_k[0]] + x_in(0) + [cp_v[0]]
    for ch in range(1, NCH):
        order += [cp_k[ch], cp_v[ch]]
    order += x_in(1) + w_set(0) + w_set(1) + x_in(2) + w_set(2) + x_in(3)
    for g in range(3, 8):
        order += w_set(g)
    order += cp_late
    for c in order:
        c.start()

    def wait_all(cps):
        for c in cps:
            c.wait()

    xio32 = xio.bitcast(U32)

    def wload(ref, r0, n):
        return jnp.concatenate([_unpk(ref[c, r0 // 2:(r0 + n) // 2, :]) for c in range(8)], axis=1)

    def wstore(ref, g, val):
        off = _mult(g * 64, 64)
        for c in range(8):
            ref[c, pl.ds(off, 64), :] = _pack(val[:, c * L:(c + 1) * L])

    def wstore_perm(ref, g, val):
        for c in range(8):
            pk = _pack(val[:, c * L:(c + 1) * L])
            for h4 in range(4):
                ref[c, pl.ds(g * 64 + h4, 16, stride=4), :] = pk[h4 * 16:(h4 + 1) * 16, :]

    def cols(ref, g):
        return ref[:, pl.ds(_mult(g * 128, 128), 128)]

    class LN:
        def __init__(self, j):
            self.j = j
            self.piv = None
            self.s1 = []
            self.s2 = []

        def add(self, xt):
            if self.piv is None:
                self.piv = jnp.broadcast_to(xt[0:1, :], (8, L))
            d = [r - self.piv for r in _rows(xt)]
            self.s1.append(_chain(jnp.add, d, 2))
            self.s2.append(_chain(jnp.add, [x * x for x in d], 2))

        def finish(self):
            j = self.j
            m1 = jnp.sum(_tree(jnp.add, self.s1), axis=0, keepdims=True) * (1.0 / D)
            m2 = jnp.sum(_tree(jnp.add, self.s2), axis=0, keepdims=True) * (1.0 / D)
            var = jnp.maximum(m2 - m1 * m1, 0.0)
            mean = jnp.broadcast_to(self.piv[0:1, :] + m1, (16, L))
            rs = jnp.broadcast_to(lax.rsqrt(var + 1e-5), (16, L))
            for r in range(D // 16):
                xn[j, r * 8:(r + 1) * 8, :] = _pack((xT[j, r * 16:(r + 1) * 16, :] - mean) * rs)

    def prep_x(src, dst):
        ln = LN(dst)
        for cc in range(8):
            xt = _unpk(xio32[cc, :, src, :]).T.astype(F32)
            xT[dst, cc * 128:(cc + 1) * 128, :] = xt
            ln.add(xt)
        ln.finish()

    def fold(g, slab):
        wstore(waT, slab, _mm_nt(_unpk(pmat[g]), cols(wa_raw, slab)) * LOG2E)

    def prep_set(g):
        fold(g, g)
        wstore(woaT, g, cols(woa_raw, g).T)
        wstore_perm(wbT, 8 + g, cols(wb_raw, 8 + g).T)
        wstore(wbT, 16 + g, cols(wb_raw, 16 + g).T)

    def prep_late(g):
        wstore_perm(wbT, g, cols(wb_raw, g).T)
        wstore(wobT, g, cols(wob_raw, g).T)

    def proj(ref, r0, n, j):
        return _mm(wload(ref, r0, n), _unpk(xn[j]))

    def emit(steps, lag):
        pend = []
        for main, late in steps:
            main()
            pend.append(late)
            if len(pend) > lag:
                f = pend.pop(0)
                if f is not None:
                    f()
        for f in pend:
            if f is not None:
                f()

    def a_kv(j, lay, last):
        steps = []
        for ch in range(NCH):
            st = {}

            def kstep(ch=ch, st=st):
                kp = proj(waT, D + ch * MC, MC, j)
                st["phi"] = []
                for u in range(GPC):
                    g = ch * GPC + u
                    ep, en, sp, sn = _phi_parts(kp[u * 128:(u + 1) * 128, :])
                    rp = 1.0 / sp
                    rn = 1.0 / sn
                    phi = jnp.concatenate([e * rp for e in ep] + [e * rn for e in en], axis=0)
                    z = zacc[lay, g * 256:(g + 1) * 256, :] + phi
                    zacc[lay, g * 256:(g + 1) * 256, :] = z
                    if last:
                        zb[g * 256:(g + 1) * 256, :] = jnp.broadcast_to(
                            jnp.sum(z, axis=1, keepdims=True), (256, L))
                    st["phi"].append(phi.astype(BF16))

            def vstep(ch=ch, st=st):
                st["v"] = proj(waT, 2 * D + ch * MC, MC, j)

            def mstep(ch=ch, st=st):
                for u in range(GPC):
                    g = ch * GPC + u
                    vg = st["v"][u * 128:(u + 1) * 128, :].astype(BF16)
                    acc = kv_acc[lay, g] + _mm_nt(vg, st["phi"][u])
                    kv_acc[lay, g] = acc
                    if last:
                        r = lax.broadcasted_iota(jnp.int32, (128, 128), 0)
                        c = lax.broadcasted_iota(jnp.int32, (128, 128), 1)
                        keep = (r // 32) == (c % 4)
                        for hf in range(2):
                            kvm[g, hf] = _pack(jnp.where(keep, acc[:, hf * 128:(hf + 1) * 128], 0.0))

            steps.append((kstep, None))
            steps.append((vstep, mstep))
        return steps

    def a_q(j, outs):
        steps = []
        for ch in range(NCH):
            st = {}

            def qstep(ch=ch, st=st):
                qp = proj(waT, ch * MC, MC, j)
                st["phi"] = []
                for u in range(GPC):
                    g = ch * GPC + u
                    ep, en, sp, sn = _phi_parts(qp[u * 128:(u + 1) * 128, :])
                    zr = _rows(zb[g * 256:(g + 1) * 256, :])
                    dp = _fold4(jnp.add, [e * zz for e, zz in zip(ep, zr[:16])])
                    dn = _fold4(jnp.add, [e * zz for e, zz in zip(en, zr[16:])])
                    rp = 1.0 / sp
                    rn = 1.0 / sn
                    rden = 1.0 / (dp * rp + dn * rn + 1e-6)
                    rp = rp * rden
                    rn = rn * rden
                    phi = jnp.concatenate([e * rp for e in ep] + [e * rn for e in en], axis=0)
                    st["phi"].append(phi.astype(BF16))

            def nstep(ch=ch, st=st):
                for u in range(GPC):
                    g = ch * GPC + u
                    kvg = jnp.concatenate([_unpk(kvm[g, 0]), _unpk(kvm[g, 1])], axis=1)
                    outs.append(_mm(kvg, st["phi"][u]))

            steps.append((qstep, nstep))
        return steps

    def out_proj(wo, outs, j):
        steps = []
        ln = LN(j)
        st = {}
        for ch in range(NCH):
            def ostep(ch=ch):
                if ch == 0:
                    st["o"] = jnp.concatenate(outs, axis=0).astype(BF16)
                m0 = ch * MC
                xt = xT[j, m0:m0 + MC, :] + _mm(wload(wo, m0, MC), st["o"])
                xT[j, m0:m0 + MC, :] = xt
                ln.add(xt)
                if ch == NCH - 1:
                    ln.finish()
            steps.append((ostep, None))
        return steps

    def b_kv(j, halo):
        steps = []
        for base, ref in ((D, kb), (2 * D, vb)):
            for m0 in range(0, D, MC):
                def step(base=base, ref=ref, m0=m0):
                    p = proj(wbT, base + m0, MC, j)
                    ref[WIN + j, m0:m0 + MC, :] = p
                    if halo:
                        ref[j - WIN, m0:m0 + MC, :] = pltpu.roll(p, 2, 1)
                steps.append((step, None))
        return steps

    def b_q(j, outs):
        even = lax.broadcasted_iota(jnp.int32, (8, L), 0) % 2 == 0
        first = lax.broadcasted_iota(jnp.int32, (8, L), 1) < 2
        cs = DH ** -0.5
        steps = []
        for G in range(4):
            def step(G=G):
                q = proj(wbT, G * 256, 256, j)
                halves = []
                for u in range(2):
                    acc = [None] * WIN
                    for r in range(16):
                        r0 = u * 128 + r * 8
                        qv = q[r0:r0 + 8, :]
                        for w in range(WIN):
                            t = qv * kb[WIN + j - w, G * 256 + r0:G * 256 + r0 + 8, :]
                            acc[w] = t if acc[w] is None else acc[w] + t
                    halves.append(acc)
                lg = []
                for w in range(WIN):
                    la, lb = halves[0][w], halves[1][w]
                    l = jnp.where(even, la + pltpu.roll(la, 7, 0), lb + pltpu.roll(lb, 1, 0))
                    l = l * cs
                    if w > 0:
                        l = jnp.where(jnp.logical_and(first, j < w), -1e9, l)
                    lg.append(l)
                mx = _tree(jnp.maximum, lg)
                ex = [jnp.exp(l - mx) for l in lg]
                rs = 1.0 / _tree(jnp.add, ex)
                at = [e * rs for e in ex]
                for hh in range(8):
                    h = G * 8 + hh
                    s = 2 * (hh % 4) + hh // 4
                    o = None
                    for w in range(WIN):
                        a = jnp.broadcast_to(at[w][s:s + 1, :], (DH, L))
                        t = a * vb[WIN + j - w, h * DH:(h + 1) * DH, :]
                        o = t if o is None else o + t
                    outs.append(o)
            steps.append((step, None))
        return steps

    def final_proj(outs, j):
        steps = []
        st = {}
        for ch in range(NCH):
            def ostep(ch=ch):
                if ch == 0:
                    st["o"] = jnp.concatenate(outs, axis=0).astype(BF16)
                m0 = ch * MC
                xt = xT[j, m0:m0 + MC, :] + _mm(wload(wobT, m0, MC), st["o"])
                for u in range(GPC):
                    y = xt[u * 128:(u + 1) * 128, :].astype(BF16).T
                    xio32[ch * GPC + u, :, j, :] = pltpu.bitcast(y, U32)
            steps.append((ostep, None))
        return steps

    kv_acc[...] = jnp.zeros(kv_acc.shape, F32)
    zacc[...] = jnp.zeros(zacc.shape, F32)

    r128 = lax.broadcasted_iota(jnp.int32, (128, 128), 0)
    c128 = lax.broadcasted_iota(jnp.int32, (128, 128), 1)
    same_head = (r128 % 4) == (c128 // 32)
    er = lax.broadcasted_iota(jnp.int32, (128, 32), 0)
    ec = lax.broadcasted_iota(jnp.int32, (128, 32), 1)
    expand = jnp.where((er // 4) == ec, 1.0, 0.0).astype(BF16)
    cp_phi.wait()
    for g in range(8):
        pg = _mm_nt(expand, wphi[g * 128:(g + 1) * 128, :])
        pmat[g] = _pack(jnp.where(same_head, pg, 0.0))

    cp_k[0].wait()
    for u in range(GPC):
        fold(u, 8 + u)
    wait_all(x_in(0))
    prep_x(0, 0)
    prep_x(1, 1)
    sa = a_kv(0, 0, False)
    sb = a_kv(1, 0, False)
    steps = []
    for ch in range(NCH):
        def pre_k(ch=ch):
            if ch > 0:
                cp_k[ch].wait()
                for u in range(GPC):
                    fold(ch * GPC + u, 8 + ch * GPC + u)

        def pre_v(ch=ch):
            cp_v[ch].wait()
            for u in range(GPC):
                wstore(waT, 16 + ch * GPC + u, cols(wa_raw, 16 + ch * GPC + u).T)
            if ch < 2:
                prep_x(2 + ch, 2 + ch)

        ka, va = sa[2 * ch], sa[2 * ch + 1]
        kb_, vb_ = sb[2 * ch], sb[2 * ch + 1]
        if ch == 0:
            steps += [(lambda f=ka[0], p=pre_v: (p(), f()), None), kb_, va]
        else:
            steps += [(lambda f=ka[0], p=pre_v: (p(), f()), None), kb_, va]
        if ch + 1 < NCH:
            steps[-1] = (lambda f=va[0], ch=ch: (pre_k(ch + 1), f()), va[1])
        steps += [vb_]
    emit(steps, LAG_KV)

    def s1(i, c):
        @pl.when(i == 1)
        def _():
            wait_all(x_in(1))

        @pl.when(i == 3)
        def _():
            wait_all(x_in(2))

        @pl.when(i == 5)
        def _():
            wait_all(x_in(3))

        wait_all(w_set(i - 1))
        j = 2 * i
        steps = a_kv(j, 0, False) + a_kv(j + 1, 0, True)
        steps.insert(2, (lambda: prep_set(i - 1), None))
        steps.insert(4, (lambda: prep_x(jnp.minimum(j + 2, NBLK - 1), j + 2), None))
        steps.insert(8, (lambda: prep_x(jnp.minimum(j + 3, NBLK - 1), j + 3), None))
        emit(steps, LAG_KV)
        return c
    lax.fori_loop(1, 8, s1, 0)
    wait_all(w_set(7))
    prep_set(7)
    wait_all(cp_late)

    def s2(i, c):
        js = [8 + i, i]
        outs = [[], []]
        steps = a_q(js[0], outs[0]) + a_q(js[1], outs[1])
        steps += out_proj(woaT, outs[0], js[0]) + out_proj(woaT, outs[1], js[1])
        steps += [(lambda: prep_late(i), None)]
        steps += b_kv(js[0], True) + b_kv(js[1], False)
        emit(steps, LAG_Q)
        return c

    def s3(i, c):
        js = [2 * i, 2 * i + 1]
        outs = [[], []]
        steps = b_q(js[0], outs[0]) + b_q(js[1], outs[1])
        steps += out_proj(wobT, outs[0], js[0]) + out_proj(wobT, outs[1], js[1])
        steps += a_kv(js[0], 1, False) + a_kv(js[1], 1, True)
        emit(steps, LAG_KV)
        return c

    def s5(i, c):
        js = [2 * i, 2 * i + 1]
        outs = [[], []]
        steps = b_q(js[0], outs[0]) + b_q(js[1], outs[1])
        steps += final_proj(outs[0], js[0]) + final_proj(outs[1], js[1])
        emit(steps, 0)

        @pl.when(i % 2 == 1)
        def _():
            for cp in x_out(i // 2):
                cp.start()
        return c

    def layer_pair(l, c):
        lax.fori_loop(0, 8, s2, 0)

        @pl.when(l == 0)
        def _():
            lax.fori_loop(0, 8, s3, 0)

        @pl.when(l == 1)
        def _():
            lax.fori_loop(0, 8, s5, 0)
        return c
    lax.fori_loop(0, 2, layer_pair, 0)

    for a in range(4):
        wait_all(x_out(a))


@jax.jit
def pallas_interleave_layers__linear_kernel_hedgehog__sliding_local_dilated__prompt_kernel(
    A_x: jax.Array,
    A_wqkv: jax.Array,
    A_w_phi: jax.Array,
    A_wo: jax.Array,
    B_x: jax.Array,
    B_wqkv: jax.Array,
    B_wo: jax.Array,
):
    del B_x
    x3 = A_x.reshape(S // 32, 32, D)
    wphi2 = A_w_phi.reshape(H * DH, DH)
    any_spec = pl.BlockSpec(memory_space=pl.ANY)
    scratch = [
        pltpu.VMEM((8, S // 32, 32, L), BF16),
        pltpu.VMEM((D, 3 * D), BF16),
        pltpu.VMEM((D, D), BF16),
        pltpu.VMEM((D, 3 * D), BF16),
        pltpu.VMEM((D, D), BF16),
        pltpu.VMEM((H * DH, DH), BF16),
        pltpu.VMEM((8, 64, 128), U32),
        pltpu.VMEM((8, 3 * D // 2, L), U32),
        pltpu.VMEM((8, D // 2, L), U32),
        pltpu.VMEM((8, 3 * D // 2, L), U32),
        pltpu.VMEM((8, D // 2, L), U32),
        pltpu.VMEM((NBLK + 2, D, L), F32),
        pltpu.VMEM((NBLK + 2, D // 2, L), U32),
        pltpu.VMEM((WIN + NBLK, D, L), F32),
        pltpu.VMEM((WIN + NBLK, D, L), F32),
        pltpu.VMEM((2, 8, 128, 256), F32),
        pltpu.VMEM((8, 2, 64, 128), U32),
        pltpu.VMEM((2, 2 * D, L), F32),
        pltpu.VMEM((2 * D, L), F32),
        pltpu.SemaphoreType.DMA((NSEM,)),
    ]
    out = pl.pallas_call(
        _kernel,
        out_shape=jax.ShapeDtypeStruct((S // 32, 32, D), BF16),
        in_specs=[any_spec] * 6,
        out_specs=any_spec,
        scratch_shapes=scratch,
        compiler_params=pltpu.CompilerParams(vmem_limit_bytes=120 * 1024 * 1024),
        name="hedgehog_dilated",
    )(x3, A_wqkv, wphi2, A_wo, B_wqkv, B_wo)
    return out.reshape(1, S, D)
```

```python
import math

import jax
import jax.numpy as jnp
from jax import lax
import jax.experimental.pallas as pl
import jax.experimental.pallas.tpu as pltpu

S = 2048
D = 1024
H = 32
DH = 32
NBLK = 16
L = 128
WIN = 8
HALO = WIN - 1
LOG2E = math.log2(math.e)
F32 = jnp.float32
BF16 = jnp.bfloat16
U32 = jnp.uint32
NT = (((1,), (1,)), ((), ()))

MC = 256
NCH = D // MC
GPC = MC // 128
LAG_Q = 1
LAG_KV = 2

SEM_X = 0
SEM_PHI = 16
SEM_KV = 17
SEM_SET = 25
SEM_LATE = 33
NSEM = 34


def _mm(a, b):
    return jnp.dot(a, b, preferred_element_type=F32)


def _mm_nt(a, b):
    return lax.dot_general(a, b, NT, preferred_element_type=F32)


def _tree(op, xs):
    xs = list(xs)
    while len(xs) > 1:
        nxt = [op(xs[i], xs[i + 1]) for i in range(0, len(xs) - 1, 2)]
        if len(xs) % 2:
            nxt.append(xs[-1])
        xs = nxt
    return xs[0]


def _chain(op, xs, ways=4):
    acc = list(xs[:ways])
    for i, x in enumerate(xs[ways:]):
        acc[i % ways] = op(acc[i % ways], x)
    return _tree(op, acc)


def _rows(a, n=8):
    return [a[i * n:(i + 1) * n, :] for i in range(a.shape[0] // n)]


def _pack(a):
    return pltpu.bitcast(a.astype(BF16), U32)


def _unpk(a):
    return pltpu.bitcast(a, BF16)


def _fold4(op, xs):
    r = _tree(op, xs)
    return op(r, pltpu.roll(r, 4, 0))


def _phi_parts(p):
    ps = _rows(p)
    mx = _fold4(jnp.maximum, ps)
    mn = _fold4(jnp.minimum, ps)
    ep = [jnp.exp2(x - mx) for x in ps]
    en = [jnp.exp2(mn - x) for x in ps]
    sp = _fold4(jnp.add, ep)
    sn = _fold4(jnp.add, en)
    return ep, en, sp, sn


def _mult(x, m):
    return x if isinstance(x, int) else pl.multiple_of(x, m)


def _kernel(x_hbm, wa_hbm, wphi_hbm, woa_hbm, wb_hbm, wob_hbm, out_hbm,
            xio, wa_raw, woa_raw, wb_raw, wob_raw, wphi, pmat,
            wqaT, wkvaT, woaT, wqbT, wkvbT, wobT, xT, xn, kb, vb, kv_acc, kvm, zacc, zb, sems):

    x32 = x_hbm.bitcast(U32)
    out32 = out_hbm.bitcast(U32)

    def x_in(j):
        return pltpu.make_async_copy(x32.at[:, j, :], xio.at[j], sems.at[SEM_X + j])

    def x_out(j):
        return pltpu.make_async_copy(xio.at[j], out32.at[:, j, :], sems.at[SEM_X + j])

    def colcopy(src, dst, c0, n, sem):
        c0 = _mult(c0, 128)
        return pltpu.make_async_copy(src.at[:, pl.ds(c0, n)], dst.at[:, pl.ds(c0, n)], sems.at[sem])

    cp_phi = pltpu.make_async_copy(wphi_hbm, wphi, sems.at[SEM_PHI])
    cp_k = [colcopy(wa_hbm, wa_raw, D + ch * MC, MC, SEM_KV + 2 * ch) for ch in range(NCH)]
    cp_v = [colcopy(wa_hbm, wa_raw, 2 * D + ch * MC, MC, SEM_KV + 2 * ch + 1) for ch in range(NCH)]

    def w_set(g):
        return [colcopy(wa_hbm, wa_raw, g * 128, 128, SEM_SET + g),
                colcopy(woa_hbm, woa_raw, g * 128, 128, SEM_SET + g),
                colcopy(wb_hbm, wb_raw, D + g * 128, 128, SEM_SET + g),
                colcopy(wb_hbm, wb_raw, 2 * D + g * 128, 128, SEM_SET + g)]

    cp_late = [colcopy(wb_hbm, wb_raw, 0, D, SEM_LATE), colcopy(wob_hbm, wob_raw, 0, D, SEM_LATE)]

    order = [cp_phi, x_in(0), cp_k[0], x_in(1), cp_v[0], cp_k[1], cp_v[1], x_in(2), x_in(3)]
    for ch in range(2, NCH):
        order += [cp_k[ch], cp_v[ch]]
    for g in range(8):
        if g < 6:
            order += [x_in(4 + 2 * g), x_in(5 + 2 * g)]
        order += w_set(g)
    order += cp_late
    for c in order:
        c.start()

    def wait_all(cps):
        for c in cps:
            c.wait()

    def wload(ref, r0, n):
        return jnp.concatenate([_unpk(ref[c, r0 // 2:(r0 + n) // 2, :]) for c in range(8)], axis=1)

    def wstore(ref, g, val):
        off = _mult(g * 64, 64)
        for c in range(8):
            ref[c, pl.ds(off, 64), :] = _pack(val[:, c * L:(c + 1) * L])

    def wstore_perm(ref, g, val):
        for c in range(8):
            pk = _pack(val[:, c * L:(c + 1) * L])
            for h4 in range(4):
                ref[c, pl.ds(g * 64 + h4, 16, stride=4), :] = pk[h4 * 16:(h4 + 1) * 16, :]

    def cols(ref, g):
        return ref[:, pl.ds(_mult(g * 128, 128), 128)]

    class LN:
        def __init__(self, j):
            self.j = j
            self.piv = None
            self.s1 = []
            self.s2 = []

        def add(self, xt):
            if self.piv is None:
                self.piv = jnp.broadcast_to(xt[0:1, :], (8, L))
            d = [r - self.piv for r in _rows(xt)]
            self.s1.append(_chain(jnp.add, d, 2))
            self.s2.append(_chain(jnp.add, [x * x for x in d], 2))

        def finish(self):
            j = self.j
            m1 = jnp.sum(_tree(jnp.add, self.s1), axis=0, keepdims=True) * (1.0 / D)
            m2 = jnp.sum(_tree(jnp.add, self.s2), axis=0, keepdims=True) * (1.0 / D)
            var = jnp.maximum(m2 - m1 * m1, 0.0)
            mean = jnp.broadcast_to(self.piv[0:1, :] + m1, (16, L))
            rs = jnp.broadcast_to(lax.rsqrt(var + 1e-5), (16, L))
            for r in range(D // 16):
                xn[j, r * 8:(r + 1) * 8, :] = _pack((xT[j, r * 16:(r + 1) * 16, :] - mean) * rs)

    def prep_x(src, dst):
        ln = LN(dst)
        for cc in range(8):
            xt = _unpk(xio[src, :, cc * L:(cc + 1) * L]).T.astype(F32)
            xT[dst, cc * 128:(cc + 1) * 128, :] = xt
            ln.add(xt)
        ln.finish()

    def fold(dst, g, slab):
        wstore(dst, g, _mm_nt(_unpk(pmat[g]), cols(wa_raw, slab)) * LOG2E)

    def prep_set(g):
        wstore(woaT, g, cols(woa_raw, g).T)
        wstore_perm(wkvbT, g, cols(wb_raw, 8 + g).T)
        wstore(wkvbT, 8 + g, cols(wb_raw, 16 + g).T)

    def prep_late(g):
        wstore_perm(wqbT, g, cols(wb_raw, g).T)
        wstore(wobT, g, cols(wob_raw, g).T)

    def proj(ref, r0, n, j):
        return _mm(wload(ref, r0, n), _unpk(xn[j]))

    def emit(steps, lag):
        pend = []
        for main, late in steps:
            main()
            pend.append(late)
            if len(pend) > lag:
                f = pend.pop(0)
                if f is not None:
                    f()
        for f in pend:
            if f is not None:
                f()

    def a_kv(j, lay, last):
        steps = []
        for ch in range(NCH):
            st = {}

            def kstep(ch=ch, st=st):
                kp = proj(wkvaT, ch * MC, MC, j)
                st["phi"] = []
                for u in range(GPC):
                    g = ch * GPC + u
                    ep, en, sp, sn = _phi_parts(kp[u * 128:(u + 1) * 128, :])
                    rp = 1.0 / sp
                    rn = 1.0 / sn
                    phi = jnp.concatenate([e * rp for e in ep] + [e * rn for e in en], axis=0)
                    z = zacc[lay, g * 256:(g + 1) * 256, :] + phi
                    zacc[lay, g * 256:(g + 1) * 256, :] = z
                    if last:
                        zb[g * 256:(g + 1) * 256, :] = jnp.broadcast_to(
                            jnp.sum(z, axis=1, keepdims=True), (256, L))
                    st["phi"].append(phi.astype(BF16))

            def vstep(ch=ch, st=st):
                st["v"] = proj(wkvaT, D + ch * MC, MC, j)

            def mstep(ch=ch, st=st):
                for u in range(GPC):
                    g = ch * GPC + u
                    vg = st["v"][u * 128:(u + 1) * 128, :].astype(BF16)
                    acc = kv_acc[lay, g] + _mm_nt(vg, st["phi"][u])
                    kv_acc[lay, g] = acc
                    if last:
                        r = lax.broadcasted_iota(jnp.int32, (128, 128), 0)
                        c = lax.broadcasted_iota(jnp.int32, (128, 128), 1)
                        keep = (r // 32) == (c % 4)
                        for hf in range(2):
                            kvm[g, hf] = _pack(jnp.where(keep, acc[:, hf * 128:(hf + 1) * 128], 0.0))

            steps.append((kstep, None))
            steps.append((vstep, mstep))
        return steps

    def a_q(j, outs):
        steps = []
        for ch in range(NCH):
            st = {}

            def qstep(ch=ch, st=st):
                qp = proj(wqaT, ch * MC, MC, j)
                st["phi"] = []
                for u in range(GPC):
                    g = ch * GPC + u
                    ep, en, sp, sn = _phi_parts(qp[u * 128:(u + 1) * 128, :])
                    zr = _rows(zb[g * 256:(g + 1) * 256, :])
                    dp = _fold4(jnp.add, [e * zz for e, zz in zip(ep, zr[:16])])
                    dn = _fold4(jnp.add, [e * zz for e, zz in zip(en, zr[16:])])
                    rp = 1.0 / sp
                    rn = 1.0 / sn
                    rden = 1.0 / (dp * rp + dn * rn + 1e-6)
                    rp = rp * rden
                    rn = rn * rden
                    phi = jnp.concatenate([e * rp for e in ep] + [e * rn for e in en], axis=0)
                    st["phi"].append(phi.astype(BF16))

            def nstep(ch=ch, st=st):
                for u in range(GPC):
                    g = ch * GPC + u
                    kvg = jnp.concatenate([_unpk(kvm[g, 0]), _unpk(kvm[g, 1])], axis=1)
                    outs.append(_mm(kvg, st["phi"][u]))

            steps.append((qstep, nstep))
        return steps

    def out_proj(wo, outs, j):
        steps = []
        ln = LN(j)
        st = {}
        for ch in range(NCH):
            def ostep(ch=ch):
                if ch == 0:
                    st["o"] = jnp.concatenate(outs, axis=0).astype(BF16)
                m0 = ch * MC
                xt = xT[j, m0:m0 + MC, :] + _mm(wload(wo, m0, MC), st["o"])
                xT[j, m0:m0 + MC, :] = xt
                ln.add(xt)
                if ch == NCH - 1:
                    ln.finish()
            steps.append((ostep, None))
        return steps

    def b_kv(j, halo):
        steps = []
        for base, ref in ((0, kb), (D, vb)):
            for m0 in range(0, D, MC):
                def step(base=base, ref=ref, m0=m0):
                    p = proj(wkvbT, base + m0, MC, j)
                    ref[WIN + j, m0:m0 + MC, :] = p
                    if halo:
                        ref[j - WIN, m0:m0 + MC, :] = pltpu.roll(p, 2, 1)
                steps.append((step, None))
        return steps

    def b_q(j, outs):
        even = lax.broadcasted_iota(jnp.int32, (8, L), 0) % 2 == 0
        first = lax.broadcasted_iota(jnp.int32, (8, L), 1) < 2
        cs = DH ** -0.5
        steps = []
        for G in range(4):
            def step(G=G):
                q = proj(wqbT, G * 256, 256, j)
                halves = []
                for u in range(2):
                    acc = [None] * WIN
                    for r in range(16):
                        r0 = u * 128 + r * 8
                        qv = q[r0:r0 + 8, :]
                        for w in range(WIN):
                            t = qv * kb[WIN + j - w, G * 256 + r0:G * 256 + r0 + 8, :]
                            acc[w] = t if acc[w] is None else acc[w] + t
                    halves.append(acc)
                lg = []
                for w in range(WIN):
                    la, lb = halves[0][w], halves[1][w]
                    l = jnp.where(even, la + pltpu.roll(la, 7, 0), lb + pltpu.roll(lb, 1, 0))
                    l = l * cs
                    if w > 0:
                        l = jnp.where(jnp.logical_and(first, j < w), -1e9, l)
                    lg.append(l)
                mx = _tree(jnp.maximum, lg)
                ex = [jnp.exp(l - mx) for l in lg]
                rs = 1.0 / _tree(jnp.add, ex)
                at = [e * rs for e in ex]
                for hh in range(8):
                    h = G * 8 + hh
                    s = 2 * (hh % 4) + hh // 4
                    o = None
                    for w in range(WIN):
                        a = jnp.broadcast_to(at[w][s:s + 1, :], (DH, L))
                        t = a * vb[WIN + j - w, h * DH:(h + 1) * DH, :]
                        o = t if o is None else o + t
                    outs.append(o)
            steps.append((step, None))
        return steps

    def final_proj(outs, j):
        steps = []
        st = {}
        for ch in range(NCH):
            def ostep(ch=ch):
                if ch == 0:
                    st["o"] = jnp.concatenate(outs, axis=0).astype(BF16)
                m0 = ch * MC
                xt = xT[j, m0:m0 + MC, :] + _mm(wload(wobT, m0, MC), st["o"])
                for u in range(GPC):
                    y = xt[u * 128:(u + 1) * 128, :].astype(BF16).T
                    cc = ch * GPC + u
                    xio[j, :, cc * L:(cc + 1) * L] = pltpu.bitcast(y, U32)
            steps.append((ostep, None))
        return steps

    kv_acc[...] = jnp.zeros(kv_acc.shape, F32)
    zacc[...] = jnp.zeros(zacc.shape, F32)

    r128 = lax.broadcasted_iota(jnp.int32, (128, 128), 0)
    c128 = lax.broadcasted_iota(jnp.int32, (128, 128), 1)
    same_head = (r128 % 4) == (c128 // 32)
    er = lax.broadcasted_iota(jnp.int32, (128, 32), 0)
    ec = lax.broadcasted_iota(jnp.int32, (128, 32), 1)
    expand = jnp.where((er // 4) == ec, 1.0, 0.0).astype(BF16)
    cp_phi.wait()
    for g in range(8):
        pg = _mm_nt(expand, wphi[g * 128:(g + 1) * 128, :])
        pmat[g] = _pack(jnp.where(same_head, pg, 0.0))

    x_in(0).wait()
    prep_x(0, 0)
    sa = a_kv(0, 0, False)
    sb = a_kv(1, 0, False)
    pend = []
    for ch in range(NCH):
        cp_k[ch].wait()
        if ch == 0:
            for u in range(GPC):
                fold(wkvaT, u, 8 + u)
            sa[0][0]()
            x_in(1).wait()
        cp_v[ch].wait()
        if ch == 2:
            x_in(2).wait()
            x_in(3).wait()
        if ch == 0:
            prep_x(1, 1)
        else:
            for u in range(GPC):
                fold(wkvaT, ch * GPC + u, 8 + ch * GPC + u)
        for u in range(GPC):
            wstore(wkvaT, 8 + ch * GPC + u, cols(wa_raw, 16 + ch * GPC + u).T)
        for f in pend:
            f()
        if ch >= 2:
            prep_x(ch, ch)
        if ch == 0:
            sa[1][0]()
            sb[0][0]()
        else:
            sa[2 * ch][0]()
            sb[2 * ch][0]()
            sa[2 * ch + 1][0]()
        sb[2 * ch + 1][0]()
        pend = [sa[2 * ch + 1][1], sb[2 * ch + 1][1]]
    for f in pend:
        f()

    def s1(i, c):
        j = 2 * i

        @pl.when(i < 7)
        def _():
            x_in(j + 2).wait()
            x_in(j + 3).wait()

        wait_all(w_set(i - 1))
        steps = a_kv(j, 0, False) + a_kv(j + 1, 0, True)
        steps.insert(14, (lambda: prep_set(i - 1), None))
        steps.insert(12, (lambda: prep_x(jnp.minimum(j + 3, NBLK - 1), j + 3), None))
        steps.insert(8, (lambda: prep_x(jnp.minimum(j + 2, NBLK - 1), j + 2), None))
        steps.insert(2, (lambda: fold(wqaT, i - 1, i - 1), None))
        emit(steps, LAG_KV)
        return c
    lax.fori_loop(1, 8, s1, 0)
    wait_all(w_set(7))
    fold(wqaT, 7, 7)
    prep_set(7)
    wait_all(cp_late)

    def s2(i, c):
        js = [8 + i, i]
        outs = [[], []]
        steps = a_q(js[0], outs[0]) + a_q(js[1], outs[1])
        steps += out_proj(woaT, outs[0], js[0]) + out_proj(woaT, outs[1], js[1])
        steps += [(lambda: prep_late(i), None)]
        steps += b_kv(js[0], True) + b_kv(js[1], False)
        emit(steps, LAG_Q)
        return c

    def s3(i, c):
        js = [2 * i, 2 * i + 1]
        outs = [[], []]
        steps = b_q(js[0], outs[0]) + b_q(js[1], outs[1])
        steps += out_proj(wobT, outs[0], js[0]) + out_proj(wobT, outs[1], js[1])
        steps += a_kv(js[0], 1, False) + a_kv(js[1], 1, True)
        emit(steps, LAG_KV)
        return c

    def s5(i, c):
        js = [2 * i, 2 * i + 1]
        outs = [[], []]
        steps = b_q(js[0], outs[0]) + b_q(js[1], outs[1])
        steps += final_proj(outs[0], js[0]) + final_proj(outs[1], js[1])
        emit(steps, 0)

        x_out(js[0]).start()
        x_out(js[1]).start()
        return c

    def layer_pair(l, c):
        lax.fori_loop(0, 8, s2, 0)

        @pl.when(l == 0)
        def _():
            lax.fori_loop(0, 8, s3, 0)

        @pl.when(l == 1)
        def _():
            lax.fori_loop(0, 8, s5, 0)
        return c
    lax.fori_loop(0, 2, layer_pair, 0)

    for j in range(NBLK):
        x_out(j).wait()


@jax.jit
def pallas_interleave_layers__linear_kernel_hedgehog__sliding_local_dilated__prompt_kernel(
    A_x: jax.Array,
    A_wqkv: jax.Array,
    A_w_phi: jax.Array,
    A_wo: jax.Array,
    B_x: jax.Array,
    B_wqkv: jax.Array,
    B_wo: jax.Array,
):
    del B_x
    x3 = A_x.reshape(S // 32, 32, D)
    wphi2 = A_w_phi.reshape(H * DH, DH)
    any_spec = pl.BlockSpec(memory_space=pl.ANY)
    scratch = [
        pltpu.VMEM((NBLK, S // 32, D), U32),
        pltpu.VMEM((D, 3 * D), BF16),
        pltpu.VMEM((D, D), BF16),
        pltpu.VMEM((D, 3 * D), BF16),
        pltpu.VMEM((D, D), BF16),
        pltpu.VMEM((H * DH, DH), BF16),
        pltpu.VMEM((8, 64, 128), U32),
        pltpu.VMEM((8, D // 2, L), U32),
        pltpu.VMEM((8, D, L), U32),
        pltpu.VMEM((8, D // 2, L), U32),
        pltpu.VMEM((8, D // 2, L), U32),
        pltpu.VMEM((8, D, L), U32),
        pltpu.VMEM((8, D // 2, L), U32),
        pltpu.VMEM((NBLK + 2, D, L), F32),
        pltpu.VMEM((NBLK + 2, D // 2, L), U32),
        pltpu.VMEM((WIN + NBLK, D, L), F32),
        pltpu.VMEM((WIN + NBLK, D, L), F32),
        pltpu.VMEM((2, 8, 128, 256), F32),
        pltpu.VMEM((8, 2, 64, 128), U32),
        pltpu.VMEM((2, 2 * D, L), F32),
        pltpu.VMEM((2 * D, L), F32),
        pltpu.SemaphoreType.DMA((NSEM,)),
    ]
    out = pl.pallas_call(
        _kernel,
        out_shape=jax.ShapeDtypeStruct((S // 32, 32, D), BF16),
        in_specs=[any_spec] * 6,
        out_specs=any_spec,
        scratch_shapes=scratch,
        compiler_params=pltpu.CompilerParams(vmem_limit_bytes=120 * 1024 * 1024),
        name="hedgehog_dilated",
    )(x3, A_wqkv, wphi2, A_wo, B_wqkv, B_wo)
    return out.reshape(1, S, D)
```

```python
import math

import jax
import jax.numpy as jnp
from jax import lax
import jax.experimental.pallas as pl
import jax.experimental.pallas.tpu as pltpu

S = 2048
D = 1024
H = 32
DH = 32
NBLK = 16
L = 128
WIN = 8
HALO = WIN - 1
LOG2E = math.log2(math.e)
F32 = jnp.float32
BF16 = jnp.bfloat16
U32 = jnp.uint32
NT = (((1,), (1,)), ((), ()))

MC = 256
NCH = D // MC
GPC = MC // 128
CFG = dict(lag_q=1, lag_kv=2, only=None, ln_ways=2, ln_serial=False, ln_late=0)

SEM_X = 0
SEM_PHI = 16
SEM_KV = 17
SEM_SET = 25
SEM_LATE = 33
NSEM = 34


def _mm(a, b):
    return jnp.dot(a, b, preferred_element_type=F32)


def _mm_nt(a, b):
    return lax.dot_general(a, b, NT, preferred_element_type=F32)


def _tree(op, xs):
    xs = list(xs)
    while len(xs) > 1:
        nxt = [op(xs[i], xs[i + 1]) for i in range(0, len(xs) - 1, 2)]
        if len(xs) % 2:
            nxt.append(xs[-1])
        xs = nxt
    return xs[0]


def _chain(op, xs, ways=4):
    acc = list(xs[:ways])
    for i, x in enumerate(xs[ways:]):
        acc[i % ways] = op(acc[i % ways], x)
    return _tree(op, acc)


def _rows(a, n=8):
    return [a[i * n:(i + 1) * n, :] for i in range(a.shape[0] // n)]


def _pack(a):
    return pltpu.bitcast(a.astype(BF16), U32)


def _unpk(a):
    return pltpu.bitcast(a, BF16)


def _pack_i(a, b):
    return pltpu.pack_elementwise([a, b], packed_dtype=BF16)


def _pack_split(a):
    r = _rows(a)
    return jnp.concatenate([_pack_i(r[2 * i], r[2 * i + 1]) for i in range(len(r) // 2)], axis=0)


def _unpack_split(p):
    out = []
    for x in _rows(p):
        out.append(pltpu.unpack_elementwise(x, index=0, packed_dtype=BF16, unpacked_dtype=F32))
        out.append(pltpu.unpack_elementwise(x, index=1, packed_dtype=BF16, unpacked_dtype=F32))
    return jnp.concatenate(out, axis=0)


def _fold4(op, xs):
    r = _tree(op, xs)
    return op(r, pltpu.roll(r, 4, 0))


def _phi_parts(p):
    ps = _rows(p)
    mx = _fold4(jnp.maximum, ps)
    mn = _fold4(jnp.minimum, ps)
    ep = [jnp.exp2(x - mx) for x in ps]
    en = [jnp.exp2(mn - x) for x in ps]
    sp = _fold4(jnp.add, ep)
    sn = _fold4(jnp.add, en)
    return ep, en, sp, sn


def _mult(x, m):
    return x if isinstance(x, int) else pl.multiple_of(x, m)


def _kernel(x_hbm, wa_hbm, wphi_hbm, woa_hbm, wb_hbm, wob_hbm, out_hbm,
            xio, wa_raw, woa_raw, wb_raw, wob_raw, wphi, pmat,
            wqaT, wkvaT, woaT, wqbT, wkvbT, wobT, xT, xn, kb, vb, kv_acc, kvm, zacc, zb, sems):

    x32 = x_hbm.bitcast(U32)
    out32 = out_hbm.bitcast(U32)

    def x_in(j):
        return pltpu.make_async_copy(x32.at[:, j, :], xio.at[j], sems.at[SEM_X + j])

    def x_out(j):
        return pltpu.make_async_copy(xio.at[j], out32.at[:, j, :], sems.at[SEM_X + j])

    def colcopy(src, dst, c0, n, sem):
        c0 = _mult(c0, 128)
        return pltpu.make_async_copy(src.at[:, pl.ds(c0, n)], dst.at[:, pl.ds(c0, n)], sems.at[sem])

    cp_phi = pltpu.make_async_copy(wphi_hbm, wphi, sems.at[SEM_PHI])
    cp_k = [colcopy(wa_hbm, wa_raw, D + ch * MC, MC, SEM_KV + 2 * ch) for ch in range(NCH)]
    cp_v = [colcopy(wa_hbm, wa_raw, 2 * D + ch * MC, MC, SEM_KV + 2 * ch + 1) for ch in range(NCH)]

    def w_set(g):
        return [colcopy(wa_hbm, wa_raw, g * 128, 128, SEM_SET + g),
                colcopy(woa_hbm, woa_raw, g * 128, 128, SEM_SET + g),
                colcopy(wb_hbm, wb_raw, D + g * 128, 128, SEM_SET + g),
                colcopy(wb_hbm, wb_raw, 2 * D + g * 128, 128, SEM_SET + g)]

    cp_late = [colcopy(wb_hbm, wb_raw, 0, D, SEM_LATE), colcopy(wob_hbm, wob_raw, 0, D, SEM_LATE)]

    order = [cp_phi, x_in(0), cp_k[0], x_in(1), cp_v[0], cp_k[1], cp_v[1], x_in(2), x_in(3)]
    for ch in range(2, NCH):
        order += [cp_k[ch], cp_v[ch]]
    for g in range(8):
        if g < 6:
            order += [x_in(4 + 2 * g), x_in(5 + 2 * g)]
        order += w_set(g)
    order += cp_late
    for c in order:
        c.start()

    def wait_all(cps):
        for c in cps:
            c.wait()

    def wload(ref, r0, n):
        return jnp.concatenate([_unpk(ref[c, r0 // 2:(r0 + n) // 2, :]) for c in range(8)], axis=1)

    def wstore(ref, g, val):
        off = _mult(g * 64, 64)
        for c in range(8):
            ref[c, pl.ds(off, 64), :] = _pack(val[:, c * L:(c + 1) * L])

    def wstore_split(ref, g, val):
        off = _mult(g * 64, 64)
        for c in range(8):
            ref[c, pl.ds(off, 64), :] = _pack(_unpack_split(pltpu.bitcast(val[:, c * L:(c + 1) * L], U32)))

    def wstore_perm(ref, g, val):
        for c in range(8):
            pk = _pack(val[:, c * L:(c + 1) * L])
            for h4 in range(4):
                ref[c, pl.ds(g * 64 + h4, 16, stride=4), :] = pk[h4 * 16:(h4 + 1) * 16, :]

    def cols(ref, g):
        return ref[:, pl.ds(_mult(g * 128, 128), 128)]

    class LN:
        def __init__(self, j):
            self.j = j
            self.piv = None
            self.s1 = []
            self.s2 = []

        def add(self, xt):
            if self.piv is None:
                self.piv = jnp.broadcast_to(xt[0:1, :], (8, L))
            d = [r - self.piv for r in _rows(xt)]
            if CFG["ln_serial"]:
                self.s1 = [_chain(jnp.add, self.s1 + d, 1)]
                self.s2 = [_chain(jnp.add, self.s2 + [x * x for x in d], 1)]
            else:
                self.s1.append(_chain(jnp.add, d, CFG["ln_ways"]))
                self.s2.append(_chain(jnp.add, [x * x for x in d], CFG["ln_ways"]))

        def finish(self):
            j = self.j
            m1 = jnp.sum(_tree(jnp.add, self.s1), axis=0, keepdims=True) * (1.0 / D)
            m2 = jnp.sum(_tree(jnp.add, self.s2), axis=0, keepdims=True) * (1.0 / D)
            var = jnp.maximum(m2 - m1 * m1, 0.0)
            rs = lax.rsqrt(var + 1e-5)
            mrs = jnp.broadcast_to((self.piv[0:1, :] + m1) * rs, (8, L))
            rs = jnp.broadcast_to(rs, (8, L))
            for r in range(D // 16):
                xn[j, r * 8:(r + 1) * 8, :] = _pack_i(xT[j, r * 16:r * 16 + 8, :] * rs - mrs,
                                                      xT[j, r * 16 + 8:r * 16 + 16, :] * rs - mrs)

    def prep_x(src, dst):
        ln = LN(dst)
        for cc in range(8):
            xt = _unpack_split(pltpu.bitcast(_unpk(xio[src, :, cc * L:(cc + 1) * L]).T, U32))
            xT[dst, cc * 128:(cc + 1) * 128, :] = xt
            ln.add(xt)
        ln.finish()

    def fold(dst, g, slab):
        val = _mm_nt(_unpk(pmat[g]), cols(wa_raw, slab)) * LOG2E
        off = _mult(g * 64, 64)
        for c in range(8):
            dst[c, pl.ds(off, 64), :] = _pack_split(val[:, c * L:(c + 1) * L])

    def prep_set(g):
        wstore_split(woaT, g, cols(woa_raw, g).T)
        wstore_perm(wkvbT, g, cols(wb_raw, 8 + g).T)
        wstore(wkvbT, 8 + g, cols(wb_raw, 16 + g).T)

    def prep_late(g):
        wstore_perm(wqbT, g, cols(wb_raw, g).T)
        wstore_split(wobT, g, cols(wob_raw, g).T)

    def proj(ref, r0, n, j):
        return _mm(wload(ref, r0, n), _unpk(xn[j]))

    def emit(steps, lag):
        pend = []
        for main, late in steps:
            main()
            pend.append(late)
            if len(pend) > lag:
                f = pend.pop(0)
                if f is not None:
                    f()
        for f in pend:
            if f is not None:
                f()

    def a_kv(j, lay, last):
        steps = []
        for ch in range(NCH):
            st = {}

            def kstep(ch=ch, st=st):
                kp = proj(wkvaT, ch * MC, MC, j)
                st["phi"] = []
                for u in range(GPC):
                    g = ch * GPC + u
                    ep, en, sp, sn = _phi_parts(kp[u * 128:(u + 1) * 128, :])
                    rp = 1.0 / sp
                    rn = 1.0 / sn
                    phi = jnp.concatenate([e * rp for e in ep] + [e * rn for e in en], axis=0)
                    z = zacc[lay, g * 256:(g + 1) * 256, :] + phi
                    zacc[lay, g * 256:(g + 1) * 256, :] = z
                    if last:
                        zb[g * 256:(g + 1) * 256, :] = jnp.broadcast_to(
                            jnp.sum(z, axis=1, keepdims=True), (256, L))
                    st["phi"].append(phi.astype(BF16))

            def vstep(ch=ch, st=st):
                st["v"] = proj(wkvaT, D + ch * MC, MC, j)

            def mstep(ch=ch, st=st):
                for u in range(GPC):
                    g = ch * GPC + u
                    vg = st["v"][u * 128:(u + 1) * 128, :].astype(BF16)
                    acc = kv_acc[lay, g] + _mm_nt(vg, st["phi"][u])
                    kv_acc[lay, g] = acc
                    if last:
                        r = lax.broadcasted_iota(jnp.int32, (128, 128), 0)
                        c = lax.broadcasted_iota(jnp.int32, (128, 128), 1)
                        keep = (r // 32) == (c % 4)
                        for hf in range(2):
                            kvm[g, hf] = _pack(jnp.where(keep, acc[:, hf * 128:(hf + 1) * 128], 0.0))

            steps.append((kstep, None))
            steps.append((vstep, mstep))
        return steps

    def a_q(j, outs):
        steps = []
        for ch in range(NCH):
            st = {}

            def qstep(ch=ch, st=st):
                qp = proj(wqaT, ch * MC, MC, j)
                st["phi"] = []
                for u in range(GPC):
                    g = ch * GPC + u
                    ep, en, sp, sn = _phi_parts(qp[u * 128:(u + 1) * 128, :])
                    zr = _rows(zb[g * 256:(g + 1) * 256, :])
                    dp = _fold4(jnp.add, [e * zz for e, zz in zip(ep, zr[:16])])
                    dn = _fold4(jnp.add, [e * zz for e, zz in zip(en, zr[16:])])
                    rp = 1.0 / sp
                    rn = 1.0 / sn
                    rden = 1.0 / (dp * rp + dn * rn + 1e-6)
                    rp = rp * rden
                    rn = rn * rden
                    phi = jnp.concatenate([e * rp for e in ep] + [e * rn for e in en], axis=0)
                    st["phi"].append(phi.astype(BF16))

            def nstep(ch=ch, st=st):
                for u in range(GPC):
                    g = ch * GPC + u
                    kvg = jnp.concatenate([_unpk(kvm[g, 0]), _unpk(kvm[g, 1])], axis=1)
                    outs.append(_mm(kvg, st["phi"][u]))

            steps.append((qstep, nstep))
        return steps

    def out_proj(wo, outs, j):
        steps = []
        ln = LN(j)
        st = {}
        for ch in range(NCH):
            def ostep(ch=ch):
                if ch == 0:
                    st["o"] = jnp.concatenate(outs, axis=0).astype(BF16)
                m0 = ch * MC
                xt = xT[j, m0:m0 + MC, :] + _mm(wload(wo, m0, MC), st["o"])
                xT[j, m0:m0 + MC, :] = xt
                ln.add(xt)
                if ch == NCH - 1 and not CFG["ln_late"]:
                    ln.finish()
            steps.append((ostep, ln.finish if (ch == NCH - 1 and CFG["ln_late"]) else None))
        return steps

    def b_kv(j, halo):
        steps = []
        for base, ref in ((0, kb), (D, vb)):
            for m0 in range(0, D, MC):
                def step(base=base, ref=ref, m0=m0):
                    p = proj(wkvbT, base + m0, MC, j)
                    ref[WIN + j, m0:m0 + MC, :] = p
                    if halo:
                        ref[j - WIN, m0:m0 + MC, :] = pltpu.roll(p, 2, 1)
                steps.append((step, None))
        return steps

    def b_q(j, outs):
        even = lax.broadcasted_iota(jnp.int32, (8, L), 0) % 2 == 0
        first = lax.broadcasted_iota(jnp.int32, (8, L), 1) < 2
        cs = DH ** -0.5
        steps = []
        for G in range(4):
            def step(G=G):
                q = proj(wqbT, G * 256, 256, j)
                halves = []
                for u in range(2):
                    acc = [None] * WIN
                    for r in range(16):
                        r0 = u * 128 + r * 8
                        qv = q[r0:r0 + 8, :]
                        for w in range(WIN):
                            t = qv * kb[WIN + j - w, G * 256 + r0:G * 256 + r0 + 8, :]
                            acc[w] = t if acc[w] is None else acc[w] + t
                    halves.append(acc)
                lg = []
                for w in range(WIN):
                    la, lb = halves[0][w], halves[1][w]
                    l = jnp.where(even, la + pltpu.roll(la, 7, 0), lb + pltpu.roll(lb, 1, 0))
                    l = l * cs
                    if w > 0:
                        l = jnp.where(jnp.logical_and(first, j < w), -1e9, l)
                    lg.append(l)
                mx = _tree(jnp.maximum, lg)
                ex = [jnp.exp(l - mx) for l in lg]
                rs = 1.0 / _tree(jnp.add, ex)
                at = [e * rs for e in ex]
                for hh in range(8):
                    h = G * 8 + hh
                    s = 2 * (hh % 4) + hh // 4
                    o = None
                    for w in range(WIN):
                        a = jnp.broadcast_to(at[w][s:s + 1, :], (DH, L))
                        t = a * vb[WIN + j - w, h * DH:(h + 1) * DH, :]
                        o = t if o is None else o + t
                    outs.append(o)
            steps.append((step, None))
        return steps

    def final_proj(outs, j):
        steps = []
        st = {}
        for ch in range(NCH):
            def ostep(ch=ch):
                if ch == 0:
                    st["o"] = jnp.concatenate(outs, axis=0).astype(BF16)
                m0 = ch * MC
                xt = xT[j, m0:m0 + MC, :] + _mm(wload(wobT, m0, MC), st["o"])
                for u in range(GPC):
                    y = _unpk(_pack_split(xt[u * 128:(u + 1) * 128, :])).T
                    cc = ch * GPC + u
                    xio[j, :, cc * L:(cc + 1) * L] = pltpu.bitcast(y, U32)
            steps.append((ostep, None))
        return steps

    kv_acc[...] = jnp.zeros(kv_acc.shape, F32)
    zacc[...] = jnp.zeros(zacc.shape, F32)

    def unsplit(r):
        return (r // 16) * 16 + 2 * (r % 8) + (r // 8) % 2

    r128 = unsplit(lax.broadcasted_iota(jnp.int32, (128, 128), 0))
    c128 = lax.broadcasted_iota(jnp.int32, (128, 128), 1)
    same_head = (r128 % 4) == (c128 // 32)
    er = unsplit(lax.broadcasted_iota(jnp.int32, (128, 32), 0))
    ec = lax.broadcasted_iota(jnp.int32, (128, 32), 1)
    expand = jnp.where((er // 4) == ec, 1.0, 0.0).astype(BF16)
    cp_phi.wait()
    for g in range(8):
        pg = _mm_nt(expand, wphi[g * 128:(g + 1) * 128, :])
        pmat[g] = _pack(jnp.where(same_head, pg, 0.0))

    only = CFG["only"]
    x_in(0).wait()
    prep_x(0, 0)
    sa = a_kv(0, 0, False)
    sb = a_kv(1, 0, False)
    pend = []
    for ch in range(NCH if only in (None, 0) else 0):
        cp_k[ch].wait()
        if ch == 0:
            for u in range(GPC):
                fold(wkvaT, u, 8 + u)
            sa[0][0]()
            x_in(1).wait()
        cp_v[ch].wait()
        if ch == 2:
            x_in(2).wait()
            x_in(3).wait()
        if ch == 0:
            prep_x(1, 1)
        else:
            for u in range(GPC):
                fold(wkvaT, ch * GPC + u, 8 + ch * GPC + u)
        for u in range(GPC):
            wstore(wkvaT, 8 + ch * GPC + u, cols(wa_raw, 16 + ch * GPC + u).T)
        for f in pend:
            f()
        if ch >= 2:
            prep_x(ch, ch)
        if ch == 0:
            sa[1][0]()
            sb[0][0]()
        else:
            sa[2 * ch][0]()
            sb[2 * ch][0]()
            sa[2 * ch + 1][0]()
        sb[2 * ch + 1][0]()
        pend = [sa[2 * ch + 1][1], sb[2 * ch + 1][1]]
    for f in pend:
        f()

    def s1(i, c):
        j = 2 * i

        @pl.when(i < 7)
        def _():
            x_in(j + 2).wait()
            x_in(j + 3).wait()

        wait_all(w_set(i - 1))
        steps = a_kv(j, 0, False) + a_kv(j + 1, 0, True)
        steps.insert(14, (lambda: prep_set(i - 1), None))
        steps.insert(12, (lambda: prep_x(jnp.minimum(j + 3, NBLK - 1), j + 3), None))
        steps.insert(8, (lambda: prep_x(jnp.minimum(j + 2, NBLK - 1), j + 2), None))
        steps.insert(2, (lambda: fold(wqaT, i - 1, i - 1), None))
        emit(steps, CFG["lag_kv"])
        return c
    if only in (None, 1):
        lax.fori_loop(1, 8, s1, 0)
    wait_all(w_set(7))
    fold(wqaT, 7, 7)
    prep_set(7)
    wait_all(cp_late)

    def s2(i, c):
        js = [8 + i, i]
        outs = [[], []]
        steps = a_q(js[0], outs[0]) + a_q(js[1], outs[1])
        steps += out_proj(woaT, outs[0], js[0]) + out_proj(woaT, outs[1], js[1])
        steps += [(lambda: prep_late(i), None)]
        steps += b_kv(js[0], True) + b_kv(js[1], False)
        emit(steps, CFG["lag_q"])
        return c

    def s3(i, c):
        js = [2 * i, 2 * i + 1]
        outs = [[], []]
        steps = b_q(js[0], outs[0]) + b_q(js[1], outs[1])
        steps += out_proj(wobT, outs[0], js[0]) + out_proj(wobT, outs[1], js[1])
        steps += a_kv(js[0], 1, False) + a_kv(js[1], 1, True)
        emit(steps, CFG["lag_kv"])
        return c

    def s5(i, c):
        js = [2 * i, 2 * i + 1]
        outs = [[], []]
        steps = b_q(js[0], outs[0]) + b_q(js[1], outs[1])
        steps += final_proj(outs[0], js[0]) + final_proj(outs[1], js[1])
        emit(steps, 0)

        x_out(js[0]).start()
        x_out(js[1]).start()
        return c

    def layer_pair(l, c):
        if only in (None, 2):
            lax.fori_loop(0, 8, s2, 0)

        @pl.when(l == 0)
        def _():
            if only in (None, 3):
                lax.fori_loop(0, 8, s3, 0)

        @pl.when(l == 1)
        def _():
            if only in (None, 5):
                lax.fori_loop(0, 8, s5, 0)
        return c
    lax.fori_loop(0, 2, layer_pair, 0)

    for j in range(NBLK):
        x_out(j).wait()


@jax.jit
def pallas_interleave_layers__linear_kernel_hedgehog__sliding_local_dilated__prompt_kernel(
    A_x: jax.Array,
    A_wqkv: jax.Array,
    A_w_phi: jax.Array,
    A_wo: jax.Array,
    B_x: jax.Array,
    B_wqkv: jax.Array,
    B_wo: jax.Array,
):
    del B_x
    x3 = A_x.reshape(S // 32, 32, D)
    wphi2 = A_w_phi.reshape(H * DH, DH)
    any_spec = pl.BlockSpec(memory_space=pl.ANY)
    scratch = [
        pltpu.VMEM((NBLK, S // 32, D), U32),
        pltpu.VMEM((D, 3 * D), BF16),
        pltpu.VMEM((D, D), BF16),
        pltpu.VMEM((D, 3 * D), BF16),
        pltpu.VMEM((D, D), BF16),
        pltpu.VMEM((H * DH, DH), BF16),
        pltpu.VMEM((8, 64, 128), U32),
        pltpu.VMEM((8, D // 2, L), U32),
        pltpu.VMEM((8, D, L), U32),
        pltpu.VMEM((8, D // 2, L), U32),
        pltpu.VMEM((8, D // 2, L), U32),
        pltpu.VMEM((8, D, L), U32),
        pltpu.VMEM((8, D // 2, L), U32),
        pltpu.VMEM((NBLK + 2, D, L), F32),
        pltpu.VMEM((NBLK + 2, D // 2, L), U32),
        pltpu.VMEM((WIN + NBLK, D, L), F32),
        pltpu.VMEM((WIN + NBLK, D, L), F32),
        pltpu.VMEM((2, 8, 128, 256), F32),
        pltpu.VMEM((8, 2, 64, 128), U32),
        pltpu.VMEM((2, 2 * D, L), F32),
        pltpu.VMEM((2 * D, L), F32),
        pltpu.SemaphoreType.DMA((NSEM,)),
    ]
    out = pl.pallas_call(
        _kernel,
        out_shape=jax.ShapeDtypeStruct((S // 32, 32, D), BF16),
        in_specs=[any_spec] * 6,
        out_specs=any_spec,
        scratch_shapes=scratch,
        compiler_params=pltpu.CompilerParams(vmem_limit_bytes=120 * 1024 * 1024),
        name="hedgehog_dilated",
    )(x3, A_wqkv, wphi2, A_wo, B_wqkv, B_wo)
    return out.reshape(1, S, D)
```

```python
import math

import jax
import jax.numpy as jnp
from jax import lax
import jax.experimental.pallas as pl
import jax.experimental.pallas.tpu as pltpu

S = 2048
D = 1024
H = 32
DH = 32
NBLK = 16
L = 128
WIN = 8
HALO = WIN - 1
LOG2E = math.log2(math.e)
F32 = jnp.float32
BF16 = jnp.bfloat16
U32 = jnp.uint32
NT = (((1,), (1,)), ((), ()))

MC = 256
NCH = D // MC
GPC = MC // 128
PPC = MC // 64
CFG = dict(lag_q=1, lag_kv=2, only=None, ln_ways=2, ln_serial=True, ln_link=4, sub=256, sub_o=256, sub_b=256)

SEM_X = 0
SEM_PHI = 16
SEM_KV = 17
SEM_SET = 25
SEM_LATE = 33
NSEM = 34


def _mm(a, b):
    return jnp.dot(a, b, preferred_element_type=F32)


def _mm_nt(a, b):
    return lax.dot_general(a, b, NT, preferred_element_type=F32)


def _tree(op, xs):
    xs = list(xs)
    while len(xs) > 1:
        nxt = [op(xs[i], xs[i + 1]) for i in range(0, len(xs) - 1, 2)]
        if len(xs) % 2:
            nxt.append(xs[-1])
        xs = nxt
    return xs[0]


def _chain(op, xs, ways=4):
    acc = list(xs[:ways])
    for i, x in enumerate(xs[ways:]):
        acc[i % ways] = op(acc[i % ways], x)
    return _tree(op, acc)


def _rows(a, n=8):
    return [a[i * n:(i + 1) * n, :] for i in range(a.shape[0] // n)]


def _pack(a):
    return pltpu.bitcast(a.astype(BF16), U32)


def _unpk(a):
    return pltpu.bitcast(a, BF16)


def _pack_i(a, b):
    return pltpu.pack_elementwise([a, b], packed_dtype=BF16)


def _pack_split(a):
    r = _rows(a)
    return jnp.concatenate([_pack_i(r[2 * i], r[2 * i + 1]) for i in range(len(r) // 2)], axis=0)


def _unpack_split(p):
    out = []
    for x in _rows(p):
        out.append(pltpu.unpack_elementwise(x, index=0, packed_dtype=BF16, unpacked_dtype=F32))
        out.append(pltpu.unpack_elementwise(x, index=1, packed_dtype=BF16, unpacked_dtype=F32))
    return jnp.concatenate(out, axis=0)


def _fold2(op, xs):
    r = _tree(op, xs)
    r = op(r, pltpu.roll(r, 4, 0))
    return op(r, pltpu.roll(r, 2, 0))


def _phi_parts(p):
    ps = _rows(p)
    mx = _fold2(jnp.maximum, ps)
    mn = _fold2(jnp.minimum, ps)
    ep = [jnp.exp2(x - mx) for x in ps]
    en = [jnp.exp2(mn - x) for x in ps]
    sp = _fold2(jnp.add, ep)
    sn = _fold2(jnp.add, en)
    return ep, en, sp, sn


def _mult(x, m):
    return x if isinstance(x, int) else pl.multiple_of(x, m)


def _kernel(x_hbm, wa_hbm, wphi_hbm, woa_hbm, wb_hbm, wob_hbm, out_hbm,
            xio, wa_raw, woa_raw, wb_raw, wob_raw, wphi, pmat,
            wqaT, wkvaT, woaT, wqbT, wkvbT, wobT, xT, xn, kb, vb, kv_acc, kvm, zacc, zb, sems):

    x32 = x_hbm.bitcast(U32)
    out32 = out_hbm.bitcast(U32)

    def x_in(j):
        return pltpu.make_async_copy(x32.at[:, j, :], xio.at[j], sems.at[SEM_X + j])

    def x_out(j):
        return pltpu.make_async_copy(xio.at[j], out32.at[:, j, :], sems.at[SEM_X + j])

    def colcopy(src, dst, c0, n, sem):
        c0 = _mult(c0, 128)
        return pltpu.make_async_copy(src.at[:, pl.ds(c0, n)], dst.at[:, pl.ds(c0, n)], sems.at[sem])

    cp_phi = pltpu.make_async_copy(wphi_hbm, wphi, sems.at[SEM_PHI])
    cp_k = [colcopy(wa_hbm, wa_raw, D + ch * MC, MC, SEM_KV + 2 * ch) for ch in range(NCH)]
    cp_v = [colcopy(wa_hbm, wa_raw, 2 * D + ch * MC, MC, SEM_KV + 2 * ch + 1) for ch in range(NCH)]

    def w_set(g):
        return [colcopy(wa_hbm, wa_raw, g * 128, 128, SEM_SET + g),
                colcopy(woa_hbm, woa_raw, g * 128, 128, SEM_SET + g),
                colcopy(wb_hbm, wb_raw, D + g * 128, 128, SEM_SET + g),
                colcopy(wb_hbm, wb_raw, 2 * D + g * 128, 128, SEM_SET + g)]

    cp_late = [colcopy(wb_hbm, wb_raw, 0, D, SEM_LATE), colcopy(wob_hbm, wob_raw, 0, D, SEM_LATE)]

    order = [cp_phi, x_in(0), cp_k[0], x_in(1), cp_v[0], cp_k[1], cp_v[1], x_in(2), x_in(3)]
    for ch in range(2, NCH):
        order += [cp_k[ch], cp_v[ch]]
    for g in range(8):
        if g < 6:
            order += [x_in(4 + 2 * g), x_in(5 + 2 * g)]
        order += w_set(g)
    order += cp_late
    for c in order:
        c.start()

    def wait_all(cps):
        for c in cps:
            c.wait()

    def wload(ref, r0, n):
        return jnp.concatenate([_unpk(ref[c, r0 // 2:(r0 + n) // 2, :]) for c in range(8)], axis=1)

    def wstore(ref, g, val):
        off = _mult(g * 64, 64)
        for c in range(8):
            ref[c, pl.ds(off, 64), :] = _pack(val[:, c * L:(c + 1) * L])

    def wstore_split(ref, g, val):
        off = _mult(g * 64, 64)
        for c in range(8):
            ref[c, pl.ds(off, 64), :] = _pack(_unpack_split(pltpu.bitcast(val[:, c * L:(c + 1) * L], U32)))

    def wstore_perm(ref, g, val):
        for c in range(8):
            pk = _pack(val[:, c * L:(c + 1) * L])
            for h4 in range(4):
                ref[c, pl.ds(g * 64 + h4, 16, stride=4), :] = pk[h4 * 16:(h4 + 1) * 16, :]

    def cols(ref, g):
        return ref[:, pl.ds(_mult(g * 128, 128), 128)]

    class LN:
        def __init__(self, j):
            self.j = j
            self.piv = None
            self.s1 = []
            self.s2 = []

        def add(self, xt):
            if self.piv is None:
                self.piv = jnp.broadcast_to(xt[0:1, :], (8, L))
            d = [r - self.piv for r in _rows(xt)]
            if CFG["ln_serial"]:
                self.s1 = [_chain(jnp.add, self.s1 + d, 1)]
                self.s2 = [_chain(jnp.add, self.s2 + [x * x for x in d], 1)]
            else:
                self.s1.append(_chain(jnp.add, d, CFG["ln_ways"]))
                self.s2.append(_chain(jnp.add, [x * x for x in d], CFG["ln_ways"]))

        def finish(self):
            j = self.j
            m1 = jnp.sum(_tree(jnp.add, self.s1), axis=0, keepdims=True) * (1.0 / D)
            m2 = jnp.sum(_tree(jnp.add, self.s2), axis=0, keepdims=True) * (1.0 / D)
            var = jnp.maximum(m2 - m1 * m1, 0.0)
            rs = lax.rsqrt(var + 1e-5)
            mrs = jnp.broadcast_to((self.piv[0:1, :] + m1) * rs, (8, L))
            rs = jnp.broadcast_to(rs, (8, L))
            never = rs < 0.0
            link = CFG["ln_link"]
            for r in range(D // 16):
                pk = _pack_i(xT[j, r * 16:r * 16 + 8, :] * rs - mrs,
                             xT[j, r * 16 + 8:r * 16 + 16, :] * rs - mrs)
                xn[j, r * 8:(r + 1) * 8, :] = pk
                if link and r % link == link - 1:
                    rs = jnp.where(never, pltpu.bitcast(pk, F32), rs)

    def prep_x(src, dst):
        ln = LN(dst)
        for cc in range(8):
            xt = _unpack_split(pltpu.bitcast(_unpk(xio[src, :, cc * L:(cc + 1) * L]).T, U32))
            xT[dst, cc * 128:(cc + 1) * 128, :] = xt
            ln.add(xt)
        ln.finish()

    def fold(dst, g, slab):
        val = _mm_nt(_unpk(pmat[g]), cols(wa_raw, slab)) * LOG2E
        off = _mult(g * 64, 64)
        for c in range(8):
            dst[c, pl.ds(off, 64), :] = _pack_split(val[:, c * L:(c + 1) * L])

    def prep_set(g):
        wstore_split(woaT, g, cols(woa_raw, g).T)
        wstore_perm(wkvbT, g, cols(wb_raw, 8 + g).T)
        wstore(wkvbT, 8 + g, cols(wb_raw, 16 + g).T)

    def prep_late(g):
        wstore_perm(wqbT, g, cols(wb_raw, g).T)
        wstore_split(wobT, g, cols(wob_raw, g).T)

    def mmw(ref, r0, n, rhs, sub):
        return jnp.concatenate([_mm(wload(ref, r, sub), rhs()) for r in range(r0, r0 + n, sub)], axis=0)

    def proj(ref, r0, n, j, sub=None):
        return mmw(ref, r0, n, lambda: _unpk(xn[j]), sub or CFG["sub"])

    def emit(steps, lag):
        pend = []
        for main, late in steps:
            main()
            pend.append(late)
            if len(pend) > lag:
                f = pend.pop(0)
                if f is not None:
                    f()
        for f in pend:
            if f is not None:
                f()

    def a_kv(j, lay, last):
        steps = []
        for ch in range(NCH):
            st = {}

            def kstep(ch=ch, st=st):
                kp = proj(wkvaT, ch * MC, MC, j)
                st["phi"] = []
                for u in range(PPC):
                    t = ch * PPC + u
                    ep, en, sp, sn = _phi_parts(kp[u * 64:(u + 1) * 64, :])
                    r = 1.0 / (sp * sn)
                    rp = r * sn
                    rn = r * sp
                    phi = jnp.concatenate([e * rp for e in ep] + [e * rn for e in en], axis=0)
                    z = zacc[lay, t * 128:(t + 1) * 128, :] + phi
                    zacc[lay, t * 128:(t + 1) * 128, :] = z
                    if last:
                        zb[t * 128:(t + 1) * 128, :] = jnp.broadcast_to(
                            jnp.sum(z, axis=1, keepdims=True), (128, L))
                    st["phi"].append(phi.astype(BF16))

            def vstep(ch=ch, st=st):
                st["v"] = proj(wkvaT, D + ch * MC, MC, j)

            def mstep(ch=ch, st=st):
                for u in range(PPC):
                    t = ch * PPC + u
                    vg = st["v"][u * 64:(u + 1) * 64, :].astype(BF16)
                    acc = kv_acc[lay, t] + _mm_nt(vg, st["phi"][u])
                    kv_acc[lay, t] = acc
                    if last:
                        r = lax.broadcasted_iota(jnp.int32, (64, 128), 0)
                        c = lax.broadcasted_iota(jnp.int32, (64, 128), 1)
                        kvm[t] = _pack(jnp.where((r // 32) == (c % 2), acc, 0.0))

            steps.append((kstep, None))
            steps.append((vstep, mstep))
        return steps

    def a_q(j, outs):
        steps = []
        for ch in range(NCH):
            st = {}

            def qstep(ch=ch, st=st):
                qp = proj(wqaT, ch * MC, MC, j)
                st["phi"] = []
                for u in range(PPC):
                    t = ch * PPC + u
                    ep, en, sp, sn = _phi_parts(qp[u * 64:(u + 1) * 64, :])
                    zr = _rows(zb[t * 128:(t + 1) * 128, :])
                    dp = _fold2(jnp.add, [e * zz for e, zz in zip(ep, zr[:8])])
                    dn = _fold2(jnp.add, [e * zz for e, zz in zip(en, zr[8:])])
                    r = 1.0 / (dp * sn + dn * sp + 1e-6 * (sp * sn))
                    rp = r * sn
                    rn = r * sp
                    phi = jnp.concatenate([e * rp for e in ep] + [e * rn for e in en], axis=0)
                    st["phi"].append(phi.astype(BF16))

            def nstep(ch=ch, st=st):
                for u in range(PPC):
                    outs.append(_mm(_unpk(kvm[ch * PPC + u]), st["phi"][u]))

            steps.append((qstep, nstep))
        return steps

    def out_proj(wo, outs, j):
        steps = []
        ln = LN(j)
        st = {}
        for ch in range(NCH):
            def ostep(ch=ch):
                if ch == 0:
                    st["o"] = jnp.concatenate(outs, axis=0).astype(BF16)
                m0 = ch * MC
                xt = xT[j, m0:m0 + MC, :] + mmw(wo, m0, MC, lambda: st["o"], CFG["sub_o"])
                xT[j, m0:m0 + MC, :] = xt
                ln.add(xt)
                if ch == NCH - 1:
                    ln.finish()
            steps.append((ostep, None))
        return steps

    def b_kv(j, halo):
        steps = []
        for base, ref in ((0, kb), (D, vb)):
            for m0 in range(0, D, MC):
                def step(base=base, ref=ref, m0=m0):
                    p = proj(wkvbT, base + m0, MC, j, CFG["sub_b"])
                    ref[WIN + j, m0:m0 + MC, :] = p
                    if halo:
                        ref[j - WIN, m0:m0 + MC, :] = pltpu.roll(p, 2, 1)
                steps.append((step, None))
        return steps

    def b_q(j, outs):
        even = lax.broadcasted_iota(jnp.int32, (8, L), 0) % 2 == 0
        first = lax.broadcasted_iota(jnp.int32, (8, L), 1) < 2
        cs = DH ** -0.5
        steps = []
        for G in range(4):
            def step(G=G):
                q = proj(wqbT, G * 256, 256, j)
                halves = []
                for u in range(2):
                    acc = [None] * WIN
                    for r in range(16):
                        r0 = u * 128 + r * 8
                        qv = q[r0:r0 + 8, :]
                        for w in range(WIN):
                            t = qv * kb[WIN + j - w, G * 256 + r0:G * 256 + r0 + 8, :]
                            acc[w] = t if acc[w] is None else acc[w] + t
                    halves.append(acc)
                lg = []
                for w in range(WIN):
                    la, lb = halves[0][w], halves[1][w]
                    l = jnp.where(even, la + pltpu.roll(la, 7, 0), lb + pltpu.roll(lb, 1, 0))
                    l = l * cs
                    if w > 0:
                        l = jnp.where(jnp.logical_and(first, j < w), -1e9, l)
                    lg.append(l)
                mx = _tree(jnp.maximum, lg)
                ex = [jnp.exp(l - mx) for l in lg]
                rs = 1.0 / _tree(jnp.add, ex)
                at = [e * rs for e in ex]
                for hh in range(8):
                    h = G * 8 + hh
                    s = 2 * (hh % 4) + hh // 4
                    o = None
                    for w in range(WIN):
                        a = jnp.broadcast_to(at[w][s:s + 1, :], (DH, L))
                        t = a * vb[WIN + j - w, h * DH:(h + 1) * DH, :]
                        o = t if o is None else o + t
                    outs.append(o)
            steps.append((step, None))
        return steps

    def final_proj(outs, j):
        steps = []
        st = {}
        for ch in range(NCH):
            def ostep(ch=ch):
                if ch == 0:
                    st["o"] = jnp.concatenate(outs, axis=0).astype(BF16)
                m0 = ch * MC
                xt = xT[j, m0:m0 + MC, :] + mmw(wobT, m0, MC, lambda: st["o"], CFG["sub_o"])
                for u in range(GPC):
                    y = _unpk(_pack_split(xt[u * 128:(u + 1) * 128, :])).T
                    cc = ch * GPC + u
                    xio[j, :, cc * L:(cc + 1) * L] = pltpu.bitcast(y, U32)
            steps.append((ostep, None))
        return steps

    kv_acc[...] = jnp.zeros(kv_acc.shape, F32)
    zacc[...] = jnp.zeros(zacc.shape, F32)

    def unsplit(r):
        return (r // 16) * 16 + 2 * (r % 8) + (r // 8) % 2

    r128 = unsplit(lax.broadcasted_iota(jnp.int32, (128, 128), 0))
    c128 = lax.broadcasted_iota(jnp.int32, (128, 128), 1)
    same_head = (2 * (r128 // 64) + r128 % 2) == (c128 // 32)
    er = unsplit(lax.broadcasted_iota(jnp.int32, (128, 32), 0))
    ec = lax.broadcasted_iota(jnp.int32, (128, 32), 1)
    expand = jnp.where(((er % 64) // 2) == ec, 1.0, 0.0).astype(BF16)
    cp_phi.wait()
    for g in range(8):
        pg = _mm_nt(expand, wphi[g * 128:(g + 1) * 128, :])
        pmat[g] = _pack(jnp.where(same_head, pg, 0.0))

    only = CFG["only"] or (0, 1, 2, 3, 5)
    x_in(0).wait()
    prep_x(0, 0)
    sa = a_kv(0, 0, False)
    sb = a_kv(1, 0, False)
    pend = []
    for ch in range(NCH if 0 in only else 0):
        cp_k[ch].wait()
        if ch == 0:
            for u in range(GPC):
                fold(wkvaT, u, 8 + u)
            sa[0][0]()
            x_in(1).wait()
        cp_v[ch].wait()
        if ch == 2:
            x_in(2).wait()
            x_in(3).wait()
        if ch == 0:
            prep_x(1, 1)
        else:
            for u in range(GPC):
                fold(wkvaT, ch * GPC + u, 8 + ch * GPC + u)
        for u in range(GPC):
            wstore(wkvaT, 8 + ch * GPC + u, cols(wa_raw, 16 + ch * GPC + u).T)
        for f in pend:
            f()
        if ch >= 2:
            prep_x(ch, ch)
        if ch == 0:
            sa[1][0]()
            sb[0][0]()
        else:
            sa[2 * ch][0]()
            sb[2 * ch][0]()
            sa[2 * ch + 1][0]()
        sb[2 * ch + 1][0]()
        pend = [sa[2 * ch + 1][1], sb[2 * ch + 1][1]]
    for f in pend:
        f()

    def s1(i, c):
        j = 2 * i

        @pl.when(i < 7)
        def _():
            x_in(j + 2).wait()
            x_in(j + 3).wait()

        wait_all(w_set(i - 1))
        steps = a_kv(j, 0, False) + a_kv(j + 1, 0, True)
        steps.insert(14, (lambda: prep_set(i - 1), None))
        steps.insert(12, (lambda: prep_x(jnp.minimum(j + 3, NBLK - 1), j + 3), None))
        steps.insert(8, (lambda: prep_x(jnp.minimum(j + 2, NBLK - 1), j + 2), None))
        steps.insert(2, (lambda: fold(wqaT, i - 1, i - 1), None))
        emit(steps, CFG["lag_kv"])
        return c
    if 1 in only:
        lax.fori_loop(1, 8, s1, 0)
    wait_all(w_set(7))
    fold(wqaT, 7, 7)
    prep_set(7)
    wait_all(cp_late)

    def s2(i, c):
        js = [8 + i, i]
        outs = [[], []]
        steps = a_q(js[0], outs[0]) + a_q(js[1], outs[1])
        steps += out_proj(woaT, outs[0], js[0]) + out_proj(woaT, outs[1], js[1])
        steps += [(lambda: prep_late(i), None)]
        steps += b_kv(js[0], True) + b_kv(js[1], False)
        emit(steps, CFG["lag_q"])
        return c

    def s3(i, c):
        js = [2 * i, 2 * i + 1]
        outs = [[], []]
        steps = b_q(js[0], outs[0]) + b_q(js[1], outs[1])
        steps += out_proj(wobT, outs[0], js[0]) + out_proj(wobT, outs[1], js[1])
        steps += a_kv(js[0], 1, False) + a_kv(js[1], 1, True)
        emit(steps, CFG["lag_kv"])
        return c

    def s5(i, c):
        js = [2 * i, 2 * i + 1]
        outs = [[], []]
        steps = b_q(js[0], outs[0]) + b_q(js[1], outs[1])
        steps += final_proj(outs[0], js[0]) + final_proj(outs[1], js[1])
        emit(steps, 0)

        x_out(js[0]).start()
        x_out(js[1]).start()
        return c

    def layer_pair(l, c):
        if 2 in only:
            lax.fori_loop(0, 8, s2, 0)

        @pl.when(l == 0)
        def _():
            if 3 in only:
                lax.fori_loop(0, 8, s3, 0)

        @pl.when(l == 1)
        def _():
            if 5 in only:
                lax.fori_loop(0, 8, s5, 0)
        return c
    lax.fori_loop(0, 2, layer_pair, 0)

    for j in range(NBLK):
        x_out(j).wait()


@jax.jit
def pallas_interleave_layers__linear_kernel_hedgehog__sliding_local_dilated__prompt_kernel(
    A_x: jax.Array,
    A_wqkv: jax.Array,
    A_w_phi: jax.Array,
    A_wo: jax.Array,
    B_x: jax.Array,
    B_wqkv: jax.Array,
    B_wo: jax.Array,
):
    del B_x
    x3 = A_x.reshape(S // 32, 32, D)
    wphi2 = A_w_phi.reshape(H * DH, DH)
    any_spec = pl.BlockSpec(memory_space=pl.ANY)
    scratch = [
        pltpu.VMEM((NBLK, S // 32, D), U32),
        pltpu.VMEM((D, 3 * D), BF16),
        pltpu.VMEM((D, D), BF16),
        pltpu.VMEM((D, 3 * D), BF16),
        pltpu.VMEM((D, D), BF16),
        pltpu.VMEM((H * DH, DH), BF16),
        pltpu.VMEM((8, 64, 128), U32),
        pltpu.VMEM((8, D // 2, L), U32),
        pltpu.VMEM((8, D, L), U32),
        pltpu.VMEM((8, D // 2, L), U32),
        pltpu.VMEM((8, D // 2, L), U32),
        pltpu.VMEM((8, D, L), U32),
        pltpu.VMEM((8, D // 2, L), U32),
        pltpu.VMEM((NBLK + 2, D, L), F32),
        pltpu.VMEM((NBLK + 2, D // 2, L), U32),
        pltpu.VMEM((WIN + NBLK, D, L), F32),
        pltpu.VMEM((WIN + NBLK, D, L), F32),
        pltpu.VMEM((2, 16, 64, 128), F32),
        pltpu.VMEM((16, 32, 128), U32),
        pltpu.VMEM((2, 2 * D, L), F32),
        pltpu.VMEM((2 * D, L), F32),
        pltpu.SemaphoreType.DMA((NSEM,)),
    ]
    out = pl.pallas_call(
        _kernel,
        out_shape=jax.ShapeDtypeStruct((S // 32, 32, D), BF16),
        in_specs=[any_spec] * 6,
        out_specs=any_spec,
        scratch_shapes=scratch,
        compiler_params=pltpu.CompilerParams(vmem_limit_bytes=120 * 1024 * 1024),
        name="hedgehog_dilated",
    )(x3, A_wqkv, wphi2, A_wo, B_wqkv, B_wo)
    return out.reshape(1, S, D)
```

```python
import math

import jax
import jax.numpy as jnp
from jax import lax
import jax.experimental.pallas as pl
import jax.experimental.pallas.tpu as pltpu

S = 2048
D = 1024
H = 32
DH = 32
NBLK = 16
L = 128
WIN = 8
HALO = WIN - 1
LOG2E = math.log2(math.e)
F32 = jnp.float32
BF16 = jnp.bfloat16
U32 = jnp.uint32
NT = (((1,), (1,)), ((), ()))

MC = 256
NCH = D // MC
GPC = MC // 128
PPC = MC // 64
CFG = dict(lag_q=1, lag_kv=2, only=None, ln_ways=2, ln_serial=True, ln_link=4, sub=256, sub_o=256, sub_b=256)

SEM_X = 0
SEM_PHI = 16
SEM_KV = 17
SEM_SET = 25
SEM_LATE = 33
NSEM = 34


def _mm(a, b):
    return jnp.dot(a, b, preferred_element_type=F32)


def _mm_nt(a, b):
    return lax.dot_general(a, b, NT, preferred_element_type=F32)


def _tree(op, xs):
    xs = list(xs)
    while len(xs) > 1:
        nxt = [op(xs[i], xs[i + 1]) for i in range(0, len(xs) - 1, 2)]
        if len(xs) % 2:
            nxt.append(xs[-1])
        xs = nxt
    return xs[0]


def _chain(op, xs, ways=4):
    acc = list(xs[:ways])
    for i, x in enumerate(xs[ways:]):
        acc[i % ways] = op(acc[i % ways], x)
    return _tree(op, acc)


def _rows(a, n=8):
    return [a[i * n:(i + 1) * n, :] for i in range(a.shape[0] // n)]


def _pack(a):
    return pltpu.bitcast(a.astype(BF16), U32)


def _unpk(a):
    return pltpu.bitcast(a, BF16)


def _pack_i(a, b):
    return pltpu.pack_elementwise([a, b], packed_dtype=BF16)


def _pack_split(a):
    r = _rows(a)
    return jnp.concatenate([_pack_i(r[2 * i], r[2 * i + 1]) for i in range(len(r) // 2)], axis=0)


def _unpack_split(p):
    out = []
    for x in _rows(p):
        out.append(pltpu.unpack_elementwise(x, index=0, packed_dtype=BF16, unpacked_dtype=F32))
        out.append(pltpu.unpack_elementwise(x, index=1, packed_dtype=BF16, unpacked_dtype=F32))
    return jnp.concatenate(out, axis=0)


def _fold2(op, xs):
    r = _tree(op, xs)
    r = op(r, pltpu.roll(r, 4, 0))
    return op(r, pltpu.roll(r, 2, 0))


def _phi_parts(p):
    ps = _rows(p)
    mx = _fold2(jnp.maximum, ps)
    mn = _fold2(jnp.minimum, ps)
    ep = [jnp.exp2(x - mx) for x in ps]
    en = [jnp.exp2(mn - x) for x in ps]
    sp = _fold2(jnp.add, ep)
    sn = _fold2(jnp.add, en)
    return ep, en, sp, sn


def _mult(x, m):
    return x if isinstance(x, int) else pl.multiple_of(x, m)


def _kernel(x_hbm, wa_hbm, wphi_hbm, woa_hbm, wb_hbm, wob_hbm, out_hbm,
            xio, wa_raw, woa_raw, wb_raw, wob_raw, wphi, pmat,
            wqaT, wkvaT, woaT, wqbT, wkvbT, wobT, xT, xn, kb, vb, kv_acc, kvm, zacc, zb, phis, vs, os_, sems):

    x32 = x_hbm.bitcast(U32)
    out32 = out_hbm.bitcast(U32)

    def x_in(j):
        return pltpu.make_async_copy(x32.at[:, j, :], xio.at[j], sems.at[SEM_X + j])

    def x_out(j):
        return pltpu.make_async_copy(xio.at[j], out32.at[:, j, :], sems.at[SEM_X + j])

    def colcopy(src, dst, c0, n, sem):
        c0 = _mult(c0, 128)
        return pltpu.make_async_copy(src.at[:, pl.ds(c0, n)], dst.at[:, pl.ds(c0, n)], sems.at[sem])

    cp_phi = pltpu.make_async_copy(wphi_hbm, wphi, sems.at[SEM_PHI])
    cp_k = [colcopy(wa_hbm, wa_raw, D + ch * MC, MC, SEM_KV + 2 * ch) for ch in range(NCH)]
    cp_v = [colcopy(wa_hbm, wa_raw, 2 * D + ch * MC, MC, SEM_KV + 2 * ch + 1) for ch in range(NCH)]

    def w_set(g):
        return [colcopy(wa_hbm, wa_raw, g * 128, 128, SEM_SET + g),
                colcopy(woa_hbm, woa_raw, g * 128, 128, SEM_SET + g),
                colcopy(wb_hbm, wb_raw, D + g * 128, 128, SEM_SET + g),
                colcopy(wb_hbm, wb_raw, 2 * D + g * 128, 128, SEM_SET + g)]

    cp_late = [colcopy(wb_hbm, wb_raw, 0, D, SEM_LATE), colcopy(wob_hbm, wob_raw, 0, D, SEM_LATE)]

    order = [cp_phi, x_in(0), cp_k[0], x_in(1), cp_v[0], cp_k[1], cp_v[1], x_in(2), x_in(3)]
    for ch in range(2, NCH):
        order += [cp_k[ch], cp_v[ch]]
    for g in range(8):
        if g < 6:
            order += [x_in(4 + 2 * g), x_in(5 + 2 * g)]
        order += w_set(g)
    order += cp_late
    for c in order:
        c.start()

    def wait_all(cps):
        for c in cps:
            c.wait()

    def wload(ref, r0, n):
        return jnp.concatenate([_unpk(ref[c, r0 // 2:(r0 + n) // 2, :]) for c in range(8)], axis=1)

    def wstore(ref, g, val):
        off = _mult(g * 64, 64)
        for c in range(8):
            ref[c, pl.ds(off, 64), :] = _pack(val[:, c * L:(c + 1) * L])

    def wstore_split(ref, g, val):
        off = _mult(g * 64, 64)
        for c in range(8):
            ref[c, pl.ds(off, 64), :] = _pack(_unpack_split(pltpu.bitcast(val[:, c * L:(c + 1) * L], U32)))

    def wstore_shuf(ref, g, val):
        off = _mult(g * 64, 64)
        for c in range(8):
            ref[c, pl.ds(off, 64), :] = _pack_split(val[:, c * L:(c + 1) * L].astype(F32))

    def wstore_perm(ref, g, val):
        for c in range(8):
            pk = _pack(val[:, c * L:(c + 1) * L])
            for h4 in range(4):
                ref[c, pl.ds(g * 64 + h4, 16, stride=4), :] = pk[h4 * 16:(h4 + 1) * 16, :]

    def cols(ref, g):
        return ref[:, pl.ds(_mult(g * 128, 128), 128)]

    class LN:
        def __init__(self, j):
            self.j = j
            self.piv = None
            self.s1 = []
            self.s2 = []

        def add(self, xt):
            if self.piv is None:
                self.piv = jnp.broadcast_to(xt[0:1, :], (8, L))
            d = [r - self.piv for r in _rows(xt)]
            if CFG["ln_serial"]:
                self.s1 = [_chain(jnp.add, self.s1 + d, 1)]
                self.s2 = [_chain(jnp.add, self.s2 + [x * x for x in d], 1)]
            else:
                self.s1.append(_chain(jnp.add, d, CFG["ln_ways"]))
                self.s2.append(_chain(jnp.add, [x * x for x in d], CFG["ln_ways"]))

        def finish(self):
            j = self.j
            m1 = jnp.sum(_tree(jnp.add, self.s1), axis=0, keepdims=True) * (1.0 / D)
            m2 = jnp.sum(_tree(jnp.add, self.s2), axis=0, keepdims=True) * (1.0 / D)
            var = jnp.maximum(m2 - m1 * m1, 0.0)
            rs = lax.rsqrt(var + 1e-5)
            mrs = jnp.broadcast_to((self.piv[0:1, :] + m1) * rs, (8, L))
            rs = jnp.broadcast_to(rs, (8, L))
            never = rs < 0.0
            link = CFG["ln_link"]
            for r in range(D // 16):
                pk = _pack_i(xT[j, r * 16:r * 16 + 8, :] * rs - mrs,
                             xT[j, r * 16 + 8:r * 16 + 16, :] * rs - mrs)
                xn[j, r * 8:(r + 1) * 8, :] = pk
                if link and r % link == link - 1:
                    rs = jnp.where(never, pltpu.bitcast(pk, F32), rs)

    def prep_x(src, dst):
        ln = LN(dst)
        for cc in range(8):
            xt = _unpack_split(pltpu.bitcast(_unpk(xio[src, :, cc * L:(cc + 1) * L]).T, U32))
            xT[dst, cc * 128:(cc + 1) * 128, :] = xt
            ln.add(xt)
        ln.finish()

    def fold(dst, g, slab):
        val = _mm_nt(_unpk(pmat[g]), cols(wa_raw, slab)) * LOG2E
        off = _mult(g * 64, 64)
        for c in range(8):
            dst[c, pl.ds(off, 64), :] = _pack_split(val[:, c * L:(c + 1) * L])

    def prep_set(g):
        wstore_split(woaT, g, cols(woa_raw, g).T)
        wstore_perm(wkvbT, g, cols(wb_raw, 8 + g).T)
        wstore_split(wkvbT, 8 + g, cols(wb_raw, 16 + g).T)

    def prep_late(g):
        wstore_perm(wqbT, g, cols(wb_raw, g).T)
        wstore_split(wobT, g, cols(wob_raw, g).T)

    def mmw(ref, r0, n, rhs, sub):
        return jnp.concatenate([_mm(wload(ref, r, sub), rhs()) for r in range(r0, r0 + n, sub)], axis=0)

    def proj(ref, r0, n, j, sub=None):
        return mmw(ref, r0, n, lambda: _unpk(xn[j]), sub or CFG["sub"])

    def emit(steps, lag):
        pend = []
        for main, late in steps:
            main()
            pend.append(late)
            if len(pend) > lag:
                f = pend.pop(0)
                if f is not None:
                    f()
        for f in pend:
            if f is not None:
                f()

    def a_kv(j, sl, lay, last):
        steps = []
        for ch in range(NCH):
            def kstep(ch=ch):
                kp = proj(wkvaT, ch * MC, MC, j)
                for u in range(PPC):
                    t = ch * PPC + u
                    ep, en, sp, sn = _phi_parts(kp[u * 64:(u + 1) * 64, :])
                    r = 1.0 / (sp * sn)
                    rp = r * sn
                    rn = r * sp
                    phi = jnp.concatenate([e * rp for e in ep] + [e * rn for e in en], axis=0)
                    phis[sl, t * 64:(t + 1) * 64, :] = _pack_split(phi)
                    z = zacc[lay, t * 128:(t + 1) * 128, :] + phi
                    zacc[lay, t * 128:(t + 1) * 128, :] = z
                    if last:
                        zb[t * 128:(t + 1) * 128, :] = jnp.broadcast_to(
                            jnp.sum(z, axis=1, keepdims=True), (128, L))

            def vstep(ch=ch):
                vs[sl, ch * (MC // 2):(ch + 1) * (MC // 2), :] = _pack_split(proj(wkvaT, D + ch * MC, MC, j))

            def mstep(ch=ch):
                for u in range(PPC):
                    t = ch * PPC + u
                    acc = kv_acc[lay, t] + _mm_nt(_unpk(vs[sl, t * 32:(t + 1) * 32, :]),
                                                  _unpk(phis[sl, t * 64:(t + 1) * 64, :]))
                    kv_acc[lay, t] = acc
                    if last:
                        r = lax.broadcasted_iota(jnp.int32, (64, 128), 0)
                        c = lax.broadcasted_iota(jnp.int32, (64, 128), 1)
                        kvm[t] = _pack_split(jnp.where((r // 32) == ((c // 2) % 2), acc, 0.0))

            steps.append((kstep, None))
            steps.append((vstep, mstep))
        return steps

    def a_q(j, sl):
        steps = []
        for ch in range(NCH):
            def qstep(ch=ch):
                qp = proj(wqaT, ch * MC, MC, j)
                for u in range(PPC):
                    t = ch * PPC + u
                    ep, en, sp, sn = _phi_parts(qp[u * 64:(u + 1) * 64, :])
                    zr = _rows(zb[t * 128:(t + 1) * 128, :])
                    dp = _fold2(jnp.add, [e * zz for e, zz in zip(ep, zr[:8])])
                    dn = _fold2(jnp.add, [e * zz for e, zz in zip(en, zr[8:])])
                    r = 1.0 / (dp * sn + dn * sp + 1e-6 * (sp * sn))
                    rp = r * sn
                    rn = r * sp
                    phi = jnp.concatenate([e * rp for e in ep] + [e * rn for e in en], axis=0)
                    phis[sl, t * 64:(t + 1) * 64, :] = _pack_split(phi)

            def nstep(ch=ch):
                for u in range(PPC):
                    t = ch * PPC + u
                    o = _mm(_unpk(kvm[t]), _unpk(phis[sl, t * 64:(t + 1) * 64, :]))
                    os_[sl, t * 32:(t + 1) * 32, :] = _pack_split(o)

            steps.append((qstep, nstep))
        return steps

    def out_proj(wo, j, sl):
        steps = []
        ln = LN(j)
        for ch in range(NCH):
            def ostep(ch=ch):
                m0 = ch * MC
                xt = xT[j, m0:m0 + MC, :] + mmw(wo, m0, MC, lambda: _unpk(os_[sl]), CFG["sub_o"])
                xT[j, m0:m0 + MC, :] = xt
                ln.add(xt)
                if ch == NCH - 1:
                    ln.finish()
            steps.append((ostep, None))
        return steps

    def b_kv(j, halo):
        steps = []
        for base, ref in ((0, kb), (D, vb)):
            for m0 in range(0, D, MC):
                def step(base=base, ref=ref, m0=m0):
                    p = proj(wkvbT, base + m0, MC, j, CFG["sub_b"])
                    ref[WIN + j, m0:m0 + MC, :] = p
                    if halo:
                        ref[j - WIN, m0:m0 + MC, :] = pltpu.roll(p, 2, 1)
                steps.append((step, None))
        return steps

    def b_q(j, sl):
        even = lax.broadcasted_iota(jnp.int32, (8, L), 0) % 2 == 0
        first = lax.broadcasted_iota(jnp.int32, (8, L), 1) < 2
        cs = DH ** -0.5
        steps = []
        for G in range(4):
            def step(G=G):
                q = proj(wqbT, G * 256, 256, j)
                halves = []
                for u in range(2):
                    acc = [None] * WIN
                    for r in range(16):
                        r0 = u * 128 + r * 8
                        qv = q[r0:r0 + 8, :]
                        for w in range(WIN):
                            t = qv * kb[WIN + j - w, G * 256 + r0:G * 256 + r0 + 8, :]
                            acc[w] = t if acc[w] is None else acc[w] + t
                    halves.append(acc)
                lg = []
                for w in range(WIN):
                    la, lb = halves[0][w], halves[1][w]
                    l = jnp.where(even, la + pltpu.roll(la, 7, 0), lb + pltpu.roll(lb, 1, 0))
                    l = l * cs
                    if w > 0:
                        l = jnp.where(jnp.logical_and(first, j < w), -1e9, l)
                    lg.append(l)
                mx = _tree(jnp.maximum, lg)
                ex = [jnp.exp(l - mx) for l in lg]
                rs = 1.0 / _tree(jnp.add, ex)
                at = [e * rs for e in ex]
                for hh in range(8):
                    h = G * 8 + hh
                    s = 2 * (hh % 4) + hh // 4
                    o = None
                    for w in range(WIN):
                        a = jnp.broadcast_to(at[w][s:s + 1, :], (DH, L))
                        t = a * vb[WIN + j - w, h * DH:(h + 1) * DH, :]
                        o = t if o is None else o + t
                    os_[sl, h * 16:(h + 1) * 16, :] = _pack_split(o)
            steps.append((step, None))
        return steps

    def final_proj(j, sl):
        steps = []
        for ch in range(NCH):
            def ostep(ch=ch):
                m0 = ch * MC
                xt = xT[j, m0:m0 + MC, :] + mmw(wobT, m0, MC, lambda: _unpk(os_[sl]), CFG["sub_o"])
                for u in range(GPC):
                    y = _unpk(_pack_split(xt[u * 128:(u + 1) * 128, :])).T
                    cc = ch * GPC + u
                    xio[j, :, cc * L:(cc + 1) * L] = pltpu.bitcast(y, U32)
            steps.append((ostep, None))
        return steps

    kv_acc[...] = jnp.zeros(kv_acc.shape, F32)
    zacc[...] = jnp.zeros(zacc.shape, F32)

    def unsplit(r):
        return (r // 16) * 16 + 2 * (r % 8) + (r // 8) % 2

    r128 = unsplit(lax.broadcasted_iota(jnp.int32, (128, 128), 0))
    c128 = lax.broadcasted_iota(jnp.int32, (128, 128), 1)
    same_head = (2 * (r128 // 64) + r128 % 2) == (c128 // 32)
    er = unsplit(lax.broadcasted_iota(jnp.int32, (128, 32), 0))
    ec = lax.broadcasted_iota(jnp.int32, (128, 32), 1)
    expand = jnp.where(((er % 64) // 2) == ec, 1.0, 0.0).astype(BF16)
    cp_phi.wait()
    for g in range(8):
        pg = _mm_nt(expand, wphi[g * 128:(g + 1) * 128, :])
        pmat[g] = _pack(jnp.where(same_head, pg, 0.0))

    only = CFG["only"] or (0, 1, 2, 3, 5)
    x_in(0).wait()
    prep_x(0, 0)
    sa = a_kv(0, 0, 0, False)
    sb = a_kv(1, 1, 0, False)
    pend = []
    for ch in range(NCH if 0 in only else 0):
        cp_k[ch].wait()
        if ch == 0:
            for u in range(GPC):
                fold(wkvaT, u, 8 + u)
            sa[0][0]()
            x_in(1).wait()
        cp_v[ch].wait()
        if ch == 2:
            x_in(2).wait()
            x_in(3).wait()
        if ch == 0:
            prep_x(1, 1)
        else:
            for u in range(GPC):
                fold(wkvaT, ch * GPC + u, 8 + ch * GPC + u)
        for u in range(GPC):
            wstore_shuf(wkvaT, 8 + ch * GPC + u, cols(wa_raw, 16 + ch * GPC + u).T)
        for f in pend:
            f()
        if ch >= 2:
            prep_x(ch, ch)
        if ch == 0:
            sa[1][0]()
            sb[0][0]()
        else:
            sa[2 * ch][0]()
            sb[2 * ch][0]()
            sa[2 * ch + 1][0]()
        sb[2 * ch + 1][0]()
        pend = [sa[2 * ch + 1][1], sb[2 * ch + 1][1]]
    for f in pend:
        f()

    def s1(i, c):
        j = 2 * i

        @pl.when(i < 7)
        def _():
            x_in(j + 2).wait()
            x_in(j + 3).wait()

        wait_all(w_set(i - 1))
        steps = a_kv(j, 0, 0, False) + a_kv(j + 1, 1, 0, True)
        steps.insert(14, (lambda: prep_set(i - 1), None))
        steps.insert(12, (lambda: prep_x(jnp.minimum(j + 3, NBLK - 1), j + 3), None))
        steps.insert(8, (lambda: prep_x(jnp.minimum(j + 2, NBLK - 1), j + 2), None))
        steps.insert(2, (lambda: fold(wqaT, i - 1, i - 1), None))
        emit(steps, CFG["lag_kv"])
        return c
    if 1 in only:
        lax.fori_loop(1, 8, s1, 0)
    wait_all(w_set(7))
    fold(wqaT, 7, 7)
    prep_set(7)
    wait_all(cp_late)

    def s2(i, c):
        js = [8 + i, i]
        steps = a_q(js[0], 0) + a_q(js[1], 1)
        steps += out_proj(woaT, js[0], 0) + out_proj(woaT, js[1], 1)
        steps += [(lambda: prep_late(i), None)]
        steps += b_kv(js[0], True) + b_kv(js[1], False)
        emit(steps, CFG["lag_q"])
        return c

    def s3(i, c):
        js = [2 * i, 2 * i + 1]
        steps = b_q(js[0], 0) + b_q(js[1], 1)
        steps += out_proj(wobT, js[0], 0) + out_proj(wobT, js[1], 1)
        steps += a_kv(js[0], 0, 1, False) + a_kv(js[1], 1, 1, True)
        emit(steps, CFG["lag_kv"])
        return c

    def s5(i, c):
        js = [2 * i, 2 * i + 1]
        steps = b_q(js[0], 0) + b_q(js[1], 1)
        steps += final_proj(js[0], 0) + final_proj(js[1], 1)
        emit(steps, 0)

        x_out(js[0]).start()
        x_out(js[1]).start()
        return c

    def layer_pair(l, c):
        if 2 in only:
            lax.fori_loop(0, 8, s2, 0)

        @pl.when(l == 0)
        def _():
            if 3 in only:
                lax.fori_loop(0, 8, s3, 0)

        @pl.when(l == 1)
        def _():
            if 5 in only:
                lax.fori_loop(0, 8, s5, 0)
        return c
    lax.fori_loop(0, 2, layer_pair, 0)

    for j in range(NBLK):
        x_out(j).wait()


@jax.jit
def pallas_interleave_layers__linear_kernel_hedgehog__sliding_local_dilated__prompt_kernel(
    A_x: jax.Array,
    A_wqkv: jax.Array,
    A_w_phi: jax.Array,
    A_wo: jax.Array,
    B_x: jax.Array,
    B_wqkv: jax.Array,
    B_wo: jax.Array,
):
    del B_x
    x3 = A_x.reshape(S // 32, 32, D)
    wphi2 = A_w_phi.reshape(H * DH, DH)
    any_spec = pl.BlockSpec(memory_space=pl.ANY)
    scratch = [
        pltpu.VMEM((NBLK, S // 32, D), U32),
        pltpu.VMEM((D, 3 * D), BF16),
        pltpu.VMEM((D, D), BF16),
        pltpu.VMEM((D, 3 * D), BF16),
        pltpu.VMEM((D, D), BF16),
        pltpu.VMEM((H * DH, DH), BF16),
        pltpu.VMEM((8, 64, 128), U32),
        pltpu.VMEM((8, D // 2, L), U32),
        pltpu.VMEM((8, D, L), U32),
        pltpu.VMEM((8, D // 2, L), U32),
        pltpu.VMEM((8, D // 2, L), U32),
        pltpu.VMEM((8, D, L), U32),
        pltpu.VMEM((8, D // 2, L), U32),
        pltpu.VMEM((NBLK + 2, D, L), F32),
        pltpu.VMEM((NBLK + 2, D // 2, L), U32),
        pltpu.VMEM((WIN + NBLK, D, L), F32),
        pltpu.VMEM((WIN + NBLK, D, L), F32),
        pltpu.VMEM((2, 16, 64, 128), F32),
        pltpu.VMEM((16, 32, 128), U32),
        pltpu.VMEM((2, 2 * D, L), F32),
        pltpu.VMEM((2 * D, L), F32),
        pltpu.VMEM((2, D, L), U32),
        pltpu.VMEM((2, D // 2, L), U32),
        pltpu.VMEM((2, D // 2, L), U32),
        pltpu.SemaphoreType.DMA((NSEM,)),
    ]
    out = pl.pallas_call(
        _kernel,
        out_shape=jax.ShapeDtypeStruct((S // 32, 32, D), BF16),
        in_specs=[any_spec] * 6,
        out_specs=any_spec,
        scratch_shapes=scratch,
        compiler_params=pltpu.CompilerParams(vmem_limit_bytes=120 * 1024 * 1024),
        name="hedgehog_dilated",
    )(x3, A_wqkv, wphi2, A_wo, B_wqkv, B_wo)
    return out.reshape(1, S, D)
```

```python
import math

import jax
import jax.numpy as jnp
from jax import lax
import jax.experimental.pallas as pl
import jax.experimental.pallas.tpu as pltpu

S = 2048
D = 1024
H = 32
DH = 32
NBLK = 16
L = 128
WIN = 8
HALO = WIN - 1
LOG2E = math.log2(math.e)
F32 = jnp.float32
BF16 = jnp.bfloat16
U32 = jnp.uint32
NT = (((1,), (1,)), ((), ()))

MC = 256
NCH = D // MC
GPC = MC // 128
PPC = MC // 64
CFG = dict(vk=False, link3=4, lag_q=1, lag_kv=2, only=None, ln_link=4, ln_rev=False, sub=256, sub_o=256, sub_b=256,
           op_acc=True, op_phi=False, op_v=False, op_o=False, op_xt=False, op_xn=False,
           fin_z=True, fin_kv=True, sub_q=128, sub_k=256, sub_v=256, arecip=False, dbg=0, att_dl=0, pv_link=0, pv_slow=0, bar3=13, ln_defer=True, side=2)

SEM_X = 0
SEM_PHI = 16
SEM_KV = 17
SEM_SET = 25
SEM_LATE = 33
NSEM = 34


def _mm(a, b):
    return jnp.dot(a, b, preferred_element_type=F32)


def _mm_nt(a, b):
    return lax.dot_general(a, b, NT, preferred_element_type=F32)


def _tree(op, xs):
    xs = list(xs)
    while len(xs) > 1:
        nxt = [op(xs[i], xs[i + 1]) for i in range(0, len(xs) - 1, 2)]
        if len(xs) % 2:
            nxt.append(xs[-1])
        xs = nxt
    return xs[0]


def _chain(op, xs, ways=4):
    acc = list(xs[:ways])
    for i, x in enumerate(xs[ways:]):
        acc[i % ways] = op(acc[i % ways], x)
    return _tree(op, acc)


def _rows(a, n=8):
    return [a[i * n:(i + 1) * n, :] for i in range(a.shape[0] // n)]


def _pack(a):
    return pltpu.bitcast(a.astype(BF16), U32)


def _unpk(a):
    return pltpu.bitcast(a, BF16)


def _pack_i(a, b):
    return pltpu.pack_elementwise([a, b], packed_dtype=BF16)


def _pack_split(a):
    r = _rows(a)
    return jnp.concatenate([_pack_i(r[2 * i], r[2 * i + 1]) for i in range(len(r) // 2)], axis=0)


def _unpack_split(p):
    out = []
    for x in _rows(p):
        out.append(pltpu.unpack_elementwise(x, index=0, packed_dtype=BF16, unpacked_dtype=F32))
        out.append(pltpu.unpack_elementwise(x, index=1, packed_dtype=BF16, unpacked_dtype=F32))
    return jnp.concatenate(out, axis=0)


def _fold2(op, xs):
    r = _tree(op, xs)
    r = op(r, pltpu.roll(r, 4, 0))
    return op(r, pltpu.roll(r, 2, 0))


def _phi_parts(p):
    ps = _rows(p)
    mx = _fold2(jnp.maximum, ps)
    mn = _fold2(jnp.minimum, ps)
    ep = [jnp.exp2(x - mx) for x in ps]
    en = [jnp.exp2(mn - x) for x in ps]
    sp = _fold2(jnp.add, ep)
    sn = _fold2(jnp.add, en)
    return ep, en, sp, sn


def _recip(x):
    if not CFG["arecip"]:
        return 1.0 / x
    r = pl.reciprocal(x, approx=True)
    return r * (2.0 - x * r)


def _mult(x, m):
    return x if isinstance(x, int) else pl.multiple_of(x, m)


def _kernel(x_hbm, wa_hbm, wphi_hbm, woa_hbm, wb_hbm, wob_hbm, out_hbm,
            xio, wa_raw, woa_raw, wb_raw, wob_raw, wphi, pmat,
            wqaT, wkvaT, woaT, wqbT, wkvbT, wobT, kb, vb, kv_acc, kvm, zacc, zb, sems, bsem, *rest):
    xT, xn, os_ = rest[0:2], rest[2:4], rest[4:6]
    phis = [rest[6:6 + NCH], rest[6 + NCH:6 + 2 * NCH]]
    vs = [rest[6 + 2 * NCH:6 + 3 * NCH], rest[6 + 3 * NCH:6 + 4 * NCH]]

    class Blk:
        def __init__(self, hf, k, opaque=True):
            self.hf, self.k = hf, k
            self.j = 8 * (1 - hf) + k
            self.zr = 0 if (isinstance(k, int) or not opaque) else k // 64

        def z(self, key):
            return self.zr if CFG[key] else 0

    x32 = x_hbm.bitcast(U32)
    out32 = out_hbm.bitcast(U32)

    def x_in(j):
        return pltpu.make_async_copy(x32.at[:, j, :], xio.at[j], sems.at[SEM_X + j])

    def x_out(j):
        return pltpu.make_async_copy(xio.at[j], out32.at[:, j, :], sems.at[SEM_X + j])

    def colcopy(src, dst, c0, n, sem):
        c0 = _mult(c0, 128)
        return pltpu.make_async_copy(src.at[:, pl.ds(c0, n)], dst.at[:, pl.ds(c0, n)], sems.at[sem])

    cp_phi = pltpu.make_async_copy(wphi_hbm, wphi, sems.at[SEM_PHI])
    cp_k = [colcopy(wa_hbm, wa_raw, D + ch * MC, MC, SEM_KV + 2 * ch) for ch in range(NCH)]
    cp_v = [colcopy(wa_hbm, wa_raw, 2 * D + ch * MC, MC, SEM_KV + 2 * ch + 1) for ch in range(NCH)]

    def w_set(g):
        return [colcopy(wa_hbm, wa_raw, g * 128, 128, SEM_SET + g),
                colcopy(woa_hbm, woa_raw, g * 128, 128, SEM_SET + g),
                colcopy(wb_hbm, wb_raw, D + g * 128, 128, SEM_SET + g),
                colcopy(wb_hbm, wb_raw, 2 * D + g * 128, 128, SEM_SET + g)]

    cp_late = [colcopy(wb_hbm, wb_raw, 0, D, SEM_LATE), colcopy(wob_hbm, wob_raw, 0, D, SEM_LATE)]

    order = [cp_phi, x_in(8), cp_k[0], x_in(0), cp_v[0], cp_k[1], cp_v[1], x_in(9), x_in(1)]
    for ch in range(2, NCH):
        order += [cp_k[ch], cp_v[ch]]
    for g in range(8):
        if g < 6:
            order += [x_in(10 + g), x_in(2 + g)]
        order += w_set(g)
    order += cp_late
    for c in order:
        c.start()

    def wait_all(cps):
        for c in cps:
            c.wait()

    deps = []

    def wload(ref, r0, n):
        parts = [ref[c, r0 // 2:(r0 + n) // 2, :] for c in range(8)]
        while deps:
            never, val = deps.pop()
            head = jnp.where(never, val, parts[0][0:8, :])
            parts[0] = jnp.concatenate([head, parts[0][8:, :]], axis=0)
        return jnp.concatenate([_unpk(x) for x in parts], axis=1)

    class Side:
        never = None
        hist = []

    def tr(x):
        w = CFG["side"]
        if Side.never is not None and w and len(Side.hist) >= w:
            x = jnp.concatenate([jnp.where(Side.never, Side.hist[-w], x[0:8, :]), x[8:, :]], axis=0)
        y = pltpu.bitcast(_unpk(x).T, U32)
        Side.hist.append(y[56:64, :])
        return y

    def side_begin(b):
        Side.never = None if b is None else jnp.full((8, L), b.zr, jnp.int32) > 0
        Side.hist = []

    def wtile(raw, slab, c):
        return tr(pltpu.bitcast(raw[c * 128:(c + 1) * 128, pl.ds(_mult(slab * 128, 128), 128)], U32))

    def wstore_split(ref, g, raw, slab):
        off = _mult(g * 64, 64)
        for c in range(8):
            ref[c, pl.ds(off, 64), :] = _pack(_unpack_split(wtile(raw, slab, c)))

    def wstore_shuf(ref, g, raw, slab):
        off = _mult(g * 64, 64)
        for c in range(8):
            ref[c, pl.ds(off, 64), :] = _pack_split(_unpk(wtile(raw, slab, c)).astype(F32))

    def wstore_perm(ref, g, raw, slab):
        for c in range(8):
            pk = wtile(raw, slab, c)
            for h4 in range(4):
                ref[c, pl.ds(g * 64 + h4, 16, stride=4), :] = pk[h4 * 16:(h4 + 1) * 16, :]

    def cols(ref, g):
        return ref[:, pl.ds(_mult(g * 128, 128), 128)]

    class LN:
        def __init__(self, b, link=None):
            self.b = b
            self.link = CFG["ln_link"] if link is None else link
            self.piv = None
            self.s1 = []
            self.s2 = []

        def add(self, xt):
            if self.piv is None:
                self.piv = jnp.broadcast_to(xt[0:1, :], (8, L))
            d = [r - self.piv for r in _rows(xt)]
            self.s1 = [_chain(jnp.add, self.s1 + d, 1)]
            self.s2 = [_chain(jnp.add, self.s2 + [x * x for x in d], 1)]

        def finish(self):
            b = self.b
            m1 = jnp.sum(self.s1[0], axis=0, keepdims=True) * (1.0 / D)
            m2 = jnp.sum(self.s2[0], axis=0, keepdims=True) * (1.0 / D)
            var = jnp.maximum(m2 - m1 * m1, 0.0)
            rs = lax.rsqrt(var + 1e-5)
            mrs = jnp.broadcast_to((self.piv[0:1, :] + m1) * rs, (8, L))
            rs = jnp.broadcast_to(rs, (8, L))
            never = rs < 0.0
            link = self.link
            kk = b.k + b.z("op_xt")
            rng = list(range(D // 16))
            if CFG["ln_rev"]:
                rng = rng[::-1]
            for n, r in enumerate(rng):
                pk = _pack_i(xT[b.hf][kk, r * 16:r * 16 + 8, :] * rs - mrs,
                             xT[b.hf][kk, r * 16 + 8:r * 16 + 16, :] * rs - mrs)
                xn[b.hf][b.k, r * 8:(r + 1) * 8, :] = pk
                if link and n % link == link - 1:
                    rs = jnp.where(never, pltpu.bitcast(pk, F32), rs)

    def prep_x(src, b):
        ln = LN(b)
        for cc in range(8):
            xt = _unpack_split(tr(xio[src, :, cc * L:(cc + 1) * L]))
            xT[b.hf][b.k, cc * 128:(cc + 1) * 128, :] = xt
            ln.add(xt)
        ln.finish()

    def fold(dst, g, slab):
        val = _mm_nt(_unpk(pmat[g]), cols(wa_raw, slab)) * LOG2E
        off = _mult(g * 64, 64)
        for c in range(8):
            dst[c, pl.ds(off, 64), :] = _pack_split(val[:, c * L:(c + 1) * L])

    def prep_set(g):
        wstore_split(woaT, g, woa_raw, g)
        wstore_perm(wkvbT, g, wb_raw, 8 + g)
        wstore_split(wkvbT, 8 + g, wb_raw, 16 + g)

    def prep_late(g):
        wstore_perm(wqbT, g, wb_raw, g)
        wstore_split(wobT, g, wob_raw, g)

    def mmw(ref, r0, n, rhs, sub):
        return jnp.concatenate([_mm(wload(ref, r, sub), rhs()) for r in range(r0, r0 + n, sub)], axis=0)

    def proj(ref, r0, n, b, sub=None, fresh=False):
        kk = b.k + b.z("op_xn") if fresh else b.k
        return mmw(ref, r0, n, lambda: _unpk(xn[b.hf][kk]), sub or CFG["sub"])

    def emit(steps, lag):
        pend = []
        for n, (main, late) in enumerate(steps):
            main()
            if late is not None:
                pend.append((n + (CFG["att_dl"] if late.__name__ == "dl" else lag), late))
            for due, f in sorted(pend, key=lambda e: e[0]):
                if due <= n:
                    f()
            pend = [e for e in pend if e[0] > n]
        for due, f in sorted(pend, key=lambda e: e[0]):
            f()
        deps.clear()

    def kv_finish(t, acc):
        r = lax.broadcasted_iota(jnp.int32, (64, 128), 0)
        c = lax.broadcasted_iota(jnp.int32, (64, 128), 1)
        kvm[t] = _pack_split(jnp.where((r // 32) == ((c // 2) % 2), acc, 0.0))

    def a_finish(lay):
        if not CFG["fin_z"]:
            zb[...] = jnp.broadcast_to(jnp.sum(zacc[lay], axis=1, keepdims=True), zb.shape)
        if not CFG["fin_kv"]:
            for t in range(16):
                kv_finish(t, kv_acc[lay, t])

    def a_kv(b, lay, last, fresh, vk=False):
        steps = []
        la = lay + b.z("op_acc") if last else lay
        for ch in range(NCH):
            def kstep(ch=ch):
                kp = proj(wkvaT, ch * MC, MC, b, CFG["sub_k"], fresh=fresh)
                for u in range(PPC):
                    t = ch * PPC + u
                    ep, en, sp, sn = _phi_parts(kp[u * 64:(u + 1) * 64, :])
                    r = _recip(sp * sn)
                    rp = r * sn
                    rn = r * sp
                    phi = jnp.concatenate([e * rp for e in ep] + [e * rn for e in en], axis=0)
                    phis[b.hf][ch][0, u * 64:(u + 1) * 64, :] = _pack_split(phi)
                    z = zacc[la, t * 128:(t + 1) * 128, :] + phi
                    zacc[la, t * 128:(t + 1) * 128, :] = z
                    if last and CFG["fin_z"]:
                        zb[t * 128:(t + 1) * 128, :] = jnp.broadcast_to(
                            jnp.sum(z, axis=1, keepdims=True), (128, L))

            def vstep(ch=ch):
                vs[b.hf][ch][0] = _pack_split(proj(wkvaT, D + ch * MC, MC, b, CFG["sub_v"], fresh=fresh))

            def mstep(ch=ch):
                for u in range(PPC):
                    t = ch * PPC + u
                    acc = kv_acc[la, t] + _mm_nt(_unpk(vs[b.hf][ch][b.z("op_v"), u * 32:(u + 1) * 32, :]),
                                                 _unpk(phis[b.hf][ch][b.z("op_phi"), u * 64:(u + 1) * 64, :]))
                    kv_acc[la, t] = acc
                    if last and CFG["fin_kv"]:
                        kv_finish(t, acc)

            if vk and not (last and ch == NCH - 1):
                steps.append((vstep, None))
                steps.append((kstep, mstep))
            else:
                steps.append((kstep, None))
                steps.append((vstep, mstep))
        return steps

    def a_q(b):
        steps = []
        for ch in range(NCH):
            def qstep(ch=ch):
                qp = proj(wqaT, ch * MC, MC, b, CFG["sub_q"])
                for u in range(PPC):
                    t = ch * PPC + u
                    ep, en, sp, sn = _phi_parts(qp[u * 64:(u + 1) * 64, :])
                    zr = _rows(zb[t * 128:(t + 1) * 128, :])
                    dp = _fold2(jnp.add, [e * zz for e, zz in zip(ep, zr[:8])])
                    dn = _fold2(jnp.add, [e * zz for e, zz in zip(en, zr[8:])])
                    r = _recip(dp * sn + dn * sp + 1e-6 * (sp * sn))
                    rp = r * sn
                    rn = r * sp
                    phi = jnp.concatenate([e * rp for e in ep] + [e * rn for e in en], axis=0)
                    phis[b.hf][ch][0, u * 64:(u + 1) * 64, :] = _pack_split(phi)

            def nstep(ch=ch):
                for u in range(PPC):
                    t = ch * PPC + u
                    o = _mm(_unpk(kvm[t]), _unpk(phis[b.hf][ch][b.z("op_phi"), u * 64:(u + 1) * 64, :]))
                    os_[b.hf][0, t * 32:(t + 1) * 32, :] = _pack_split(o)

            steps.append((qstep, nstep))
        return steps

    def barrier():
        pl.semaphore_signal(bsem, 1)
        pl.semaphore_wait(bsem, 1)

    def o_rhs(b):
        return lambda: _unpk(os_[b.hf][b.z("op_o")])

    def out_proj(wo, b, link=None, defer=None):
        steps = []
        ln = LN(b, link)
        if defer is not None:
            defer.append((ln.finish, None))
        for ch in range(NCH):
            def ostep(ch=ch):
                m0 = ch * MC
                xt = xT[b.hf][b.k, m0:m0 + MC, :] + mmw(wo, m0, MC, o_rhs(b), CFG["sub_o"])
                xT[b.hf][b.k, m0:m0 + MC, :] = xt
                ln.add(xt)
                if ch == NCH - 1 and defer is None:
                    ln.finish()
            steps.append((ostep, None))
        return steps

    def b_kv(b):
        steps = []
        for base, ref in ((0, kb), (D, vb)):
            for m0 in range(0, D, MC):
                def step(base=base, ref=ref, m0=m0):
                    p = proj(wkvbT, base + m0, MC, b, CFG["sub_b"], fresh=True)
                    ref[WIN + b.j, m0:m0 + MC, :] = p
                    if b.hf == 0:
                        ref[b.k, m0:m0 + MC, :] = pltpu.roll(p, 2, 1)
                steps.append((step, None))
        return steps

    def b_q(b):
        j = b.j
        even = lax.broadcasted_iota(jnp.int32, (8, L), 0) % 2 == 0
        first = lax.broadcasted_iota(jnp.int32, (8, L), 1) < 2
        cs = DH ** -0.5
        steps = []
        for G in range(4):
            st = {}

            def step(G=G, st=st):
                q = proj(wqbT, G * 256, 256, b)
                halves = []
                for u in range(2):
                    acc = [None] * WIN
                    for r in range(16):
                        r0 = u * 128 + r * 8
                        qv = q[r0:r0 + 8, :]
                        for w in range(WIN):
                            t = qv * kb[WIN + j - w, G * 256 + r0:G * 256 + r0 + 8, :]
                            acc[w] = t if acc[w] is None else acc[w] + t
                    halves.append(acc)
                lg = []
                for w in range(WIN):
                    la, lb = halves[0][w], halves[1][w]
                    l = jnp.where(even, la + pltpu.roll(la, 7, 0), lb + pltpu.roll(lb, 1, 0))
                    l = l * cs
                    if w > 0 and b.hf == 1:
                        l = jnp.where(jnp.logical_and(first, j < w), -1e9, l)
                    lg.append(l)
                mx = _tree(jnp.maximum, lg)
                ex = [jnp.exp(l - mx) for l in lg]
                rs = 1.0 / _tree(jnp.add, ex)
                at = [e * rs for e in ex]
                never = rs < 0.0
                for hh in range(8):
                    h = G * 8 + hh
                    s = 2 * (hh % 4) + hh // 4
                    o = None
                    for w in range(WIN if CFG['dbg'] != 3 else 2):
                        a = jnp.broadcast_to(at[w][s:s + 1, :], (DH, L))
                        t = a * vb[WIN + j - w, h * DH:(h + 1) * DH, :]
                        o = t if o is None else o + t
                    pk = _pack_split(o)
                    os_[b.hf][0, h * 16:(h + 1) * 16, :] = pk
                    st["pk"] = pk[0:8, :] if hh == 0 else st["pk"] | pk[8:16, :]
                    if CFG["pv_link"] and hh % CFG["pv_link"] == CFG["pv_link"] - 1 and hh < 7:
                        lk = pltpu.bitcast(pk[0:8, :] | pk[8:16, :], F32)
                        for _ in range(CFG['pv_slow']):
                            lk = pltpu.roll(lk, 1, 0)
                        at = [jnp.where(never, lk, a) for a in at]

            def dl(st=st):
                deps.append((jnp.full((8, L), b.zr, jnp.int32) > 0, st["pk"]))
            steps.append((step, dl if CFG["att_dl"] else None))
        return steps

    def final_proj(b):
        steps = []
        for ch in range(NCH):
            def ostep(ch=ch):
                m0 = ch * MC
                xt = xT[b.hf][b.k, m0:m0 + MC, :] + mmw(wobT, m0, MC, o_rhs(b), CFG["sub_o"])
                for u in range(GPC):
                    y = _unpk(_pack_split(xt[u * 128:(u + 1) * 128, :])).T
                    cc = ch * GPC + u
                    xio[b.j, :, cc * L:(cc + 1) * L] = pltpu.bitcast(y, U32)
            steps.append((ostep, None))
        return steps

    kv_acc[...] = jnp.zeros(kv_acc.shape, F32)
    zacc[...] = jnp.zeros(zacc.shape, F32)

    def unsplit(r):
        return (r // 16) * 16 + 2 * (r % 8) + (r // 8) % 2

    r128 = unsplit(lax.broadcasted_iota(jnp.int32, (128, 128), 0))
    c128 = lax.broadcasted_iota(jnp.int32, (128, 128), 1)
    same_head = (2 * (r128 // 64) + r128 % 2) == (c128 // 32)
    er = unsplit(lax.broadcasted_iota(jnp.int32, (128, 32), 0))
    ec = lax.broadcasted_iota(jnp.int32, (128, 32), 1)
    expand = jnp.where(((er % 64) // 2) == ec, 1.0, 0.0).astype(BF16)
    cp_phi.wait()
    for g in range(8):
        pg = _mm_nt(expand, wphi[g * 128:(g + 1) * 128, :])
        pmat[g] = _pack(jnp.where(same_head, pg, 0.0))

    only = CFG["only"] or (0, 1, 2, 3, 5)
    x_in(8).wait()
    prep_x(8, Blk(0, 0))
    sa = a_kv(Blk(0, 0), 0, False, False)
    sb = a_kv(Blk(1, 0), 0, False, False)
    pend = []
    for ch in range(NCH if 0 in only else 0):
        cp_k[ch].wait()
        if ch == 0:
            for u in range(GPC):
                fold(wkvaT, u, 8 + u)
            sa[0][0]()
            x_in(0).wait()
        cp_v[ch].wait()
        if ch == 2:
            x_in(9).wait()
            x_in(1).wait()
        if ch == 0:
            prep_x(0, Blk(1, 0))
        else:
            for u in range(GPC):
                fold(wkvaT, ch * GPC + u, 8 + ch * GPC + u)
        for u in range(GPC):
            wstore_shuf(wkvaT, 8 + ch * GPC + u, wa_raw, 16 + ch * GPC + u)
        for f in pend:
            f()
        if ch >= 2:
            prep_x(Blk(ch - 2, 1).j, Blk(ch - 2, 1))
        if ch == 0:
            sa[1][0]()
            sb[0][0]()
        else:
            sa[2 * ch][0]()
            sb[2 * ch][0]()
            sa[2 * ch + 1][0]()
        sb[2 * ch + 1][0]()
        pend = [sa[2 * ch + 1][1], sb[2 * ch + 1][1]]
    for f in pend:
        f()

    def s1(i, c):
        @pl.when(i < 7)
        def _():
            x_in(9 + i).wait()
            x_in(1 + i).wait()

        wait_all(w_set(i - 1))
        side_begin(Blk(0, i))
        steps = a_kv(Blk(0, i), 0, False, False, CFG["vk"]) + a_kv(Blk(1, i), 0, True, False, CFG["vk"])
        nxt = jnp.minimum(i + 1, 7)
        steps.insert(14, (lambda: prep_set(i - 1), None))
        steps.insert(12, (lambda: prep_x(nxt, Blk(1, i + 1)), None))
        steps.insert(8, (lambda: prep_x(8 + nxt, Blk(0, i + 1)), None))
        steps.insert(2, (lambda: fold(wqaT, i - 1, i - 1), None))
        emit(steps, CFG["lag_kv"])
        return c
    if 1 in only:
        lax.fori_loop(1, 8, s1, 0)
    side_begin(None)
    wait_all(w_set(7))
    fold(wqaT, 7, 7)
    prep_set(7)
    a_finish(0)
    wait_all(cp_late)

    def s2(i, c):
        b0, b1 = Blk(0, i), Blk(1, i)
        steps = a_q(b0) + a_q(b1) + out_proj(woaT, b0) + out_proj(woaT, b1)
        steps += [(lambda: prep_late(i), None)]
        steps += b_kv(b0) + b_kv(b1)
        emit(steps, CFG["lag_q"])
        return c

    def s3(i, c):
        b0, b1 = Blk(0, i), Blk(1, i)
        dfr = [] if CFG["ln_defer"] else None
        steps = b_q(b0) + b_q(b1) + out_proj(wobT, b0, CFG["link3"], dfr) + out_proj(wobT, b1, CFG["link3"])
        if CFG["dbg"] == 1:
            steps = steps[8:]
        if CFG["dbg"] == 2:
            steps = steps[4:]
        steps += a_kv(b0, 1, False, True, CFG["vk"]) + a_kv(b1, 1, True, True, CFG["vk"])
        if CFG["bar3"]:
            steps[CFG["bar3"]:CFG["bar3"]] = [(barrier, None)] + (dfr or [])
        if CFG["dbg"] == 4:
            qs = b_q(Blk(0, i + 1)) + b_q(Blk(1, i + 1))
            kv = steps[16:]
            steps = steps[8:16]
            for n in range(8):
                steps += [qs[n], kv[2 * n], kv[2 * n + 1]]
        if CFG["dbg"] == 5:
            qs = b_q(Blk(0, i + 1)) + b_q(Blk(1, i + 1))
            kv = steps[16:]
            steps = steps[8:16]
            for n in range(8):
                steps += [kv[2 * n], qs[n], kv[2 * n + 1]]
        emit(steps, CFG["lag_kv"])
        return c

    def s5(i, c):
        b0, b1 = Blk(0, i), Blk(1, i)
        steps = b_q(b0) + b_q(b1) + final_proj(b0) + final_proj(b1)
        if CFG["dbg"] in (4, 5):
            qa, qb = b_q(Blk(0, i + 1)), b_q(b1)
            oa, ob = final_proj(b0), final_proj(b1)
            steps = []
            for n in range(4):
                steps += [qb[n], oa[n]]
            for n in range(4):
                steps += [qa[n], ob[n]]
        emit(steps, 0)
        x_out(b0.j).start()
        x_out(b1.j).start()
        return c

    def layer_pair(l, c):
        if 2 in only:
            lax.fori_loop(0, 8, s2, 0)

        @pl.when(l == 0)
        def _():
            if 3 in only:
                lax.fori_loop(0, 8, s3, 0)
                a_finish(1)

        @pl.when(l == 1)
        def _():
            if 5 in only:
                lax.fori_loop(0, 8, s5, 0)
        return c
    lax.fori_loop(0, 2, layer_pair, 0)

    for j in range(NBLK):
        x_out(j).wait()


@jax.jit
def pallas_interleave_layers__linear_kernel_hedgehog__sliding_local_dilated__prompt_kernel(
    A_x: jax.Array,
    A_wqkv: jax.Array,
    A_w_phi: jax.Array,
    A_wo: jax.Array,
    B_x: jax.Array,
    B_wqkv: jax.Array,
    B_wo: jax.Array,
):
    del B_x
    x3 = A_x.reshape(S // 32, 32, D)
    wphi2 = A_w_phi.reshape(H * DH, DH)
    any_spec = pl.BlockSpec(memory_space=pl.ANY)
    scratch = [
        pltpu.VMEM((NBLK, S // 32, D), U32),
        pltpu.VMEM((D, 3 * D), BF16),
        pltpu.VMEM((D, D), BF16),
        pltpu.VMEM((D, 3 * D), BF16),
        pltpu.VMEM((D, D), BF16),
        pltpu.VMEM((H * DH, DH), BF16),
        pltpu.VMEM((8, 64, 128), U32),
        pltpu.VMEM((8, D // 2, L), U32),
        pltpu.VMEM((8, D, L), U32),
        pltpu.VMEM((8, D // 2, L), U32),
        pltpu.VMEM((8, D // 2, L), U32),
        pltpu.VMEM((8, D, L), U32),
        pltpu.VMEM((8, D // 2, L), U32),
        pltpu.VMEM((WIN + NBLK, D, L), F32),
        pltpu.VMEM((WIN + NBLK, D, L), F32),
        pltpu.VMEM((2, 16, 64, 128), F32),
        pltpu.VMEM((16, 32, 128), U32),
        pltpu.VMEM((2, 2 * D, L), F32),
        pltpu.VMEM((2 * D, L), F32),
        pltpu.SemaphoreType.DMA((NSEM,)),
        pltpu.SemaphoreType.REGULAR,
    ]
    scratch += [pltpu.VMEM((9, D, L), F32)] * 2
    scratch += [pltpu.VMEM((9, D // 2, L), U32)] * 2
    scratch += [pltpu.VMEM((1, D // 2, L), U32)] * 2
    scratch += [pltpu.VMEM((1, MC, L), U32)] * (2 * NCH)
    scratch += [pltpu.VMEM((1, MC // 2, L), U32)] * (2 * NCH)
    out = pl.pallas_call(
        _kernel,
        out_shape=jax.ShapeDtypeStruct((S // 32, 32, D), BF16),
        in_specs=[any_spec] * 6,
        out_specs=any_spec,
        scratch_shapes=scratch,
        compiler_params=pltpu.CompilerParams(vmem_limit_bytes=120 * 1024 * 1024),
        name="hedgehog_dilated",
    )(x3, A_wqkv, wphi2, A_wo, B_wqkv, B_wo)
    return out.reshape(1, S, D)
```

```python
import math

import jax
import jax.numpy as jnp
from jax import lax
import jax.experimental.pallas as pl
import jax.experimental.pallas.tpu as pltpu

S = 2048
D = 1024
H = 32
DH = 32
NBLK = 16
L = 128
WIN = 8
HALO = WIN - 1
LOG2E = math.log2(math.e)
F32 = jnp.float32
BF16 = jnp.bfloat16
U32 = jnp.uint32
NT = (((1,), (1,)), ((), ()))

MC = 256
NCH = D // MC
GPC = MC // 128
PPC = MC // 64
CFG = dict(vk=False, link3=4, lag_q=1, lag_kv=2, only=None, ln_link=4, ln_rev=False, sub=256, sub_o=256, sub_b=256,
           op_acc=True, op_phi=False, op_v=False, op_o=False, op_xt=False, op_xn=False,
           fin_z=True, fin_kv=True, sub_q=128, sub_k=128, sub_v=256, arecip=True, dbg=0, att_dl=0, pv_link=0, pv_slow=0, bar3=13, ln_defer=True, side=2, out_defer=2, u2=1, u5=1)

SEM_X = 0
SEM_PHI = 16
SEM_KV = 17
SEM_SET = 25
SEM_LATE = 33
NSEM = 34


def _mm(a, b):
    return jnp.dot(a, b, preferred_element_type=F32)


def _mm_nt(a, b):
    return lax.dot_general(a, b, NT, preferred_element_type=F32)


def _tree(op, xs):
    xs = list(xs)
    while len(xs) > 1:
        nxt = [op(xs[i], xs[i + 1]) for i in range(0, len(xs) - 1, 2)]
        if len(xs) % 2:
            nxt.append(xs[-1])
        xs = nxt
    return xs[0]


def _chain(op, xs, ways=4):
    acc = list(xs[:ways])
    for i, x in enumerate(xs[ways:]):
        acc[i % ways] = op(acc[i % ways], x)
    return _tree(op, acc)


def _rows(a, n=8):
    return [a[i * n:(i + 1) * n, :] for i in range(a.shape[0] // n)]


def _pack(a):
    return pltpu.bitcast(a.astype(BF16), U32)


def _unpk(a):
    return pltpu.bitcast(a, BF16)


def _pack_i(a, b):
    return pltpu.pack_elementwise([a, b], packed_dtype=BF16)


def _pack_split(a):
    r = _rows(a)
    return jnp.concatenate([_pack_i(r[2 * i], r[2 * i + 1]) for i in range(len(r) // 2)], axis=0)


def _unpack_split(p):
    out = []
    for x in _rows(p):
        out.append(pltpu.unpack_elementwise(x, index=0, packed_dtype=BF16, unpacked_dtype=F32))
        out.append(pltpu.unpack_elementwise(x, index=1, packed_dtype=BF16, unpacked_dtype=F32))
    return jnp.concatenate(out, axis=0)


def _fold2(op, xs):
    r = _tree(op, xs)
    r = op(r, pltpu.roll(r, 4, 0))
    return op(r, pltpu.roll(r, 2, 0))


def _phi_parts(p):
    ps = _rows(p)
    mx = _fold2(jnp.maximum, ps)
    mn = _fold2(jnp.minimum, ps)
    ep = [jnp.exp2(x - mx) for x in ps]
    en = [jnp.exp2(mn - x) for x in ps]
    sp = _fold2(jnp.add, ep)
    sn = _fold2(jnp.add, en)
    return ep, en, sp, sn


def _recip(x):
    if not CFG["arecip"]:
        return 1.0 / x
    r = pl.reciprocal(x, approx=True)
    return r * (2.0 - x * r)


def _mult(x, m):
    return x if isinstance(x, int) else pl.multiple_of(x, m)


def _kernel(x_hbm, wa_hbm, wphi_hbm, woa_hbm, wb_hbm, wob_hbm, out_hbm,
            xio, wa_raw, woa_raw, wb_raw, wob_raw, wphi, pmat,
            wqaT, wkvaT, woaT, wqbT, wkvbT, wobT, kb, vb, kv_acc, kvm, zacc, zb, ystage, sems, bsem, *rest):
    xT, xn, os_ = rest[0:2], rest[2:4], rest[4:6]
    phis = [rest[6:6 + NCH], rest[6 + NCH:6 + 2 * NCH]]
    vs = [rest[6 + 2 * NCH:6 + 3 * NCH], rest[6 + 3 * NCH:6 + 4 * NCH]]

    class Blk:
        def __init__(self, hf, k, opaque=True):
            self.hf, self.k = hf, k
            self.j = 8 * (1 - hf) + k
            self.zr = 0 if (isinstance(k, int) or not opaque) else k // 64

        def z(self, key):
            return self.zr if CFG[key] else 0

    x32 = x_hbm.bitcast(U32)
    out32 = out_hbm.bitcast(U32)

    def x_in(j):
        return pltpu.make_async_copy(x32.at[:, j, :], xio.at[j], sems.at[SEM_X + j])

    def x_out(j):
        return pltpu.make_async_copy(xio.at[j], out32.at[:, j, :], sems.at[SEM_X + j])

    def colcopy(src, dst, c0, n, sem):
        c0 = _mult(c0, 128)
        return pltpu.make_async_copy(src.at[:, pl.ds(c0, n)], dst.at[:, pl.ds(c0, n)], sems.at[sem])

    cp_phi = pltpu.make_async_copy(wphi_hbm, wphi, sems.at[SEM_PHI])
    cp_k = [colcopy(wa_hbm, wa_raw, D + ch * MC, MC, SEM_KV + 2 * ch) for ch in range(NCH)]
    cp_v = [colcopy(wa_hbm, wa_raw, 2 * D + ch * MC, MC, SEM_KV + 2 * ch + 1) for ch in range(NCH)]

    def w_set(g):
        return [colcopy(wa_hbm, wa_raw, g * 128, 128, SEM_SET + g),
                colcopy(woa_hbm, woa_raw, g * 128, 128, SEM_SET + g),
                colcopy(wb_hbm, wb_raw, D + g * 128, 128, SEM_SET + g),
                colcopy(wb_hbm, wb_raw, 2 * D + g * 128, 128, SEM_SET + g)]

    cp_late = [colcopy(wb_hbm, wb_raw, 0, D, SEM_LATE), colcopy(wob_hbm, wob_raw, 0, D, SEM_LATE)]

    order = [cp_phi, x_in(8), cp_k[0], x_in(0), cp_v[0], cp_k[1], cp_v[1], x_in(9), x_in(1)]
    for ch in range(2, NCH):
        order += [cp_k[ch], cp_v[ch]]
    for g in range(8):
        if g < 6:
            order += [x_in(10 + g), x_in(2 + g)]
        order += w_set(g)
    order += cp_late
    for c in order:
        c.start()

    def wait_all(cps):
        for c in cps:
            c.wait()

    deps = []

    def wload(ref, r0, n):
        parts = [ref[c, r0 // 2:(r0 + n) // 2, :] for c in range(8)]
        while deps:
            never, val = deps.pop()
            head = jnp.where(never, val, parts[0][0:8, :])
            parts[0] = jnp.concatenate([head, parts[0][8:, :]], axis=0)
        return jnp.concatenate([_unpk(x) for x in parts], axis=1)

    class Side:
        never = None
        hist = []

    def tr(x):
        w = CFG["side"]
        if Side.never is not None and w and len(Side.hist) >= w:
            x = jnp.concatenate([jnp.where(Side.never, Side.hist[-w], x[0:8, :]), x[8:, :]], axis=0)
        y = pltpu.bitcast(_unpk(x).T, U32)
        Side.hist.append(y[56:64, :])
        return y

    def side_begin(b):
        Side.never = None if b is None else jnp.full((8, L), b.zr, jnp.int32) > 0
        Side.hist = []

    def wtile(raw, slab, c):
        return tr(pltpu.bitcast(raw[c * 128:(c + 1) * 128, pl.ds(_mult(slab * 128, 128), 128)], U32))

    def wstore_split(ref, g, raw, slab):
        off = _mult(g * 64, 64)
        for c in range(8):
            ref[c, pl.ds(off, 64), :] = _pack(_unpack_split(wtile(raw, slab, c)))

    def wstore_shuf(ref, g, raw, slab):
        off = _mult(g * 64, 64)
        for c in range(8):
            ref[c, pl.ds(off, 64), :] = _pack_split(_unpk(wtile(raw, slab, c)).astype(F32))

    def wstore_perm(ref, g, raw, slab):
        for c in range(8):
            pk = wtile(raw, slab, c)
            for h4 in range(4):
                ref[c, pl.ds(g * 64 + h4, 16, stride=4), :] = pk[h4 * 16:(h4 + 1) * 16, :]

    def cols(ref, g):
        return ref[:, pl.ds(_mult(g * 128, 128), 128)]

    class LN:
        def __init__(self, b, link=None):
            self.b = b
            self.link = CFG["ln_link"] if link is None else link
            self.piv = None
            self.s1 = []
            self.s2 = []

        def add(self, xt):
            if self.piv is None:
                self.piv = jnp.broadcast_to(xt[0:1, :], (8, L))
            d = [r - self.piv for r in _rows(xt)]
            self.s1 = [_chain(jnp.add, self.s1 + d, 1)]
            self.s2 = [_chain(jnp.add, self.s2 + [x * x for x in d], 1)]

        def finish(self):
            b = self.b
            m1 = jnp.sum(self.s1[0], axis=0, keepdims=True) * (1.0 / D)
            m2 = jnp.sum(self.s2[0], axis=0, keepdims=True) * (1.0 / D)
            var = jnp.maximum(m2 - m1 * m1, 0.0)
            rs = lax.rsqrt(var + 1e-5)
            mrs = jnp.broadcast_to((self.piv[0:1, :] + m1) * rs, (8, L))
            rs = jnp.broadcast_to(rs, (8, L))
            never = rs < 0.0
            link = self.link
            kk = b.k + b.z("op_xt")
            rng = list(range(D // 16))
            if CFG["ln_rev"]:
                rng = rng[::-1]
            for n, r in enumerate(rng):
                pk = _pack_i(xT[b.hf][kk, r * 16:r * 16 + 8, :] * rs - mrs,
                             xT[b.hf][kk, r * 16 + 8:r * 16 + 16, :] * rs - mrs)
                xn[b.hf][b.k, r * 8:(r + 1) * 8, :] = pk
                if link and n % link == link - 1:
                    rs = jnp.where(never, pltpu.bitcast(pk, F32), rs)

    def prep_x(src, b):
        ln = LN(b)
        for cc in range(8):
            xt = _unpack_split(tr(xio[src, :, cc * L:(cc + 1) * L]))
            xT[b.hf][b.k, cc * 128:(cc + 1) * 128, :] = xt
            ln.add(xt)
        ln.finish()

    def fold(dst, g, slab):
        val = _mm_nt(_unpk(pmat[g]), cols(wa_raw, slab)) * LOG2E
        off = _mult(g * 64, 64)
        for c in range(8):
            dst[c, pl.ds(off, 64), :] = _pack_split(val[:, c * L:(c + 1) * L])

    def prep_set(g):
        wstore_split(woaT, g, woa_raw, g)
        wstore_perm(wkvbT, g, wb_raw, 8 + g)
        wstore_split(wkvbT, 8 + g, wb_raw, 16 + g)

    def prep_late(g):
        wstore_perm(wqbT, g, wb_raw, g)
        wstore_split(wobT, g, wob_raw, g)

    def mmw(ref, r0, n, rhs, sub):
        return jnp.concatenate([_mm(wload(ref, r, sub), rhs()) for r in range(r0, r0 + n, sub)], axis=0)

    def proj(ref, r0, n, b, sub=None, fresh=False):
        kk = b.k + b.z("op_xn") if fresh else b.k
        return mmw(ref, r0, n, lambda: _unpk(xn[b.hf][kk]), sub or CFG["sub"])

    def emit(steps, lag):
        pend = []
        for n, (main, late) in enumerate(steps):
            main()
            if late is not None:
                pend.append((n + (CFG["att_dl"] if late.__name__ == "dl" else lag), late))
            for due, f in sorted(pend, key=lambda e: e[0]):
                if due <= n:
                    f()
            pend = [e for e in pend if e[0] > n]
        for due, f in sorted(pend, key=lambda e: e[0]):
            f()
        deps.clear()

    def kv_finish(t, acc):
        r = lax.broadcasted_iota(jnp.int32, (64, 128), 0)
        c = lax.broadcasted_iota(jnp.int32, (64, 128), 1)
        kvm[t] = _pack_split(jnp.where((r // 32) == ((c // 2) % 2), acc, 0.0))

    def a_finish(lay):
        if not CFG["fin_z"]:
            zb[...] = jnp.broadcast_to(jnp.sum(zacc[lay], axis=1, keepdims=True), zb.shape)
        if not CFG["fin_kv"]:
            for t in range(16):
                kv_finish(t, kv_acc[lay, t])

    def a_kv(b, lay, last, fresh, vk=False):
        steps = []
        la = lay + b.z("op_acc") if last else lay
        for ch in range(NCH):
            def kstep(ch=ch):
                kp = proj(wkvaT, ch * MC, MC, b, CFG["sub_k"], fresh=fresh)
                for u in range(PPC):
                    t = ch * PPC + u
                    ep, en, sp, sn = _phi_parts(kp[u * 64:(u + 1) * 64, :])
                    r = _recip(sp * sn)
                    rp = r * sn
                    rn = r * sp
                    phi = jnp.concatenate([e * rp for e in ep] + [e * rn for e in en], axis=0)
                    phis[b.hf][ch][0, u * 64:(u + 1) * 64, :] = _pack_split(phi)
                    z = zacc[la, t * 128:(t + 1) * 128, :] + phi
                    zacc[la, t * 128:(t + 1) * 128, :] = z
                    if last and CFG["fin_z"]:
                        zb[t * 128:(t + 1) * 128, :] = jnp.broadcast_to(
                            jnp.sum(z, axis=1, keepdims=True), (128, L))

            def vstep(ch=ch):
                vs[b.hf][ch][0] = _pack_split(proj(wkvaT, D + ch * MC, MC, b, CFG["sub_v"], fresh=fresh))

            def mstep(ch=ch):
                for u in range(PPC):
                    t = ch * PPC + u
                    acc = kv_acc[la, t] + _mm_nt(_unpk(vs[b.hf][ch][b.z("op_v"), u * 32:(u + 1) * 32, :]),
                                                 _unpk(phis[b.hf][ch][b.z("op_phi"), u * 64:(u + 1) * 64, :]))
                    kv_acc[la, t] = acc
                    if last and CFG["fin_kv"]:
                        kv_finish(t, acc)

            if vk and not (last and ch == NCH - 1):
                steps.append((vstep, None))
                steps.append((kstep, mstep))
            else:
                steps.append((kstep, None))
                steps.append((vstep, mstep))
        return steps

    def a_q(b):
        steps = []
        for ch in range(NCH):
            def qstep(ch=ch):
                qp = proj(wqaT, ch * MC, MC, b, CFG["sub_q"])
                for u in range(PPC):
                    t = ch * PPC + u
                    ep, en, sp, sn = _phi_parts(qp[u * 64:(u + 1) * 64, :])
                    zr = _rows(zb[t * 128:(t + 1) * 128, :])
                    dp = _fold2(jnp.add, [e * zz for e, zz in zip(ep, zr[:8])])
                    dn = _fold2(jnp.add, [e * zz for e, zz in zip(en, zr[8:])])
                    r = _recip(dp * sn + dn * sp + 1e-6 * (sp * sn))
                    rp = r * sn
                    rn = r * sp
                    phi = jnp.concatenate([e * rp for e in ep] + [e * rn for e in en], axis=0)
                    phis[b.hf][ch][0, u * 64:(u + 1) * 64, :] = _pack_split(phi)

            def nstep(ch=ch):
                for u in range(PPC):
                    t = ch * PPC + u
                    o = _mm(_unpk(kvm[t]), _unpk(phis[b.hf][ch][b.z("op_phi"), u * 64:(u + 1) * 64, :]))
                    os_[b.hf][0, t * 32:(t + 1) * 32, :] = _pack_split(o)

            steps.append((qstep, nstep))
        return steps

    def barrier():
        pl.semaphore_signal(bsem, 1)
        pl.semaphore_wait(bsem, 1)

    def o_rhs(b):
        return lambda: _unpk(os_[b.hf][b.z("op_o")])

    def out_proj(wo, b, link=None, defer=None):
        steps = []
        ln = LN(b, link)
        if defer is not None:
            defer.append((ln.finish, None))
        for ch in range(NCH):
            def ostep(ch=ch):
                m0 = ch * MC
                xt = xT[b.hf][b.k, m0:m0 + MC, :] + mmw(wo, m0, MC, o_rhs(b), CFG["sub_o"])
                xT[b.hf][b.k, m0:m0 + MC, :] = xt
                ln.add(xt)
                if ch == NCH - 1 and defer is None:
                    ln.finish()
            steps.append((ostep, None))
        return steps

    def b_kv(b):
        steps = []
        for base, ref in ((0, kb), (D, vb)):
            for m0 in range(0, D, MC):
                def step(base=base, ref=ref, m0=m0):
                    p = proj(wkvbT, base + m0, MC, b, CFG["sub_b"], fresh=True)
                    ref[WIN + b.j, m0:m0 + MC, :] = p
                    if b.hf == 0:
                        ref[b.k, m0:m0 + MC, :] = pltpu.roll(p, 2, 1)
                steps.append((step, None))
        return steps

    def b_q(b):
        j = b.j
        even = lax.broadcasted_iota(jnp.int32, (8, L), 0) % 2 == 0
        first = lax.broadcasted_iota(jnp.int32, (8, L), 1) < 2
        cs = DH ** -0.5
        steps = []
        for G in range(4):
            st = {}

            def step(G=G, st=st):
                q = proj(wqbT, G * 256, 256, b)
                halves = []
                for u in range(2):
                    acc = [None] * WIN
                    for r in range(16):
                        r0 = u * 128 + r * 8
                        qv = q[r0:r0 + 8, :]
                        for w in range(WIN):
                            t = qv * kb[WIN + j - w, G * 256 + r0:G * 256 + r0 + 8, :]
                            acc[w] = t if acc[w] is None else acc[w] + t
                    halves.append(acc)
                lg = []
                for w in range(WIN):
                    la, lb = halves[0][w], halves[1][w]
                    l = jnp.where(even, la + pltpu.roll(la, 7, 0), lb + pltpu.roll(lb, 1, 0))
                    if w > 0 and b.hf == 1:
                        l = jnp.where(jnp.logical_and(first, j < w), -1e9 / cs, l)
                    lg.append(l)
                mx = _tree(jnp.maximum, lg)
                ex = [jnp.exp2((l - mx) * (cs * LOG2E)) for l in lg]
                rs = _recip(_tree(jnp.add, ex))
                at = [e * rs for e in ex]
                never = rs < 0.0
                for hh in range(8):
                    h = G * 8 + hh
                    s = 2 * (hh % 4) + hh // 4
                    o = None
                    for w in range(WIN if CFG['dbg'] != 3 else 2):
                        a = jnp.broadcast_to(at[w][s:s + 1, :], (DH, L))
                        t = a * vb[WIN + j - w, h * DH:(h + 1) * DH, :]
                        o = t if o is None else o + t
                    pk = _pack_split(o)
                    os_[b.hf][0, h * 16:(h + 1) * 16, :] = pk
                    st["pk"] = pk[0:8, :] if hh == 0 else st["pk"] | pk[8:16, :]
                    if CFG["pv_link"] and hh % CFG["pv_link"] == CFG["pv_link"] - 1 and hh < 7:
                        lk = pltpu.bitcast(pk[0:8, :] | pk[8:16, :], F32)
                        for _ in range(CFG['pv_slow']):
                            lk = pltpu.roll(lk, 1, 0)
                        at = [jnp.where(never, lk, a) for a in at]

            def dl(st=st):
                deps.append((jnp.full((8, L), b.zr, jnp.int32) > 0, st["pk"]))
            steps.append((step, dl if CFG["att_dl"] else None))
        return steps

    def final_proj(b, defer=0):
        steps = []
        for ch in range(NCH):
            def ostep(ch=ch):
                m0 = ch * MC
                xt = xT[b.hf][b.k, m0:m0 + MC, :] + mmw(wobT, m0, MC, o_rhs(b), CFG["sub_o"])
                for u in range(GPC):
                    cc = ch * GPC + u
                    y = _pack_split(xt[u * 128:(u + 1) * 128, :])
                    if cc >= 8 - defer:
                        ystage[b.k + 1, cc * 64:(cc + 1) * 64, :] = y
                    else:
                        xio[b.j, :, cc * L:(cc + 1) * L] = tr(y)
            steps.append((ostep, None))
        return steps

    def flush_out(k, slot):
        for cc in range(8 - CFG["out_defer"], 8):
            xio[slot, :, cc * L:(cc + 1) * L] = tr(ystage[k, cc * 64:(cc + 1) * 64, :])

    kv_acc[...] = jnp.zeros(kv_acc.shape, F32)
    zacc[...] = jnp.zeros(zacc.shape, F32)
    ystage[0] = jnp.zeros(ystage.shape[1:], U32)

    def unsplit(r):
        return (r // 16) * 16 + 2 * (r % 8) + (r // 8) % 2

    r128 = unsplit(lax.broadcasted_iota(jnp.int32, (128, 128), 0))
    c128 = lax.broadcasted_iota(jnp.int32, (128, 128), 1)
    same_head = (2 * (r128 // 64) + r128 % 2) == (c128 // 32)
    er = unsplit(lax.broadcasted_iota(jnp.int32, (128, 32), 0))
    ec = lax.broadcasted_iota(jnp.int32, (128, 32), 1)
    expand = jnp.where(((er % 64) // 2) == ec, 1.0, 0.0).astype(BF16)
    cp_phi.wait()
    for g in range(8):
        pg = _mm_nt(expand, wphi[g * 128:(g + 1) * 128, :])
        pmat[g] = _pack(jnp.where(same_head, pg, 0.0))

    only = CFG["only"] or (0, 1, 2, 3, 5)
    x_in(8).wait()
    prep_x(8, Blk(0, 0))
    sa = a_kv(Blk(0, 0), 0, False, False)
    sb = a_kv(Blk(1, 0), 0, False, False)
    pend = []
    for ch in range(NCH if 0 in only else 0):
        cp_k[ch].wait()
        if ch == 0:
            for u in range(GPC):
                fold(wkvaT, u, 8 + u)
            sa[0][0]()
            x_in(0).wait()
        cp_v[ch].wait()
        if ch == 2:
            x_in(9).wait()
            x_in(1).wait()
        if ch == 0:
            prep_x(0, Blk(1, 0))
        else:
            for u in range(GPC):
                fold(wkvaT, ch * GPC + u, 8 + ch * GPC + u)
        for u in range(GPC):
            wstore_shuf(wkvaT, 8 + ch * GPC + u, wa_raw, 16 + ch * GPC + u)
        for f in pend:
            f()
        if ch >= 2:
            prep_x(Blk(ch - 2, 1).j, Blk(ch - 2, 1))
        if ch == 0:
            sa[1][0]()
            sb[0][0]()
        else:
            sa[2 * ch][0]()
            sb[2 * ch][0]()
            sa[2 * ch + 1][0]()
        sb[2 * ch + 1][0]()
        pend = [sa[2 * ch + 1][1], sb[2 * ch + 1][1]]
    for f in pend:
        f()

    def s1(i, c):
        @pl.when(i < 7)
        def _():
            x_in(9 + i).wait()
            x_in(1 + i).wait()

        wait_all(w_set(i - 1))
        side_begin(Blk(0, i))
        steps = a_kv(Blk(0, i), 0, False, False, CFG["vk"]) + a_kv(Blk(1, i), 0, True, False, CFG["vk"])
        nxt = jnp.minimum(i + 1, 7)
        steps.insert(14, (lambda: prep_set(i - 1), None))
        steps.insert(12, (lambda: prep_x(nxt, Blk(1, i + 1)), None))
        steps.insert(8, (lambda: prep_x(8 + nxt, Blk(0, i + 1)), None))
        steps.insert(2, (lambda: fold(wqaT, i - 1, i - 1), None))
        emit(steps, CFG["lag_kv"])
        return c
    if 1 in only:
        lax.fori_loop(1, 8, s1, 0)
    side_begin(None)
    wait_all(w_set(7))
    fold(wqaT, 7, 7)
    prep_set(7)
    a_finish(0)
    wait_all(cp_late)

    def s2(ii, c):
        steps = []
        for u in range(CFG["u2"]):
            i = ii * CFG["u2"] + u
            b0, b1 = Blk(0, i), Blk(1, i)
            steps += a_q(b0) + a_q(b1) + out_proj(woaT, b0) + out_proj(woaT, b1)
            steps += [(lambda i=i: prep_late(i), None)]
            steps += b_kv(b0) + b_kv(b1)
        emit(steps, CFG["lag_q"])
        return c

    def s3(i, c):
        b0, b1 = Blk(0, i), Blk(1, i)
        dfr = [] if CFG["ln_defer"] else None
        steps = b_q(b0) + b_q(b1) + out_proj(wobT, b0, CFG["link3"], dfr) + out_proj(wobT, b1, CFG["link3"])
        if CFG["dbg"] == 1:
            steps = steps[8:]
        if CFG["dbg"] == 2:
            steps = steps[4:]
        steps += a_kv(b0, 1, False, True, CFG["vk"]) + a_kv(b1, 1, True, True, CFG["vk"])
        if CFG["bar3"]:
            steps[CFG["bar3"]:CFG["bar3"]] = [(barrier, None)] + (dfr or [])
        if CFG["dbg"] == 4:
            qs = b_q(Blk(0, i + 1)) + b_q(Blk(1, i + 1))
            kv = steps[16:]
            steps = steps[8:16]
            for n in range(8):
                steps += [qs[n], kv[2 * n], kv[2 * n + 1]]
        if CFG["dbg"] == 5:
            qs = b_q(Blk(0, i + 1)) + b_q(Blk(1, i + 1))
            kv = steps[16:]
            steps = steps[8:16]
            for n in range(8):
                steps += [kv[2 * n], qs[n], kv[2 * n + 1]]
        emit(steps, CFG["lag_kv"])
        return c

    def s5(i, c):
        b0, b1 = Blk(0, i), Blk(1, i)
        steps = b_q(b0) + b_q(b1) + final_proj(b0) + final_proj(b1, CFG["out_defer"])
        if CFG["out_defer"]:
            steps.insert(8, (lambda: flush_out(i, jnp.where(i > 0, i - 1, NBLK)), None))
        emit(steps, 0)
        x_out(b0.j).start()
        if CFG["out_defer"]:
            @pl.when(i > 0)
            def _():
                x_out(i - 1).start()
        else:
            x_out(b1.j).start()
        return c

    def layer_pair(l, c):
        if 2 in only:
            lax.fori_loop(0, 8 // CFG["u2"], s2, 0)

        @pl.when(l == 0)
        def _():
            if 3 in only:
                lax.fori_loop(0, 8, s3, 0)
                a_finish(1)

        @pl.when(l == 1)
        def _():
            if 5 in only:
                lax.fori_loop(0, 8, s5, 0)
        return c
    lax.fori_loop(0, 2, layer_pair, 0)

    if CFG["out_defer"]:
        flush_out(8, 7)
        x_out(7).start()
    for j in range(NBLK):
        x_out(j).wait()


@jax.jit
def pallas_interleave_layers__linear_kernel_hedgehog__sliding_local_dilated__prompt_kernel(
    A_x: jax.Array,
    A_wqkv: jax.Array,
    A_w_phi: jax.Array,
    A_wo: jax.Array,
    B_x: jax.Array,
    B_wqkv: jax.Array,
    B_wo: jax.Array,
):
    del B_x
    x3 = A_x.reshape(S // 32, 32, D)
    wphi2 = A_w_phi.reshape(H * DH, DH)
    any_spec = pl.BlockSpec(memory_space=pl.ANY)
    scratch = [
        pltpu.VMEM((NBLK + 1, S // 32, D), U32),
        pltpu.VMEM((D, 3 * D), BF16),
        pltpu.VMEM((D, D), BF16),
        pltpu.VMEM((D, 3 * D), BF16),
        pltpu.VMEM((D, D), BF16),
        pltpu.VMEM((H * DH, DH), BF16),
        pltpu.VMEM((8, 64, 128), U32),
        pltpu.VMEM((8, D // 2, L), U32),
        pltpu.VMEM((8, D, L), U32),
        pltpu.VMEM((8, D // 2, L), U32),
        pltpu.VMEM((8, D // 2, L), U32),
        pltpu.VMEM((8, D, L), U32),
        pltpu.VMEM((8, D // 2, L), U32),
        pltpu.VMEM((WIN + NBLK, D, L), F32),
        pltpu.VMEM((WIN + NBLK, D, L), F32),
        pltpu.VMEM((2, 16, 64, 128), F32),
        pltpu.VMEM((16, 32, 128), U32),
        pltpu.VMEM((2, 2 * D, L), F32),
        pltpu.VMEM((2 * D, L), F32),
        pltpu.VMEM((9, D // 2, L), U32),
        pltpu.SemaphoreType.DMA((NSEM,)),
        pltpu.SemaphoreType.REGULAR,
    ]
    scratch += [pltpu.VMEM((9, D, L), F32)] * 2
    scratch += [pltpu.VMEM((9, D // 2, L), U32)] * 2
    scratch += [pltpu.VMEM((1, D // 2, L), U32)] * 2
    scratch += [pltpu.VMEM((1, MC, L), U32)] * (2 * NCH)
    scratch += [pltpu.VMEM((1, MC // 2, L), U32)] * (2 * NCH)
    out = pl.pallas_call(
        _kernel,
        out_shape=jax.ShapeDtypeStruct((S // 32, 32, D), BF16),
        in_specs=[any_spec] * 6,
        out_specs=any_spec,
        scratch_shapes=scratch,
        compiler_params=pltpu.CompilerParams(vmem_limit_bytes=120 * 1024 * 1024),
        name="hedgehog_dilated",
    )(x3, A_wqkv, wphi2, A_wo, B_wqkv, B_wo)
    return out.reshape(1, S, D)
```

```python
import math

import jax
import jax.numpy as jnp
from jax import lax
import jax.experimental.pallas as pl
import jax.experimental.pallas.tpu as pltpu

S = 2048
D = 1024
H = 32
DH = 32
NBLK = 16
L = 128
WIN = 8
HALO = WIN - 1
LOG2E = math.log2(math.e)
F32 = jnp.float32
BF16 = jnp.bfloat16
U32 = jnp.uint32
NT = (((1,), (1,)), ((), ()))

MC = 256
NCH = D // MC
GPC = MC // 128
PPC = MC // 64
CFG = dict(vk=False, link3=4, lag_q=1, lag_kv=2, only=None, ln_link=4, ln_rev=False, sub=256, sub_o=256, sub_b=256,
           op_acc=True, op_phi=False, op_v=False, op_o=False, op_xt=False, op_xn=False,
           fin_z=True, fin_kv=True, sub_q=128, sub_k=128, sub_v=256, arecip=True, dbg=0, att_dl=0, pv_link=0, pv_slow=0, bar3=13, ln_defer=True, side=2, out_defer=2, u2=1, out_at=17, cp=dict(disable_semaphore_checks=True), fold_at=2, hold=7, att4=False)

SEM_X = 0
SEM_PHI = 16
SEM_KV = 17
SEM_SET = 25
SEM_LATE = 33
NSEM = 34


def _mm(a, b):
    return jnp.dot(a, b, preferred_element_type=F32)


def _mm_nt(a, b):
    return lax.dot_general(a, b, NT, preferred_element_type=F32)


def _tree(op, xs):
    xs = list(xs)
    while len(xs) > 1:
        nxt = [op(xs[i], xs[i + 1]) for i in range(0, len(xs) - 1, 2)]
        if len(xs) % 2:
            nxt.append(xs[-1])
        xs = nxt
    return xs[0]


def _chain(op, xs, ways=4):
    acc = list(xs[:ways])
    for i, x in enumerate(xs[ways:]):
        acc[i % ways] = op(acc[i % ways], x)
    return _tree(op, acc)


def _rows(a, n=8):
    return [a[i * n:(i + 1) * n, :] for i in range(a.shape[0] // n)]


def _pack(a):
    return pltpu.bitcast(a.astype(BF16), U32)


def _unpk(a):
    return pltpu.bitcast(a, BF16)


def _pack_i(a, b):
    return pltpu.pack_elementwise([a, b], packed_dtype=BF16)


def _pack_split(a):
    r = _rows(a)
    return jnp.concatenate([_pack_i(r[2 * i], r[2 * i + 1]) for i in range(len(r) // 2)], axis=0)


def _unpack_split(p):
    out = []
    for x in _rows(p):
        out.append(pltpu.unpack_elementwise(x, index=0, packed_dtype=BF16, unpacked_dtype=F32))
        out.append(pltpu.unpack_elementwise(x, index=1, packed_dtype=BF16, unpacked_dtype=F32))
    return jnp.concatenate(out, axis=0)


def _fold2(op, xs):
    r = _tree(op, xs)
    r = op(r, pltpu.roll(r, 4, 0))
    return op(r, pltpu.roll(r, 2, 0))


def _phi_parts(p):
    ps = _rows(p)
    mx = _fold2(jnp.maximum, ps)
    mn = _fold2(jnp.minimum, ps)
    ep = [jnp.exp2(x - mx) for x in ps]
    en = [jnp.exp2(mn - x) for x in ps]
    sp = _fold2(jnp.add, ep)
    sn = _fold2(jnp.add, en)
    return ep, en, sp, sn


def _recip(x):
    if not CFG["arecip"]:
        return 1.0 / x
    r = pl.reciprocal(x, approx=True)
    return r * (2.0 - x * r)


def _mult(x, m):
    return x if isinstance(x, int) else pl.multiple_of(x, m)


def _kernel(x_hbm, wa_hbm, wphi_hbm, woa_hbm, wb_hbm, wob_hbm, out_hbm,
            xio, wa_raw, woa_raw, wb_raw, wob_raw, wphi, pmat,
            wqaT, wkvaT, woaT, wqbT, wkvbT, wobT, kb, vb, kv_acc, kvm, zacc, zb, ystage, sems, bsem, *rest):
    xT, xn, os_ = rest[0:2], rest[2:4], rest[4:6]
    phis = [rest[6:6 + NCH], rest[6 + NCH:6 + 2 * NCH]]
    vs = [rest[6 + 2 * NCH:6 + 3 * NCH], rest[6 + 3 * NCH:6 + 4 * NCH]]

    class Blk:
        def __init__(self, hf, k, opaque=True):
            self.hf, self.k = hf, k
            self.j = 8 * (1 - hf) + k
            self.zr = 0 if (isinstance(k, int) or not opaque) else k // 64

        def z(self, key):
            return self.zr if CFG[key] else 0

    x32 = x_hbm.bitcast(U32)
    out32 = out_hbm.bitcast(U32)

    def x_in(j):
        return pltpu.make_async_copy(x32.at[:, j, :], xio.at[j], sems.at[SEM_X + j])

    def x_out(j, c0=0, c1=8, sem=None):
        cs = pl.ds(c0 * L, (c1 - c0) * L)
        return pltpu.make_async_copy(xio.at[j, :, cs], out32.at[:, j, cs],
                                     sems.at[SEM_X + j if sem is None else sem])

    def colcopy(src, dst, c0, n, sem):
        c0 = _mult(c0, 128)
        return pltpu.make_async_copy(src.at[:, pl.ds(c0, n)], dst.at[:, pl.ds(c0, n)], sems.at[sem])

    cp_phi = pltpu.make_async_copy(wphi_hbm, wphi, sems.at[SEM_PHI])
    cp_k = [colcopy(wa_hbm, wa_raw, D + ch * MC, MC, SEM_KV + 2 * ch) for ch in range(NCH)]
    cp_v = [colcopy(wa_hbm, wa_raw, 2 * D + ch * MC, MC, SEM_KV + 2 * ch + 1) for ch in range(NCH)]

    def w_set(g):
        return [colcopy(wa_hbm, wa_raw, g * 128, 128, SEM_SET + g),
                colcopy(woa_hbm, woa_raw, g * 128, 128, SEM_SET + g),
                colcopy(wb_hbm, wb_raw, D + g * 128, 128, SEM_SET + g),
                colcopy(wb_hbm, wb_raw, 2 * D + g * 128, 128, SEM_SET + g)]

    cp_late = [colcopy(wb_hbm, wb_raw, 0, D, SEM_LATE), colcopy(wob_hbm, wob_raw, 0, D, SEM_LATE)]

    order = [cp_phi, x_in(8), cp_k[0], x_in(0), cp_v[0], cp_k[1], cp_v[1], x_in(9), x_in(1)]
    for ch in range(2, NCH):
        order += [cp_k[ch], cp_v[ch]]
    for g in range(8):
        if g < 6:
            order += [x_in(10 + g), x_in(2 + g)]
        order += w_set(g)
    order += cp_late
    for c in order:
        c.start()

    def wait_all(cps):
        for c in cps:
            c.wait()

    deps = []

    def wload(ref, r0, n):
        parts = [ref[c, r0 // 2:(r0 + n) // 2, :] for c in range(8)]
        while deps:
            never, val = deps.pop()
            head = jnp.where(never, val, parts[0][0:8, :])
            parts[0] = jnp.concatenate([head, parts[0][8:, :]], axis=0)
        return jnp.concatenate([_unpk(x) for x in parts], axis=1)

    class Side:
        never = None
        hist = []

    def tr(x):
        w = CFG["side"]
        if Side.never is not None and w and len(Side.hist) >= w:
            x = jnp.concatenate([jnp.where(Side.never, Side.hist[-w], x[0:8, :]), x[8:, :]], axis=0)
        y = pltpu.bitcast(_unpk(x).T, U32)
        Side.hist.append(y[56:64, :])
        return y

    def side_begin(b):
        Side.never = None if b is None else jnp.full((8, L), b.zr, jnp.int32) > 0
        Side.hist = []

    def wtile(raw, slab, c):
        return tr(pltpu.bitcast(raw[c * 128:(c + 1) * 128, pl.ds(_mult(slab * 128, 128), 128)], U32))

    def wstore_split(ref, g, raw, slab):
        off = _mult(g * 64, 64)
        for c in range(8):
            ref[c, pl.ds(off, 64), :] = _pack(_unpack_split(wtile(raw, slab, c)))

    def wstore_shuf(ref, g, raw, slab):
        off = _mult(g * 64, 64)
        for c in range(8):
            ref[c, pl.ds(off, 64), :] = _pack_split(_unpk(wtile(raw, slab, c)).astype(F32))

    def wstore_perm(ref, g, raw, slab):
        for c in range(8):
            pk = wtile(raw, slab, c)
            for h4 in range(4):
                ref[c, pl.ds(g * 64 + h4, 16, stride=4), :] = pk[h4 * 16:(h4 + 1) * 16, :]

    def cols(ref, g):
        return ref[:, pl.ds(_mult(g * 128, 128), 128)]

    class LN:
        def __init__(self, b, link=None):
            self.b = b
            self.link = CFG["ln_link"] if link is None else link
            self.piv = None
            self.s1 = []
            self.s2 = []

        def add(self, xt):
            if self.piv is None:
                self.piv = jnp.broadcast_to(xt[0:1, :], (8, L))
            d = [r - self.piv for r in _rows(xt)]
            self.s1 = [_chain(jnp.add, self.s1 + d, 1)]
            self.s2 = [_chain(jnp.add, self.s2 + [x * x for x in d], 1)]

        def finish(self):
            b = self.b
            m1 = jnp.sum(self.s1[0], axis=0, keepdims=True) * (1.0 / D)
            m2 = jnp.sum(self.s2[0], axis=0, keepdims=True) * (1.0 / D)
            var = jnp.maximum(m2 - m1 * m1, 0.0)
            rs = lax.rsqrt(var + 1e-5)
            mrs = jnp.broadcast_to((self.piv[0:1, :] + m1) * rs, (8, L))
            rs = jnp.broadcast_to(rs, (8, L))
            never = rs < 0.0
            link = self.link
            kk = b.k + b.z("op_xt")
            rng = list(range(D // 16))
            if CFG["ln_rev"]:
                rng = rng[::-1]
            for n, r in enumerate(rng):
                pk = _pack_i(xT[b.hf][kk, r * 16:r * 16 + 8, :] * rs - mrs,
                             xT[b.hf][kk, r * 16 + 8:r * 16 + 16, :] * rs - mrs)
                xn[b.hf][b.k, r * 8:(r + 1) * 8, :] = pk
                if link and n % link == link - 1:
                    rs = jnp.where(never, pltpu.bitcast(pk, F32), rs)

    def prep_x(src, b):
        ln = LN(b)
        for cc in range(8):
            xt = _unpack_split(tr(xio[src, :, cc * L:(cc + 1) * L]))
            xT[b.hf][b.k, cc * 128:(cc + 1) * 128, :] = xt
            ln.add(xt)
        ln.finish()

    def fold(dst, g, slab):
        val = _mm_nt(_unpk(pmat[g]), cols(wa_raw, slab)) * LOG2E
        off = _mult(g * 64, 64)
        for c in range(8):
            dst[c, pl.ds(off, 64), :] = _pack_split(val[:, c * L:(c + 1) * L])

    def prep_set(g):
        wstore_split(woaT, g, woa_raw, g)
        wstore_perm(wkvbT, g, wb_raw, 8 + g)
        wstore_split(wkvbT, 8 + g, wb_raw, 16 + g)

    def prep_late(g):
        wstore_perm(wqbT, g, wb_raw, g)
        wstore_split(wobT, g, wob_raw, g)

    def mmw(ref, r0, n, rhs, sub):
        return jnp.concatenate([_mm(wload(ref, r, sub), rhs()) for r in range(r0, r0 + n, sub)], axis=0)

    def proj(ref, r0, n, b, sub=None, fresh=False):
        kk = b.k + b.z("op_xn") if fresh else b.k
        return mmw(ref, r0, n, lambda: _unpk(xn[b.hf][kk]), sub or CFG["sub"])

    def emit(steps, lag):
        pend = []
        for n, (main, late) in enumerate(steps):
            main()
            if late is not None:
                due = n + lag
                if n >= len(steps) - CFG["hold"]:
                    due = len(steps) + n
                pend.append((due, late))
            for due, f in sorted(pend, key=lambda e: e[0]):
                if due <= n:
                    f()
            pend = [e for e in pend if e[0] > n]
        for due, f in sorted(pend, key=lambda e: e[0]):
            f()
        deps.clear()

    def kv_finish(t, acc):
        r = lax.broadcasted_iota(jnp.int32, (64, 128), 0)
        c = lax.broadcasted_iota(jnp.int32, (64, 128), 1)
        kvm[t] = _pack_split(jnp.where((r // 32) == ((c // 2) % 2), acc, 0.0))

    def a_finish(lay):
        if not CFG["fin_z"]:
            zb[...] = jnp.broadcast_to(jnp.sum(zacc[lay], axis=1, keepdims=True), zb.shape)
        if not CFG["fin_kv"]:
            for t in range(16):
                kv_finish(t, kv_acc[lay, t])

    def a_kv(b, lay, last, fresh, vk=False):
        steps = []
        la = lay + b.z("op_acc") if last else lay
        for ch in range(NCH):
            def kstep(ch=ch):
                kp = proj(wkvaT, ch * MC, MC, b, CFG["sub_k"], fresh=fresh)
                for u in range(PPC):
                    t = ch * PPC + u
                    ep, en, sp, sn = _phi_parts(kp[u * 64:(u + 1) * 64, :])
                    r = _recip(sp * sn)
                    rp = r * sn
                    rn = r * sp
                    phi = jnp.concatenate([e * rp for e in ep] + [e * rn for e in en], axis=0)
                    phis[b.hf][ch][0, u * 64:(u + 1) * 64, :] = _pack_split(phi)
                    z = zacc[la, t * 128:(t + 1) * 128, :] + phi
                    zacc[la, t * 128:(t + 1) * 128, :] = z
                    if last and CFG["fin_z"]:
                        zb[t * 128:(t + 1) * 128, :] = jnp.broadcast_to(
                            jnp.sum(z, axis=1, keepdims=True), (128, L))

            def vstep(ch=ch):
                vs[b.hf][ch][0] = _pack_split(proj(wkvaT, D + ch * MC, MC, b, CFG["sub_v"], fresh=fresh))

            def mstep(ch=ch):
                for u in range(PPC):
                    t = ch * PPC + u
                    acc = kv_acc[la, t] + _mm_nt(_unpk(vs[b.hf][ch][b.z("op_v"), u * 32:(u + 1) * 32, :]),
                                                 _unpk(phis[b.hf][ch][b.z("op_phi"), u * 64:(u + 1) * 64, :]))
                    kv_acc[la, t] = acc
                    if last and CFG["fin_kv"]:
                        kv_finish(t, acc)

            if vk and not (last and ch == NCH - 1):
                steps.append((vstep, None))
                steps.append((kstep, mstep))
            else:
                steps.append((kstep, None))
                steps.append((vstep, mstep))
        return steps

    def a_q(b):
        steps = []
        for ch in range(NCH):
            def qstep(ch=ch):
                qp = proj(wqaT, ch * MC, MC, b, CFG["sub_q"])
                for u in range(PPC):
                    t = ch * PPC + u
                    ep, en, sp, sn = _phi_parts(qp[u * 64:(u + 1) * 64, :])
                    zr = _rows(zb[t * 128:(t + 1) * 128, :])
                    dp = _fold2(jnp.add, [e * zz for e, zz in zip(ep, zr[:8])])
                    dn = _fold2(jnp.add, [e * zz for e, zz in zip(en, zr[8:])])
                    r = _recip(dp * sn + dn * sp + 1e-6 * (sp * sn))
                    rp = r * sn
                    rn = r * sp
                    phi = jnp.concatenate([e * rp for e in ep] + [e * rn for e in en], axis=0)
                    phis[b.hf][ch][0, u * 64:(u + 1) * 64, :] = _pack_split(phi)

            def nstep(ch=ch):
                for u in range(PPC):
                    t = ch * PPC + u
                    o = _mm(_unpk(kvm[t]), _unpk(phis[b.hf][ch][b.z("op_phi"), u * 64:(u + 1) * 64, :]))
                    os_[b.hf][0, t * 32:(t + 1) * 32, :] = _pack_split(o)

            steps.append((qstep, nstep))
        return steps

    def barrier():
        pl.semaphore_signal(bsem, 1)
        pl.semaphore_wait(bsem, 1)

    def o_rhs(b):
        return lambda: _unpk(os_[b.hf][b.z("op_o")])

    def out_proj(wo, b, link=None, defer=None):
        steps = []
        ln = LN(b, link)
        if defer is not None:
            defer.append((ln.finish, None))
        for ch in range(NCH):
            def ostep(ch=ch):
                m0 = ch * MC
                xt = xT[b.hf][b.k, m0:m0 + MC, :] + mmw(wo, m0, MC, o_rhs(b), CFG["sub_o"])
                xT[b.hf][b.k, m0:m0 + MC, :] = xt
                ln.add(xt)
                if ch == NCH - 1 and defer is None:
                    ln.finish()
            steps.append((ostep, None))
        return steps

    def b_kv(b):
        steps = []
        for base, ref in ((0, kb), (D, vb)):
            for m0 in range(0, D, MC):
                def step(base=base, ref=ref, m0=m0):
                    p = proj(wkvbT, base + m0, MC, b, CFG["sub_b"], fresh=True)
                    ref[WIN + b.j, m0:m0 + MC, :] = p
                    if b.hf == 0:
                        ref[b.k, m0:m0 + MC, :] = pltpu.roll(p, 2, 1)
                steps.append((step, None))
        return steps

    def b_q(b):
        j = b.j
        even = lax.broadcasted_iota(jnp.int32, (8, L), 0) % 2 == 0
        first = lax.broadcasted_iota(jnp.int32, (8, L), 1) < 2
        cs = DH ** -0.5

        def logits(q, g):
            acc = [None] * WIN
            for r in range(16):
                qv = q[r * 8:r * 8 + 8, :]
                for w in range(WIN):
                    t = qv * kb[WIN + j - w, g * 128 + r * 8:g * 128 + r * 8 + 8, :]
                    acc[w] = t if acc[w] is None else acc[w] + t
            return acc

        def attend(lg, heads):
            if b.hf == 1:
                lg = [l if w == 0 else jnp.where(jnp.logical_and(first, j < w), -1e9 / cs, l)
                      for w, l in enumerate(lg)]
            mx = _tree(jnp.maximum, lg)
            ex = [jnp.exp2((l - mx) * (cs * LOG2E)) for l in lg]
            rs = _recip(_tree(jnp.add, ex))
            at = [e * rs for e in ex]
            never = rs < 0.0
            for n, (h, s) in enumerate(heads):
                o = None
                for w in range(WIN):
                    a = jnp.broadcast_to(at[w][s:s + 1, :], (DH, L))
                    t = a * vb[WIN + j - w, h * DH:(h + 1) * DH, :]
                    o = t if o is None else o + t
                pk = _pack_split(o)
                os_[b.hf][0, h * 16:(h + 1) * 16, :] = pk
                if CFG["pv_link"] and n % CFG["pv_link"] == CFG["pv_link"] - 1 and n < len(heads) - 1:
                    lk = pltpu.bitcast(pk[0:8, :] | pk[8:16, :], F32)
                    at = [jnp.where(never, lk, a) for a in at]

        steps = []
        for G in range(4):
            def step(G=G):
                if CFG["att4"]:
                    for g in (2 * G, 2 * G + 1):
                        la = logits(proj(wqbT, g * 128, 128, b, 128), g)
                        attend([x + pltpu.roll(x, 7, 0) for x in la], [(4 * g + s, 2 * s) for s in range(4)])
                    return
                q = proj(wqbT, G * 256, 256, b)
                la, lb = logits(q[0:128, :], 2 * G), logits(q[128:256, :], 2 * G + 1)
                lg = [jnp.where(even, x + pltpu.roll(x, 7, 0), y + pltpu.roll(y, 1, 0)) for x, y in zip(la, lb)]
                attend(lg, [(G * 8 + hh, 2 * (hh % 4) + hh // 4) for hh in range(8)])
            steps.append((step, None))
        return steps

    def final_proj(b, defer=0):
        steps = []
        for ch in range(NCH):
            def ostep(ch=ch):
                m0 = ch * MC
                xt = xT[b.hf][b.k, m0:m0 + MC, :] + mmw(wobT, m0, MC, o_rhs(b), CFG["sub_o"])
                for u in range(GPC):
                    cc = ch * GPC + u
                    y = _pack_split(xt[u * 128:(u + 1) * 128, :])
                    if cc >= 8 - defer:
                        ystage[b.k + 1, cc * 64:(cc + 1) * 64, :] = y
                    else:
                        xio[b.j, :, cc * L:(cc + 1) * L] = tr(y)
            steps.append((ostep, None))
        return steps

    def flush_out(k, slot):
        for cc in range(8 - CFG["out_defer"], 8):
            xio[slot, :, cc * L:(cc + 1) * L] = tr(ystage[k, cc * 64:(cc + 1) * 64, :])

    kv_acc[...] = jnp.zeros(kv_acc.shape, F32)
    zacc[...] = jnp.zeros(zacc.shape, F32)
    ystage[0] = jnp.zeros(ystage.shape[1:], U32)

    def unsplit(r):
        return (r // 16) * 16 + 2 * (r % 8) + (r // 8) % 2

    r128 = unsplit(lax.broadcasted_iota(jnp.int32, (128, 128), 0))
    c128 = lax.broadcasted_iota(jnp.int32, (128, 128), 1)
    same_head = (2 * (r128 // 64) + r128 % 2) == (c128 // 32)
    er = unsplit(lax.broadcasted_iota(jnp.int32, (128, 32), 0))
    ec = lax.broadcasted_iota(jnp.int32, (128, 32), 1)
    expand = jnp.where(((er % 64) // 2) == ec, 1.0, 0.0).astype(BF16)
    cp_phi.wait()
    for g in range(8):
        pg = _mm_nt(expand, wphi[g * 128:(g + 1) * 128, :])
        pmat[g] = _pack(jnp.where(same_head, pg, 0.0))

    only = CFG["only"] or (0, 1, 2, 3, 5)
    x_in(8).wait()
    prep_x(8, Blk(0, 0))
    sa = a_kv(Blk(0, 0), 0, False, False)
    sb = a_kv(Blk(1, 0), 0, False, False)
    pend = []
    for ch in range(NCH if 0 in only else 0):
        cp_k[ch].wait()
        if ch == 0:
            for u in range(GPC):
                fold(wkvaT, u, 8 + u)
            sa[0][0]()
            x_in(0).wait()
        cp_v[ch].wait()
        if ch == 2:
            x_in(9).wait()
            x_in(1).wait()
        if ch == 0:
            prep_x(0, Blk(1, 0))
        else:
            for u in range(GPC):
                fold(wkvaT, ch * GPC + u, 8 + ch * GPC + u)
        for u in range(GPC):
            wstore_shuf(wkvaT, 8 + ch * GPC + u, wa_raw, 16 + ch * GPC + u)
        for f in pend:
            f()
        if ch >= 2:
            prep_x(Blk(ch - 2, 1).j, Blk(ch - 2, 1))
        if ch == 0:
            sa[1][0]()
            sb[0][0]()
        else:
            sa[2 * ch][0]()
            sb[2 * ch][0]()
            sa[2 * ch + 1][0]()
        sb[2 * ch + 1][0]()
        pend = [sa[2 * ch + 1][1], sb[2 * ch + 1][1]]
    for f in pend:
        f()

    def s1(i, c):
        @pl.when(i < 7)
        def _():
            x_in(9 + i).wait()
            x_in(1 + i).wait()

        wait_all(w_set(i - 1))
        side_begin(Blk(0, i))
        steps = a_kv(Blk(0, i), 0, False, False, CFG["vk"]) + a_kv(Blk(1, i), 0, True, False, CFG["vk"])
        nxt = jnp.minimum(i + 1, 7)
        prep_x(8 + nxt, Blk(0, i + 1))
        prep_x(nxt, Blk(1, i + 1))
        prep_set(i - 1)
        steps.insert(CFG["fold_at"], (lambda: fold(wqaT, i - 1, i - 1), None))
        emit(steps, CFG["lag_kv"])
        return c
    if 1 in only:
        lax.fori_loop(1, 8, s1, 0)
    side_begin(None)
    wait_all(w_set(7))
    fold(wqaT, 7, 7)
    prep_set(7)
    a_finish(0)
    wait_all(cp_late)

    def s2(ii, c):
        steps = []
        for u in range(CFG["u2"]):
            i = ii * CFG["u2"] + u
            b0, b1 = Blk(0, i), Blk(1, i)
            steps += a_q(b0) + a_q(b1) + out_proj(woaT, b0) + out_proj(woaT, b1)
            steps += [(lambda i=i: prep_late(i), None)]
            steps += b_kv(b0) + b_kv(b1)
        emit(steps, CFG["lag_q"])
        return c

    def s3(i, c):
        b0, b1 = Blk(0, i), Blk(1, i)
        dfr = [] if CFG["ln_defer"] else None
        steps = b_q(b0) + b_q(b1) + out_proj(wobT, b0, CFG["link3"], dfr) + out_proj(wobT, b1, CFG["link3"])
        if CFG["dbg"] == 1:
            steps = steps[8:]
        if CFG["dbg"] == 2:
            steps = steps[4:]
        steps += a_kv(b0, 1, False, True, CFG["vk"]) + a_kv(b1, 1, True, True, CFG["vk"])
        if CFG["bar3"]:
            steps[CFG["bar3"]:CFG["bar3"]] = [(barrier, None)] + (dfr or [])
        if CFG["dbg"] == 4:
            qs = b_q(Blk(0, i + 1)) + b_q(Blk(1, i + 1))
            kv = steps[16:]
            steps = steps[8:16]
            for n in range(8):
                steps += [qs[n], kv[2 * n], kv[2 * n + 1]]
        if CFG["dbg"] == 5:
            qs = b_q(Blk(0, i + 1)) + b_q(Blk(1, i + 1))
            kv = steps[16:]
            steps = steps[8:16]
            for n in range(8):
                steps += [kv[2 * n], qs[n], kv[2 * n + 1]]
        emit(steps, CFG["lag_kv"])
        return c

    ND = CFG["out_defer"]

    def s5(i, c):
        b0, b1 = Blk(0, i), Blk(1, i)

        def flush():
            flush_out(i, jnp.where(i > 0, i - 1, NBLK))

        steps = b_q(b0) + b_q(b1) + [(flush, None)] + final_proj(b0) + final_proj(b1, ND)
        steps.insert(CFG["out_at"], (x_out(b0.j).start, None))
        emit(steps, 0)
        x_out(b1.j, 0, 8 - ND).start()

        @pl.when(i > 0)
        def _():
            x_out(i - 1, 8 - ND, 8, SEM_KV + i - 1).start()
        return c

    def layer_pair(l, c):
        if 2 in only:
            lax.fori_loop(0, 8 // CFG["u2"], s2, 0)

        @pl.when(l == 0)
        def _():
            if 3 in only:
                lax.fori_loop(0, 8, s3, 0)
                a_finish(1)

        @pl.when(l == 1)
        def _():
            if 5 in only:
                lax.fori_loop(0, 8, s5, 0)
        return c
    lax.fori_loop(0, 2, layer_pair, 0)

    flush_out(8, 7)
    x_out(7, 8 - ND, 8, SEM_KV + 7).start()
    for k in range(8):
        x_out(8 + k).wait()
        x_out(k, 0, 8 - ND).wait()
        x_out(k, 8 - ND, 8, SEM_KV + k).wait()


@jax.jit
def pallas_interleave_layers__linear_kernel_hedgehog__sliding_local_dilated__prompt_kernel(
    A_x: jax.Array,
    A_wqkv: jax.Array,
    A_w_phi: jax.Array,
    A_wo: jax.Array,
    B_x: jax.Array,
    B_wqkv: jax.Array,
    B_wo: jax.Array,
):
    del B_x
    x3 = A_x.reshape(S // 32, 32, D)
    wphi2 = A_w_phi.reshape(H * DH, DH)
    any_spec = pl.BlockSpec(memory_space=pl.ANY)
    scratch = [
        pltpu.VMEM((NBLK + 1, S // 32, D), U32),
        pltpu.VMEM((D, 3 * D), BF16),
        pltpu.VMEM((D, D), BF16),
        pltpu.VMEM((D, 3 * D), BF16),
        pltpu.VMEM((D, D), BF16),
        pltpu.VMEM((H * DH, DH), BF16),
        pltpu.VMEM((8, 64, 128), U32),
        pltpu.VMEM((8, D // 2, L), U32),
        pltpu.VMEM((8, D, L), U32),
        pltpu.VMEM((8, D // 2, L), U32),
        pltpu.VMEM((8, D // 2, L), U32),
        pltpu.VMEM((8, D, L), U32),
        pltpu.VMEM((8, D // 2, L), U32),
        pltpu.VMEM((WIN + NBLK, D, L), F32),
        pltpu.VMEM((WIN + NBLK, D, L), F32),
        pltpu.VMEM((2, 16, 64, 128), F32),
        pltpu.VMEM((16, 32, 128), U32),
        pltpu.VMEM((2, 2 * D, L), F32),
        pltpu.VMEM((2 * D, L), F32),
        pltpu.VMEM((9, D // 2, L), U32),
        pltpu.SemaphoreType.DMA((NSEM,)),
        pltpu.SemaphoreType.REGULAR,
    ]
    scratch += [pltpu.VMEM((9, D, L), F32)] * 2
    scratch += [pltpu.VMEM((9, D // 2, L), U32)] * 2
    scratch += [pltpu.VMEM((1, D // 2, L), U32)] * 2
    scratch += [pltpu.VMEM((1, MC, L), U32)] * (2 * NCH)
    scratch += [pltpu.VMEM((1, MC // 2, L), U32)] * (2 * NCH)
    out = pl.pallas_call(
        _kernel,
        out_shape=jax.ShapeDtypeStruct((S // 32, 32, D), BF16),
        in_specs=[any_spec] * 6,
        out_specs=any_spec,
        scratch_shapes=scratch,
        compiler_params=pltpu.CompilerParams(vmem_limit_bytes=120 * 1024 * 1024, **CFG["cp"]),
        name="hedgehog_dilated",
    )(x3, A_wqkv, wphi2, A_wo, B_wqkv, B_wo)
    return out.reshape(1, S, D)
```

```python
import math

import jax
import jax.numpy as jnp
from jax import lax
import jax.experimental.pallas as pl
import jax.experimental.pallas.tpu as pltpu

S = 2048
D = 1024
H = 32
DH = 32
NBLK = 16
L = 128
WIN = 8
HALO = WIN - 1
LOG2E = math.log2(math.e)
F32 = jnp.float32
BF16 = jnp.bfloat16
U32 = jnp.uint32
NT = (((1,), (1,)), ((), ()))

MC = 256
NCH = D // MC
GPC = MC // 128
PPC = MC // 64
CFG = dict(vk=False, link3=4, lag_q=1, lag_kv=2, only=None, ln_link=4, ln_rev=False, sub=256, sub_o=256, sub_b=256,
           op_acc=True, op_phi=False, op_v=False, op_o=False, op_xt=False, op_xn=False,
           fin_z=True, fin_kv=True, sub_q=128, sub_k=128, sub_v=256, arecip=True, dbg=0, att_dl=0, pv_link=0, pv_slow=0, bar3=13, ln_defer=True, side=2, out_defer=2, u2=1, out_at=17, cp=dict(disable_semaphore_checks=True), fold_at=2, hold=7, att4=False, b2_at=1, side0=True)

SEM_X = 0
SEM_PHI = 16
SEM_KV = 18
SEM_SET = 26
SEM_LATE = 34
NSEM = 35


def _mm(a, b):
    return jnp.dot(a, b, preferred_element_type=F32)


def _mm_nt(a, b):
    return lax.dot_general(a, b, NT, preferred_element_type=F32)


def _tree(op, xs):
    xs = list(xs)
    while len(xs) > 1:
        nxt = [op(xs[i], xs[i + 1]) for i in range(0, len(xs) - 1, 2)]
        if len(xs) % 2:
            nxt.append(xs[-1])
        xs = nxt
    return xs[0]


def _chain(op, xs, ways=4):
    acc = list(xs[:ways])
    for i, x in enumerate(xs[ways:]):
        acc[i % ways] = op(acc[i % ways], x)
    return _tree(op, acc)


def _rows(a, n=8):
    return [a[i * n:(i + 1) * n, :] for i in range(a.shape[0] // n)]


def _pack(a):
    return pltpu.bitcast(a.astype(BF16), U32)


def _unpk(a):
    return pltpu.bitcast(a, BF16)


def _pack_i(a, b):
    return pltpu.pack_elementwise([a, b], packed_dtype=BF16)


def _pack_split(a):
    r = _rows(a)
    return jnp.concatenate([_pack_i(r[2 * i], r[2 * i + 1]) for i in range(len(r) // 2)], axis=0)


def _unpack_split(p):
    out = []
    for x in _rows(p):
        out.append(pltpu.unpack_elementwise(x, index=0, packed_dtype=BF16, unpacked_dtype=F32))
        out.append(pltpu.unpack_elementwise(x, index=1, packed_dtype=BF16, unpacked_dtype=F32))
    return jnp.concatenate(out, axis=0)


def _fold2(op, xs):
    r = _tree(op, xs)
    r = op(r, pltpu.roll(r, 4, 0))
    return op(r, pltpu.roll(r, 2, 0))


def _phi_parts(p):
    ps = _rows(p)
    mx = _fold2(jnp.maximum, ps)
    mn = _fold2(jnp.minimum, ps)
    ep = [jnp.exp2(x - mx) for x in ps]
    en = [jnp.exp2(mn - x) for x in ps]
    sp = _fold2(jnp.add, ep)
    sn = _fold2(jnp.add, en)
    return ep, en, sp, sn


def _recip(x):
    if not CFG["arecip"]:
        return 1.0 / x
    r = pl.reciprocal(x, approx=True)
    return r * (2.0 - x * r)


def _mult(x, m):
    return x if isinstance(x, int) else pl.multiple_of(x, m)


def _kernel(x_hbm, wa_hbm, wphi_hbm, woa_hbm, wb_hbm, wob_hbm, out_hbm,
            xio, wa_raw, woa_raw, wb_raw, wob_raw, wphi, pmat,
            wqaT, wkvaT, woaT, wqbT, wkvbT, wobT, kb, vb, kv_acc, kvm, zacc, zb, ystage, sems, bsem, *rest):
    xT, xn, os_ = rest[0:2], rest[2:4], rest[4:6]
    phis = [rest[6:6 + NCH], rest[6 + NCH:6 + 2 * NCH]]
    vs = [rest[6 + 2 * NCH:6 + 3 * NCH], rest[6 + 3 * NCH:6 + 4 * NCH]]

    class Blk:
        def __init__(self, hf, k, opaque=True):
            self.hf, self.k = hf, k
            self.j = 8 * (1 - hf) + k
            self.zr = 0 if (isinstance(k, int) or not opaque) else k >> 6

        def z(self, key):
            return self.zr if CFG[key] else 0

    x32 = x_hbm.bitcast(U32)
    out32 = out_hbm.bitcast(U32)

    def x_in(j):
        return pltpu.make_async_copy(x32.at[:, j, :], xio.at[j], sems.at[SEM_X + j])

    def x_out(j, c0=0, c1=8, sem=None):
        cs = pl.ds(c0 * L, (c1 - c0) * L)
        return pltpu.make_async_copy(xio.at[j, :, cs], out32.at[:, j, cs],
                                     sems.at[SEM_X + j if sem is None else sem])

    wa32, woa32, wb32, wob32 = [w.bitcast(U32) for w in (wa_hbm, woa_hbm, wb_hbm, wob_hbm)]

    def slabs(src, dst, g0, n, sem):
        return [pltpu.make_async_copy(src.at[:, pl.ds(_mult((g0 + u) * 128, 128), 128)], dst.at[g0 + u],
                                      sems.at[sem]) for u in range(n)]

    cp_phi = pltpu.make_async_copy(wphi_hbm.at[0:MC], wphi.at[0:MC], sems.at[SEM_PHI])
    cp_phi2 = pltpu.make_async_copy(wphi_hbm.at[MC:D], wphi.at[MC:D], sems.at[SEM_PHI + 1])
    cp_k = [slabs(wa32, wa_raw, 8 + ch * GPC, GPC, SEM_KV + 2 * ch) for ch in range(NCH)]
    cp_v = [slabs(wa32, wa_raw, 16 + ch * GPC, GPC, SEM_KV + 2 * ch + 1) for ch in range(NCH)]

    def w_set(g):
        return (slabs(wa32, wa_raw, g, 1, SEM_SET + g) + slabs(woa32, woa_raw, g, 1, SEM_SET + g)
                + slabs(wb32, wb_raw, 8 + g, 1, SEM_SET + g) + slabs(wb32, wb_raw, 16 + g, 1, SEM_SET + g))

    cp_late = slabs(wb32, wb_raw, 0, 8, SEM_LATE) + slabs(wob32, wob_raw, 0, 8, SEM_LATE)

    batch = [[cp_phi, x_in(8)] + cp_k[0] + [x_in(0)] + cp_v[0] + [cp_phi2] + cp_k[1] + cp_v[1], [], []]
    batch[1] += cp_k[2] + cp_v[2] + cp_k[3] + cp_v[3] + [x_in(9), x_in(1)]
    for g in range(8):
        n = 1 if g < 6 else 2
        if g < 6:
            batch[n] += [x_in(10 + g), x_in(2 + g)]
        batch[n] += w_set(g)
    batch[2] += cp_late

    def start_all(cps):
        for c in cps:
            c.start()

    start_all(batch[0])

    def wait_all(cps):
        for c in cps:
            c.wait()

    deps = []

    def wload(ref, r0, n):
        parts = [ref[c, r0 // 2:(r0 + n) // 2, :] for c in range(8)]
        while deps:
            never, val = deps.pop()
            head = jnp.where(never, val, parts[0][0:8, :])
            parts[0] = jnp.concatenate([head, parts[0][8:, :]], axis=0)
        return jnp.concatenate([_unpk(x) for x in parts], axis=1)

    class Side:
        never = None
        hist = []

    def tr(x):
        w = CFG["side"]
        if Side.never is not None and w and len(Side.hist) >= w:
            x = jnp.concatenate([jnp.where(Side.never, Side.hist[-w], x[0:8, :]), x[8:, :]], axis=0)
        y = pltpu.bitcast(_unpk(x).T, U32)
        Side.hist.append(y[56:64, :])
        return y

    def side_begin(b):
        Side.never = None if b is None else jnp.full((8, L), b.zr, jnp.int32) > 0
        Side.hist = []

    def wtile(raw, slab, c):
        return tr(raw[slab, c * 64:(c + 1) * 64, :])

    def wstore_split(ref, g, raw, slab):
        off = _mult(g * 64, 64)
        for c in range(8):
            ref[c, pl.ds(off, 64), :] = _pack(_unpack_split(wtile(raw, slab, c)))

    def wstore_shuf(ref, g, raw, slab):
        off = _mult(g * 64, 64)
        for c in range(8):
            ref[c, pl.ds(off, 64), :] = _pack_split(_unpk(wtile(raw, slab, c)).astype(F32))

    def wstore_perm(ref, g, raw, slab):
        for c in range(8):
            pk = wtile(raw, slab, c)
            for h4 in range(4):
                ref[c, pl.ds(g * 64 + h4, 16, stride=4), :] = pk[h4 * 16:(h4 + 1) * 16, :]

    class LN:
        def __init__(self, b, link=None):
            self.b = b
            self.link = CFG["ln_link"] if link is None else link
            self.piv = None
            self.s1 = []
            self.s2 = []

        def add(self, xt):
            if self.piv is None:
                self.piv = jnp.broadcast_to(xt[0:1, :], (8, L))
            d = [r - self.piv for r in _rows(xt)]
            self.s1 = [_chain(jnp.add, self.s1 + d, 1)]
            self.s2 = [_chain(jnp.add, self.s2 + [x * x for x in d], 1)]

        def finish(self):
            b = self.b
            m1 = jnp.sum(self.s1[0], axis=0, keepdims=True) * (1.0 / D)
            m2 = jnp.sum(self.s2[0], axis=0, keepdims=True) * (1.0 / D)
            var = jnp.maximum(m2 - m1 * m1, 0.0)
            rs = lax.rsqrt(var + 1e-5)
            mrs = jnp.broadcast_to((self.piv[0:1, :] + m1) * rs, (8, L))
            rs = jnp.broadcast_to(rs, (8, L))
            never = rs < 0.0
            link = self.link
            kk = b.k + b.z("op_xt")
            rng = list(range(D // 16))
            if CFG["ln_rev"]:
                rng = rng[::-1]
            for n, r in enumerate(rng):
                pk = _pack_i(xT[b.hf][kk, r * 16:r * 16 + 8, :] * rs - mrs,
                             xT[b.hf][kk, r * 16 + 8:r * 16 + 16, :] * rs - mrs)
                xn[b.hf][b.k, r * 8:(r + 1) * 8, :] = pk
                if link and n % link == link - 1:
                    rs = jnp.where(never, pltpu.bitcast(pk, F32), rs)

    def prep_x(src, b):
        ln = LN(b)
        for cc in range(8):
            xt = _unpack_split(tr(xio[src, :, cc * L:(cc + 1) * L]))
            xT[b.hf][b.k, cc * 128:(cc + 1) * 128, :] = xt
            ln.add(xt)
        ln.finish()

    def fold(dst, g, slab):
        val = _mm_nt(_unpk(pmat[g]), _unpk(wa_raw[slab])) * LOG2E
        off = _mult(g * 64, 64)
        for c in range(8):
            dst[c, pl.ds(off, 64), :] = _pack_split(val[:, c * L:(c + 1) * L])

    def prep_set(g):
        wstore_split(woaT, g, woa_raw, g)
        wstore_perm(wkvbT, g, wb_raw, 8 + g)
        wstore_split(wkvbT, 8 + g, wb_raw, 16 + g)

    def prep_late(g):
        if CFG["dbg"] == 7:
            return
        if CFG["dbg"] == 8:
            wstore_split(wqbT, g, wb_raw, g)
        else:
            wstore_perm(wqbT, g, wb_raw, g)
        wstore_split(wobT, g, wob_raw, g)

    def mmw(ref, r0, n, rhs, sub):
        return jnp.concatenate([_mm(wload(ref, r, sub), rhs()) for r in range(r0, r0 + n, sub)], axis=0)

    def proj(ref, r0, n, b, sub=None, fresh=False):
        kk = b.k + b.z("op_xn") if fresh else b.k
        return mmw(ref, r0, n, lambda: _unpk(xn[b.hf][kk]), sub or CFG["sub"])

    def emit(steps, lag):
        pend = []
        for n, (main, late) in enumerate(steps):
            main()
            if late is not None:
                due = n + lag
                if n >= len(steps) - CFG["hold"]:
                    due = len(steps) + n
                pend.append((due, late))
            for due, f in sorted(pend, key=lambda e: e[0]):
                if due <= n:
                    f()
            pend = [e for e in pend if e[0] > n]
        for due, f in sorted(pend, key=lambda e: e[0]):
            f()
        deps.clear()

    def kv_finish(t, acc):
        r = lax.broadcasted_iota(jnp.int32, (64, 128), 0)
        c = lax.broadcasted_iota(jnp.int32, (64, 128), 1)
        kvm[t] = _pack_split(jnp.where((r >> 5) == ((c >> 1) & 1), acc, 0.0))

    def a_finish(lay):
        if not CFG["fin_z"]:
            zb[...] = jnp.broadcast_to(jnp.sum(zacc[lay], axis=1, keepdims=True), zb.shape)
        if not CFG["fin_kv"]:
            for t in range(16):
                kv_finish(t, kv_acc[lay, t])

    def a_kv(b, lay, last, fresh, vk=False):
        steps = []
        la = lay + b.z("op_acc") if last else lay
        for ch in range(NCH):
            def kstep(ch=ch):
                kp = proj(wkvaT, ch * MC, MC, b, CFG["sub_k"], fresh=fresh)
                for u in range(PPC):
                    t = ch * PPC + u
                    ep, en, sp, sn = _phi_parts(kp[u * 64:(u + 1) * 64, :])
                    r = _recip(sp * sn)
                    rp = r * sn
                    rn = r * sp
                    phi = jnp.concatenate([e * rp for e in ep] + [e * rn for e in en], axis=0)
                    phis[b.hf][ch][0, u * 64:(u + 1) * 64, :] = _pack_split(phi)
                    z = zacc[la, t * 128:(t + 1) * 128, :] + phi
                    zacc[la, t * 128:(t + 1) * 128, :] = z
                    if last and CFG["fin_z"]:
                        zb[t * 128:(t + 1) * 128, :] = jnp.broadcast_to(
                            jnp.sum(z, axis=1, keepdims=True), (128, L))

            def vstep(ch=ch):
                vs[b.hf][ch][0] = _pack_split(proj(wkvaT, D + ch * MC, MC, b, CFG["sub_v"], fresh=fresh))

            def mstep(ch=ch):
                for u in range(PPC):
                    t = ch * PPC + u
                    acc = kv_acc[la, t] + _mm_nt(_unpk(vs[b.hf][ch][b.z("op_v"), u * 32:(u + 1) * 32, :]),
                                                 _unpk(phis[b.hf][ch][b.z("op_phi"), u * 64:(u + 1) * 64, :]))
                    kv_acc[la, t] = acc
                    if last and CFG["fin_kv"]:
                        kv_finish(t, acc)

            if vk and not (last and ch == NCH - 1):
                steps.append((vstep, None))
                steps.append((kstep, mstep))
            else:
                steps.append((kstep, None))
                steps.append((vstep, mstep))
        return steps

    def a_q(b):
        steps = []
        for ch in range(NCH):
            def qstep(ch=ch):
                qp = proj(wqaT, ch * MC, MC, b, CFG["sub_q"])
                for u in range(PPC):
                    t = ch * PPC + u
                    ep, en, sp, sn = _phi_parts(qp[u * 64:(u + 1) * 64, :])
                    zr = _rows(zb[t * 128:(t + 1) * 128, :])
                    dp = _fold2(jnp.add, [e * zz for e, zz in zip(ep, zr[:8])])
                    dn = _fold2(jnp.add, [e * zz for e, zz in zip(en, zr[8:])])
                    r = _recip(dp * sn + dn * sp + 1e-6 * (sp * sn))
                    rp = r * sn
                    rn = r * sp
                    phi = jnp.concatenate([e * rp for e in ep] + [e * rn for e in en], axis=0)
                    phis[b.hf][ch][0, u * 64:(u + 1) * 64, :] = _pack_split(phi)

            def nstep(ch=ch):
                for u in range(PPC):
                    t = ch * PPC + u
                    o = _mm(_unpk(kvm[t]), _unpk(phis[b.hf][ch][b.z("op_phi"), u * 64:(u + 1) * 64, :]))
                    os_[b.hf][0, t * 32:(t + 1) * 32, :] = _pack_split(o)

            steps.append((qstep, nstep))
        return steps

    def barrier():
        pl.semaphore_signal(bsem, 1)
        pl.semaphore_wait(bsem, 1)

    def o_rhs(b):
        return lambda: _unpk(os_[b.hf][b.z("op_o")])

    def out_proj(wo, b, link=None, defer=None):
        steps = []
        ln = LN(b, link)
        if defer is not None:
            defer.append((ln.finish, None))
        for ch in range(NCH):
            def ostep(ch=ch):
                m0 = ch * MC
                xt = xT[b.hf][b.k, m0:m0 + MC, :] + mmw(wo, m0, MC, o_rhs(b), CFG["sub_o"])
                xT[b.hf][b.k, m0:m0 + MC, :] = xt
                ln.add(xt)
                if ch == NCH - 1 and defer is None:
                    ln.finish()
            steps.append((ostep, None))
        return steps

    def b_kv(b):
        steps = []
        for base, ref in ((0, kb), (D, vb)):
            for m0 in range(0, D, MC):
                def step(base=base, ref=ref, m0=m0):
                    p = proj(wkvbT, base + m0, MC, b, CFG["sub_b"], fresh=True)
                    ref[WIN + b.j, m0:m0 + MC, :] = p
                    if b.hf == 0:
                        ref[b.k, m0:m0 + MC, :] = pltpu.roll(p, 2, 1)
                steps.append((step, None))
        return steps

    def b_q(b):
        j = b.j
        even = (lax.broadcasted_iota(jnp.int32, (8, L), 0) & 1) == 0
        first = lax.broadcasted_iota(jnp.int32, (8, L), 1) < 2
        cs = DH ** -0.5

        def logits(q, g):
            acc = [None] * WIN
            for r in range(16):
                qv = q[r * 8:r * 8 + 8, :]
                for w in range(WIN):
                    t = qv * kb[WIN + j - w, g * 128 + r * 8:g * 128 + r * 8 + 8, :]
                    acc[w] = t if acc[w] is None else acc[w] + t
            return acc

        def attend(lg, heads):
            if b.hf == 1:
                lg = [l if w == 0 else jnp.where(jnp.logical_and(first, j < w), -1e9 / cs, l)
                      for w, l in enumerate(lg)]
            mx = _tree(jnp.maximum, lg)
            ex = [jnp.exp2((l - mx) * (cs * LOG2E)) for l in lg]
            rs = _recip(_tree(jnp.add, ex))
            at = [e * rs for e in ex]
            never = rs < 0.0
            for n, (h, s) in enumerate(heads):
                o = None
                for w in range(WIN):
                    a = jnp.broadcast_to(at[w][s:s + 1, :], (DH, L))
                    t = a * vb[WIN + j - w, h * DH:(h + 1) * DH, :]
                    o = t if o is None else o + t
                pk = _pack_split(o)
                os_[b.hf][0, h * 16:(h + 1) * 16, :] = pk
                if CFG["pv_link"] and n % CFG["pv_link"] == CFG["pv_link"] - 1 and n < len(heads) - 1:
                    lk = pltpu.bitcast(pk[0:8, :] | pk[8:16, :], F32)
                    at = [jnp.where(never, lk, a) for a in at]

        steps = []
        for G in range(4):
            def step(G=G):
                if CFG["att4"]:
                    for g in (2 * G, 2 * G + 1):
                        la = logits(proj(wqbT, g * 128, 128, b, 128), g)
                        attend([x + pltpu.roll(x, 7, 0) for x in la], [(4 * g + s, 2 * s) for s in range(4)])
                    return
                q = proj(wqbT, G * 256, 256, b)
                la, lb = logits(q[0:128, :], 2 * G), logits(q[128:256, :], 2 * G + 1)
                lg = [jnp.where(even, x + pltpu.roll(x, 7, 0), y + pltpu.roll(y, 1, 0)) for x, y in zip(la, lb)]
                attend(lg, [(G * 8 + hh, 2 * (hh % 4) + hh // 4) for hh in range(8)])
            steps.append((step, None))
        return steps

    def final_proj(b, defer=0):
        steps = []
        for ch in range(NCH):
            def ostep(ch=ch):
                m0 = ch * MC
                xt = xT[b.hf][b.k, m0:m0 + MC, :] + mmw(wobT, m0, MC, o_rhs(b), CFG["sub_o"])
                for u in range(GPC):
                    cc = ch * GPC + u
                    y = _pack_split(xt[u * 128:(u + 1) * 128, :])
                    if cc >= 8 - defer:
                        ystage[b.k + 1, cc * 64:(cc + 1) * 64, :] = y
                    else:
                        xio[b.j, :, cc * L:(cc + 1) * L] = tr(y)
            steps.append((ostep, None))
        return steps

    def flush_out(k, slot):
        for cc in range(8 - CFG["out_defer"], 8):
            xio[slot, :, cc * L:(cc + 1) * L] = tr(ystage[k, cc * 64:(cc + 1) * 64, :])

    kv_acc[...] = jnp.zeros(kv_acc.shape, F32)
    zacc[...] = jnp.zeros(zacc.shape, F32)
    ystage[0] = jnp.zeros(ystage.shape[1:], U32)

    def unsplit(r):
        return (r & ~15) + 2 * (r & 7) + ((r >> 3) & 1)

    def make_pmat(gs):
        r128 = unsplit(lax.broadcasted_iota(jnp.int32, (128, 128), 0))
        c128 = lax.broadcasted_iota(jnp.int32, (128, 128), 1)
        same_head = (2 * (r128 >> 6) + (r128 & 1)) == (c128 >> 5)
        er = unsplit(lax.broadcasted_iota(jnp.int32, (128, 32), 0))
        ec = lax.broadcasted_iota(jnp.int32, (128, 32), 1)
        expand = jnp.where(((er & 63) >> 1) == ec, 1.0, 0.0).astype(BF16)
        for g in gs:
            pg = _mm_nt(expand, wphi[g * 128:(g + 1) * 128, :])
            pmat[g] = _pack(jnp.where(same_head, pg, 0.0))

    only = CFG["only"] or (0, 1, 2, 3, 5)
    cp_phi.wait()
    x_in(8).wait()
    make_pmat(range(GPC))
    prep_x(8, Blk(0, 0))
    start_all(batch[1])
    sa = a_kv(Blk(0, 0), 0, False, False)
    sb = a_kv(Blk(1, 0), 0, False, False)
    pend = []
    for ch in range(NCH if 0 in only else 0):
        if ch == CFG["b2_at"]:
            start_all(batch[2])
        wait_all(cp_k[ch])
        if ch == 0:
            for u in range(GPC):
                fold(wkvaT, u, 8 + u)
            sa[0][0]()
            x_in(0).wait()
        wait_all(cp_v[ch])
        if ch == 0:
            cp_phi2.wait()
            prep_x(0, Blk(1, 0))
            make_pmat(range(GPC, 8))
        else:
            if ch == 3:
                x_in(9).wait()
                x_in(1).wait()
            for u in range(GPC):
                fold(wkvaT, ch * GPC + u, 8 + ch * GPC + u)
        for u in range(GPC):
            wstore_shuf(wkvaT, 8 + ch * GPC + u, wa_raw, 16 + ch * GPC + u)
        for f in pend:
            f()
        if ch == 3:
            if CFG["side0"]:
                Side.never = zacc[0, 0:8, :] < 0.0
                Side.hist = []
            prep_x(9, Blk(0, 1))
            prep_x(1, Blk(1, 1))
            side_begin(None)
        if ch == 0:
            sa[1][0]()
            sb[0][0]()
        else:
            sa[2 * ch][0]()
            sb[2 * ch][0]()
            sa[2 * ch + 1][0]()
        sb[2 * ch + 1][0]()
        pend = [sa[2 * ch + 1][1], sb[2 * ch + 1][1]]
    for f in pend:
        f()

    def s1(i, c):
        @pl.when(i < 7)
        def _():
            x_in(9 + i).wait()
            x_in(1 + i).wait()

        wait_all(w_set(i - 1))
        side_begin(Blk(0, i))
        steps = a_kv(Blk(0, i), 0, False, False, CFG["vk"]) + a_kv(Blk(1, i), 0, True, False, CFG["vk"])
        nxt = jnp.minimum(i + 1, 7)
        prep_x(8 + nxt, Blk(0, i + 1))
        prep_x(nxt, Blk(1, i + 1))
        prep_set(i - 1)
        steps.insert(CFG["fold_at"], (lambda: fold(wqaT, i - 1, i - 1), None))
        emit(steps, CFG["lag_kv"])
        return c
    if 1 in only:
        lax.fori_loop(1, 8, s1, 0)
    side_begin(None)
    wait_all(w_set(7))
    fold(wqaT, 7, 7)
    prep_set(7)
    a_finish(0)
    wait_all(cp_late)

    def s2(ii, c):
        steps = []
        for u in range(CFG["u2"]):
            i = ii * CFG["u2"] + u
            b0, b1 = Blk(0, i), Blk(1, i)
            steps += a_q(b0) + a_q(b1) + out_proj(woaT, b0) + out_proj(woaT, b1)
            steps += [(lambda i=i: prep_late(i), None)]
            steps += b_kv(b0) + b_kv(b1)
        emit(steps, CFG["lag_q"])
        return c

    def s3(i, c):
        b0, b1 = Blk(0, i), Blk(1, i)
        dfr = [] if CFG["ln_defer"] else None
        steps = b_q(b0) + b_q(b1) + out_proj(wobT, b0, CFG["link3"], dfr) + out_proj(wobT, b1, CFG["link3"])
        if CFG["dbg"] == 1:
            steps = steps[8:]
        if CFG["dbg"] == 2:
            steps = steps[4:]
        steps += a_kv(b0, 1, False, True, CFG["vk"]) + a_kv(b1, 1, True, True, CFG["vk"])
        if CFG["bar3"]:
            steps[CFG["bar3"]:CFG["bar3"]] = [(barrier, None)] + (dfr or [])
        if CFG["dbg"] == 4:
            qs = b_q(Blk(0, i + 1)) + b_q(Blk(1, i + 1))
            kv = steps[16:]
            steps = steps[8:16]
            for n in range(8):
                steps += [qs[n], kv[2 * n], kv[2 * n + 1]]
        if CFG["dbg"] == 5:
            qs = b_q(Blk(0, i + 1)) + b_q(Blk(1, i + 1))
            kv = steps[16:]
            steps = steps[8:16]
            for n in range(8):
                steps += [kv[2 * n], qs[n], kv[2 * n + 1]]
        emit(steps, CFG["lag_kv"])
        return c

    ND = CFG["out_defer"]

    def s5(i, c):
        b0, b1 = Blk(0, i), Blk(1, i)

        def flush():
            flush_out(i, jnp.where(i > 0, i - 1, NBLK))

        steps = b_q(b0) + b_q(b1) + [(flush, None)] + final_proj(b0) + final_proj(b1, ND)
        steps.insert(CFG["out_at"], (x_out(b0.j).start, None))
        emit(steps, 0)
        x_out(b1.j, 0, 8 - ND).start()

        @pl.when(i > 0)
        def _():
            x_out(i - 1, 8 - ND, 8, SEM_KV + i - 1).start()
        return c

    def layer_pair(l, c):
        if 2 in only:
            lax.fori_loop(0, 8 // CFG["u2"], s2, 0)

        @pl.when(l == 0)
        def _():
            if 3 in only:
                lax.fori_loop(0, 8, s3, 0)
                a_finish(1)

        @pl.when(l == 1)
        def _():
            if 5 in only:
                lax.fori_loop(0, 8, s5, 0)
        return c
    lax.fori_loop(0, 2, layer_pair, 0)

    flush_out(8, 7)
    x_out(7, 8 - ND, 8, SEM_KV + 7).start()
    for k in range(8):
        x_out(8 + k).wait()
        x_out(k, 0, 8 - ND).wait()
        x_out(k, 8 - ND, 8, SEM_KV + k).wait()


@jax.jit
def pallas_interleave_layers__linear_kernel_hedgehog__sliding_local_dilated__prompt_kernel(
    A_x: jax.Array,
    A_wqkv: jax.Array,
    A_w_phi: jax.Array,
    A_wo: jax.Array,
    B_x: jax.Array,
    B_wqkv: jax.Array,
    B_wo: jax.Array,
):
    del B_x
    x3 = A_x.reshape(S // 32, 32, D)
    wphi2 = A_w_phi.reshape(H * DH, DH)
    any_spec = pl.BlockSpec(memory_space=pl.ANY)
    scratch = [
        pltpu.VMEM((NBLK + 1, S // 32, D), U32),
        pltpu.VMEM((24, D // 2, L), U32),
        pltpu.VMEM((8, D // 2, L), U32),
        pltpu.VMEM((24, D // 2, L), U32),
        pltpu.VMEM((8, D // 2, L), U32),
        pltpu.VMEM((H * DH, DH), BF16),
        pltpu.VMEM((8, 64, 128), U32),
        pltpu.VMEM((8, D // 2, L), U32),
        pltpu.VMEM((8, D, L), U32),
        pltpu.VMEM((8, D // 2, L), U32),
        pltpu.VMEM((8, D // 2, L), U32),
        pltpu.VMEM((8, D, L), U32),
        pltpu.VMEM((8, D // 2, L), U32),
        pltpu.VMEM((WIN + NBLK, D, L), F32),
        pltpu.VMEM((WIN + NBLK, D, L), F32),
        pltpu.VMEM((2, 16, 64, 128), F32),
        pltpu.VMEM((16, 32, 128), U32),
        pltpu.VMEM((2, 2 * D, L), F32),
        pltpu.VMEM((2 * D, L), F32),
        pltpu.VMEM((9, D // 2, L), U32),
        pltpu.SemaphoreType.DMA((NSEM,)),
        pltpu.SemaphoreType.REGULAR,
    ]
    scratch += [pltpu.VMEM((9, D, L), F32)] * 2
    scratch += [pltpu.VMEM((9, D // 2, L), U32)] * 2
    scratch += [pltpu.VMEM((1, D // 2, L), U32)] * 2
    scratch += [pltpu.VMEM((1, MC, L), U32)] * (2 * NCH)
    scratch += [pltpu.VMEM((1, MC // 2, L), U32)] * (2 * NCH)
    out = pl.pallas_call(
        _kernel,
        out_shape=jax.ShapeDtypeStruct((S // 32, 32, D), BF16),
        in_specs=[any_spec] * 6,
        out_specs=any_spec,
        scratch_shapes=scratch,
        compiler_params=pltpu.CompilerParams(vmem_limit_bytes=120 * 1024 * 1024, **CFG["cp"]),
        name="hedgehog_dilated",
    )(x3, A_wqkv, wphi2, A_wo, B_wqkv, B_wo)
    return out.reshape(1, S, D)
```

```python
import math

import jax
import jax.numpy as jnp
from jax import lax
import jax.experimental.pallas as pl
import jax.experimental.pallas.tpu as pltpu

S = 2048
D = 1024
H = 32
DH = 32
NBLK = 16
L = 128
WIN = 8
LOG2E = math.log2(math.e)
F32 = jnp.float32
BF16 = jnp.bfloat16
U32 = jnp.uint32
NT = (((1,), (1,)), ((), ()))

MC = 256
NCH = D // MC
GPC = MC // 128
PPC = MC // 64
ND = 2

CFG = dict(only=None, lag_q=1, lag_kv=2, hold=7, ln_link=4, side=2, bar3=13, fold_at=2,
           sub_q=128, sub_k=128, sub_v=256, sub_qb=256, sub_o=256, sub_b=256)

SEM_X = 0
SEM_PHI = 16
SEM_KV = 18
SEM_SET = 26
SEM_LATE = 34
NSEM = 35


def _mm(a, b):
    return jnp.dot(a, b, preferred_element_type=F32)


def _mm_nt(a, b):
    return lax.dot_general(a, b, NT, preferred_element_type=F32)


def _tree(op, xs):
    xs = list(xs)
    while len(xs) > 1:
        nxt = [op(xs[i], xs[i + 1]) for i in range(0, len(xs) - 1, 2)]
        if len(xs) % 2:
            nxt.append(xs[-1])
        xs = nxt
    return xs[0]


def _running_sum(acc, xs):
    for x in xs:
        acc = x if acc is None else acc + x
    return acc


def _rows(a, n=8):
    return [a[i * n:(i + 1) * n, :] for i in range(a.shape[0] // n)]


def _pack(a):
    return pltpu.bitcast(a.astype(BF16), U32)


def _unpk(a):
    return pltpu.bitcast(a, BF16)


def _pack_i(a, b):
    return pltpu.pack_elementwise([a, b], packed_dtype=BF16)


def _pack_split(a):
    r = _rows(a)
    return jnp.concatenate([_pack_i(r[2 * i], r[2 * i + 1]) for i in range(len(r) // 2)], axis=0)


def _unpack_split(p):
    out = []
    for x in _rows(p):
        out.append(pltpu.unpack_elementwise(x, index=0, packed_dtype=BF16, unpacked_dtype=F32))
        out.append(pltpu.unpack_elementwise(x, index=1, packed_dtype=BF16, unpacked_dtype=F32))
    return jnp.concatenate(out, axis=0)


def _fold2(op, xs):
    r = _tree(op, xs)
    r = op(r, pltpu.roll(r, 4, 0))
    return op(r, pltpu.roll(r, 2, 0))


def _phi_parts(p):
    ps = _rows(p)
    mx = _fold2(jnp.maximum, ps)
    mn = _fold2(jnp.minimum, ps)
    ep = [jnp.exp2(x - mx) for x in ps]
    en = [jnp.exp2(mn - x) for x in ps]
    return ep, en, _fold2(jnp.add, ep), _fold2(jnp.add, en)


def _recip(x):
    r = pl.reciprocal(x, approx=True)
    return r * (2.0 - x * r)


def _mult(x, m):
    return x if isinstance(x, int) else pl.multiple_of(x, m)


def _kernel(x_hbm, wa_hbm, wphi_hbm, woa_hbm, wb_hbm, wob_hbm, out_hbm,
            xio, wa_raw, woa_raw, wb_raw, wob_raw, wphi, pmat,
            wqaT, wkvaT, woaT, wqbT, wkvbT, wobT, kb, vb, kv_acc, kvm, zacc, zb, ystage, sems, bsem, *rest):
    xT, xn, os_ = rest[0:2], rest[2:4], rest[4:6]
    phis = [rest[6:6 + NCH], rest[6 + NCH:6 + 2 * NCH]]
    vs = [rest[6 + 2 * NCH:6 + 3 * NCH], rest[6 + 3 * NCH:6 + 4 * NCH]]
    only = CFG["only"] or (0, 1, 2, 3, 5)

    class Blk:
        def __init__(self, hf, k):
            self.hf, self.k = hf, k
            self.j = 8 * (1 - hf) + k
            self.zr = 0 if isinstance(k, int) else k >> 6

    x32, out32, wa32, woa32, wb32, wob32 = [
        r.bitcast(U32) for r in (x_hbm, out_hbm, wa_hbm, woa_hbm, wb_hbm, wob_hbm)]

    def x_in(j):
        return pltpu.make_async_copy(x32.at[:, j, :], xio.at[j], sems.at[SEM_X + j])

    def x_out(j, c0=0, c1=8, sem=None):
        cs = pl.ds(c0 * L, (c1 - c0) * L)
        return pltpu.make_async_copy(xio.at[j, :, cs], out32.at[:, j, cs],
                                     sems.at[SEM_X + j if sem is None else sem])

    def slabs(src, dst, g0, n, sem):
        return [pltpu.make_async_copy(src.at[:, pl.ds(_mult((g0 + u) * 128, 128), 128)], dst.at[g0 + u],
                                      sems.at[sem]) for u in range(n)]

    cp_phi = pltpu.make_async_copy(wphi_hbm.at[0:MC], wphi.at[0:MC], sems.at[SEM_PHI])
    cp_phi2 = pltpu.make_async_copy(wphi_hbm.at[MC:D], wphi.at[MC:D], sems.at[SEM_PHI + 1])
    cp_k = [slabs(wa32, wa_raw, 8 + ch * GPC, GPC, SEM_KV + 2 * ch) for ch in range(NCH)]
    cp_v = [slabs(wa32, wa_raw, 16 + ch * GPC, GPC, SEM_KV + 2 * ch + 1) for ch in range(NCH)]

    def w_set(g):
        return (slabs(wa32, wa_raw, g, 1, SEM_SET + g) + slabs(woa32, woa_raw, g, 1, SEM_SET + g)
                + slabs(wb32, wb_raw, 8 + g, 1, SEM_SET + g) + slabs(wb32, wb_raw, 16 + g, 1, SEM_SET + g))

    cp_late = slabs(wb32, wb_raw, 0, 8, SEM_LATE) + slabs(wob32, wob_raw, 0, 8, SEM_LATE)

    batch = [[cp_phi, x_in(8)] + cp_k[0] + [x_in(0)] + cp_v[0] + [cp_phi2] + cp_k[1] + cp_v[1],
             cp_k[2] + cp_v[2] + cp_k[3] + cp_v[3] + [x_in(9), x_in(1)], []]
    for g in range(8):
        if g < 6:
            batch[1] += [x_in(10 + g), x_in(2 + g)] + w_set(g)
        else:
            batch[2] += w_set(g)
    batch[2] += cp_late

    def start_all(cps):
        for c in cps:
            c.start()

    def wait_all(cps):
        for c in cps:
            c.wait()

    start_all(batch[0])

    class Side:
        never = None
        hist = []

    def side_begin(never):
        Side.never = never
        Side.hist = []

    def tr(x):
        w = CFG["side"]
        if Side.never is not None and len(Side.hist) >= w:
            x = jnp.concatenate([jnp.where(Side.never, Side.hist[-w], x[0:8, :]), x[8:, :]], axis=0)
        y = pltpu.bitcast(_unpk(x).T, U32)
        Side.hist.append(y[56:64, :])
        return y

    def wtile(raw, slab, c):
        return tr(raw[slab, c * 64:(c + 1) * 64, :])

    def wstore_split(ref, g, raw, slab):
        for c in range(8):
            ref[c, pl.ds(_mult(g * 64, 64), 64), :] = _pack(_unpack_split(wtile(raw, slab, c)))

    def wstore_shuf(ref, g, raw, slab):
        for c in range(8):
            ref[c, pl.ds(_mult(g * 64, 64), 64), :] = _pack_split(_unpk(wtile(raw, slab, c)).astype(F32))

    def wstore_perm(ref, g, raw, slab):
        for c in range(8):
            pk = wtile(raw, slab, c)
            for h4 in range(4):
                ref[c, pl.ds(g * 64 + h4, 16, stride=4), :] = pk[h4 * 16:(h4 + 1) * 16, :]

    def make_pmat(gs):
        def unsplit(r):
            return (r & ~15) + 2 * (r & 7) + ((r >> 3) & 1)

        r128 = unsplit(lax.broadcasted_iota(jnp.int32, (128, 128), 0))
        c128 = lax.broadcasted_iota(jnp.int32, (128, 128), 1)
        same_head = (2 * (r128 >> 6) + (r128 & 1)) == (c128 >> 5)
        er = unsplit(lax.broadcasted_iota(jnp.int32, (128, 32), 0))
        ec = lax.broadcasted_iota(jnp.int32, (128, 32), 1)
        expand = jnp.where(((er & 63) >> 1) == ec, 1.0, 0.0).astype(BF16)
        for g in gs:
            pg = _mm_nt(expand, wphi[g * 128:(g + 1) * 128, :])
            pmat[g] = _pack(jnp.where(same_head, pg, 0.0))

    def fold(dst, g, slab):
        val = _mm_nt(_unpk(pmat[g]), _unpk(wa_raw[slab])) * LOG2E
        for c in range(8):
            dst[c, pl.ds(_mult(g * 64, 64), 64), :] = _pack_split(val[:, c * L:(c + 1) * L])

    def prep_set(g):
        wstore_split(woaT, g, woa_raw, g)
        wstore_perm(wkvbT, g, wb_raw, 8 + g)
        wstore_split(wkvbT, 8 + g, wb_raw, 16 + g)

    def prep_late(g):
        wstore_perm(wqbT, g, wb_raw, g)
        wstore_split(wobT, g, wob_raw, g)

    class LN:
        def __init__(self, b):
            self.b = b
            self.piv = self.s1 = self.s2 = None

        def add(self, xt):
            if self.piv is None:
                self.piv = jnp.broadcast_to(xt[0:1, :], (8, L))
            d = [r - self.piv for r in _rows(xt)]
            self.s1 = _running_sum(self.s1, d)
            self.s2 = _running_sum(self.s2, [x * x for x in d])

        def finish(self):
            b = self.b
            m1 = jnp.sum(self.s1, axis=0, keepdims=True) * (1.0 / D)
            m2 = jnp.sum(self.s2, axis=0, keepdims=True) * (1.0 / D)
            var = jnp.maximum(m2 - m1 * m1, 0.0)
            rs = lax.rsqrt(var + 1e-5)
            mrs = jnp.broadcast_to((self.piv[0:1, :] + m1) * rs, (8, L))
            rs = jnp.broadcast_to(rs, (8, L))
            never = rs < 0.0
            for r in range(D // 16):
                pk = _pack_i(xT[b.hf][b.k, r * 16:r * 16 + 8, :] * rs - mrs,
                             xT[b.hf][b.k, r * 16 + 8:r * 16 + 16, :] * rs - mrs)
                xn[b.hf][b.k, r * 8:(r + 1) * 8, :] = pk
                if r % CFG["ln_link"] == CFG["ln_link"] - 1:
                    rs = jnp.where(never, pltpu.bitcast(pk, F32), rs)

    def prep_x(src, b):
        ln = LN(b)
        for cc in range(8):
            xt = _unpack_split(tr(xio[src, :, cc * L:(cc + 1) * L]))
            xT[b.hf][b.k, cc * 128:(cc + 1) * 128, :] = xt
            ln.add(xt)
        ln.finish()

    def mmw(ref, r0, n, rhs, sub):
        def wload(r):
            return jnp.concatenate([_unpk(ref[c, r // 2:(r + sub) // 2, :]) for c in range(8)], axis=1)
        return jnp.concatenate([_mm(wload(r), rhs()) for r in range(r0, r0 + n, sub)], axis=0)

    def proj(ref, r0, n, b, sub):
        return mmw(ref, r0, n, lambda: _unpk(xn[b.hf][b.k]), sub)

    def out_mm(wo, ch, b):
        m0 = ch * MC
        return xT[b.hf][b.k, m0:m0 + MC, :] + mmw(wo, m0, MC, lambda: _unpk(os_[b.hf][...]), CFG["sub_o"])

    def emit(steps, lag):
        pend = []
        for n, (main, late) in enumerate(steps):
            main()
            if late is not None:
                pend.append((n + lag if n < len(steps) - CFG["hold"] else len(steps) + n, late))
            for due, f in pend:
                if due <= n:
                    f()
            pend = [e for e in pend if e[0] > n]
        for _, f in sorted(pend, key=lambda e: e[0]):
            f()

    def barrier():
        pl.semaphore_signal(bsem, 1)
        pl.semaphore_wait(bsem, 1)

    def a_kv(b, lay, last):
        steps = []
        la = lay + b.zr if last else lay
        for ch in range(NCH):
            def kstep(ch=ch):
                kp = proj(wkvaT, ch * MC, MC, b, CFG["sub_k"])
                for u in range(PPC):
                    t = ch * PPC + u
                    ep, en, sp, sn = _phi_parts(kp[u * 64:(u + 1) * 64, :])
                    r = _recip(sp * sn)
                    rp = r * sn
                    rn = r * sp
                    phi = jnp.concatenate([e * rp for e in ep] + [e * rn for e in en], axis=0)
                    phis[b.hf][ch][u * 64:(u + 1) * 64, :] = _pack_split(phi)
                    z = zacc[la, t * 128:(t + 1) * 128, :] + phi
                    zacc[la, t * 128:(t + 1) * 128, :] = z
                    if last:
                        zb[t * 128:(t + 1) * 128, :] = jnp.broadcast_to(
                            jnp.sum(z, axis=1, keepdims=True), (128, L))

            def vstep(ch=ch):
                vs[b.hf][ch][...] = _pack_split(proj(wkvaT, D + ch * MC, MC, b, CFG["sub_v"]))

            def mstep(ch=ch):
                for u in range(PPC):
                    t = ch * PPC + u
                    acc = kv_acc[la, t] + _mm_nt(_unpk(vs[b.hf][ch][u * 32:(u + 1) * 32, :]),
                                                 _unpk(phis[b.hf][ch][u * 64:(u + 1) * 64, :]))
                    kv_acc[la, t] = acc
                    if last:
                        r = lax.broadcasted_iota(jnp.int32, (64, 128), 0)
                        c = lax.broadcasted_iota(jnp.int32, (64, 128), 1)
                        kvm[t] = _pack_split(jnp.where((r >> 5) == ((c >> 1) & 1), acc, 0.0))

            steps += [(kstep, None), (vstep, mstep)]
        return steps

    def a_q(b):
        steps = []
        for ch in range(NCH):
            def qstep(ch=ch):
                qp = proj(wqaT, ch * MC, MC, b, CFG["sub_q"])
                for u in range(PPC):
                    t = ch * PPC + u
                    ep, en, sp, sn = _phi_parts(qp[u * 64:(u + 1) * 64, :])
                    zr = _rows(zb[t * 128:(t + 1) * 128, :])
                    dp = _fold2(jnp.add, [e * zz for e, zz in zip(ep, zr[:8])])
                    dn = _fold2(jnp.add, [e * zz for e, zz in zip(en, zr[8:])])
                    r = _recip(dp * sn + dn * sp + 1e-6 * (sp * sn))
                    rp = r * sn
                    rn = r * sp
                    phi = jnp.concatenate([e * rp for e in ep] + [e * rn for e in en], axis=0)
                    phis[b.hf][ch][u * 64:(u + 1) * 64, :] = _pack_split(phi)

            def nstep(ch=ch):
                for u in range(PPC):
                    t = ch * PPC + u
                    o = _mm(_unpk(kvm[t]), _unpk(phis[b.hf][ch][u * 64:(u + 1) * 64, :]))
                    os_[b.hf][t * 32:(t + 1) * 32, :] = _pack_split(o)

            steps.append((qstep, nstep))
        return steps

    def out_proj(wo, b, defer=None):
        steps = []
        ln = LN(b)
        for ch in range(NCH):
            def ostep(ch=ch):
                xt = out_mm(wo, ch, b)
                xT[b.hf][b.k, ch * MC:(ch + 1) * MC, :] = xt
                ln.add(xt)
                if ch == NCH - 1 and defer is None:
                    ln.finish()
            steps.append((ostep, None))
        if defer is not None:
            defer.append((ln.finish, None))
        return steps

    def b_kv(b):
        steps = []
        for base, ref in ((0, kb), (D, vb)):
            for m0 in range(0, D, MC):
                def step(base=base, ref=ref, m0=m0):
                    p = proj(wkvbT, base + m0, MC, b, CFG["sub_b"])
                    ref[WIN + b.j, m0:m0 + MC, :] = p
                    if b.hf == 0:
                        ref[b.k, m0:m0 + MC, :] = pltpu.roll(p, 2, 1)
                steps.append((step, None))
        return steps

    def b_q(b):
        j = b.j
        even = (lax.broadcasted_iota(jnp.int32, (8, L), 0) & 1) == 0
        first = lax.broadcasted_iota(jnp.int32, (8, L), 1) < 2
        cs = DH ** -0.5

        def logits(q, g):
            acc = [None] * WIN
            for r in range(16):
                qv = q[r * 8:r * 8 + 8, :]
                for w in range(WIN):
                    t = qv * kb[WIN + j - w, g * 128 + r * 8:g * 128 + r * 8 + 8, :]
                    acc[w] = t if acc[w] is None else acc[w] + t
            return acc

        steps = []
        for G in range(4):
            def step(G=G):
                q = proj(wqbT, G * 256, 256, b, CFG["sub_qb"])
                la, lb = logits(q[0:128, :], 2 * G), logits(q[128:256, :], 2 * G + 1)
                lg = [jnp.where(even, x + pltpu.roll(x, 7, 0), y + pltpu.roll(y, 1, 0)) for x, y in zip(la, lb)]
                if b.hf == 1:
                    lg = [l if w == 0 else jnp.where(jnp.logical_and(first, j < w), -1e9 / cs, l)
                          for w, l in enumerate(lg)]
                mx = _tree(jnp.maximum, lg)
                ex = [jnp.exp2((l - mx) * (cs * LOG2E)) for l in lg]
                rs = _recip(_tree(jnp.add, ex))
                at = [e * rs for e in ex]
                for hh in range(8):
                    h = G * 8 + hh
                    s = 2 * (hh % 4) + hh // 4
                    o = _running_sum(None, [
                        jnp.broadcast_to(at[w][s:s + 1, :], (DH, L)) * vb[WIN + j - w, h * DH:(h + 1) * DH, :]
                        for w in range(WIN)])
                    os_[b.hf][h * 16:(h + 1) * 16, :] = _pack_split(o)
            steps.append((step, None))
        return steps

    def final_proj(b, defer):
        steps = []
        for ch in range(NCH):
            def ostep(ch=ch):
                xt = out_mm(wobT, ch, b)
                for u in range(GPC):
                    cc = ch * GPC + u
                    y = _pack_split(xt[u * 128:(u + 1) * 128, :])
                    if cc >= 8 - defer:
                        ystage[b.k + 1, (cc - 8 + ND) * 64:(cc - 7 + ND) * 64, :] = y
                    else:
                        xio[b.j, :, cc * L:(cc + 1) * L] = tr(y)
            steps.append((ostep, None))
        return steps

    def flush_out(k, slot):
        for u in range(ND):
            xio[slot, :, (8 - ND + u) * L:(9 - ND + u) * L] = tr(ystage[k, u * 64:(u + 1) * 64, :])

    kv_acc[...] = jnp.zeros(kv_acc.shape, F32)
    zacc[...] = jnp.zeros(zacc.shape, F32)
    ystage[0] = jnp.zeros(ystage.shape[1:], U32)
    cp_phi.wait()
    x_in(8).wait()
    make_pmat(range(GPC))
    prep_x(8, Blk(0, 0))
    start_all(batch[1])

    sa = a_kv(Blk(0, 0), 0, False)
    sb = a_kv(Blk(1, 0), 0, False)
    pend = []
    for ch in range(NCH if 0 in only else 0):
        if ch == 1:
            start_all(batch[2])
        wait_all(cp_k[ch])
        if ch == 0:
            for u in range(GPC):
                fold(wkvaT, u, 8 + u)
            sa[0][0]()
            x_in(0).wait()
        wait_all(cp_v[ch])
        if ch == 0:
            cp_phi2.wait()
            prep_x(0, Blk(1, 0))
            make_pmat(range(GPC, 8))
        else:
            if ch == NCH - 1:
                x_in(9).wait()
                x_in(1).wait()
            for u in range(GPC):
                fold(wkvaT, ch * GPC + u, 8 + ch * GPC + u)
        for u in range(GPC):
            wstore_shuf(wkvaT, 8 + ch * GPC + u, wa_raw, 16 + ch * GPC + u)
        for f in pend:
            f()
        if ch == NCH - 1:
            side_begin(zacc[0, 0:8, :] < 0.0)
            prep_x(9, Blk(0, 1))
            prep_x(1, Blk(1, 1))
            side_begin(None)
        if ch == 0:
            sa[1][0]()
            sb[0][0]()
        else:
            sa[2 * ch][0]()
            sb[2 * ch][0]()
            sa[2 * ch + 1][0]()
        sb[2 * ch + 1][0]()
        pend = [sa[2 * ch + 1][1], sb[2 * ch + 1][1]]
    for f in pend:
        f()

    def s1(i, c):
        @pl.when(i < 7)
        def _():
            x_in(9 + i).wait()
            x_in(1 + i).wait()

        wait_all(w_set(i - 1))
        side_begin(jnp.full((8, L), i >> 6, jnp.int32) > 0)
        nxt = jnp.minimum(i + 1, 7)
        prep_x(8 + nxt, Blk(0, i + 1))
        prep_x(nxt, Blk(1, i + 1))
        prep_set(i - 1)
        side_begin(None)
        steps = a_kv(Blk(0, i), 0, False) + a_kv(Blk(1, i), 0, True)
        steps.insert(CFG["fold_at"], (lambda: fold(wqaT, i - 1, i - 1), None))
        emit(steps, CFG["lag_kv"])
        return c

    if 1 in only:
        lax.fori_loop(1, 8, s1, 0)
    wait_all(w_set(7))
    fold(wqaT, 7, 7)
    prep_set(7)
    wait_all(cp_late)

    def s2(i, c):
        b0, b1 = Blk(0, i), Blk(1, i)
        steps = a_q(b0) + a_q(b1) + out_proj(woaT, b0) + out_proj(woaT, b1)
        steps += [(lambda: prep_late(i), None)] + b_kv(b0) + b_kv(b1)
        emit(steps, CFG["lag_q"])
        return c

    def s3(i, c):
        b0, b1 = Blk(0, i), Blk(1, i)
        late_ln = []
        steps = b_q(b0) + b_q(b1) + out_proj(wobT, b0, late_ln) + out_proj(wobT, b1)
        steps += a_kv(b0, 1, False) + a_kv(b1, 1, True)
        steps[CFG["bar3"]:CFG["bar3"]] = [(barrier, None)] + late_ln
        emit(steps, CFG["lag_kv"])
        return c

    def s5(i, c):
        b0, b1 = Blk(0, i), Blk(1, i)
        flush = (lambda: flush_out(i, jnp.where(i > 0, i - 1, NBLK)), None)
        emit(b_q(b0) + b_q(b1) + [flush] + final_proj(b0, 0) + final_proj(b1, ND), 0)
        x_out(b0.j).start()
        x_out(b1.j, 0, 8 - ND).start()

        @pl.when(i > 0)
        def _():
            x_out(i - 1, 8 - ND, 8, SEM_KV + i - 1).start()
        return c

    def layer_pair(l, c):
        if 2 in only:
            lax.fori_loop(0, 8, s2, 0)

        @pl.when(l == 0)
        def _():
            if 3 in only:
                lax.fori_loop(0, 8, s3, 0)

        @pl.when(l == 1)
        def _():
            if 5 in only:
                lax.fori_loop(0, 8, s5, 0)
        return c

    lax.fori_loop(0, 2, layer_pair, 0)

    flush_out(8, 7)
    x_out(7, 8 - ND, 8, SEM_KV + 7).start()
    for k in range(8):
        x_out(8 + k).wait()
        x_out(k, 0, 8 - ND).wait()
        x_out(k, 8 - ND, 8, SEM_KV + k).wait()


def _compiler_params():
    vmem = 120 * 1024 * 1024
    try:
        return pltpu.CompilerParams(vmem_limit_bytes=vmem, disable_semaphore_checks=True)
    except TypeError:
        return pltpu.CompilerParams(vmem_limit_bytes=vmem)


@jax.jit
def pallas_interleave_layers__linear_kernel_hedgehog__sliding_local_dilated__prompt_kernel(
    A_x: jax.Array,
    A_wqkv: jax.Array,
    A_w_phi: jax.Array,
    A_wo: jax.Array,
    B_x: jax.Array,
    B_wqkv: jax.Array,
    B_wo: jax.Array,
):
    del B_x
    x3 = A_x.reshape(S // 32, 32, D)
    wphi2 = A_w_phi.reshape(H * DH, DH)
    any_spec = pl.BlockSpec(memory_space=pl.ANY)
    scratch = [
        pltpu.VMEM((NBLK + 1, S // 32, D), U32),
        pltpu.VMEM((24, D // 2, L), U32),
        pltpu.VMEM((8, D // 2, L), U32),
        pltpu.VMEM((24, D // 2, L), U32),
        pltpu.VMEM((8, D // 2, L), U32),
        pltpu.VMEM((H * DH, DH), BF16),
        pltpu.VMEM((8, 64, 128), U32),
        pltpu.VMEM((8, D // 2, L), U32),
        pltpu.VMEM((8, D, L), U32),
        pltpu.VMEM((8, D // 2, L), U32),
        pltpu.VMEM((8, D // 2 + 8, L), U32),
        pltpu.VMEM((8, D, L), U32),
        pltpu.VMEM((8, D // 2, L), U32),
        pltpu.VMEM((WIN + NBLK, D, L), F32),
        pltpu.VMEM((WIN + NBLK, D, L), F32),
        pltpu.VMEM((2, 16, 64, 128), F32),
        pltpu.VMEM((16, 32, 128), U32),
        pltpu.VMEM((2, 2 * D, L), F32),
        pltpu.VMEM((2 * D, L), F32),
        pltpu.VMEM((9, ND * 64, L), U32),
        pltpu.SemaphoreType.DMA((NSEM,)),
        pltpu.SemaphoreType.REGULAR,
    ]
    scratch += [pltpu.VMEM((9, D, L), F32)] * 2
    scratch += [pltpu.VMEM((9, D // 2, L), U32)] * 2
    scratch += [pltpu.VMEM((D // 2, L), U32)] * 2
    scratch += [pltpu.VMEM((MC, L), U32)] * (2 * NCH)
    scratch += [pltpu.VMEM((MC // 2, L), U32)] * (2 * NCH)
    out = pl.pallas_call(
        _kernel,
        out_shape=jax.ShapeDtypeStruct((S // 32, 32, D), BF16),
        in_specs=[any_spec] * 6,
        out_specs=any_spec,
        scratch_shapes=scratch,
        compiler_params=_compiler_params(),
        name="hedgehog_dilated",
    )(x3, A_wqkv, wphi2, A_wo, B_wqkv, B_wo)
    return out.reshape(1, S, D)
```

```python
import math

import jax
import jax.numpy as jnp
from jax import lax
import jax.experimental.pallas as pl
import jax.experimental.pallas.tpu as pltpu

S = 2048
D = 1024
H = 32
DH = 32
NBLK = 16
L = 128
WIN = 8
LOG2E = math.log2(math.e)
F32 = jnp.float32
BF16 = jnp.bfloat16
U32 = jnp.uint32
NT = (((1,), (1,)), ((), ()))

MC = 256
NCH = D // MC
GPC = MC // 128
PPC = MC // 64
ND = 2

CFG = dict(only=None, lag_q=2, lag_kv=4, hold=7, ln_link=4, side=3, bar3=14, tail=2,
           sub_q=128, sub_k=64, sub_v=256, sub_qb=128, sub_o=256, sub_b=256,
           hold_1=0, sub_v_1=128, ln_link_3=2)


class _Stage:
    cur = 0


def _cfg(key):
    return CFG.get("%s_%d" % (key, _Stage.cur), CFG[key])


SEM_X = 0
SEM_PHI = 16
SEM_KV = 18
SEM_SET = 26
SEM_LATE = 34
NSEM = 35


def _mm(a, b):
    return jnp.dot(a, b, preferred_element_type=F32)


def _mm_nt(a, b):
    return lax.dot_general(a, b, NT, preferred_element_type=F32)


def _tree(op, xs):
    xs = list(xs)
    while len(xs) > 1:
        nxt = [op(xs[i], xs[i + 1]) for i in range(0, len(xs) - 1, 2)]
        if len(xs) % 2:
            nxt.append(xs[-1])
        xs = nxt
    return xs[0]


def _running_sum(acc, xs):
    for x in xs:
        acc = x if acc is None else acc + x
    return acc


def _rows(a, n=8):
    return [a[i * n:(i + 1) * n, :] for i in range(a.shape[0] // n)]


def _pack(a):
    return pltpu.bitcast(a.astype(BF16), U32)


def _unpk(a):
    return pltpu.bitcast(a, BF16)


def _pack_i(a, b):
    return pltpu.pack_elementwise([a, b], packed_dtype=BF16)


def _pack_split(a):
    r = _rows(a)
    return jnp.concatenate([_pack_i(r[2 * i], r[2 * i + 1]) for i in range(len(r) // 2)], axis=0)


def _unpack_split(p):
    out = []
    for x in _rows(p):
        out.append(pltpu.unpack_elementwise(x, index=0, packed_dtype=BF16, unpacked_dtype=F32))
        out.append(pltpu.unpack_elementwise(x, index=1, packed_dtype=BF16, unpacked_dtype=F32))
    return jnp.concatenate(out, axis=0)


def _fold2(op, xs):
    r = _tree(op, xs)
    r = op(r, pltpu.roll(r, 4, 0))
    return op(r, pltpu.roll(r, 2, 0))


def _phi_parts(p):
    ps = _rows(p)
    mx = _fold2(jnp.maximum, ps)
    mn = _fold2(jnp.minimum, ps)
    ep = [jnp.exp2(x - mx) for x in ps]
    en = [jnp.exp2(mn - x) for x in ps]
    return ep, en, _fold2(jnp.add, ep), _fold2(jnp.add, en)


def _recip(x):
    r = pl.reciprocal(x, approx=True)
    return r * (2.0 - x * r)


def _mult(x, m):
    return x if isinstance(x, int) else pl.multiple_of(x, m)


def _kernel(x_hbm, wa_hbm, wphi_hbm, woa_hbm, wb_hbm, wob_hbm, out_hbm,
            xio, wa_raw, woa_raw, wb_raw, wob_raw, wphi, pmat,
            wqaT, wkvaT, woaT, wqbT, wkvbT, wobT, kb, vb, kv_acc, kvm, zacc, zb, ystage, sems, bsem, *rest):
    xT, xn, os_ = rest[0:2], rest[2:4], rest[4:6]
    phis = [rest[6:6 + NCH], rest[6 + NCH:6 + 2 * NCH]]
    vs = [rest[6 + 2 * NCH:6 + 3 * NCH], rest[6 + 3 * NCH:6 + 4 * NCH]]
    only = CFG["only"] or (0, 1, 2, 3, 5)

    class Blk:
        def __init__(self, hf, k):
            self.hf, self.k = hf, k
            self.j = 8 * (1 - hf) + k
            self.zr = 0 if isinstance(k, int) else k >> 6

    x32, out32, wa32, woa32, wb32, wob32 = [
        r.bitcast(U32) for r in (x_hbm, out_hbm, wa_hbm, woa_hbm, wb_hbm, wob_hbm)]

    def x_in(j):
        return pltpu.make_async_copy(x32.at[:, j, :], xio.at[j], sems.at[SEM_X + j])

    def x_out(j, c0=0, c1=8, sem=None):
        cs = pl.ds(c0 * L, (c1 - c0) * L)
        return pltpu.make_async_copy(xio.at[j, :, cs], out32.at[:, j, cs],
                                     sems.at[SEM_X + j if sem is None else sem])

    def slabs(src, dst, g0, n, sem):
        return [pltpu.make_async_copy(src.at[:, pl.ds(_mult((g0 + u) * 128, 128), 128)], dst.at[g0 + u],
                                      sems.at[sem]) for u in range(n)]

    cp_phi = pltpu.make_async_copy(wphi_hbm.at[0:MC], wphi.at[0:MC], sems.at[SEM_PHI])
    cp_phi2 = pltpu.make_async_copy(wphi_hbm.at[MC:D], wphi.at[MC:D], sems.at[SEM_PHI + 1])
    cp_k = [slabs(wa32, wa_raw, 8 + ch * GPC, GPC, SEM_KV + 2 * ch) for ch in range(NCH)]
    cp_v = [slabs(wa32, wa_raw, 16 + ch * GPC, GPC, SEM_KV + 2 * ch + 1) for ch in range(NCH)]

    def w_set(g):
        return (slabs(wa32, wa_raw, g, 1, SEM_SET + g) + slabs(woa32, woa_raw, g, 1, SEM_SET + g)
                + slabs(wb32, wb_raw, 8 + g, 1, SEM_SET + g) + slabs(wb32, wb_raw, 16 + g, 1, SEM_SET + g))

    cp_late = slabs(wb32, wb_raw, 0, 8, SEM_LATE) + slabs(wob32, wob_raw, 0, 8, SEM_LATE)

    batch = [[cp_phi, x_in(8)] + cp_k[0] + [x_in(0)] + cp_v[0] + [cp_phi2] + cp_k[1] + cp_v[1],
             cp_k[2] + cp_v[2] + cp_k[3] + cp_v[3] + [x_in(9), x_in(1)], []]
    for g in range(8):
        if g < 6:
            batch[1] += [x_in(10 + g), x_in(2 + g)] + w_set(g)
        else:
            batch[2] += w_set(g)
    batch[2] += cp_late

    def start_all(cps):
        for c in cps:
            c.start()

    def wait_all(cps):
        for c in cps:
            c.wait()

    start_all(batch[0])
    _Stage.cur = 0

    class Side:
        never = None
        hist = []

    def side_begin(never):
        Side.never = never
        Side.hist = []

    def tr(x):
        w = _cfg("side")
        if Side.never is not None and len(Side.hist) >= w:
            x = jnp.concatenate([jnp.where(Side.never, Side.hist[-w], x[0:8, :]), x[8:, :]], axis=0)
        y = pltpu.bitcast(_unpk(x).T, U32)
        Side.hist.append(y[56:64, :])
        return y

    def wtile(raw, slab, c):
        return tr(raw[slab, c * 64:(c + 1) * 64, :])

    def wstore_split(ref, g, raw, slab):
        for c in range(8):
            ref[c, pl.ds(_mult(g * 64, 64), 64), :] = _pack(_unpack_split(wtile(raw, slab, c)))

    def wstore_shuf(ref, g, raw, slab):
        for c in range(8):
            ref[c, pl.ds(_mult(g * 64, 64), 64), :] = _pack_split(_unpk(wtile(raw, slab, c)).astype(F32))

    def wstore_perm(ref, g, raw, slab):
        for c in range(8):
            pk = wtile(raw, slab, c)
            for h4 in range(4):
                ref[c, pl.ds(g * 64 + h4, 16, stride=4), :] = pk[h4 * 16:(h4 + 1) * 16, :]

    def make_pmat(gs):
        def unsplit(r):
            return (r & ~15) + 2 * (r & 7) + ((r >> 3) & 1)

        r128 = unsplit(lax.broadcasted_iota(jnp.int32, (128, 128), 0))
        c128 = lax.broadcasted_iota(jnp.int32, (128, 128), 1)
        same_head = (2 * (r128 >> 6) + (r128 & 1)) == (c128 >> 5)
        er = unsplit(lax.broadcasted_iota(jnp.int32, (128, 32), 0))
        ec = lax.broadcasted_iota(jnp.int32, (128, 32), 1)
        expand = jnp.where(((er & 63) >> 1) == ec, 1.0, 0.0).astype(BF16)
        for g in gs:
            pg = _mm_nt(expand, wphi[g * 128:(g + 1) * 128, :])
            pmat[g] = _pack(jnp.where(same_head, pg, 0.0))

    def fold(dst, g, slab):
        val = _mm_nt(_unpk(pmat[g]), _unpk(wa_raw[slab])) * LOG2E
        for c in range(8):
            dst[c, pl.ds(_mult(g * 64, 64), 64), :] = _pack_split(val[:, c * L:(c + 1) * L])

    def prep_set(g):
        wstore_split(woaT, g, woa_raw, g)
        wstore_perm(wkvbT, g, wb_raw, 8 + g)
        wstore_split(wkvbT, 8 + g, wb_raw, 16 + g)

    def prep_late(g):
        wstore_perm(wqbT, g, wb_raw, g)
        wstore_split(wobT, g, wob_raw, g)

    class LN:
        def __init__(self, b):
            self.b = b
            self.piv = self.s1 = self.s2 = None

        def add(self, xt):
            if self.piv is None:
                self.piv = jnp.broadcast_to(xt[0:1, :], (8, L))
            d = [r - self.piv for r in _rows(xt)]
            self.s1 = _running_sum(self.s1, d)
            self.s2 = _running_sum(self.s2, [x * x for x in d])

        def finish(self):
            b = self.b
            m1 = jnp.sum(self.s1, axis=0, keepdims=True) * (1.0 / D)
            m2 = jnp.sum(self.s2, axis=0, keepdims=True) * (1.0 / D)
            var = jnp.maximum(m2 - m1 * m1, 0.0)
            rs = lax.rsqrt(var + 1e-5)
            mrs = jnp.broadcast_to((self.piv[0:1, :] + m1) * rs, (8, L))
            rs = jnp.broadcast_to(rs, (8, L))
            never = rs < 0.0
            for r in range(D // 16):
                pk = _pack_i(xT[b.hf][b.k, r * 16:r * 16 + 8, :] * rs - mrs,
                             xT[b.hf][b.k, r * 16 + 8:r * 16 + 16, :] * rs - mrs)
                xn[b.hf][b.k, r * 8:(r + 1) * 8, :] = pk
                if r % _cfg("ln_link") == _cfg("ln_link") - 1:
                    rs = jnp.where(never, pltpu.bitcast(pk, F32), rs)

    def prep_x(src, b):
        ln = LN(b)
        for cc in range(8):
            xt = _unpack_split(tr(xio[src, :, cc * L:(cc + 1) * L]))
            xT[b.hf][b.k, cc * 128:(cc + 1) * 128, :] = xt
            ln.add(xt)
        ln.finish()

    def mmw(ref, r0, n, rhs, sub):
        def wload(r):
            return jnp.concatenate([_unpk(ref[c, r // 2:(r + sub) // 2, :]) for c in range(8)], axis=1)
        return jnp.concatenate([_mm(wload(r), rhs()) for r in range(r0, r0 + n, sub)], axis=0)

    def proj(ref, r0, n, b, sub):
        return mmw(ref, r0, n, lambda: _unpk(xn[b.hf][b.k]), sub)

    def out_mm(wo, ch, b):
        m0 = ch * MC
        return xT[b.hf][b.k, m0:m0 + MC, :] + mmw(wo, m0, MC, lambda: _unpk(os_[b.hf][...]), _cfg("sub_o"))

    def emit(steps, lag):
        pend = []
        for n, (main, late) in enumerate(steps):
            main()
            if late is not None:
                pend.append((n + lag if n < len(steps) - _cfg("hold") else len(steps) + n, late))
            for due, f in pend:
                if due <= n:
                    f()
            pend = [e for e in pend if e[0] > n]
        for _, f in sorted(pend, key=lambda e: e[0]):
            f()

    def barrier():
        pl.semaphore_signal(bsem, 1)
        pl.semaphore_wait(bsem, 1)

    def z_finish(t, z):
        zb[t * 128:(t + 1) * 128, :] = jnp.broadcast_to(jnp.sum(z, axis=1, keepdims=True), (128, L))

    def kv_finish(t, acc):
        r = lax.broadcasted_iota(jnp.int32, (64, 128), 0)
        c = lax.broadcasted_iota(jnp.int32, (64, 128), 1)
        kvm[t] = _pack_split(jnp.where((r >> 5) == ((c >> 1) & 1), acc, 0.0))

    def a_kv(b, lay, last):
        steps = []
        la = lay + b.zr if b.hf == 1 else lay
        for ch in range(NCH):
            def kstep(ch=ch):
                kp = proj(wkvaT, ch * MC, MC, b, _cfg("sub_k"))
                for u in range(PPC):
                    t = ch * PPC + u
                    ep, en, sp, sn = _phi_parts(kp[u * 64:(u + 1) * 64, :])
                    r = _recip(sp * sn)
                    rp = r * sn
                    rn = r * sp
                    phi = jnp.concatenate([e * rp for e in ep] + [e * rn for e in en], axis=0)
                    phis[b.hf][ch][u * 64:(u + 1) * 64, :] = _pack_split(phi)
                    z = zacc[la, t * 128:(t + 1) * 128, :] + phi
                    zacc[la, t * 128:(t + 1) * 128, :] = z
                    if last:
                        z_finish(t, z)

            def vstep(ch=ch):
                vs[b.hf][ch][...] = _pack_split(proj(wkvaT, D + ch * MC, MC, b, _cfg("sub_v")))

            def mstep(ch=ch):
                for u in range(PPC):
                    t = ch * PPC + u
                    acc = kv_acc[la, t] + _mm_nt(_unpk(vs[b.hf][ch][u * 32:(u + 1) * 32, :]),
                                                 _unpk(phis[b.hf][ch][u * 64:(u + 1) * 64, :]))
                    kv_acc[la, t] = acc
                    if last:
                        kv_finish(t, acc)

            steps += [(kstep, None), (vstep, mstep)]
        return steps

    def a_q(b):
        steps = []
        for ch in range(NCH):
            def qstep(ch=ch):
                qp = proj(wqaT, ch * MC, MC, b, _cfg("sub_q"))
                for u in range(PPC):
                    t = ch * PPC + u
                    ep, en, sp, sn = _phi_parts(qp[u * 64:(u + 1) * 64, :])
                    zr = _rows(zb[t * 128:(t + 1) * 128, :])
                    dp = _fold2(jnp.add, [e * zz for e, zz in zip(ep, zr[:8])])
                    dn = _fold2(jnp.add, [e * zz for e, zz in zip(en, zr[8:])])
                    r = _recip(dp * sn + dn * sp + 1e-6 * (sp * sn))
                    rp = r * sn
                    rn = r * sp
                    phi = jnp.concatenate([e * rp for e in ep] + [e * rn for e in en], axis=0)
                    phis[b.hf][ch][u * 64:(u + 1) * 64, :] = _pack_split(phi)

            def nstep(ch=ch):
                for u in range(PPC):
                    t = ch * PPC + u
                    o = _mm(_unpk(kvm[t]), _unpk(phis[b.hf][ch][u * 64:(u + 1) * 64, :]))
                    os_[b.hf][t * 32:(t + 1) * 32, :] = _pack_split(o)

            steps.append((qstep, nstep))
        return steps

    def out_proj(wo, b, defer=None):
        steps = []
        ln = LN(b)
        for ch in range(NCH):
            def ostep(ch=ch):
                xt = out_mm(wo, ch, b)
                xT[b.hf][b.k, ch * MC:(ch + 1) * MC, :] = xt
                ln.add(xt)
                if ch == NCH - 1 and defer is None:
                    ln.finish()
            steps.append((ostep, None))
        if defer is not None:
            defer.append((ln.finish, None))
        return steps

    def b_kv(b):
        steps = []
        for base, ref in ((0, kb), (D, vb)):
            for m0 in range(0, D, MC):
                def step(base=base, ref=ref, m0=m0):
                    p = proj(wkvbT, base + m0, MC, b, _cfg("sub_b"))
                    ref[WIN + b.j, m0:m0 + MC, :] = p
                    if b.hf == 0:
                        ref[b.k, m0:m0 + MC, :] = pltpu.roll(p, 2, 1)
                steps.append((step, None))
        return steps

    def b_q(b):
        j = b.j
        even = (lax.broadcasted_iota(jnp.int32, (8, L), 0) & 1) == 0
        first = lax.broadcasted_iota(jnp.int32, (8, L), 1) < 2
        cs = DH ** -0.5

        def logits(q, g):
            acc = [None] * WIN
            for r in range(16):
                qv = q[r * 8:r * 8 + 8, :]
                for w in range(WIN):
                    t = qv * kb[WIN + j - w, g * 128 + r * 8:g * 128 + r * 8 + 8, :]
                    acc[w] = t if acc[w] is None else acc[w] + t
            return acc

        steps = []
        for G in range(4):
            def step(G=G):
                q = proj(wqbT, G * 256, 256, b, _cfg("sub_qb"))
                la, lb = logits(q[0:128, :], 2 * G), logits(q[128:256, :], 2 * G + 1)
                lg = [jnp.where(even, x + pltpu.roll(x, 7, 0), y + pltpu.roll(y, 1, 0)) for x, y in zip(la, lb)]
                if b.hf == 1:
                    lg = [l if w == 0 else jnp.where(jnp.logical_and(first, j < w), -1e9 / cs, l)
                          for w, l in enumerate(lg)]
                mx = _tree(jnp.maximum, lg)
                ex = [jnp.exp2((l - mx) * (cs * LOG2E)) for l in lg]
                rs = _recip(_tree(jnp.add, ex))
                at = [e * rs for e in ex]
                for hh in range(8):
                    h = G * 8 + hh
                    s = 2 * (hh % 4) + hh // 4
                    o = _running_sum(None, [
                        jnp.broadcast_to(at[w][s:s + 1, :], (DH, L)) * vb[WIN + j - w, h * DH:(h + 1) * DH, :]
                        for w in range(WIN)])
                    os_[b.hf][h * 16:(h + 1) * 16, :] = _pack_split(o)
            steps.append((step, None))
        return steps

    def final_proj(b, defer):
        steps = []
        for ch in range(NCH):
            def ostep(ch=ch):
                xt = out_mm(wobT, ch, b)
                for u in range(GPC):
                    cc = ch * GPC + u
                    y = _pack_split(xt[u * 128:(u + 1) * 128, :])
                    if cc >= 8 - defer:
                        ystage[b.k + 1, (cc - 8 + ND) * 64:(cc - 7 + ND) * 64, :] = y
                    else:
                        xio[b.j, :, cc * L:(cc + 1) * L] = tr(y)
            steps.append((ostep, None))
        return steps

    def flush_out(k, slot):
        for u in range(ND):
            xio[slot, :, (8 - ND + u) * L:(9 - ND + u) * L] = tr(ystage[k, u * 64:(u + 1) * 64, :])

    kv_acc[...] = jnp.zeros(kv_acc.shape, F32)
    zacc[...] = jnp.zeros(zacc.shape, F32)
    ystage[0] = jnp.zeros(ystage.shape[1:], U32)
    cp_phi.wait()
    x_in(8).wait()
    make_pmat(range(GPC))
    prep_x(8, Blk(0, 0))
    start_all(batch[1])

    sa = a_kv(Blk(0, 0), 0, False)
    sb = a_kv(Blk(1, 0), 0, False)
    pend = []
    for ch in range(NCH if 0 in only else 0):
        if ch == 1:
            start_all(batch[2])
        wait_all(cp_k[ch])
        if ch == 0:
            for u in range(GPC):
                fold(wkvaT, u, 8 + u)
            sa[0][0]()
            x_in(0).wait()
        wait_all(cp_v[ch])
        if ch == 0:
            cp_phi2.wait()
            prep_x(0, Blk(1, 0))
            make_pmat(range(GPC, 8))
        else:
            if ch == NCH - 1:
                x_in(9).wait()
                x_in(1).wait()
            for u in range(GPC):
                fold(wkvaT, ch * GPC + u, 8 + ch * GPC + u)
        for u in range(GPC):
            wstore_shuf(wkvaT, 8 + ch * GPC + u, wa_raw, 16 + ch * GPC + u)
        for f in pend:
            f()
        if ch == NCH - 1:
            side_begin(zacc[0, 0:8, :] < 0.0)
            prep_x(9, Blk(0, 1))
            prep_x(1, Blk(1, 1))
            side_begin(None)
        if ch == 0:
            sa[1][0]()
            sb[0][0]()
        else:
            sa[2 * ch][0]()
            sb[2 * ch][0]()
            sa[2 * ch + 1][0]()
        sb[2 * ch + 1][0]()
        pend = [sa[2 * ch + 1][1], sb[2 * ch + 1][1]]
    for f in pend:
        f()

    def s1(i, c):
        _Stage.cur = 1
        @pl.when(i < 7)
        def _():
            x_in(9 + i).wait()
            x_in(1 + i).wait()

        wait_all(w_set(i - 1))
        side_begin(jnp.full((8, L), i >> 6, jnp.int32) > 0)
        nxt = jnp.minimum(i + 1, 7)
        prep_x(8 + nxt, Blk(0, i + 1))
        prep_x(nxt, Blk(1, i + 1))
        prep_set(i - 1)
        side_begin(None)
        steps = a_kv(Blk(0, i), 0, False) + a_kv(Blk(1, i), 0, CFG["tail"] < 2)
        if not CFG["tail"]:
            steps.insert(CFG["fold_at"], (lambda: fold(wqaT, i - 1, i - 1), None))
        emit(steps, _cfg("lag_kv"))
        return c

    if 1 in only:
        lax.fori_loop(1, 8, s1, 0)
    _Stage.cur = 0
    wait_all(w_set(7))
    for g in range(0 if CFG["tail"] else 7, 8):
        fold(wqaT, g, g)
    prep_set(7)
    if CFG["tail"] == 2:
        for t in range(16):
            z_finish(t, zacc[0, t * 128:(t + 1) * 128, :])
            kv_finish(t, kv_acc[0, t])
    wait_all(cp_late)

    def s2(i, c):
        _Stage.cur = 2
        b0, b1 = Blk(0, i), Blk(1, i)
        steps = a_q(b0) + a_q(b1) + out_proj(woaT, b0) + out_proj(woaT, b1)
        steps += [(lambda: prep_late(i), None)] + b_kv(b0) + b_kv(b1)
        emit(steps, _cfg("lag_q"))
        return c

    def s3(i, c):
        _Stage.cur = 3
        b0, b1 = Blk(0, i), Blk(1, i)
        late_ln = []
        steps = b_q(b0) + b_q(b1) + out_proj(wobT, b0, late_ln) + out_proj(wobT, b1)
        steps += a_kv(b0, 1, False) + a_kv(b1, 1, True)
        steps[CFG["bar3"]:CFG["bar3"]] = [(barrier, None)] + late_ln
        emit(steps, _cfg("lag_kv"))
        return c

    def s5(i, c):
        _Stage.cur = 5
        b0, b1 = Blk(0, i), Blk(1, i)
        flush = (lambda: flush_out(i, jnp.where(i > 0, i - 1, NBLK)), None)
        emit(b_q(b0) + b_q(b1) + [flush] + final_proj(b0, 0) + final_proj(b1, ND), 0)
        x_out(b0.j).start()
        x_out(b1.j, 0, 8 - ND).start()

        @pl.when(i > 0)
        def _():
            x_out(i - 1, 8 - ND, 8, SEM_KV + i - 1).start()
        return c

    def layer_pair(l, c):
        if 2 in only:
            lax.fori_loop(0, 8, s2, 0)

        @pl.when(l == 0)
        def _():
            if 3 in only:
                lax.fori_loop(0, 8, s3, 0)

        @pl.when(l == 1)
        def _():
            if 5 in only:
                lax.fori_loop(0, 8, s5, 0)
        return c

    lax.fori_loop(0, 2, layer_pair, 0)

    flush_out(8, 7)
    x_out(7, 8 - ND, 8, SEM_KV + 7).start()
    for k in range(8):
        x_out(8 + k).wait()
        x_out(k, 0, 8 - ND).wait()
        x_out(k, 8 - ND, 8, SEM_KV + k).wait()


def _compiler_params():
    vmem = 120 * 1024 * 1024
    try:
        return pltpu.CompilerParams(vmem_limit_bytes=vmem, disable_semaphore_checks=True)
    except TypeError:
        return pltpu.CompilerParams(vmem_limit_bytes=vmem)


@jax.jit
def pallas_interleave_layers__linear_kernel_hedgehog__sliding_local_dilated__prompt_kernel(
    A_x: jax.Array,
    A_wqkv: jax.Array,
    A_w_phi: jax.Array,
    A_wo: jax.Array,
    B_x: jax.Array,
    B_wqkv: jax.Array,
    B_wo: jax.Array,
):
    del B_x
    x3 = A_x.reshape(S // 32, 32, D)
    wphi2 = A_w_phi.reshape(H * DH, DH)
    any_spec = pl.BlockSpec(memory_space=pl.ANY)
    scratch = [
        pltpu.VMEM((NBLK + 1, S // 32, D), U32),
        pltpu.VMEM((24, D // 2, L), U32),
        pltpu.VMEM((8, D // 2, L), U32),
        pltpu.VMEM((24, D // 2, L), U32),
        pltpu.VMEM((8, D // 2, L), U32),
        pltpu.VMEM((H * DH, DH), BF16),
        pltpu.VMEM((8, 64, 128), U32),
        pltpu.VMEM((8, D // 2, L), U32),
        pltpu.VMEM((8, D, L), U32),
        pltpu.VMEM((8, D // 2, L), U32),
        pltpu.VMEM((8, D // 2 + 8, L), U32),
        pltpu.VMEM((8, D, L), U32),
        pltpu.VMEM((8, D // 2, L), U32),
        pltpu.VMEM((WIN + NBLK, D, L), F32),
        pltpu.VMEM((WIN + NBLK, D, L), F32),
        pltpu.VMEM((2, 16, 64, 128), F32),
        pltpu.VMEM((16, 32, 128), U32),
        pltpu.VMEM((2, 2 * D, L), F32),
        pltpu.VMEM((2 * D, L), F32),
        pltpu.VMEM((9, ND * 64, L), U32),
        pltpu.SemaphoreType.DMA((NSEM,)),
        pltpu.SemaphoreType.REGULAR,
    ]
    scratch += [pltpu.VMEM((9, D, L), F32)] * 2
    scratch += [pltpu.VMEM((9, D // 2, L), U32)] * 2
    scratch += [pltpu.VMEM((D // 2, L), U32)] * 2
    scratch += [pltpu.VMEM((MC, L), U32)] * (2 * NCH)
    scratch += [pltpu.VMEM((MC // 2, L), U32)] * (2 * NCH)
    out = pl.pallas_call(
        _kernel,
        out_shape=jax.ShapeDtypeStruct((S // 32, 32, D), BF16),
        in_specs=[any_spec] * 6,
        out_specs=any_spec,
        scratch_shapes=scratch,
        compiler_params=_compiler_params(),
        name="hedgehog_dilated",
    )(x3, A_wqkv, wphi2, A_wo, B_wqkv, B_wo)
    return out.reshape(1, S, D)
```

```python
import math

import jax
import jax.numpy as jnp
from jax import lax
import jax.experimental.pallas as pl
import jax.experimental.pallas.tpu as pltpu

S = 2048
D = 1024
H = 32
DH = 32
NBLK = 16
L = 128
WIN = 8
LOG2E = math.log2(math.e)
F32 = jnp.float32
BF16 = jnp.bfloat16
U32 = jnp.uint32
NT = (((1,), (1,)), ((), ()))

MC = 256
NCH = D // MC
GPC = MC // 128
PPC = MC // 64
ND = 2

CFG = dict(only=None, lag_q=2, lag_kv=4, hold=7, ln_link=4, side=3, bar3=14, tail=2,
           sub_q=128, sub_k=64, sub_v=256, sub_qb=128, sub_o=256, sub_b=256,
           hold_1=0, sub_v_1=128, ln_link_3=2)


class _Stage:
    cur = 0


def _cfg(key):
    return CFG.get("%s_%d" % (key, _Stage.cur), CFG[key])


SEM_X = 0
SEM_PHI = 16
SEM_KV = 18
SEM_SET = 26
SEM_LATE = 34
NSEM = 35


def _mm(a, b):
    return jnp.dot(a, b, preferred_element_type=F32)


def _mm_nt(a, b):
    return lax.dot_general(a, b, NT, preferred_element_type=F32)


def _tree(op, xs):
    xs = list(xs)
    while len(xs) > 1:
        nxt = [op(xs[i], xs[i + 1]) for i in range(0, len(xs) - 1, 2)]
        if len(xs) % 2:
            nxt.append(xs[-1])
        xs = nxt
    return xs[0]


def _running_sum(acc, xs):
    for x in xs:
        acc = x if acc is None else acc + x
    return acc


def _rows(a, n=8):
    return [a[i * n:(i + 1) * n, :] for i in range(a.shape[0] // n)]


def _pack(a):
    return pltpu.bitcast(a.astype(BF16), U32)


def _unpk(a):
    return pltpu.bitcast(a, BF16)


def _pack_i(a, b):
    return pltpu.pack_elementwise([a, b], packed_dtype=BF16)


def _pack_split(a):
    r = _rows(a)
    return jnp.concatenate([_pack_i(r[2 * i], r[2 * i + 1]) for i in range(len(r) // 2)], axis=0)


def _unpack_split(p):
    out = []
    for x in _rows(p):
        out.append(pltpu.unpack_elementwise(x, index=0, packed_dtype=BF16, unpacked_dtype=F32))
        out.append(pltpu.unpack_elementwise(x, index=1, packed_dtype=BF16, unpacked_dtype=F32))
    return jnp.concatenate(out, axis=0)


def _fold2(op, xs):
    r = _tree(op, xs)
    r = op(r, pltpu.roll(r, 4, 0))
    return op(r, pltpu.roll(r, 2, 0))


def _phi_parts(p):
    ps = _rows(p)
    mx = _fold2(jnp.maximum, ps)
    mn = _fold2(jnp.minimum, ps)
    ep = [jnp.exp2(x - mx) for x in ps]
    en = [jnp.exp2(mn - x) for x in ps]
    return ep, en, _fold2(jnp.add, ep), _fold2(jnp.add, en)


def _recip(x):
    r = pl.reciprocal(x, approx=True)
    return r * (2.0 - x * r)


def _mult(x, m):
    return x if isinstance(x, int) else pl.multiple_of(x, m)


def _kernel(x_hbm, wa_hbm, wphi_hbm, woa_hbm, wb_hbm, wob_hbm, out_hbm,
            xio, wa_raw, woa_raw, wb_raw, wob_raw, wphi, pmat,
            wqaT, wkvaT, woaT, wqbT, wkvbT, wobT, kb, vb, kv_acc, kvm, zacc, zb, ystage, sems, bsem, *rest):
    xT, xn, os_ = rest[0:2], rest[2:4], rest[4:6]
    phis = [rest[6:6 + NCH], rest[6 + NCH:6 + 2 * NCH]]
    vs = [rest[6 + 2 * NCH:6 + 3 * NCH], rest[6 + 3 * NCH:6 + 4 * NCH]]
    only = CFG["only"] or (0, 1, 2, 3, 5)

    class Blk:
        def __init__(self, hf, k):
            self.hf, self.k = hf, k
            self.j = 8 * (1 - hf) + k
            self.zr = 0 if isinstance(k, int) else k >> 6

    x32, out32, wa32, woa32, wb32, wob32 = [
        r.bitcast(U32) for r in (x_hbm, out_hbm, wa_hbm, woa_hbm, wb_hbm, wob_hbm)]

    def x_in(j):
        return pltpu.make_async_copy(x32.at[:, j, :], xio.at[j], sems.at[SEM_X + j])

    def x_out(j, c0=0, c1=8, sem=None):
        cs = pl.ds(c0 * L, (c1 - c0) * L)
        return pltpu.make_async_copy(xio.at[j, :, cs], out32.at[:, j, cs],
                                     sems.at[SEM_X + j if sem is None else sem])

    def slabs(src, dst, g0, n, sem):
        return [pltpu.make_async_copy(src.at[:, pl.ds(_mult((g0 + u) * 128, 128), 128)], dst.at[g0 + u],
                                      sems.at[sem]) for u in range(n)]

    cp_phi = pltpu.make_async_copy(wphi_hbm.at[0:MC], wphi.at[0:MC], sems.at[SEM_PHI])
    cp_phi2 = pltpu.make_async_copy(wphi_hbm.at[MC:D], wphi.at[MC:D], sems.at[SEM_PHI + 1])
    cp_k = [slabs(wa32, wa_raw, 8 + ch * GPC, GPC, SEM_KV + 2 * ch) for ch in range(NCH)]
    cp_v = [slabs(wa32, wa_raw, 16 + ch * GPC, GPC, SEM_KV + 2 * ch + 1) for ch in range(NCH)]

    def w_set(g):
        return (slabs(wa32, wa_raw, g, 1, SEM_SET + g) + slabs(woa32, woa_raw, g, 1, SEM_SET + g)
                + slabs(wb32, wb_raw, 8 + g, 1, SEM_SET + g) + slabs(wb32, wb_raw, 16 + g, 1, SEM_SET + g))

    cp_late = slabs(wb32, wb_raw, 0, 8, SEM_LATE) + slabs(wob32, wob_raw, 0, 8, SEM_LATE)

    batch = [[cp_phi, x_in(8)] + cp_k[0] + [x_in(0)] + cp_v[0] + [cp_phi2] + cp_k[1] + cp_v[1],
             cp_k[2] + cp_v[2] + cp_k[3] + cp_v[3] + [x_in(9), x_in(1)], []]
    for g in range(8):
        if g < 6:
            batch[1] += [x_in(10 + g), x_in(2 + g)] + w_set(g)
        else:
            batch[2] += w_set(g)
    batch[2] += cp_late

    def start_all(cps):
        for c in cps:
            c.start()

    def wait_all(cps):
        for c in cps:
            c.wait()

    start_all(batch[0])

    class Side:
        never = None
        hist = []

    def side_begin(never):
        Side.never = never
        Side.hist = []

    def tr(x):
        w = _cfg("side")
        if Side.never is not None and len(Side.hist) >= w:
            x = jnp.concatenate([jnp.where(Side.never, Side.hist[-w], x[0:8, :]), x[8:, :]], axis=0)
        y = pltpu.bitcast(_unpk(x).T, U32)
        Side.hist.append(y[56:64, :])
        return y

    def wtile(raw, slab, c):
        return tr(raw[slab, c * 64:(c + 1) * 64, :])

    def wstore_split(ref, g, raw, slab):
        for c in range(8):
            ref[c, pl.ds(_mult(g * 64, 64), 64), :] = _pack(_unpack_split(wtile(raw, slab, c)))

    def wstore_shuf(ref, g, raw, slab):
        for c in range(8):
            ref[c, pl.ds(_mult(g * 64, 64), 64), :] = _pack_split(_unpk(wtile(raw, slab, c)).astype(F32))

    def wstore_perm(ref, g, raw, slab):
        for c in range(8):
            pk = wtile(raw, slab, c)
            for h4 in range(4):
                ref[c, pl.ds(g * 64 + h4, 16, stride=4), :] = pk[h4 * 16:(h4 + 1) * 16, :]

    def make_pmat(gs):
        def unsplit(r):
            return (r & ~15) + 2 * (r & 7) + ((r >> 3) & 1)

        r128 = unsplit(lax.broadcasted_iota(jnp.int32, (128, 128), 0))
        c128 = lax.broadcasted_iota(jnp.int32, (128, 128), 1)
        same_head = (2 * (r128 >> 6) + (r128 & 1)) == (c128 >> 5)
        er = unsplit(lax.broadcasted_iota(jnp.int32, (128, 32), 0))
        ec = lax.broadcasted_iota(jnp.int32, (128, 32), 1)
        expand = jnp.where(((er & 63) >> 1) == ec, 1.0, 0.0).astype(BF16)
        for g in gs:
            pg = _mm_nt(expand, wphi[g * 128:(g + 1) * 128, :])
            pmat[g] = _pack(jnp.where(same_head, pg, 0.0))

    def fold(dst, g, slab):
        val = _mm_nt(_unpk(pmat[g]), _unpk(wa_raw[slab])) * LOG2E
        for c in range(8):
            dst[c, pl.ds(_mult(g * 64, 64), 64), :] = _pack_split(val[:, c * L:(c + 1) * L])

    def prep_set(g):
        wstore_split(woaT, g, woa_raw, g)
        wstore_perm(wkvbT, g, wb_raw, 8 + g)
        wstore_split(wkvbT, 8 + g, wb_raw, 16 + g)

    def prep_late(g):
        wstore_perm(wqbT, g, wb_raw, g)
        wstore_split(wobT, g, wob_raw, g)

    class LN:
        def __init__(self, b):
            self.b = b
            self.piv = self.s1 = self.s2 = None

        def add(self, xt):
            if self.piv is None:
                self.piv = jnp.broadcast_to(xt[0:1, :], (8, L))
            d = [r - self.piv for r in _rows(xt)]
            self.s1 = _running_sum(self.s1, d)
            self.s2 = _running_sum(self.s2, [x * x for x in d])

        def finish(self):
            b = self.b
            m1 = jnp.sum(self.s1, axis=0, keepdims=True) * (1.0 / D)
            m2 = jnp.sum(self.s2, axis=0, keepdims=True) * (1.0 / D)
            var = jnp.maximum(m2 - m1 * m1, 0.0)
            rs = lax.rsqrt(var + 1e-5)
            mrs = jnp.broadcast_to((self.piv[0:1, :] + m1) * rs, (8, L))
            rs = jnp.broadcast_to(rs, (8, L))
            never = rs < 0.0
            for r in range(D // 16):
                pk = _pack_i(xT[b.hf][b.k, r * 16:r * 16 + 8, :] * rs - mrs,
                             xT[b.hf][b.k, r * 16 + 8:r * 16 + 16, :] * rs - mrs)
                xn[b.hf][b.k, r * 8:(r + 1) * 8, :] = pk
                if r % _cfg("ln_link") == _cfg("ln_link") - 1:
                    rs = jnp.where(never, pltpu.bitcast(pk, F32), rs)

    def prep_x(src, b):
        ln = LN(b)
        for cc in range(8):
            xt = _unpack_split(tr(xio[src, :, cc * L:(cc + 1) * L]))
            xT[b.hf][b.k, cc * 128:(cc + 1) * 128, :] = xt
            ln.add(xt)
        ln.finish()

    def mmw(ref, r0, n, rhs, sub):
        def wload(r):
            return jnp.concatenate([_unpk(ref[c, r // 2:(r + sub) // 2, :]) for c in range(8)], axis=1)
        return jnp.concatenate([_mm(wload(r), rhs()) for r in range(r0, r0 + n, sub)], axis=0)

    def proj(ref, r0, n, b, sub):
        return mmw(ref, r0, n, lambda: _unpk(xn[b.hf][b.k]), sub)

    def out_mm(wo, ch, b):
        m0 = ch * MC
        return xT[b.hf][b.k, m0:m0 + MC, :] + mmw(wo, m0, MC, lambda: _unpk(os_[b.hf][...]), _cfg("sub_o"))

    def emit(steps, lag):
        pend = []
        for n, (main, late) in enumerate(steps):
            main()
            if late is not None:
                pend.append((n + lag if n < len(steps) - _cfg("hold") else len(steps) + n, late))
            for due, f in pend:
                if due <= n:
                    f()
            pend = [e for e in pend if e[0] > n]
        for _, f in sorted(pend, key=lambda e: e[0]):
            f()

    def barrier():
        pl.semaphore_signal(bsem, 1)
        pl.semaphore_wait(bsem, 1)

    def z_finish(t, z):
        zb[t * 128:(t + 1) * 128, :] = jnp.broadcast_to(jnp.sum(z, axis=1, keepdims=True), (128, L))

    def kv_finish(t, acc):
        r = lax.broadcasted_iota(jnp.int32, (64, 128), 0)
        c = lax.broadcasted_iota(jnp.int32, (64, 128), 1)
        kvm[t] = _pack_split(jnp.where((r >> 5) == ((c >> 1) & 1), acc, 0.0))

    def a_kv(b, lay, last):
        steps = []
        la = lay + b.zr if b.hf == 1 else lay
        for ch in range(NCH):
            def kstep(ch=ch):
                kp = proj(wkvaT, ch * MC, MC, b, _cfg("sub_k"))
                for u in range(PPC):
                    t = ch * PPC + u
                    ep, en, sp, sn = _phi_parts(kp[u * 64:(u + 1) * 64, :])
                    r = _recip(sp * sn)
                    rp = r * sn
                    rn = r * sp
                    phi = jnp.concatenate([e * rp for e in ep] + [e * rn for e in en], axis=0)
                    phis[b.hf][ch][u * 64:(u + 1) * 64, :] = _pack_split(phi)
                    z = zacc[la, t * 128:(t + 1) * 128, :] + phi
                    zacc[la, t * 128:(t + 1) * 128, :] = z
                    if last:
                        z_finish(t, z)

            def vstep(ch=ch):
                vs[b.hf][ch][...] = _pack_split(proj(wkvaT, D + ch * MC, MC, b, _cfg("sub_v")))

            def mstep(ch=ch):
                for u in range(PPC):
                    t = ch * PPC + u
                    acc = kv_acc[la, t] + _mm_nt(_unpk(vs[b.hf][ch][u * 32:(u + 1) * 32, :]),
                                                 _unpk(phis[b.hf][ch][u * 64:(u + 1) * 64, :]))
                    kv_acc[la, t] = acc
                    if last:
                        kv_finish(t, acc)

            steps += [(kstep, None), (vstep, mstep)]
        return steps

    def a_q(b):
        steps = []
        for ch in range(NCH):
            def qstep(ch=ch):
                qp = proj(wqaT, ch * MC, MC, b, _cfg("sub_q"))
                for u in range(PPC):
                    t = ch * PPC + u
                    ep, en, sp, sn = _phi_parts(qp[u * 64:(u + 1) * 64, :])
                    zr = _rows(zb[t * 128:(t + 1) * 128, :])
                    dp = _fold2(jnp.add, [e * zz for e, zz in zip(ep, zr[:8])])
                    dn = _fold2(jnp.add, [e * zz for e, zz in zip(en, zr[8:])])
                    r = _recip(dp * sn + dn * sp + 1e-6 * (sp * sn))
                    rp = r * sn
                    rn = r * sp
                    phi = jnp.concatenate([e * rp for e in ep] + [e * rn for e in en], axis=0)
                    phis[b.hf][ch][u * 64:(u + 1) * 64, :] = _pack_split(phi)

            def nstep(ch=ch):
                for u in range(PPC):
                    t = ch * PPC + u
                    o = _mm(_unpk(kvm[t]), _unpk(phis[b.hf][ch][u * 64:(u + 1) * 64, :]))
                    os_[b.hf][t * 32:(t + 1) * 32, :] = _pack_split(o)

            steps.append((qstep, nstep))
        return steps

    def out_proj(wo, b, defer=None):
        steps = []
        ln = LN(b)
        for ch in range(NCH):
            def ostep(ch=ch):
                xt = out_mm(wo, ch, b)
                xT[b.hf][b.k, ch * MC:(ch + 1) * MC, :] = xt
                ln.add(xt)
                if ch == NCH - 1 and defer is None:
                    ln.finish()
            steps.append((ostep, None))
        if defer is not None:
            defer.append((ln.finish, None))
        return steps

    def b_kv(b):
        steps = []
        for base, ref in ((0, kb), (D, vb)):
            for m0 in range(0, D, MC):
                def step(base=base, ref=ref, m0=m0):
                    p = proj(wkvbT, base + m0, MC, b, _cfg("sub_b"))
                    ref[WIN + b.j, m0:m0 + MC, :] = p
                    if b.hf == 0:
                        ref[b.k, m0:m0 + MC, :] = pltpu.roll(p, 2, 1)
                steps.append((step, None))
        return steps

    def b_q(b):
        j = b.j
        even = (lax.broadcasted_iota(jnp.int32, (8, L), 0) & 1) == 0
        first = lax.broadcasted_iota(jnp.int32, (8, L), 1) < 2
        cs = DH ** -0.5

        def logits(q, g):
            acc = [None] * WIN
            for r in range(16):
                qv = q[r * 8:r * 8 + 8, :]
                for w in range(WIN):
                    t = qv * kb[WIN + j - w, g * 128 + r * 8:g * 128 + r * 8 + 8, :]
                    acc[w] = t if acc[w] is None else acc[w] + t
            return acc

        steps = []
        for G in range(4):
            def step(G=G):
                q = proj(wqbT, G * 256, 256, b, _cfg("sub_qb"))
                la, lb = logits(q[0:128, :], 2 * G), logits(q[128:256, :], 2 * G + 1)
                lg = [jnp.where(even, x + pltpu.roll(x, 7, 0), y + pltpu.roll(y, 1, 0)) for x, y in zip(la, lb)]
                if b.hf == 1:
                    lg = [l if w == 0 else jnp.where(jnp.logical_and(first, j < w), -1e9 / cs, l)
                          for w, l in enumerate(lg)]
                mx = _tree(jnp.maximum, lg)
                ex = [jnp.exp2((l - mx) * (cs * LOG2E)) for l in lg]
                rs = _recip(_tree(jnp.add, ex))
                at = [e * rs for e in ex]
                for hh in range(8):
                    h = G * 8 + hh
                    s = 2 * (hh % 4) + hh // 4
                    o = _running_sum(None, [
                        jnp.broadcast_to(at[w][s:s + 1, :], (DH, L)) * vb[WIN + j - w, h * DH:(h + 1) * DH, :]
                        for w in range(WIN)])
                    os_[b.hf][h * 16:(h + 1) * 16, :] = _pack_split(o)
            steps.append((step, None))
        return steps

    def final_proj(b, defer):
        steps = []
        for ch in range(NCH):
            def ostep(ch=ch):
                xt = out_mm(wobT, ch, b)
                for u in range(GPC):
                    cc = ch * GPC + u
                    y = _pack_split(xt[u * 128:(u + 1) * 128, :])
                    if cc >= 8 - defer:
                        ystage[b.k + 1, (cc - 8 + ND) * 64:(cc - 7 + ND) * 64, :] = y
                    else:
                        xio[b.j, :, cc * L:(cc + 1) * L] = tr(y)
            steps.append((ostep, None))
        return steps

    def flush_out(k, slot):
        for u in range(ND):
            xio[slot, :, (8 - ND + u) * L:(9 - ND + u) * L] = tr(ystage[k, u * 64:(u + 1) * 64, :])

    def stage1():
        _Stage.cur = 0
        kv_acc[...] = jnp.zeros(kv_acc.shape, F32)
        zacc[...] = jnp.zeros(zacc.shape, F32)
        ystage[0] = jnp.zeros(ystage.shape[1:], U32)
        cp_phi.wait()
        x_in(8).wait()
        make_pmat(range(GPC))
        prep_x(8, Blk(0, 0))
        start_all(batch[1])

        sa = a_kv(Blk(0, 0), 0, False)
        sb = a_kv(Blk(1, 0), 0, False)
        pend = []
        for ch in range(NCH if 0 in only else 0):
            if ch == 1:
                start_all(batch[2])
            wait_all(cp_k[ch])
            if ch == 0:
                for u in range(GPC):
                    fold(wkvaT, u, 8 + u)
                sa[0][0]()
                x_in(0).wait()
            wait_all(cp_v[ch])
            if ch == 0:
                cp_phi2.wait()
                prep_x(0, Blk(1, 0))
                make_pmat(range(GPC, 8))
            else:
                if ch == NCH - 1:
                    x_in(9).wait()
                    x_in(1).wait()
                for u in range(GPC):
                    fold(wkvaT, ch * GPC + u, 8 + ch * GPC + u)
            for u in range(GPC):
                wstore_shuf(wkvaT, 8 + ch * GPC + u, wa_raw, 16 + ch * GPC + u)
            for f in pend:
                f()
            if ch == NCH - 1:
                side_begin(zacc[0, 0:8, :] < 0.0)
                prep_x(9, Blk(0, 1))
                prep_x(1, Blk(1, 1))
                side_begin(None)
            if ch == 0:
                sa[1][0]()
                sb[0][0]()
            else:
                sa[2 * ch][0]()
                sb[2 * ch][0]()
                sa[2 * ch + 1][0]()
            sb[2 * ch + 1][0]()
            pend = [sa[2 * ch + 1][1], sb[2 * ch + 1][1]]
        for f in pend:
            f()

        def s1(i, c):
            _Stage.cur = 1
            @pl.when(i < 7)
            def _():
                x_in(9 + i).wait()
                x_in(1 + i).wait()

            wait_all(w_set(i - 1))
            side_begin(jnp.full((8, L), i >> 6, jnp.int32) > 0)
            nxt = jnp.minimum(i + 1, 7)
            prep_x(8 + nxt, Blk(0, i + 1))
            prep_x(nxt, Blk(1, i + 1))
            prep_set(i - 1)
            side_begin(None)
            steps = a_kv(Blk(0, i), 0, False) + a_kv(Blk(1, i), 0, CFG["tail"] < 2)
            if not CFG["tail"]:
                steps.insert(CFG["fold_at"], (lambda: fold(wqaT, i - 1, i - 1), None))
            emit(steps, _cfg("lag_kv"))
            return c

        if 1 in only:
            lax.fori_loop(1, 8, s1, 0)
        _Stage.cur = 0
        wait_all(w_set(7))
        for g in range(0 if CFG["tail"] else 7, 8):
            fold(wqaT, g, g)
        prep_set(7)
        if CFG["tail"] == 2:
            for t in range(16):
                z_finish(t, zacc[0, t * 128:(t + 1) * 128, :])
                kv_finish(t, kv_acc[0, t])
        wait_all(cp_late)

    def s2(i, c):
        _Stage.cur = 2
        b0, b1 = Blk(0, i), Blk(1, i)
        steps = a_q(b0) + a_q(b1) + out_proj(woaT, b0) + out_proj(woaT, b1)
        steps += [(lambda: prep_late(i), None)] + b_kv(b0) + b_kv(b1)
        emit(steps, _cfg("lag_q"))
        return c

    def s3(i, c):
        _Stage.cur = 3
        b0, b1 = Blk(0, i), Blk(1, i)
        late_ln = []
        steps = b_q(b0) + b_q(b1) + out_proj(wobT, b0, late_ln) + out_proj(wobT, b1)
        steps += a_kv(b0, 1, False) + a_kv(b1, 1, True)
        steps[CFG["bar3"]:CFG["bar3"]] = [(barrier, None)] + late_ln
        emit(steps, _cfg("lag_kv"))
        return c

    def s5(i, c):
        _Stage.cur = 5
        b0, b1 = Blk(0, i), Blk(1, i)
        flush = (lambda: flush_out(i, jnp.where(i > 0, i - 1, NBLK)), None)
        emit(b_q(b0) + b_q(b1) + [flush] + final_proj(b0, 0) + final_proj(b1, ND), 0)
        x_out(b0.j).start()
        x_out(b1.j, 0, 8 - ND).start()

        @pl.when(i > 0)
        def _():
            x_out(i - 1, 8 - ND, 8, SEM_KV + i - 1).start()
        return c

    def layer_pair(l, c):
        pl.when(l == 0)(stage1)
        if 2 in only:
            lax.fori_loop(0, 8, s2, 0)

        @pl.when(l == 0)
        def _():
            if 3 in only:
                lax.fori_loop(0, 8, s3, 0)

        @pl.when(l == 1)
        def _():
            if 5 in only:
                lax.fori_loop(0, 8, s5, 0)
            flush_out(8, 7)
            x_out(7, 8 - ND, 8, SEM_KV + 7).start()
        return c

    lax.fori_loop(0, 2, layer_pair, 0)

    for k in range(8):
        x_out(8 + k).wait()
        x_out(k, 0, 8 - ND).wait()
        x_out(k, 8 - ND, 8, SEM_KV + k).wait()


def _compiler_params():
    vmem = 120 * 1024 * 1024
    try:
        return pltpu.CompilerParams(vmem_limit_bytes=vmem, disable_semaphore_checks=True)
    except TypeError:
        return pltpu.CompilerParams(vmem_limit_bytes=vmem)


@jax.jit
def pallas_interleave_layers__linear_kernel_hedgehog__sliding_local_dilated__prompt_kernel(
    A_x: jax.Array,
    A_wqkv: jax.Array,
    A_w_phi: jax.Array,
    A_wo: jax.Array,
    B_x: jax.Array,
    B_wqkv: jax.Array,
    B_wo: jax.Array,
):
    del B_x
    x3 = A_x.reshape(S // 32, 32, D)
    wphi2 = A_w_phi.reshape(H * DH, DH)
    any_spec = pl.BlockSpec(memory_space=pl.ANY)
    scratch = [
        pltpu.VMEM((NBLK + 1, S // 32, D), U32),
        pltpu.VMEM((24, D // 2, L), U32),
        pltpu.VMEM((8, D // 2, L), U32),
        pltpu.VMEM((24, D // 2, L), U32),
        pltpu.VMEM((8, D // 2, L), U32),
        pltpu.VMEM((H * DH, DH), BF16),
        pltpu.VMEM((8, 64, 128), U32),
        pltpu.VMEM((8, D // 2, L), U32),
        pltpu.VMEM((8, D, L), U32),
        pltpu.VMEM((8, D // 2, L), U32),
        pltpu.VMEM((8, D // 2 + 8, L), U32),
        pltpu.VMEM((8, D, L), U32),
        pltpu.VMEM((8, D // 2, L), U32),
        pltpu.VMEM((WIN + NBLK, D, L), F32),
        pltpu.VMEM((WIN + NBLK, D, L), F32),
        pltpu.VMEM((2, 16, 64, 128), F32),
        pltpu.VMEM((16, 32, 128), U32),
        pltpu.VMEM((2, 2 * D, L), F32),
        pltpu.VMEM((2 * D, L), F32),
        pltpu.VMEM((9, ND * 64, L), U32),
        pltpu.SemaphoreType.DMA((NSEM,)),
        pltpu.SemaphoreType.REGULAR,
    ]
    scratch += [pltpu.VMEM((9, D, L), F32)] * 2
    scratch += [pltpu.VMEM((9, D // 2, L), U32)] * 2
    scratch += [pltpu.VMEM((D // 2, L), U32)] * 2
    scratch += [pltpu.VMEM((MC, L), U32)] * (2 * NCH)
    scratch += [pltpu.VMEM((MC // 2, L), U32)] * (2 * NCH)
    out = pl.pallas_call(
        _kernel,
        out_shape=jax.ShapeDtypeStruct((S // 32, 32, D), BF16),
        in_specs=[any_spec] * 6,
        out_specs=any_spec,
        scratch_shapes=scratch,
        compiler_params=_compiler_params(),
        name="hedgehog_dilated",
    )(x3, A_wqkv, wphi2, A_wo, B_wqkv, B_wo)
    return out.reshape(1, S, D)
```

```python
import math

import jax
import jax.numpy as jnp
from jax import lax
import jax.experimental.pallas as pl
import jax.experimental.pallas.tpu as pltpu

S = 2048
D = 1024
H = 32
DH = 32
NBLK = 16
L = 128
WIN = 8
LOG2E = math.log2(math.e)
F32 = jnp.float32
BF16 = jnp.bfloat16
U32 = jnp.uint32
NT = (((1,), (1,)), ((), ()))

MC = 256
NCH = D // MC
GPC = MC // 128
PPC = MC // 64
ND = 2

CFG = dict(only=None, lag_q=2, lag_kv=4, hold=7, ln_link=4, side=3, bar3=14,
           sub_q=128, sub_k=64, sub_v=256, sub_qb=128, sub_o=256, sub_b=256,
           hold_1=0, sub_v_1=128, ln_link_3=2)


class _Stage:
    cur = 0


def _cfg(key):
    return CFG.get("%s_%d" % (key, _Stage.cur), CFG[key])


SEM_X = 0
SEM_PHI = 16
SEM_KV = 18
SEM_SET = 26
SEM_LATE = 34
NSEM = 35


def _mm(a, b):
    return jnp.dot(a, b, preferred_element_type=F32)


def _mm_nt(a, b):
    return lax.dot_general(a, b, NT, preferred_element_type=F32)


def _tree(op, xs):
    xs = list(xs)
    while len(xs) > 1:
        nxt = [op(xs[i], xs[i + 1]) for i in range(0, len(xs) - 1, 2)]
        if len(xs) % 2:
            nxt.append(xs[-1])
        xs = nxt
    return xs[0]


def _running_sum(acc, xs):
    for x in xs:
        acc = x if acc is None else acc + x
    return acc


def _rows(a, n=8):
    return [a[i * n:(i + 1) * n, :] for i in range(a.shape[0] // n)]


def _pack(a):
    return pltpu.bitcast(a.astype(BF16), U32)


def _unpk(a):
    return pltpu.bitcast(a, BF16)


def _pack_i(a, b):
    return pltpu.pack_elementwise([a, b], packed_dtype=BF16)


def _pack_split(a):
    r = _rows(a)
    return jnp.concatenate([_pack_i(r[2 * i], r[2 * i + 1]) for i in range(len(r) // 2)], axis=0)


def _unpack_split(p):
    out = []
    for x in _rows(p):
        out.append(pltpu.unpack_elementwise(x, index=0, packed_dtype=BF16, unpacked_dtype=F32))
        out.append(pltpu.unpack_elementwise(x, index=1, packed_dtype=BF16, unpacked_dtype=F32))
    return jnp.concatenate(out, axis=0)


def _fold2(op, xs):
    r = _tree(op, xs)
    r = op(r, pltpu.roll(r, 4, 0))
    return op(r, pltpu.roll(r, 2, 0))


def _phi_parts(p):
    ps = _rows(p)
    mx = _fold2(jnp.maximum, ps)
    mn = _fold2(jnp.minimum, ps)
    ep = [jnp.exp2(x - mx) for x in ps]
    en = [jnp.exp2(mn - x) for x in ps]
    return ep, en, _fold2(jnp.add, ep), _fold2(jnp.add, en)


def _recip(x):
    r = pl.reciprocal(x, approx=True)
    return r * (2.0 - x * r)


def _mult(x, m):
    return x if isinstance(x, int) else pl.multiple_of(x, m)


def _kernel(x_hbm, wa_hbm, wphi_hbm, woa_hbm, wb_hbm, wob_hbm, out_hbm,
            xio, wa_raw, woa_raw, wb_raw, wob_raw, wphi, pmat,
            wqaT, wkvaT, woaT, wqbT, wkvbT, wobT, kb, vb, kv_acc, kvm, zacc, zb, ystage, sems, *rest):
    xT, xn, os_ = rest[0:2], rest[2:4], rest[4:6]
    phis = [rest[6:6 + NCH], rest[6 + NCH:6 + 2 * NCH]]
    vs = [rest[6 + 2 * NCH:6 + 3 * NCH], rest[6 + 3 * NCH:6 + 4 * NCH]]
    only = CFG["only"] or (0, 1, 2, 3, 5)

    class Blk:
        def __init__(self, hf, k):
            self.hf, self.k = hf, k
            self.j = 8 * (1 - hf) + k
            self.zr = 0 if isinstance(k, int) else k >> 6

    x32, out32, wa32, woa32, wb32, wob32 = [
        r.bitcast(U32) for r in (x_hbm, out_hbm, wa_hbm, woa_hbm, wb_hbm, wob_hbm)]

    def x_in(j):
        return pltpu.make_async_copy(x32.at[:, j, :], xio.at[j], sems.at[SEM_X + j])

    def x_out(j, c0=0, c1=8, sem=None):
        cs = pl.ds(c0 * L, (c1 - c0) * L)
        return pltpu.make_async_copy(xio.at[j, :, cs], out32.at[:, j, cs],
                                     sems.at[SEM_X + j if sem is None else sem])

    def slabs(src, dst, g0, n, sem):
        return [pltpu.make_async_copy(src.at[:, pl.ds(_mult((g0 + u) * 128, 128), 128)], dst.at[g0 + u],
                                      sems.at[sem]) for u in range(n)]

    cp_phi = pltpu.make_async_copy(wphi_hbm.at[0:MC], wphi.at[0:MC], sems.at[SEM_PHI])
    cp_phi2 = pltpu.make_async_copy(wphi_hbm.at[MC:D], wphi.at[MC:D], sems.at[SEM_PHI + 1])
    cp_k = [slabs(wa32, wa_raw, 8 + ch * GPC, GPC, SEM_KV + 2 * ch) for ch in range(NCH)]
    cp_v = [slabs(wa32, wa_raw, 16 + ch * GPC, GPC, SEM_KV + 2 * ch + 1) for ch in range(NCH)]

    def w_set(g):
        return (slabs(wa32, wa_raw, g, 1, SEM_SET + g) + slabs(woa32, woa_raw, g, 1, SEM_SET + g)
                + slabs(wb32, wb_raw, 8 + g, 1, SEM_SET + g) + slabs(wb32, wb_raw, 16 + g, 1, SEM_SET + g))

    cp_late = slabs(wb32, wb_raw, 0, 8, SEM_LATE) + slabs(wob32, wob_raw, 0, 8, SEM_LATE)

    batch = [[cp_phi, x_in(8)] + cp_k[0] + [x_in(0)] + cp_v[0] + [cp_phi2] + cp_k[1] + cp_v[1],
             cp_k[2] + cp_v[2] + cp_k[3] + cp_v[3] + [x_in(9), x_in(1)], []]
    for g in range(8):
        if g < 6:
            batch[1] += [x_in(10 + g), x_in(2 + g)] + w_set(g)
        else:
            batch[2] += w_set(g)
    batch[2] += cp_late

    def start_all(cps):
        for c in cps:
            c.start()

    def wait_all(cps):
        for c in cps:
            c.wait()

    start_all(batch[0])

    class Side:
        never = None
        hist = []

    def side_begin(never):
        Side.never = never
        Side.hist = []

    def tr(x):
        w = _cfg("side")
        if Side.never is not None and len(Side.hist) >= w:
            x = jnp.concatenate([jnp.where(Side.never, Side.hist[-w], x[0:8, :]), x[8:, :]], axis=0)
        y = pltpu.bitcast(_unpk(x).T, U32)
        Side.hist.append(y[56:64, :])
        return y

    def wtile(raw, slab, c):
        return tr(raw[slab, c * 64:(c + 1) * 64, :])

    def wstore_split(ref, g, raw, slab):
        for c in range(8):
            ref[c, pl.ds(_mult(g * 64, 64), 64), :] = _pack(_unpack_split(wtile(raw, slab, c)))

    def wstore_shuf(ref, g, raw, slab):
        for c in range(8):
            ref[c, pl.ds(_mult(g * 64, 64), 64), :] = _pack_split(_unpk(wtile(raw, slab, c)).astype(F32))

    def wstore_perm(ref, g, raw, slab):
        for c in range(8):
            pk = wtile(raw, slab, c)
            for h4 in range(4):
                ref[c, pl.ds(g * 64 + h4, 16, stride=4), :] = pk[h4 * 16:(h4 + 1) * 16, :]

    def make_pmat(gs):
        def unsplit(r):
            return (r & ~15) + 2 * (r & 7) + ((r >> 3) & 1)

        r128 = unsplit(lax.broadcasted_iota(jnp.int32, (128, 128), 0))
        c128 = lax.broadcasted_iota(jnp.int32, (128, 128), 1)
        same_head = (2 * (r128 >> 6) + (r128 & 1)) == (c128 >> 5)
        er = unsplit(lax.broadcasted_iota(jnp.int32, (128, 32), 0))
        ec = lax.broadcasted_iota(jnp.int32, (128, 32), 1)
        expand = jnp.where(((er & 63) >> 1) == ec, 1.0, 0.0).astype(BF16)
        for g in gs:
            pg = _mm_nt(expand, wphi[g * 128:(g + 1) * 128, :])
            pmat[g] = _pack(jnp.where(same_head, pg, 0.0))

    def fold(dst, g, slab):
        val = _mm_nt(_unpk(pmat[g]), _unpk(wa_raw[slab])) * LOG2E
        for c in range(8):
            dst[c, pl.ds(_mult(g * 64, 64), 64), :] = _pack_split(val[:, c * L:(c + 1) * L])

    def prep_set(g):
        wstore_split(woaT, g, woa_raw, g)
        wstore_perm(wkvbT, g, wb_raw, 8 + g)
        wstore_split(wkvbT, 8 + g, wb_raw, 16 + g)

    def prep_late(g):
        wstore_perm(wqbT, g, wb_raw, g)
        wstore_split(wobT, g, wob_raw, g)

    class LN:
        def __init__(self, b):
            self.b = b
            self.piv = self.s1 = self.s2 = None

        def add(self, xt):
            if self.piv is None:
                self.piv = jnp.broadcast_to(xt[0:1, :], (8, L))
            d = [r - self.piv for r in _rows(xt)]
            self.s1 = _running_sum(self.s1, d)
            self.s2 = _running_sum(self.s2, [x * x for x in d])

        def finish(self):
            b = self.b
            m1 = jnp.sum(self.s1, axis=0, keepdims=True) * (1.0 / D)
            m2 = jnp.sum(self.s2, axis=0, keepdims=True) * (1.0 / D)
            var = jnp.maximum(m2 - m1 * m1, 0.0)
            rs = lax.rsqrt(var + 1e-5)
            mrs = jnp.broadcast_to((self.piv[0:1, :] + m1) * rs, (8, L))
            rs = jnp.broadcast_to(rs, (8, L))
            never = rs < 0.0
            for r in range(D // 16):
                pk = _pack_i(xT[b.hf][b.k, r * 16:r * 16 + 8, :] * rs - mrs,
                             xT[b.hf][b.k, r * 16 + 8:r * 16 + 16, :] * rs - mrs)
                xn[b.hf][b.k, r * 8:(r + 1) * 8, :] = pk
                if r % _cfg("ln_link") == _cfg("ln_link") - 1:
                    rs = jnp.where(never, pltpu.bitcast(pk, F32), rs)

    def prep_x(src, b):
        ln = LN(b)
        for cc in range(8):
            xt = _unpack_split(tr(xio[src, :, cc * L:(cc + 1) * L]))
            xT[b.hf][b.k, cc * 128:(cc + 1) * 128, :] = xt
            ln.add(xt)
        ln.finish()

    def mmw(ref, r0, n, rhs, sub):
        def wload(r):
            return jnp.concatenate([_unpk(ref[c, r // 2:(r + sub) // 2, :]) for c in range(8)], axis=1)
        return jnp.concatenate([_mm(wload(r), rhs()) for r in range(r0, r0 + n, sub)], axis=0)

    def proj(ref, r0, n, b, sub):
        return mmw(ref, r0, n, lambda: _unpk(xn[b.hf][b.k]), sub)

    def out_mm(wo, ch, b):
        m0 = ch * MC
        return xT[b.hf][b.k, m0:m0 + MC, :] + mmw(wo, m0, MC, lambda: _unpk(os_[b.hf][...]), _cfg("sub_o"))

    def emit(steps, lag):
        pend = []
        for n, (main, late) in enumerate(steps):
            main()
            if late is not None:
                pend.append((n + lag if n < len(steps) - _cfg("hold") else len(steps) + n, late))
            for due, f in pend:
                if due <= n:
                    f()
            pend = [e for e in pend if e[0] > n]
        for _, f in sorted(pend, key=lambda e: e[0]):
            f()

    def split(i):
        @pl.when((i >> 6) > 0)
        def _():
            zb[2 * D:2 * D + 8, :] = jnp.zeros((8, L), F32)

    def z_finish(t, z):
        zb[t * 128:(t + 1) * 128, :] = jnp.broadcast_to(jnp.sum(z, axis=1, keepdims=True), (128, L))

    def kv_finish(t, acc):
        r = lax.broadcasted_iota(jnp.int32, (64, 128), 0)
        c = lax.broadcasted_iota(jnp.int32, (64, 128), 1)
        kvm[t] = _pack_split(jnp.where((r >> 5) == ((c >> 1) & 1), acc, 0.0))

    def a_kv(b, lay, last):
        steps = []
        la = lay + b.zr if b.hf == 1 else lay
        for ch in range(NCH):
            def kstep(ch=ch):
                kp = proj(wkvaT, ch * MC, MC, b, _cfg("sub_k"))
                for u in range(PPC):
                    t = ch * PPC + u
                    ep, en, sp, sn = _phi_parts(kp[u * 64:(u + 1) * 64, :])
                    r = _recip(sp * sn)
                    rp = r * sn
                    rn = r * sp
                    phi = jnp.concatenate([e * rp for e in ep] + [e * rn for e in en], axis=0)
                    phis[b.hf][ch][u * 64:(u + 1) * 64, :] = _pack_split(phi)
                    z = zacc[la, t * 128:(t + 1) * 128, :] + phi
                    zacc[la, t * 128:(t + 1) * 128, :] = z
                    if last:
                        z_finish(t, z)

            def vstep(ch=ch):
                vs[b.hf][ch][...] = _pack_split(proj(wkvaT, D + ch * MC, MC, b, _cfg("sub_v")))

            def mstep(ch=ch):
                for u in range(PPC):
                    t = ch * PPC + u
                    acc = kv_acc[la, t] + _mm_nt(_unpk(vs[b.hf][ch][u * 32:(u + 1) * 32, :]),
                                                 _unpk(phis[b.hf][ch][u * 64:(u + 1) * 64, :]))
                    kv_acc[la, t] = acc
                    if last:
                        kv_finish(t, acc)

            steps += [(kstep, None), (vstep, mstep)]
        return steps

    def a_q(b):
        steps = []
        for ch in range(NCH):
            def qstep(ch=ch):
                qp = proj(wqaT, ch * MC, MC, b, _cfg("sub_q"))
                for u in range(PPC):
                    t = ch * PPC + u
                    ep, en, sp, sn = _phi_parts(qp[u * 64:(u + 1) * 64, :])
                    zr = _rows(zb[t * 128:(t + 1) * 128, :])
                    dp = _fold2(jnp.add, [e * zz for e, zz in zip(ep, zr[:8])])
                    dn = _fold2(jnp.add, [e * zz for e, zz in zip(en, zr[8:])])
                    r = _recip(dp * sn + dn * sp + 1e-6 * (sp * sn))
                    rp = r * sn
                    rn = r * sp
                    phi = jnp.concatenate([e * rp for e in ep] + [e * rn for e in en], axis=0)
                    phis[b.hf][ch][u * 64:(u + 1) * 64, :] = _pack_split(phi)

            def nstep(ch=ch):
                for u in range(PPC):
                    t = ch * PPC + u
                    o = _mm(_unpk(kvm[t]), _unpk(phis[b.hf][ch][u * 64:(u + 1) * 64, :]))
                    os_[b.hf][t * 32:(t + 1) * 32, :] = _pack_split(o)

            steps.append((qstep, nstep))
        return steps

    def out_proj(wo, b, defer=None):
        steps = []
        ln = LN(b)
        for ch in range(NCH):
            def ostep(ch=ch):
                xt = out_mm(wo, ch, b)
                xT[b.hf][b.k, ch * MC:(ch + 1) * MC, :] = xt
                ln.add(xt)
                if ch == NCH - 1 and defer is None:
                    ln.finish()
            steps.append((ostep, None))
        if defer is not None:
            defer.append((ln.finish, None))
        return steps

    def b_kv(b):
        steps = []
        for base, ref in ((0, kb), (D, vb)):
            for m0 in range(0, D, MC):
                def step(base=base, ref=ref, m0=m0):
                    p = proj(wkvbT, base + m0, MC, b, _cfg("sub_b"))
                    ref[WIN + b.j, m0:m0 + MC, :] = p
                    if b.hf == 0:
                        ref[b.k, m0:m0 + MC, :] = pltpu.roll(p, 2, 1)
                steps.append((step, None))
        return steps

    def b_q(b):
        j = b.j
        even = (lax.broadcasted_iota(jnp.int32, (8, L), 0) & 1) == 0
        first = lax.broadcasted_iota(jnp.int32, (8, L), 1) < 2
        cs = DH ** -0.5

        def logits(q, g):
            acc = [None] * WIN
            for r in range(16):
                qv = q[r * 8:r * 8 + 8, :]
                for w in range(WIN):
                    t = qv * kb[WIN + j - w, g * 128 + r * 8:g * 128 + r * 8 + 8, :]
                    acc[w] = t if acc[w] is None else acc[w] + t
            return acc

        steps = []
        for G in range(4):
            def step(G=G):
                q = proj(wqbT, G * 256, 256, b, _cfg("sub_qb"))
                la, lb = logits(q[0:128, :], 2 * G), logits(q[128:256, :], 2 * G + 1)
                lg = [jnp.where(even, x + pltpu.roll(x, 7, 0), y + pltpu.roll(y, 1, 0)) for x, y in zip(la, lb)]
                if b.hf == 1:
                    lg = [l if w == 0 else jnp.where(jnp.logical_and(first, j < w), -1e9 / cs, l)
                          for w, l in enumerate(lg)]
                mx = _tree(jnp.maximum, lg)
                ex = [jnp.exp2((l - mx) * (cs * LOG2E)) for l in lg]
                rs = _recip(_tree(jnp.add, ex))
                at = [e * rs for e in ex]
                for hh in range(8):
                    h = G * 8 + hh
                    s = 2 * (hh % 4) + hh // 4
                    o = _running_sum(None, [
                        jnp.broadcast_to(at[w][s:s + 1, :], (DH, L)) * vb[WIN + j - w, h * DH:(h + 1) * DH, :]
                        for w in range(WIN)])
                    os_[b.hf][h * 16:(h + 1) * 16, :] = _pack_split(o)
            steps.append((step, None))
        return steps

    def final_proj(b, defer):
        steps = []
        for ch in range(NCH):
            def ostep(ch=ch):
                xt = out_mm(wobT, ch, b)
                for u in range(GPC):
                    cc = ch * GPC + u
                    y = _pack_split(xt[u * 128:(u + 1) * 128, :])
                    if cc >= 8 - defer:
                        ystage[b.k + 1, (cc - 8 + ND) * 64:(cc - 7 + ND) * 64, :] = y
                    else:
                        xio[b.j, :, cc * L:(cc + 1) * L] = tr(y)
            steps.append((ostep, None))
        return steps

    def flush_out(k, slot):
        for u in range(ND):
            xio[slot, :, (8 - ND + u) * L:(9 - ND + u) * L] = tr(ystage[k, u * 64:(u + 1) * 64, :])

    def stage1():
        _Stage.cur = 0
        kv_acc[...] = jnp.zeros(kv_acc.shape, F32)
        zacc[...] = jnp.zeros(zacc.shape, F32)
        ystage[0] = jnp.zeros(ystage.shape[1:], U32)
        cp_phi.wait()
        x_in(8).wait()
        make_pmat(range(GPC))
        prep_x(8, Blk(0, 0))
        start_all(batch[1])

        sa = a_kv(Blk(0, 0), 0, False)
        sb = a_kv(Blk(1, 0), 0, False)
        pend = []
        for ch in range(NCH if 0 in only else 0):
            if ch == 1:
                start_all(batch[2])
            wait_all(cp_k[ch])
            if ch == 0:
                for u in range(GPC):
                    fold(wkvaT, u, 8 + u)
                sa[0][0]()
                x_in(0).wait()
            wait_all(cp_v[ch])
            if ch == 0:
                cp_phi2.wait()
                prep_x(0, Blk(1, 0))
                make_pmat(range(GPC, 8))
            else:
                if ch == NCH - 1:
                    x_in(9).wait()
                    x_in(1).wait()
                for u in range(GPC):
                    fold(wkvaT, ch * GPC + u, 8 + ch * GPC + u)
            for u in range(GPC):
                wstore_shuf(wkvaT, 8 + ch * GPC + u, wa_raw, 16 + ch * GPC + u)
            for f in pend:
                f()
            if ch == NCH - 1:
                side_begin(zacc[0, 0:8, :] < 0.0)
                prep_x(9, Blk(0, 1))
                prep_x(1, Blk(1, 1))
                side_begin(None)
            if ch == 0:
                sa[1][0]()
                sb[0][0]()
            else:
                sa[2 * ch][0]()
                sb[2 * ch][0]()
                sa[2 * ch + 1][0]()
            sb[2 * ch + 1][0]()
            pend = [sa[2 * ch + 1][1], sb[2 * ch + 1][1]]
        for f in pend:
            f()

        def s1(i, c):
            _Stage.cur = 1
            @pl.when(i < 7)
            def _():
                x_in(9 + i).wait()
                x_in(1 + i).wait()

            wait_all(w_set(i - 1))
            side_begin(jnp.full((8, L), i >> 6, jnp.int32) > 0)
            nxt = jnp.minimum(i + 1, 7)
            prep_x(8 + nxt, Blk(0, i + 1))
            prep_x(nxt, Blk(1, i + 1))
            prep_set(i - 1)
            side_begin(None)
            steps = a_kv(Blk(0, i), 0, False) + a_kv(Blk(1, i), 0, False)
            emit(steps, _cfg("lag_kv"))
            return c

        if 1 in only:
            lax.fori_loop(1, 8, s1, 0)
        _Stage.cur = 0
        wait_all(w_set(7))
        for g in range(8):
            fold(wqaT, g, g)
        prep_set(7)
        for t in range(16):
            z_finish(t, zacc[0, t * 128:(t + 1) * 128, :])
            kv_finish(t, kv_acc[0, t])
        wait_all(cp_late)

    def s2(i, c):
        _Stage.cur = 2
        b0, b1 = Blk(0, i), Blk(1, i)
        steps = a_q(b0) + a_q(b1) + out_proj(woaT, b0) + out_proj(woaT, b1)
        steps += [(lambda: prep_late(i), None)] + b_kv(b0) + b_kv(b1)
        emit(steps, _cfg("lag_q"))
        return c

    def s3(i, c):
        _Stage.cur = 3
        b0, b1 = Blk(0, i), Blk(1, i)
        late_ln = []
        steps = b_q(b0) + b_q(b1) + out_proj(wobT, b0, late_ln) + out_proj(wobT, b1)
        steps += a_kv(b0, 1, False) + a_kv(b1, 1, True)
        steps[CFG["bar3"]:CFG["bar3"]] = [(lambda: split(i), None)] + late_ln
        emit(steps, _cfg("lag_kv"))
        return c

    def s5(i, c):
        _Stage.cur = 5
        b0, b1 = Blk(0, i), Blk(1, i)
        flush = (lambda: flush_out(i, jnp.where(i > 0, i - 1, NBLK)), None)
        emit(b_q(b0) + b_q(b1) + [flush] + final_proj(b0, 0) + final_proj(b1, ND), 0)
        x_out(b0.j).start()
        x_out(b1.j, 0, 8 - ND).start()

        @pl.when(i > 0)
        def _():
            x_out(i - 1, 8 - ND, 8, SEM_KV + i - 1).start()
        return c

    def layer_pair(l, c):
        pl.when(l == 0)(stage1)
        if 2 in only:
            lax.fori_loop(0, 8, s2, 0)

        @pl.when(l == 0)
        def _():
            if 3 in only:
                lax.fori_loop(0, 8, s3, 0)

        @pl.when(l == 1)
        def _():
            if 5 in only:
                lax.fori_loop(0, 8, s5, 0)
            flush_out(8, 7)
            x_out(7, 8 - ND, 8, SEM_KV + 7).start()
        return c

    lax.fori_loop(0, 2, layer_pair, 0)

    for k in range(8):
        x_out(8 + k).wait()
        x_out(k, 0, 8 - ND).wait()
        x_out(k, 8 - ND, 8, SEM_KV + k).wait()


def _compiler_params():
    vmem = 120 * 1024 * 1024
    try:
        return pltpu.CompilerParams(vmem_limit_bytes=vmem, disable_semaphore_checks=True)
    except TypeError:
        return pltpu.CompilerParams(vmem_limit_bytes=vmem)


@jax.jit
def pallas_interleave_layers__linear_kernel_hedgehog__sliding_local_dilated__prompt_kernel(
    A_x: jax.Array,
    A_wqkv: jax.Array,
    A_w_phi: jax.Array,
    A_wo: jax.Array,
    B_x: jax.Array,
    B_wqkv: jax.Array,
    B_wo: jax.Array,
):
    del B_x
    x3 = A_x.reshape(S // 32, 32, D)
    wphi2 = A_w_phi.reshape(H * DH, DH)
    any_spec = pl.BlockSpec(memory_space=pl.ANY)
    scratch = [
        pltpu.VMEM((NBLK + 1, S // 32, D), U32),
        pltpu.VMEM((24, D // 2, L), U32),
        pltpu.VMEM((8, D // 2, L), U32),
        pltpu.VMEM((24, D // 2, L), U32),
        pltpu.VMEM((8, D // 2, L), U32),
        pltpu.VMEM((H * DH, DH), BF16),
        pltpu.VMEM((8, 64, 128), U32),
        pltpu.VMEM((8, D // 2, L), U32),
        pltpu.VMEM((8, D, L), U32),
        pltpu.VMEM((8, D // 2, L), U32),
        pltpu.VMEM((8, D // 2 + 8, L), U32),
        pltpu.VMEM((8, D, L), U32),
        pltpu.VMEM((8, D // 2, L), U32),
        pltpu.VMEM((WIN + NBLK, D, L), F32),
        pltpu.VMEM((WIN + NBLK, D, L), F32),
        pltpu.VMEM((2, 16, 64, 128), F32),
        pltpu.VMEM((16, 32, 128), U32),
        pltpu.VMEM((2, 2 * D, L), F32),
        pltpu.VMEM((2 * D + 64, L), F32),
        pltpu.VMEM((9, ND * 64, L), U32),
        pltpu.SemaphoreType.DMA((NSEM,)),
    ]
    scratch += [pltpu.VMEM((9, D, L), F32)] * 2
    scratch += [pltpu.VMEM((9, D // 2, L), U32)] * 2
    scratch += [pltpu.VMEM((D // 2, L), U32)] * 2
    scratch += [pltpu.VMEM((MC, L), U32)] * (2 * NCH)
    scratch += [pltpu.VMEM((MC // 2, L), U32)] * (2 * NCH)
    out = pl.pallas_call(
        _kernel,
        out_shape=jax.ShapeDtypeStruct((S // 32, 32, D), BF16),
        in_specs=[any_spec] * 6,
        out_specs=any_spec,
        scratch_shapes=scratch,
        compiler_params=_compiler_params(),
        name="hedgehog_dilated",
    )(x3, A_wqkv, wphi2, A_wo, B_wqkv, B_wo)
    return out.reshape(1, S, D)
```

```python
import math

import jax
import jax.numpy as jnp
from jax import lax
import jax.experimental.pallas as pl
import jax.experimental.pallas.tpu as pltpu

S = 2048
D = 1024
H = 32
DH = 32
NBLK = 16
L = 128
WIN = 8
LOG2E = math.log2(math.e)
F32 = jnp.float32
BF16 = jnp.bfloat16
U32 = jnp.uint32
NT = (((1,), (1,)), ((), ()))

MC = 256
NCH = D // MC
GPC = MC // 128
PPC = MC // 64
ND = 2

CFG = dict(only=None, lag_q=2, lag_kv=4, hold=7, ln_link=4, side=3, bar3=14,
           sub_q=128, sub_k=64, sub_v=256, sub_qb=128, sub_o=256, sub_b=256, ln_link_3=2)


class _Stage:
    cur = 0


def _cfg(key):
    return CFG.get("%s_%d" % (key, _Stage.cur), CFG[key])


SEM_X = 0
SEM_PHI = 16
SEM_KV = 18
SEM_SET = 26
SEM_LATE = 34
NSEM = 35


def _mm(a, b):
    return jnp.dot(a, b, preferred_element_type=F32)


def _mm_nt(a, b):
    return lax.dot_general(a, b, NT, preferred_element_type=F32)


def _tree(op, xs):
    xs = list(xs)
    while len(xs) > 1:
        nxt = [op(xs[i], xs[i + 1]) for i in range(0, len(xs) - 1, 2)]
        if len(xs) % 2:
            nxt.append(xs[-1])
        xs = nxt
    return xs[0]


def _running_sum(acc, xs):
    for x in xs:
        acc = x if acc is None else acc + x
    return acc


def _rows(a, n=8):
    return [a[i * n:(i + 1) * n, :] for i in range(a.shape[0] // n)]


def _unpk(a):
    return pltpu.bitcast(a, BF16)


def _fold2(op, xs):
    r = _tree(op, xs)
    r = op(r, pltpu.roll(r, 4, 0))
    return op(r, pltpu.roll(r, 2, 0))


def _phi_parts(p):
    ps = _rows(p)
    mx = _fold2(jnp.maximum, ps)
    mn = _fold2(jnp.minimum, ps)
    ep = [jnp.exp2(x - mx) for x in ps]
    en = [jnp.exp2(mn - x) for x in ps]
    return ep, en, _fold2(jnp.add, ep), _fold2(jnp.add, en)


def _recip(x):
    r = pl.reciprocal(x, approx=True)
    return r * (2.0 - x * r)


def _mult(x, m):
    return x if isinstance(x, int) else pl.multiple_of(x, m)


def _kernel(x_hbm, wa_hbm, wphi_hbm, woa_hbm, wb_hbm, wob_hbm, out_hbm,
            xio, wa_raw, woa_raw, wb_raw, wob_raw, wphi, pmat,
            wqaT, wkaT, wvaT, woaT, wqbT, wkvbT, wobT, kb, vb, kv_acc, kvm, zacc, zb, ystage, sems, *rest):
    xT, xn, os_ = rest[0:2], rest[2:4], rest[4:6]
    phis = [rest[6:6 + NCH], rest[6 + NCH:6 + 2 * NCH]]
    vs = [rest[6 + 2 * NCH:6 + 3 * NCH], rest[6 + 3 * NCH:6 + 4 * NCH]]

    def u32(ref):
        return ref.bitcast(U32)

    only = CFG["only"] or (0, 1, 2, 3, 5)

    class Blk:
        def __init__(self, hf, k):
            self.hf, self.k = hf, k
            self.j = 8 * (1 - hf) + k
            self.zr = 0 if isinstance(k, int) else k >> 6

    x32, out32 = u32(x_hbm), u32(out_hbm)

    def x_in(j):
        return pltpu.make_async_copy(x32.at[:, j, :], xio.at[j], sems.at[SEM_X + j])

    def x_out(j, c0=0, c1=8, sem=None):
        cs = pl.ds(c0 * L, (c1 - c0) * L)
        return pltpu.make_async_copy(xio.at[j, :, cs], out32.at[:, j, cs],
                                     sems.at[SEM_X + j if sem is None else sem])

    def slabs(src, dst, g0, n, sem):
        return [pltpu.make_async_copy(src.at[:, pl.ds(_mult((g0 + u) * 128, 128), 128)], dst.at[g0 + u],
                                      sems.at[sem]) for u in range(n)]

    cp_phi = pltpu.make_async_copy(wphi_hbm.at[0:MC], wphi.at[0:MC], sems.at[SEM_PHI])
    cp_phi2 = pltpu.make_async_copy(wphi_hbm.at[MC:D], wphi.at[MC:D], sems.at[SEM_PHI + 1])
    cp_k = [slabs(wa_hbm, wa_raw, 8 + ch * GPC, GPC, SEM_KV + 2 * ch) for ch in range(NCH)]
    cp_v = [slabs(wa_hbm, wa_raw, 16 + ch * GPC, GPC, SEM_KV + 2 * ch + 1) for ch in range(NCH)]

    def w_set(g):
        return (slabs(wa_hbm, wa_raw, g, 1, SEM_SET + g) + slabs(woa_hbm, woa_raw, g, 1, SEM_SET + g)
                + slabs(wb_hbm, wb_raw, 8 + g, 1, SEM_SET + g) + slabs(wb_hbm, wb_raw, 16 + g, 1, SEM_SET + g))

    cp_late = slabs(wb_hbm, wb_raw, 0, 8, SEM_LATE) + slabs(wob_hbm, wob_raw, 0, 8, SEM_LATE)

    batch = [[cp_phi, x_in(8)] + cp_k[0] + [x_in(0)] + cp_v[0] + [cp_phi2] + cp_k[1] + cp_v[1],
             cp_k[2] + cp_v[2] + cp_k[3] + cp_v[3] + [x_in(9), x_in(1)], []]
    for g in range(8):
        if g < 6:
            batch[1] += [x_in(10 + g), x_in(2 + g)] + w_set(g)
        else:
            batch[2] += w_set(g)
    batch[2] += cp_late

    def start_all(cps):
        for c in cps:
            c.start()

    def wait_all(cps):
        for c in cps:
            c.wait()

    start_all(batch[0])

    class Side:
        never = None
        hist = []

    def side_begin(never):
        Side.never = never
        Side.hist = []

    def tr(x):
        w = _cfg("side")
        if Side.never is not None and len(Side.hist) >= w:
            x = jnp.concatenate([jnp.where(Side.never, Side.hist[-w], x[0:8, :]), x[8:, :]], axis=0)
        y = pltpu.bitcast(_unpk(x).T, U32)
        Side.hist.append(y[56:64, :])
        return y

    def wtile(raw, slab, c):
        return tr(u32(raw)[slab, c * 64:(c + 1) * 64, :])

    def wstore(ref, g, raw, slab):
        for c in range(8):
            ref[c, pl.ds(_mult(g * 64, 64), 64), :] = wtile(raw, slab, c)

    def wstore_perm(ref, g, raw, slab):
        for c in range(8):
            pk = wtile(raw, slab, c)
            for h4 in range(4):
                ref[c, pl.ds(g * 64 + h4, 16, stride=4), :] = pk[h4 * 16:(h4 + 1) * 16, :]

    def make_pmat(gs):
        r128 = lax.broadcasted_iota(jnp.int32, (128, 128), 0)
        c128 = lax.broadcasted_iota(jnp.int32, (128, 128), 1)
        same_head = (2 * (r128 >> 6) + (r128 & 1)) == (c128 >> 5)
        er = lax.broadcasted_iota(jnp.int32, (128, 32), 0)
        ec = lax.broadcasted_iota(jnp.int32, (128, 32), 1)
        expand = jnp.where(((er & 63) >> 1) == ec, 1.0, 0.0).astype(BF16)
        for g in gs:
            pg = _mm_nt(expand, wphi[g * 128:(g + 1) * 128, :])
            pmat[g] = jnp.where(same_head, pg, 0.0).astype(BF16)

    def fold(dst, g, slab):
        val = _mm_nt(_unpk(u32(pmat)[g]), _unpk(u32(wa_raw)[slab])) * LOG2E
        for c in range(8):
            dst[c, g * 128:(g + 1) * 128, :] = val[:, c * L:(c + 1) * L].astype(BF16)

    def prep_set(g):
        wstore(woaT, g, woa_raw, g)
        wstore_perm(wkvbT, g, wb_raw, 8 + g)
        wstore(wkvbT, 8 + g, wb_raw, 16 + g)

    def prep_late(g):
        wstore_perm(wqbT, g, wb_raw, g)
        wstore(wobT, g, wob_raw, g)

    class LN:
        def __init__(self, b):
            self.b = b
            self.piv = self.s1 = self.s2 = None

        def add(self, xt):
            if self.piv is None:
                self.piv = jnp.broadcast_to(xt[0:1, :], (8, L))
            d = [r - self.piv for r in _rows(xt)]
            self.s1 = _running_sum(self.s1, d)
            self.s2 = _running_sum(self.s2, [x * x for x in d])

        def finish(self):
            b = self.b
            m1 = jnp.sum(self.s1, axis=0, keepdims=True) * (1.0 / D)
            m2 = jnp.sum(self.s2, axis=0, keepdims=True) * (1.0 / D)
            var = jnp.maximum(m2 - m1 * m1, 0.0)
            rs = lax.rsqrt(var + 1e-5)
            mrs = jnp.broadcast_to((self.piv[0:1, :] + m1) * rs, (8, L))
            rs = jnp.broadcast_to(rs, (8, L))
            never = rs < 0.0
            for r in range(D // 16):
                y = [xT[b.hf][b.k, r * 16 + 8 * u:r * 16 + 8 * u + 8, :] * rs - mrs for u in range(2)]
                xn[b.hf][b.k, r * 16:(r + 1) * 16, :] = jnp.concatenate(y, axis=0).astype(BF16)
                if r % _cfg("ln_link") == _cfg("ln_link") - 1:
                    rs = jnp.where(never, y[0] + y[1], rs)

    def prep_x(src, b):
        ln = LN(b)
        for cc in range(8):
            xt = _unpk(tr(xio[src, :, cc * L:(cc + 1) * L])).astype(F32)
            xT[b.hf][b.k, cc * 128:(cc + 1) * 128, :] = xt
            ln.add(xt)
        ln.finish()

    def mmw(ref, r0, n, rhs, sub):
        def wload(r):
            return jnp.concatenate([_unpk(ref[c, r // 2:(r + sub) // 2, :]) for c in range(8)], axis=1)
        return jnp.concatenate([_mm(wload(r), rhs()) for r in range(r0, r0 + n, sub)], axis=0)

    def proj(ref, r0, n, b, sub):
        return mmw(ref, r0, n, lambda: _unpk(u32(xn[b.hf])[b.k]), sub)

    def out_mm(wo, ch, b):
        m0 = ch * MC
        return xT[b.hf][b.k, m0:m0 + MC, :] + mmw(wo, m0, MC, lambda: _unpk(u32(os_[b.hf])[...]), _cfg("sub_o"))

    def emit(steps, lag):
        pend = []
        for n, (main, late) in enumerate(steps):
            main()
            if late is not None:
                pend.append((n + lag if n < len(steps) - _cfg("hold") else len(steps) + n, late))
            for due, f in pend:
                if due <= n:
                    f()
            pend = [e for e in pend if e[0] > n]
        for _, f in sorted(pend, key=lambda e: e[0]):
            f()

    def split(i):
        @pl.when((i >> 6) > 0)
        def _():
            zb[2 * D:2 * D + 8, :] = jnp.zeros((8, L), F32)

    def z_finish(t, z):
        zb[t * 128:(t + 1) * 128, :] = jnp.broadcast_to(jnp.sum(z, axis=1, keepdims=True), (128, L))

    def kv_finish(t, acc):
        r = lax.broadcasted_iota(jnp.int32, (64, 128), 0)
        c = lax.broadcasted_iota(jnp.int32, (64, 128), 1)
        kvm[t] = jnp.where((r >> 5) == (c & 1), acc, 0.0).astype(BF16)

    def a_kv(b, lay, last):
        steps = []
        la = lay + b.zr if b.hf == 1 else lay
        for ch in range(NCH):
            def kstep(ch=ch):
                kp = proj(u32(wkaT), ch * MC, MC, b, _cfg("sub_k"))
                for u in range(PPC):
                    t = ch * PPC + u
                    ep, en, sp, sn = _phi_parts(kp[u * 64:(u + 1) * 64, :])
                    r = _recip(sp * sn)
                    rp = r * sn
                    rn = r * sp
                    phi = jnp.concatenate([e * rp for e in ep] + [e * rn for e in en], axis=0)
                    phis[b.hf][ch][u * 128:(u + 1) * 128, :] = phi.astype(BF16)
                    z = zacc[la, t * 128:(t + 1) * 128, :] + phi
                    zacc[la, t * 128:(t + 1) * 128, :] = z
                    if last:
                        z_finish(t, z)

            def vstep(ch=ch):
                vs[b.hf][ch][...] = proj(wvaT, ch * MC, MC, b, _cfg("sub_v")).astype(BF16)

            def mstep(ch=ch):
                for u in range(PPC):
                    t = ch * PPC + u
                    acc = kv_acc[la, t] + _mm_nt(_unpk(u32(vs[b.hf][ch])[u * 32:(u + 1) * 32, :]),
                                                 _unpk(u32(phis[b.hf][ch])[u * 64:(u + 1) * 64, :]))
                    kv_acc[la, t] = acc
                    if last:
                        kv_finish(t, acc)

            steps += [(kstep, None), (vstep, mstep)]
        return steps

    def a_q(b):
        steps = []
        for ch in range(NCH):
            def qstep(ch=ch):
                qp = proj(u32(wqaT), ch * MC, MC, b, _cfg("sub_q"))
                for u in range(PPC):
                    t = ch * PPC + u
                    ep, en, sp, sn = _phi_parts(qp[u * 64:(u + 1) * 64, :])
                    zr = _rows(zb[t * 128:(t + 1) * 128, :])
                    dp = _fold2(jnp.add, [e * zz for e, zz in zip(ep, zr[:8])])
                    dn = _fold2(jnp.add, [e * zz for e, zz in zip(en, zr[8:])])
                    r = _recip(dp * sn + dn * sp + 1e-6 * (sp * sn))
                    rp = r * sn
                    rn = r * sp
                    phi = jnp.concatenate([e * rp for e in ep] + [e * rn for e in en], axis=0)
                    phis[b.hf][ch][u * 128:(u + 1) * 128, :] = phi.astype(BF16)

            def nstep(ch=ch):
                for u in range(PPC):
                    t = ch * PPC + u
                    o = _mm(_unpk(u32(kvm)[t]), _unpk(u32(phis[b.hf][ch])[u * 64:(u + 1) * 64, :]))
                    os_[b.hf][t * 64:(t + 1) * 64, :] = o.astype(BF16)

            steps.append((qstep, nstep))
        return steps

    def out_proj(wo, b, defer=None):
        steps = []
        ln = LN(b)
        for ch in range(NCH):
            def ostep(ch=ch):
                xt = out_mm(wo, ch, b)
                xT[b.hf][b.k, ch * MC:(ch + 1) * MC, :] = xt
                ln.add(xt)
                if ch == NCH - 1 and defer is None:
                    ln.finish()
            steps.append((ostep, None))
        if defer is not None:
            defer.append((ln.finish, None))
        return steps

    def b_kv(b):
        steps = []
        for base, ref in ((0, kb), (D, vb)):
            for m0 in range(0, D, MC):
                def step(base=base, ref=ref, m0=m0):
                    p = proj(wkvbT, base + m0, MC, b, _cfg("sub_b"))
                    ref[WIN + b.j, m0:m0 + MC, :] = p
                    if b.hf == 0:
                        ref[b.k, m0:m0 + MC, :] = pltpu.roll(p, 2, 1)
                steps.append((step, None))
        return steps

    def b_q(b):
        j = b.j
        even = (lax.broadcasted_iota(jnp.int32, (8, L), 0) & 1) == 0
        first = lax.broadcasted_iota(jnp.int32, (8, L), 1) < 2
        cs = DH ** -0.5

        def logits(q, g):
            acc = [None] * WIN
            for r in range(16):
                qv = q[r * 8:r * 8 + 8, :]
                for w in range(WIN):
                    t = qv * kb[WIN + j - w, g * 128 + r * 8:g * 128 + r * 8 + 8, :]
                    acc[w] = t if acc[w] is None else acc[w] + t
            return acc

        steps = []
        for G in range(4):
            def step(G=G):
                q = proj(wqbT, G * 256, 256, b, _cfg("sub_qb"))
                la, lb = logits(q[0:128, :], 2 * G), logits(q[128:256, :], 2 * G + 1)
                lg = [jnp.where(even, x + pltpu.roll(x, 7, 0), y + pltpu.roll(y, 1, 0)) for x, y in zip(la, lb)]
                if b.hf == 1:
                    lg = [l if w == 0 else jnp.where(jnp.logical_and(first, j < w), -1e9 / cs, l)
                          for w, l in enumerate(lg)]
                mx = _tree(jnp.maximum, lg)
                ex = [jnp.exp2((l - mx) * (cs * LOG2E)) for l in lg]
                rs = _recip(_tree(jnp.add, ex))
                at = [e * rs for e in ex]
                for hh in range(8):
                    h = G * 8 + hh
                    s = 2 * (hh % 4) + hh // 4
                    o = _running_sum(None, [
                        jnp.broadcast_to(at[w][s:s + 1, :], (DH, L)) * vb[WIN + j - w, h * DH:(h + 1) * DH, :]
                        for w in range(WIN)])
                    os_[b.hf][h * DH:(h + 1) * DH, :] = o.astype(BF16)
            steps.append((step, None))
        return steps

    def final_proj(b, defer):
        steps = []
        for ch in range(NCH):
            def ostep(ch=ch):
                xt = out_mm(wobT, ch, b)
                for u in range(GPC):
                    cc = ch * GPC + u
                    y = xt[u * 128:(u + 1) * 128, :].astype(BF16)
                    if cc >= 8 - defer:
                        ystage[b.k + 1, (cc - 8 + ND) * 128:(cc - 7 + ND) * 128, :] = y
                    else:
                        xio[b.j, :, cc * L:(cc + 1) * L] = pltpu.bitcast(y.T, U32)
            steps.append((ostep, None))
        return steps

    def flush_out(k, slot):
        for u in range(ND):
            xio[slot, :, (8 - ND + u) * L:(9 - ND + u) * L] = tr(u32(ystage)[k, u * 64:(u + 1) * 64, :])

    def stage1():
        _Stage.cur = 0
        kv_acc[...] = jnp.zeros(kv_acc.shape, F32)
        zacc[...] = jnp.zeros(zacc.shape, F32)
        ystage[0] = jnp.zeros(ystage.shape[1:], BF16)
        cp_phi.wait()
        x_in(8).wait()
        make_pmat(range(GPC))
        prep_x(8, Blk(0, 0))
        start_all(batch[1])

        sa = a_kv(Blk(0, 0), 0, False)
        sb = a_kv(Blk(1, 0), 0, False)
        pend = []
        for ch in range(NCH if 0 in only else 0):
            if ch == 1:
                start_all(batch[2])
            wait_all(cp_k[ch])
            if ch == 0:
                for u in range(GPC):
                    fold(wkaT, u, 8 + u)
                sa[0][0]()
                x_in(0).wait()
            wait_all(cp_v[ch])
            if ch == 0:
                cp_phi2.wait()
                prep_x(0, Blk(1, 0))
                make_pmat(range(GPC, 8))
            else:
                if ch == NCH - 1:
                    x_in(9).wait()
                    x_in(1).wait()
                for u in range(GPC):
                    fold(wkaT, ch * GPC + u, 8 + ch * GPC + u)
            for u in range(GPC):
                wstore(wvaT, ch * GPC + u, wa_raw, 16 + ch * GPC + u)
            for f in pend:
                f()
            if ch == NCH - 1:
                side_begin(zacc[0, 0:8, :] < 0.0)
                prep_x(9, Blk(0, 1))
                prep_x(1, Blk(1, 1))
                side_begin(None)
            if ch == 0:
                sa[1][0]()
                sb[0][0]()
            else:
                sa[2 * ch][0]()
                sb[2 * ch][0]()
                sa[2 * ch + 1][0]()
            sb[2 * ch + 1][0]()
            pend = [sa[2 * ch + 1][1], sb[2 * ch + 1][1]]
        for f in pend:
            f()

        def s1(i, c):
            _Stage.cur = 1

            @pl.when(i < 7)
            def _():
                x_in(9 + i).wait()
                x_in(1 + i).wait()

            wait_all(w_set(i - 1))
            side_begin(jnp.full((8, L), i >> 6, jnp.int32) > 0)
            nxt = jnp.minimum(i + 1, 7)
            prep_x(8 + nxt, Blk(0, i + 1))
            prep_x(nxt, Blk(1, i + 1))
            prep_set(i - 1)
            side_begin(None)
            steps = a_kv(Blk(0, i), 0, False) + a_kv(Blk(1, i), 0, False)
            emit(steps, _cfg("lag_kv"))
            return c

        if 1 in only:
            lax.fori_loop(1, 8, s1, 0)
        _Stage.cur = 0
        wait_all(w_set(7))
        for g in range(8):
            fold(wqaT, g, g)
        prep_set(7)
        for t in range(16):
            z_finish(t, zacc[0, t * 128:(t + 1) * 128, :])
            kv_finish(t, kv_acc[0, t])
        wait_all(cp_late)

    def s2(i, c):
        _Stage.cur = 2
        b0, b1 = Blk(0, i), Blk(1, i)
        steps = a_q(b0) + a_q(b1) + out_proj(woaT, b0) + out_proj(woaT, b1)
        steps += [(lambda: prep_late(i), None)] + b_kv(b0) + b_kv(b1)
        emit(steps, _cfg("lag_q"))
        return c

    def s3(i, c):
        _Stage.cur = 3
        b0, b1 = Blk(0, i), Blk(1, i)
        late_ln = []
        steps = b_q(b0) + b_q(b1) + out_proj(wobT, b0, late_ln) + out_proj(wobT, b1)
        steps += a_kv(b0, 1, False) + a_kv(b1, 1, True)
        steps[CFG["bar3"]:CFG["bar3"]] = [(lambda: split(i), None)] + late_ln
        emit(steps, _cfg("lag_kv"))
        return c

    def s5(i, c):
        _Stage.cur = 5
        b0, b1 = Blk(0, i), Blk(1, i)
        flush = (lambda: flush_out(i, jnp.where(i > 0, i - 1, NBLK)), None)
        emit(b_q(b0) + b_q(b1) + [flush] + final_proj(b0, 0) + final_proj(b1, ND), 0)
        x_out(b0.j).start()
        x_out(b1.j, 0, 8 - ND).start()

        @pl.when(i > 0)
        def _():
            x_out(i - 1, 8 - ND, 8, SEM_KV + i - 1).start()
        return c

    def layer_pair(l, c):
        pl.when(l == 0)(stage1)
        if 2 in only:
            lax.fori_loop(0, 8, s2, 0)

        @pl.when(l == 0)
        def _():
            if 3 in only:
                lax.fori_loop(0, 8, s3, 0)

        @pl.when(l == 1)
        def _():
            if 5 in only:
                lax.fori_loop(0, 8, s5, 0)
            flush_out(8, 7)
            x_out(7, 8 - ND, 8, SEM_KV + 7).start()
        return c

    lax.fori_loop(0, 2, layer_pair, 0)

    for k in range(8):
        x_out(8 + k).wait()
        x_out(k, 0, 8 - ND).wait()
        x_out(k, 8 - ND, 8, SEM_KV + k).wait()


def _compiler_params():
    vmem = 120 * 1024 * 1024
    try:
        return pltpu.CompilerParams(vmem_limit_bytes=vmem, disable_semaphore_checks=True)
    except TypeError:
        return pltpu.CompilerParams(vmem_limit_bytes=vmem)


@jax.jit
def pallas_interleave_layers__linear_kernel_hedgehog__sliding_local_dilated__prompt_kernel(
    A_x: jax.Array,
    A_wqkv: jax.Array,
    A_w_phi: jax.Array,
    A_wo: jax.Array,
    B_x: jax.Array,
    B_wqkv: jax.Array,
    B_wo: jax.Array,
):
    del B_x
    x3 = A_x.reshape(S // 32, 32, D)
    wphi2 = A_w_phi.reshape(H * DH, DH)
    any_spec = pl.BlockSpec(memory_space=pl.ANY)
    scratch = [
        pltpu.VMEM((NBLK + 1, S // 32, D), U32),
        pltpu.VMEM((24, D, L), BF16),
        pltpu.VMEM((8, D, L), BF16),
        pltpu.VMEM((24, D, L), BF16),
        pltpu.VMEM((8, D, L), BF16),
        pltpu.VMEM((H * DH, DH), BF16),
        pltpu.VMEM((8, 128, 128), BF16),
        pltpu.VMEM((8, D, L), BF16),
        pltpu.VMEM((8, D, L), BF16),
        pltpu.VMEM((8, D // 2, L), U32),
        pltpu.VMEM((8, D // 2, L), U32),
        pltpu.VMEM((8, D // 2 + 8, L), U32),
        pltpu.VMEM((8, D, L), U32),
        pltpu.VMEM((8, D // 2, L), U32),
        pltpu.VMEM((WIN + NBLK, D, L), F32),
        pltpu.VMEM((WIN + NBLK, D, L), F32),
        pltpu.VMEM((2, 16, 64, 128), F32),
        pltpu.VMEM((16, 64, 128), BF16),
        pltpu.VMEM((2, 2 * D, L), F32),
        pltpu.VMEM((2 * D + 64, L), F32),
        pltpu.VMEM((9, ND * 128, L), BF16),
        pltpu.SemaphoreType.DMA((NSEM,)),
    ]
    scratch += [pltpu.VMEM((9, D, L), F32)] * 2
    scratch += [pltpu.VMEM((9, D, L), BF16)] * 2
    scratch += [pltpu.VMEM((D, L), BF16)] * 2
    scratch += [pltpu.VMEM((2 * MC, L), BF16)] * (2 * NCH)
    scratch += [pltpu.VMEM((MC, L), BF16)] * (2 * NCH)
    out = pl.pallas_call(
        _kernel,
        out_shape=jax.ShapeDtypeStruct((S // 32, 32, D), BF16),
        in_specs=[any_spec] * 6,
        out_specs=any_spec,
        scratch_shapes=scratch,
        compiler_params=_compiler_params(),
        name="hedgehog_dilated",
    )(x3, A_wqkv, wphi2, A_wo, B_wqkv, B_wo)
    return out.reshape(1, S, D)
```

```python
import math

import jax
import jax.numpy as jnp
from jax import lax
import jax.experimental.pallas as pl
import jax.experimental.pallas.tpu as pltpu

S = 2048
D = 1024
H = 32
DH = 32
NBLK = 16
L = 128
WIN = 8
LOG2E = math.log2(math.e)
F32 = jnp.float32
BF16 = jnp.bfloat16
U32 = jnp.uint32
NT = (((1,), (1,)), ((), ()))

MC = 256
NCH = D // MC
GPC = MC // 128
PPC = MC // 64
ND = 2

CFG = dict(only=None, lag_n=5, lag_m=5, hold=2, ln_link=2, side=3, split_at=10, hk=2, tk=2,
           sub_q=64, sub_k=64, sub_v=128, sub_qb=128, sub_o=128, sub_b=128)


class _Stage:
    cur = 0


def _cfg(key):
    return CFG.get("%s_%d" % (key, _Stage.cur), CFG[key])


SEM_X = 0
SEM_PHI = 16
SEM_KV = 18
SEM_SET = 26
SEM_LATE = 34
NSEM = 35


def _mm(a, b):
    return jnp.dot(a, b, preferred_element_type=F32)


def _mm_nt(a, b):
    return lax.dot_general(a, b, NT, preferred_element_type=F32)


def _tree(op, xs):
    xs = list(xs)
    while len(xs) > 1:
        nxt = [op(xs[i], xs[i + 1]) for i in range(0, len(xs) - 1, 2)]
        if len(xs) % 2:
            nxt.append(xs[-1])
        xs = nxt
    return xs[0]


def _running_sum(acc, xs):
    for x in xs:
        acc = x if acc is None else acc + x
    return acc


def _rows(a, n=8):
    return [a[i * n:(i + 1) * n, :] for i in range(a.shape[0] // n)]


def _unpk(a):
    return pltpu.bitcast(a, BF16)


def _fold2(op, xs):
    r = _tree(op, xs)
    r = op(r, pltpu.roll(r, 4, 0))
    return op(r, pltpu.roll(r, 2, 0))


def _phi_parts(p):
    ps = _rows(p)
    mx = _fold2(jnp.maximum, ps)
    mn = _fold2(jnp.minimum, ps)
    ep = [jnp.exp2(x - mx) for x in ps]
    en = [jnp.exp2(mn - x) for x in ps]
    return ep, en, _fold2(jnp.add, ep), _fold2(jnp.add, en)


def _recip(x):
    r = pl.reciprocal(x, approx=True)
    return r * (2.0 - x * r)


def _lhs_ops(a11, a12, a21, a22):
    return [a11 + a22, a21 + a22, a11, a22, a11 + a12, a21 - a11, a12 - a22]


def _mult(x, m):
    return x if isinstance(x, int) else pl.multiple_of(x, m)


def _kernel(x_hbm, wa_hbm, wphi_hbm, woa_hbm, wb_hbm, wob_hbm, out_hbm,
            xio, wa_raw, woa_raw, wb_raw, wob_raw, wphi, pmat,
            wqaT, wkaT, wvaT, woaT, wqbT, wkbT, wvbT, wobT, xr, orr, kb, vb, kv_acc, kvm, zacc, zb, ystage,
            sems, *rest):
    xT = rest[0:2]
    phis = [rest[2:2 + NCH], rest[2 + NCH:2 + 2 * NCH]]
    vs = [rest[2 + 2 * NCH:2 + 3 * NCH], rest[2 + 3 * NCH:2 + 4 * NCH]]

    def u32(ref):
        return ref.bitcast(U32)

    only = CFG["only"] or (0, 1, 2, 3, 5)

    x32, out32 = u32(x_hbm), u32(out_hbm)

    def x_in(j):
        return pltpu.make_async_copy(x32.at[:, j, :], xio.at[j], sems.at[SEM_X + j])

    def x_out(j, c0=0, c1=8, sem=None):
        cs = pl.ds(c0 * L, (c1 - c0) * L)
        return pltpu.make_async_copy(xio.at[j, :, cs], out32.at[:, j, cs],
                                     sems.at[SEM_X + j if sem is None else sem])

    def slabs(src, dst, g0, n, sem):
        return [pltpu.make_async_copy(src.at[:, pl.ds(_mult((g0 + u) * 128, 128), 128)], dst.at[g0 + u],
                                      sems.at[sem]) for u in range(n)]

    cp_phi = pltpu.make_async_copy(wphi_hbm.at[0:MC], wphi.at[0:MC], sems.at[SEM_PHI])
    cp_phi2 = pltpu.make_async_copy(wphi_hbm.at[MC:D], wphi.at[MC:D], sems.at[SEM_PHI + 1])
    cp_k = [slabs(wa_hbm, wa_raw, 8 + ch * GPC, GPC, SEM_KV + 2 * ch) for ch in range(NCH)]
    cp_v = [slabs(wa_hbm, wa_raw, 16 + ch * GPC, GPC, SEM_KV + 2 * ch + 1) for ch in range(NCH)]

    def w_set(g):
        rows = pl.ds(_mult((g & 1) * 512, 512), 512)
        cps = []
        for src, dst, g0 in ((woa_hbm, woa_raw, 0), (wb_hbm, wb_raw, 8), (wb_hbm, wb_raw, 16)):
            for u in range(2):
                sl = g0 + 2 * (g >> 1) + u
                cps.append(pltpu.make_async_copy(src.at[rows, pl.ds(_mult(sl * 128, 128), 128)],
                                                 dst.at[sl, rows, :], sems.at[SEM_SET + g]))
        return cps

    cp_late = (slabs(wa_hbm, wa_raw, 0, 8, SEM_LATE) + slabs(wb_hbm, wb_raw, 0, 8, SEM_LATE)
               + slabs(wob_hbm, wob_raw, 0, 8, SEM_LATE))

    batch = [[cp_phi, x_in(8), x_in(0)] + cp_k[0] + cp_v[0] + [cp_phi2] + cp_k[1] + cp_v[1],
             cp_k[2] + cp_v[2] + cp_k[3] + cp_v[3] + [x_in(9), x_in(1)], [], cp_late]
    for g in range(8):
        n = 1 if g < 4 else 2
        if g < 6:
            batch[n] += [x_in(10 + g), x_in(2 + g)]
        batch[n] += w_set(g)

    def start_all(cps):
        for c in cps:
            c.start()

    def wait_all(cps):
        for c in cps:
            c.wait()

    start_all(batch[0])

    class Side:
        never = None
        hist = []

    def side_begin(never):
        Side.never = never
        Side.hist = []

    def gate(x):
        w = _cfg("side")
        if Side.never is not None and len(Side.hist) >= w:
            x = jnp.concatenate([jnp.where(Side.never, Side.hist[-w], x[0:8, :]), x[8:, :]], axis=0)
        return x

    def tr(x):
        y = pltpu.bitcast(x.T, U32)
        Side.hist.append(y[56:64, :])
        return y

    def wprep(ref, raw, g0, st, c, perm=False):
        def tile(u, kt):
            return _unpk(gate(u32(raw)[g0 + 2 * st + u, pl.ds(_mult(kt * 64, 64), 64), :]))
        t = [tile(0, 2 * c), tile(0, 2 * c + 1), tile(1, 2 * c), tile(1, 2 * c + 1)]
        ops = _lhs_ops(*[x.astype(F32) for x in t])
        for q in range(7):
            pk = tr(t[0] if q == 2 else t[3] if q == 3 else ops[q].astype(BF16))
            if perm:
                for h4 in range(4):
                    ref[q, c, pl.ds(st * 64 + h4, 16, stride=4), :] = pk[h4 * 16:(h4 + 1) * 16, :]
            else:
                ref[q, c, pl.ds(_mult(st * 64, 64), 64), :] = pk

    def make_pmat(gs):
        r128 = lax.broadcasted_iota(jnp.int32, (128, 128), 0)
        c128 = lax.broadcasted_iota(jnp.int32, (128, 128), 1)
        same_head = (2 * (r128 >> 6) + (r128 & 1)) == (c128 >> 5)
        er = lax.broadcasted_iota(jnp.int32, (128, 32), 0)
        ec = lax.broadcasted_iota(jnp.int32, (128, 32), 1)
        expand = jnp.where(((er & 63) >> 1) == ec, 1.0, 0.0).astype(BF16)
        for g in gs:
            pg = _mm_nt(expand, wphi[g * 128:(g + 1) * 128, :])
            pmat[g] = jnp.where(same_head, pg, 0.0).astype(BF16)

    def fold(dst, g0, st):
        for c in range(4):
            f = [_mm_nt(_unpk(u32(pmat)[2 * st + u]),
                        _unpk(u32(wa_raw)[g0 + 2 * st + u, kt * 64:(kt + 1) * 64, :])) * LOG2E
                 for u in range(2) for kt in (2 * c, 2 * c + 1)]
            for q, v in enumerate(_lhs_ops(*f)):
                dst[q, c, st * 128:(st + 1) * 128, :] = v.astype(BF16)

    def prep_set(g):
        for u in range(2):
            c = 2 * (g & 1) + u
            wprep(woaT, woa_raw, 0, g >> 1, c)
            wprep(wkbT, wb_raw, 8, g >> 1, c, True)
            wprep(wvbT, wb_raw, 16, g >> 1, c)

    def prep_late(g):
        for u in range(2):
            c = 2 * (g & 1) + u
            wprep(wqbT, wb_raw, 0, g >> 1, c, True)
            wprep(wobT, wob_raw, 0, g >> 1, c)

    def put_a(dst, r0, alo, ahi):
        n = alo.shape[0]
        dst[1, r0:r0 + n, :] = alo.astype(BF16)
        dst[3, r0:r0 + n, :] = (ahi - alo).astype(BF16)

    def put_b(dst, r0, alo, ahi, blo, bhi):
        n = alo.shape[0]
        dst[4, r0:r0 + n, :] = bhi.astype(BF16)
        dst[2, r0:r0 + n, :] = (blo - bhi).astype(BF16)
        dst[0, r0:r0 + n, :] = (alo + bhi).astype(BF16)
        dst[6, r0:r0 + n, :] = (ahi + bhi).astype(BF16)
        dst[5, r0:r0 + n, :] = (alo + blo).astype(BF16)

    class LN:
        def __init__(self, k):
            self.k = k
            self.piv, self.s1, self.s2, self.sc = [None] * 2, [None] * 2, [None] * 2, [None] * 2

        def add(self, hf, xt):
            if self.piv[hf] is None:
                self.piv[hf] = jnp.broadcast_to(xt[0:1, :], (8, L))
            d = [r - self.piv[hf] for r in _rows(xt)]
            self.s1[hf] = _running_sum(self.s1[hf], d)
            self.s2[hf] = _running_sum(self.s2[hf], [x * x for x in d])

        def stats(self, hf):
            m1 = jnp.sum(self.s1[hf], axis=0, keepdims=True) * (1.0 / D)
            m2 = jnp.sum(self.s2[hf], axis=0, keepdims=True) * (1.0 / D)
            rs = lax.rsqrt(jnp.maximum(m2 - m1 * m1, 0.0) + 1e-5)
            self.sc[hf] = (jnp.broadcast_to(rs, (16, L)), jnp.broadcast_to((self.piv[hf][0:1, :] + m1) * rs, (16, L)))

        def finish(self, do_a, do_b):
            for hf in range(2):
                if (do_a, do_b)[hf]:
                    self.stats(hf)
            dst = xr.at[self.k]
            rs = [None if sc is None else sc[0] for sc in self.sc]
            never = rs[1 if do_b else 0] < 0.0
            if do_b and not do_a:
                rs[0] = jnp.where(never, rs[1], rs[0])
            for r in range(D // 32):
                r0 = (r // 8) * 256 + (r % 8) * 16
                y = [[xT[hf][self.k, r0 + o:r0 + o + 16, :] * rs[hf] - self.sc[hf][1] for o in (0, 128)]
                     for hf in range(2 if do_b else 1)]
                if do_a:
                    put_a(dst, r * 16, *y[0])
                if do_b:
                    put_b(dst, r * 16, *y[0], *y[1])
                if r % _cfg("ln_link") == _cfg("ln_link") - 1:
                    lk = y[0][1] + y[-1][1]
                    rs = [None if x is None else jnp.where(never, lk, x) for x in rs]

    def prep_x(src, k):
        ln = LN(k)
        for hf in range(2):
            for cc in range(8):
                xt = _unpk(tr(_unpk(gate(xio[8 * (1 - hf) + src, :, cc * L:(cc + 1) * L])))).astype(F32)
                xT[hf][k, cc * 128:(cc + 1) * 128, :] = xt
                ln.add(hf, xt)
        ln.finish(True, True)

    class Emit:
        def __init__(self):
            self.n = 0
            self.pend = []

        def later(self, lag, f):
            self.pend.append((self.n + lag, f))

        def tick(self, w=1):
            self.n += w
            due = [e for e in self.pend if e[0] <= self.n]
            self.pend = [e for e in self.pend if e[0] > self.n]
            for _, f in due:
                f()

        def flush(self):
            self.tick(1 << 20)

    def phase(em, steps, rhs, hk, tk):
        units = [(n, u) for n, stp in enumerate(steps) for u in range(128 // stp[2])]
        order = [(n, u, q) for n, u in units if n < hk for q in (3, 1)]
        for n, u in units:
            qs = (3, 1, 4, 2, 0, 6, 5) if n < len(steps) - tk else (3, 1, 4, 0, 6)
            order += [(n, u, q) for q in qs if n >= hk or q not in (3, 1)]
        order += [(n, u, q) for n, u in units if n >= len(steps) - tk for q in (2, 5)]
        uses = {0: [((0, 0), 1), ((1, 1), 1)], 1: [((0, 1), 1), ((1, 1), -1)], 2: [((1, 0), 1), ((1, 1), 1)],
                3: [((0, 0), 1), ((0, 1), 1)], 4: [((0, 0), -1), ((1, 0), 1)], 5: [((1, 1), 1)], 6: [((0, 0), 1)]}
        need = {(0, 0): 4, (0, 1): 2, (1, 0): 2, (1, 1): 4}
        acc = {}
        for n, u, q in order:
            ref, st, sub, consumer = steps[n]
            r = (st * 128 + u * sub) // 2
            lhs = jnp.concatenate([_unpk(ref[q, c, r:r + sub // 2, :]) for c in range(4)], axis=1)
            m = _mm(lhs, _unpk(rhs(q)))
            for quad, sign in uses[q]:
                val, sg, cnt = acc.get((n, u, quad), (None, 1, 0))
                if val is None:
                    val, sg = m, sign
                elif sg == sign:
                    val = val + m
                else:
                    val, sg = (val - m, 1) if sg == 1 else (m - val, 1)
                acc[(n, u, quad)] = (val, sg, cnt + 1)
                if cnt + 1 == need[quad]:
                    consumer(quad[0], quad[1], u, val)
            em.tick(sub // 64)

    def x_rhs(k):
        return lambda q: u32(xr)[k, q]

    def o_rhs(q):
        return u32(orr)[q]

    def split(i):
        @pl.when((i >> 6) > 0)
        def _():
            zb[2 * D:2 * D + 8, :] = jnp.zeros((8, L), F32)

    def z_finish(t, z):
        zb[t * 128:(t + 1) * 128, :] = jnp.broadcast_to(jnp.sum(z, axis=1, keepdims=True), (128, L))

    def kv_finish(t, acc):
        r = lax.broadcasted_iota(jnp.int32, (64, 128), 0)
        c = lax.broadcasted_iota(jnp.int32, (64, 128), 1)
        kvm[t] = jnp.where((r >> 5) == (c & 1), acc, 0.0).astype(BF16)

    def pairs_of(bot, u, sub, val):
        return [(2 * bot + (u * sub) // 64 + w, val[w * 64:(w + 1) * 64, :]) for w in range(sub // 64)]

    def a_kv(em, lay, last):
        steps = []
        for ch in range(NCH):
            seen = {}

            def kcons(hf, bot, u, val, ch=ch, seen=seen):
                for pp, kp in pairs_of(bot, u, _cfg("sub_k"), val):
                    t = ch * PPC + pp
                    ep, en, sp, sn = _phi_parts(kp)
                    r = _recip(sp * sn)
                    rp = r * sn
                    rn = r * sp
                    phi = jnp.concatenate([e * rp for e in ep] + [e * rn for e in en], axis=0)
                    phis[hf][ch][pp * 128:(pp + 1) * 128, :] = phi.astype(BF16)
                    z = zacc[lay, t * 128:(t + 1) * 128, :] + phi
                    zacc[lay, t * 128:(t + 1) * 128, :] = z
                    seen[pp] = seen.get(pp, 0) + 1
                    if last and seen[pp] == 2:
                        z_finish(t, z)

            def mstep(ch=ch):
                for pp in range(PPC):
                    t = ch * PPC + pp
                    acc = kv_acc[lay, t]
                    for hf in range(2):
                        acc = acc + _mm_nt(_unpk(u32(vs[hf][ch])[pp * 32:(pp + 1) * 32, :]),
                                           _unpk(u32(phis[hf][ch])[pp * 64:(pp + 1) * 64, :]))
                    kv_acc[lay, t] = acc
                    if last:
                        kv_finish(t, acc)

            def vcons(hf, bot, u, val, ch=ch, seen=seen, mstep=mstep):
                sub = _cfg("sub_v")
                vs[hf][ch][bot * 128 + u * sub:bot * 128 + (u + 1) * sub, :] = val.astype(BF16)
                seen["v"] = seen.get("v", 0) + 1
                if seen["v"] == 4 * (128 // sub):
                    em.later(_cfg("lag_m") if ch < NCH - _cfg("hold") else 1 << 10, mstep)

            steps += [(u32(wkaT), ch, _cfg("sub_k"), kcons), (wvaT, ch, _cfg("sub_v"), vcons)]
        return steps

    def a_q(em, tk):
        steps = []
        for ch in range(NCH):
            seen = {0: 0, 1: 0}
            o = {}

            def num(hf, pp, ch=ch):
                return _mm(_unpk(u32(kvm)[ch * PPC + pp]), _unpk(u32(phis[hf][ch])[pp * 64:(pp + 1) * 64, :]))

            def nstep(hfs, ch=ch, o=o, num=num):
                for w in range(2):
                    for hf in hfs:
                        o[hf, w] = (num(hf, w), num(hf, 2 + w))
                    if 0 in hfs:
                        put_a(orr, ch * 128 + w * 64, *o[0, w])
                    if 1 in hfs:
                        put_b(orr, ch * 128 + w * 64, *o[0, w], *o[1, w])

            def qcons(hf, bot, u, val, ch=ch, seen=seen, nstep=nstep):
                for pp, qp in pairs_of(bot, u, _cfg("sub_q"), val):
                    t = ch * PPC + pp
                    ep, en, sp, sn = _phi_parts(qp)
                    zr = _rows(zb[t * 128:(t + 1) * 128, :])
                    dp = _fold2(jnp.add, [e * zz for e, zz in zip(ep, zr[:8])])
                    dn = _fold2(jnp.add, [e * zz for e, zz in zip(en, zr[8:])])
                    r = _recip(dp * sn + dn * sp + 1e-6 * (sp * sn))
                    rp = r * sn
                    rn = r * sp
                    phi = jnp.concatenate([e * rp for e in ep] + [e * rn for e in en], axis=0)
                    phis[hf][ch][pp * 128:(pp + 1) * 128, :] = phi.astype(BF16)
                    seen[hf] += 1
                    if seen[hf] == PPC:
                        if ch >= NCH - tk:
                            em.later(_cfg("lag_n"), lambda hf=hf: nstep((hf,)))
                        elif seen[1 - hf] == PPC:
                            em.later(_cfg("lag_n"), lambda: nstep((0, 1)))

            steps.append((u32(wqaT), ch, _cfg("sub_q"), qcons))
        return steps

    def out_proj(wo, k):
        ln = LN(k)
        seen = {0: 0, 1: 0}
        sub = _cfg("sub_o")
        steps = []
        for ch in range(NCH):
            def cons(hf, bot, u, val, ch=ch):
                r0 = ch * MC + bot * 128 + u * sub
                xt = xT[hf][k, r0:r0 + sub, :] + val
                xT[hf][k, r0:r0 + sub, :] = xt
                ln.add(hf, xt)
                seen[hf] += 1
                if seen[hf] == D // sub:
                    ln.finish(hf == 0, hf == 1)
            steps.append((wo, ch, sub, cons))
        return steps

    def b_kv(k):
        sub = _cfg("sub_b")
        steps = []
        for w, ref in ((wkbT, kb), (wvbT, vb)):
            for ch in range(NCH):
                def cons(hf, bot, u, val, ch=ch, ref=ref):
                    r0 = ch * MC + bot * 128 + u * sub
                    ref[WIN + 8 * (1 - hf) + k, r0:r0 + sub, :] = val
                    if hf == 0:
                        ref[k, r0:r0 + sub, :] = pltpu.roll(val, 2, 1)
                steps.append((w, ch, sub, cons))
        return steps

    def b_q(k):
        even = (lax.broadcasted_iota(jnp.int32, (8, L), 0) & 1) == 0
        first = lax.broadcasted_iota(jnp.int32, (8, L), 1) < 2
        cs = DH ** -0.5
        sub = _cfg("sub_qb")
        steps = []
        for G in range(4):
            lacc = {}
            seen = {0: 0, 1: 0}
            oa = {}

            def cons(hf, bot, u, q, G=G, lacc=lacc, seen=seen, oa=oa):
                j = 8 * (1 - hf) + k
                acc = lacc.setdefault((hf, bot), [None] * WIN)
                for r in range(sub // 8):
                    r0 = G * 256 + bot * 128 + u * sub + r * 8
                    for w in range(WIN):
                        t = q[r * 8:r * 8 + 8, :] * kb[WIN + j - w, r0:r0 + 8, :]
                        acc[w] = t if acc[w] is None else acc[w] + t
                seen[hf] += 1
                if seen[hf] < 256 // sub:
                    return
                lg = [jnp.where(even, x + pltpu.roll(x, 7, 0), y + pltpu.roll(y, 1, 0))
                      for x, y in zip(lacc[hf, 0], lacc[hf, 1])]
                if hf == 1:
                    lg = [l if w == 0 else jnp.where(jnp.logical_and(first, j < w), -1e9 / cs, l)
                          for w, l in enumerate(lg)]
                mx = _tree(jnp.maximum, lg)
                ex = [jnp.exp2((l - mx) * (cs * LOG2E)) for l in lg]
                rs = _recip(_tree(jnp.add, ex))
                at = [e * rs for e in ex]

                def pv(hh):
                    h = G * 8 + hh
                    s = 2 * (hh % 4) + hh // 4
                    return _running_sum(None, [
                        jnp.broadcast_to(at[w][s:s + 1, :], (DH, L)) * vb[WIN + j - w, h * DH:(h + 1) * DH, :]
                        for w in range(WIN)])

                for h4 in range(4):
                    o = (pv(h4), pv(4 + h4))
                    if hf == 0:
                        oa[h4] = o
                        put_a(orr, G * 128 + h4 * DH, *o)
                    else:
                        put_b(orr, G * 128 + h4 * DH, *oa[h4], *o)

            steps.append((wqbT, G, sub, cons))
        return steps

    def final_proj(k):
        steps = []
        for ch in range(NCH):
            def cons(hf, bot, u, val, ch=ch):
                cc = ch * GPC + bot
                y = (xT[hf][k, cc * 128:(cc + 1) * 128, :] + val).astype(BF16)
                if hf == 1 and cc >= 8 - ND:
                    ystage[k + 1, (cc - 8 + ND) * 128:(cc - 7 + ND) * 128, :] = y
                else:
                    xio[8 * (1 - hf) + k, :, cc * L:(cc + 1) * L] = tr(y)
            steps.append((wobT, ch, 128, cons))
        return steps

    def flush_out(k, slot):
        for u in range(ND):
            xio[slot, :, (8 - ND + u) * L:(9 - ND + u) * L] = tr(_unpk(u32(ystage)[k, u * 64:(u + 1) * 64, :]))

    def stage1():
        _Stage.cur = 0
        kv_acc[...] = jnp.zeros(kv_acc.shape, F32)
        zacc[...] = jnp.zeros(zacc.shape, F32)
        ystage[0] = jnp.zeros(ystage.shape[1:], BF16)
        cp_phi.wait()
        x_in(8).wait()
        x_in(0).wait()
        make_pmat(range(GPC))
        prep_x(0, 0)
        start_all(batch[1])

        em = Emit()
        steps = a_kv(em, 0, False)
        for ch in range(NCH if 0 in only else 0):
            if ch in (1, 2):
                start_all(batch[ch + 1])
            wait_all(cp_k[ch])
            if ch == 0:
                fold(wkaT, 8, 0)
                phase(em, steps[0:1], x_rhs(0), 0, 0)
            wait_all(cp_v[ch])
            if ch == 0:
                cp_phi2.wait()
                make_pmat(range(GPC, 8))
            else:
                if ch == NCH - 1:
                    x_in(9).wait()
                    x_in(1).wait()
                fold(wkaT, 8, ch)
            for c in range(4):
                wprep(wvaT, wa_raw, 16, ch, c)
            em.flush()
            if ch == NCH - 1:
                side_begin(zacc[0, 0:8, :] < 0.0)
                prep_x(1, 1)
                side_begin(None)
            phase(em, steps[max(2 * ch, 1):2 * ch + 2], x_rhs(0), 0, 0)
        em.flush()

        def s1(i, c):
            _Stage.cur = 1

            @pl.when(i < 7)
            def _():
                x_in(9 + i).wait()
                x_in(1 + i).wait()

            wait_all(w_set(i - 1))
            side_begin(jnp.full((8, L), i >> 6, jnp.int32) > 0)
            prep_x(jnp.minimum(i + 1, 7), i + 1)
            prep_set(i - 1)
            side_begin(None)
            em = Emit()
            phase(em, a_kv(em, 0, False), x_rhs(i), 0, 0)
            em.flush()
            return c

        if 1 in only:
            lax.fori_loop(1, 8, s1, 0)
        _Stage.cur = 0
        wait_all(w_set(7))
        wait_all(cp_late)
        for st in range(NCH):
            fold(wqaT, 0, st)
        prep_set(7)
        for t in range(16):
            z_finish(t, zacc[0, t * 128:(t + 1) * 128, :])
            kv_finish(t, kv_acc[0, t])

    def s2(i, c):
        _Stage.cur = 2
        hk, tk = _cfg("hk"), _cfg("tk")
        em = Emit()
        phase(em, a_q(em, tk), x_rhs(i), 0, tk)
        phase(em, out_proj(woaT, i), o_rhs, hk, tk)
        prep_late(i)
        phase(em, b_kv(i), x_rhs(i), hk, 1)
        return c

    def s3(i, c):
        _Stage.cur = 3
        hk, tk = _cfg("hk"), _cfg("tk")
        em = Emit()
        phase(em, b_q(i), x_rhs(i), 0, tk)
        em.later(2 * _cfg("split_at"), lambda: split(i))
        phase(em, out_proj(wobT, i), o_rhs, hk, tk)
        phase(em, a_kv(em, 1, True), x_rhs(i), hk, 0)
        em.flush()
        return c

    def s5(i, c):
        _Stage.cur = 5
        em = Emit()
        phase(em, b_q(i), x_rhs(i), 0, _cfg("tk"))
        flush_out(i, jnp.where(i > 0, i - 1, NBLK))
        phase(em, final_proj(i), o_rhs, _cfg("hk"), 1)
        x_out(8 + i).start()
        x_out(i, 0, 8 - ND).start()

        @pl.when(i > 0)
        def _():
            x_out(i - 1, 8 - ND, 8, SEM_KV + i - 1).start()
        return c

    def layer_pair(l, c):
        pl.when(l == 0)(stage1)
        if 2 in only:
            lax.fori_loop(0, 8, s2, 0)

        @pl.when(l == 0)
        def _():
            if 3 in only:
                lax.fori_loop(0, 8, s3, 0)

        @pl.when(l == 1)
        def _():
            if 5 in only:
                lax.fori_loop(0, 8, s5, 0)
            flush_out(8, 7)
            x_out(7, 8 - ND, 8, SEM_KV + 7).start()
        return c

    lax.fori_loop(0, 2, layer_pair, 0)

    for k in range(8):
        x_out(8 + k).wait()
        x_out(k, 0, 8 - ND).wait()
        x_out(k, 8 - ND, 8, SEM_KV + k).wait()


def _compiler_params():
    vmem = 120 * 1024 * 1024
    try:
        return pltpu.CompilerParams(vmem_limit_bytes=vmem, disable_semaphore_checks=True)
    except TypeError:
        return pltpu.CompilerParams(vmem_limit_bytes=vmem)


@jax.jit
def pallas_interleave_layers__linear_kernel_hedgehog__sliding_local_dilated__prompt_kernel(
    A_x: jax.Array,
    A_wqkv: jax.Array,
    A_w_phi: jax.Array,
    A_wo: jax.Array,
    B_x: jax.Array,
    B_wqkv: jax.Array,
    B_wo: jax.Array,
):
    del B_x
    x3 = A_x.reshape(S // 32, 32, D)
    wphi2 = A_w_phi.reshape(H * DH, DH)
    any_spec = pl.BlockSpec(memory_space=pl.ANY)
    scratch = [
        pltpu.VMEM((NBLK + 1, S // 32, D), U32),
        pltpu.VMEM((24, D, L), BF16),
        pltpu.VMEM((8, D, L), BF16),
        pltpu.VMEM((24, D, L), BF16),
        pltpu.VMEM((8, D, L), BF16),
        pltpu.VMEM((H * DH, DH), BF16),
        pltpu.VMEM((8, 128, 128), BF16),
        pltpu.VMEM((7, 4, D // 2, L), BF16),
        pltpu.VMEM((7, 4, D // 2, L), BF16),
        pltpu.VMEM((7, 4, D // 4, L), U32),
        pltpu.VMEM((7, 4, D // 4, L), U32),
        pltpu.VMEM((7, 4, D // 4 + 16, L), U32),
        pltpu.VMEM((7, 4, D // 4 + 16, L), U32),
        pltpu.VMEM((7, 4, D // 4, L), U32),
        pltpu.VMEM((7, 4, D // 4, L), U32),
        pltpu.VMEM((9, 7, D // 2, L), BF16),
        pltpu.VMEM((7, D // 2, L), BF16),
        pltpu.VMEM((WIN + NBLK, D, L), F32),
        pltpu.VMEM((WIN + NBLK, D, L), F32),
        pltpu.VMEM((2, 16, 64, 128), F32),
        pltpu.VMEM((16, 64, 128), BF16),
        pltpu.VMEM((2, 2 * D, L), F32),
        pltpu.VMEM((2 * D + 64, L), F32),
        pltpu.VMEM((9, ND * 128, L), BF16),
        pltpu.SemaphoreType.DMA((NSEM,)),
    ]
    scratch += [pltpu.VMEM((9, D, L), F32)] * 2
    scratch += [pltpu.VMEM((2 * MC, L), BF16)] * (2 * NCH)
    scratch += [pltpu.VMEM((MC, L), BF16)] * (2 * NCH)
    out = pl.pallas_call(
        _kernel,
        out_shape=jax.ShapeDtypeStruct((S // 32, 32, D), BF16),
        in_specs=[any_spec] * 6,
        out_specs=any_spec,
        scratch_shapes=scratch,
        compiler_params=_compiler_params(),
        name="hedgehog_dilated",
    )(x3, A_wqkv, wphi2, A_wo, B_wqkv, B_wo)
    return out.reshape(1, S, D)
```

```python
import math

import jax
import jax.numpy as jnp
from jax import lax
import jax.experimental.pallas as pl
import jax.experimental.pallas.tpu as pltpu

S = 2048
D = 1024
H = 32
DH = 32
NBLK = 16
L = 128
WIN = 8
LOG2E = math.log2(math.e)
F32 = jnp.float32
BF16 = jnp.bfloat16
U32 = jnp.uint32
NT = (((1,), (1,)), ((), ()))

MC = 256
NCH = D // MC
GPC = MC // 128
PPC = MC // 64
ND = 2

CFG = dict(only=None, lag_n=5, lag_m=5, hold=2, lnk_a=1, dep_a=1, lnk_b=1, dep_b=4, side2=True, zfin=0, kvhead=(1, 3, 5), split2=0, side=3, split_at=5, tkq=2, hko=3, keep=99, late6=False, att4=(3,), sub_k_3=128, hk=3, tk=2,
           sub_q=64, sub_k=64, sub_v=128, sub_qb=128, sub_o=128, sub_b=128)


class _Stage:
    cur = 0


def _cfg(key):
    return CFG.get("%s_%d" % (key, _Stage.cur), CFG[key])


SEM_X = 0
SEM_PHI = 16
SEM_KV = 18
SEM_SET = 26
SEM_LATE = 34
NSEM = 35


def _mm(a, b):
    return jnp.dot(a, b, preferred_element_type=F32)


def _mm_nt(a, b):
    return lax.dot_general(a, b, NT, preferred_element_type=F32)


def _tree(op, xs):
    xs = list(xs)
    while len(xs) > 1:
        nxt = [op(xs[i], xs[i + 1]) for i in range(0, len(xs) - 1, 2)]
        if len(xs) % 2:
            nxt.append(xs[-1])
        xs = nxt
    return xs[0]


def _running_sum(acc, xs):
    for x in xs:
        acc = x if acc is None else acc + x
    return acc


def _rows(a, n=8):
    return [a[i * n:(i + 1) * n, :] for i in range(a.shape[0] // n)]


def _unpk(a):
    return pltpu.bitcast(a, BF16)


def _fold2(op, xs):
    r = _tree(op, xs)
    r = op(r, pltpu.roll(r, 4, 0))
    return op(r, pltpu.roll(r, 2, 0))


def _phi_parts(p):
    ps = _rows(p)
    mx = _fold2(jnp.maximum, ps)
    mn = _fold2(jnp.minimum, ps)
    ep = [jnp.exp2(x - mx) for x in ps]
    en = [jnp.exp2(mn - x) for x in ps]
    return ep, en, _fold2(jnp.add, ep), _fold2(jnp.add, en)


def _recip(x):
    r = pl.reciprocal(x, approx=True)
    return r * (2.0 - x * r)


def _lhs_ops(a11, a12, a21, a22):
    return [a11 + a22, a21 + a22, a11, a22, a11 + a12, a21 - a11, a12 - a22]


def _mult(x, m):
    return x if isinstance(x, int) else pl.multiple_of(x, m)


def _kernel(x_hbm, wa_hbm, wphi_hbm, woa_hbm, wb_hbm, wob_hbm, out_hbm,
            xio, wa_raw, woa_raw, wb_raw, wob_raw, wphi, pmat,
            wqaT, wkaT, wvaT, woaT, wqbT, wkbT, wvbT, wobT, xr, orr, kb, vb, kv_acc, kvm, zacc, zb, ystage,
            sems, *rest):
    xT = rest[0:2]
    phis = [rest[2:2 + NCH], rest[2 + NCH:2 + 2 * NCH]]
    vs = [rest[2 + 2 * NCH:2 + 3 * NCH], rest[2 + 3 * NCH:2 + 4 * NCH]]

    def u32(ref):
        return ref.bitcast(U32)

    only = CFG["only"] or (0, 1, 2, 3, 5)

    x32, out32 = u32(x_hbm), u32(out_hbm)

    def x_in(j):
        return pltpu.make_async_copy(x32.at[:, j, :], xio.at[j], sems.at[SEM_X + j])

    def x_out(j, c0=0, c1=8, sem=None):
        cs = pl.ds(c0 * L, (c1 - c0) * L)
        return pltpu.make_async_copy(xio.at[j, :, cs], out32.at[:, j, cs],
                                     sems.at[SEM_X + j if sem is None else sem])

    def slabs(src, dst, g0, n, sem):
        return [pltpu.make_async_copy(src.at[:, pl.ds(_mult((g0 + u) * 128, 128), 128)], dst.at[g0 + u],
                                      sems.at[sem]) for u in range(n)]

    cp_phi = pltpu.make_async_copy(wphi_hbm.at[0:MC], wphi.at[0:MC], sems.at[SEM_PHI])
    cp_phi2 = pltpu.make_async_copy(wphi_hbm.at[MC:D], wphi.at[MC:D], sems.at[SEM_PHI + 1])
    cp_k = [slabs(wa_hbm, wa_raw, 8 + ch * GPC, GPC, SEM_KV + 2 * ch) for ch in range(NCH)]
    cp_v = [slabs(wa_hbm, wa_raw, 16 + ch * GPC, GPC, SEM_KV + 2 * ch + 1) for ch in range(NCH)]

    def w_set(g):
        rows = pl.ds(_mult((g & 1) * 512, 512), 512)
        cps = []
        for src, dst, g0 in ((woa_hbm, woa_raw, 0), (wb_hbm, wb_raw, 8), (wb_hbm, wb_raw, 16)):
            for u in range(2):
                sl = g0 + 2 * (g >> 1) + u
                cps.append(pltpu.make_async_copy(src.at[rows, pl.ds(_mult(sl * 128, 128), 128)],
                                                 dst.at[sl, rows, :], sems.at[SEM_SET + g]))
        return cps

    cp_late = (slabs(wa_hbm, wa_raw, 0, 8, SEM_LATE) + slabs(wb_hbm, wb_raw, 0, 8, SEM_LATE)
               + slabs(wob_hbm, wob_raw, 0, 8, SEM_LATE))

    batch = [[cp_phi, x_in(8), x_in(0)] + cp_k[0] + cp_v[0] + [cp_phi2] + cp_k[1] + cp_v[1],
             cp_k[2] + cp_v[2] + cp_k[3] + cp_v[3] + [x_in(9), x_in(1)], [], cp_late]
    for g in range(8):
        n = 1 if g < 4 else 2
        if g < 6:
            batch[n] += [x_in(10 + g), x_in(2 + g)]
        batch[n] += w_set(g)

    def start_all(cps):
        for c in cps:
            c.start()

    def wait_all(cps):
        for c in cps:
            c.wait()

    start_all(batch[0])

    class Side:
        never = None
        hist = []

    def side_begin(never):
        Side.never = never
        Side.hist = []

    def gate(x):
        w = _cfg("side")
        if Side.never is not None and len(Side.hist) >= w:
            x = jnp.concatenate([jnp.where(Side.never, Side.hist[-w], x[0:8, :]), x[8:, :]], axis=0)
        return x

    def tr(x):
        y = pltpu.bitcast(x.T, U32)
        Side.hist.append(y[56:64, :])
        return y

    def wprep(ref, raw, g0, st, c, perm=False):
        def tile(u, kt):
            return _unpk(gate(u32(raw)[g0 + 2 * st + u, pl.ds(_mult(kt * 64, 64), 64), :]))
        t = [tile(0, 2 * c), tile(0, 2 * c + 1), tile(1, 2 * c), tile(1, 2 * c + 1)]
        ops = _lhs_ops(*[x.astype(F32) for x in t])
        for q in range(7):
            pk = tr(t[0] if q == 2 else t[3] if q == 3 else ops[q].astype(BF16))
            if perm:
                for h4 in range(4):
                    ref[q, c, pl.ds(st * 64 + h4, 16, stride=4), :] = pk[h4 * 16:(h4 + 1) * 16, :]
            else:
                ref[q, c, pl.ds(_mult(st * 64, 64), 64), :] = pk

    def make_pmat(gs):
        r128 = lax.broadcasted_iota(jnp.int32, (128, 128), 0)
        c128 = lax.broadcasted_iota(jnp.int32, (128, 128), 1)
        same_head = (2 * (r128 >> 6) + (r128 & 1)) == (c128 >> 5)
        er = lax.broadcasted_iota(jnp.int32, (128, 32), 0)
        ec = lax.broadcasted_iota(jnp.int32, (128, 32), 1)
        expand = jnp.where(((er & 63) >> 1) == ec, 1.0, 0.0).astype(BF16)
        for g in gs:
            pg = _mm_nt(expand, wphi[g * 128:(g + 1) * 128, :])
            pmat[g] = jnp.where(same_head, pg, 0.0).astype(BF16)

    def fold(dst, g0, st):
        for c in range(4):
            f = [_mm_nt(_unpk(u32(pmat)[2 * st + u]),
                        _unpk(u32(wa_raw)[g0 + 2 * st + u, kt * 64:(kt + 1) * 64, :])) * LOG2E
                 for u in range(2) for kt in (2 * c, 2 * c + 1)]
            for q, v in enumerate(_lhs_ops(*f)):
                dst[q, c, st * 128:(st + 1) * 128, :] = v.astype(BF16)

    def prep_set(g):
        for u in range(2):
            c = 2 * (g & 1) + u
            wprep(woaT, woa_raw, 0, g >> 1, c)
            wprep(wkbT, wb_raw, 8, g >> 1, c, True)
            wprep(wvbT, wb_raw, 16, g >> 1, c)

    def prep_late(g):
        for u in range(2):
            c = 2 * (g & 1) + u
            wprep(wqbT, wb_raw, 0, g >> 1, c, True)
            wprep(wobT, wob_raw, 0, g >> 1, c)

    def put_a(dst, r0, alo, ahi):
        n = alo.shape[0]
        ops = {1: alo, 3: ahi - alo}
        for q, v in ops.items():
            dst[q, r0:r0 + n, :] = v.astype(BF16)
        return [ops[3]]

    def put_b(dst, r0, alo, ahi, blo, bhi):
        n = alo.shape[0]
        ops = {4: bhi, 2: blo - bhi, 0: alo + bhi, 6: ahi + bhi, 5: alo + blo}
        for q, v in ops.items():
            dst[q, r0:r0 + n, :] = v.astype(BF16)
        return [ops[q] for q in (2, 0, 6, 5)]

    class LN:
        def __init__(self, k):
            self.k = k
            self.piv, self.s1, self.s2, self.sc = [None] * 2, [None] * 2, [None] * 2, [None] * 2

        def add(self, hf, xt):
            if self.piv[hf] is None:
                self.piv[hf] = jnp.broadcast_to(xt[0:1, :], (8, L))
            d = [r - self.piv[hf] for r in _rows(xt)]
            self.s1[hf] = _running_sum(self.s1[hf], d)
            self.s2[hf] = _running_sum(self.s2[hf], [x * x for x in d])

        def stats(self, hf):
            m1 = jnp.sum(self.s1[hf], axis=0, keepdims=True) * (1.0 / D)
            m2 = jnp.sum(self.s2[hf], axis=0, keepdims=True) * (1.0 / D)
            rs = lax.rsqrt(jnp.maximum(m2 - m1 * m1, 0.0) + 1e-5)
            self.sc[hf] = (jnp.broadcast_to(rs, (8, L)), jnp.broadcast_to((self.piv[hf][0:1, :] + m1) * rs, (8, L)))

        def finish(self, do_a, do_b):
            for hf in range(2):
                if (do_a, do_b)[hf]:
                    self.stats(hf)
            dst = xr.at[self.k]
            nh = 2 if do_b else 1
            rs = [self.sc[hf][0] for hf in range(nh)]
            never = rs[-1] < 0.0
            if do_b and not do_a:
                rs[0] = jnp.where(never, rs[1], rs[0])
            link, depth = (_cfg("lnk_b"), _cfg("dep_b")) if do_b else (_cfg("lnk_a"), _cfg("dep_a"))
            for r in range(D // 32):
                r0 = (r // 8) * 256 + (r % 8) * 16
                y = [[jnp.concatenate([xT[hf][self.k, r0 + o + e:r0 + o + e + 8, :] * rs[hf] - self.sc[hf][1]
                                       for e in (0, 8)], axis=0) for o in (0, 128)] for hf in range(nh)]
                outs = []
                if do_a:
                    outs += put_a(dst, r * 16, *y[0])
                if do_b:
                    outs += put_b(dst, r * 16, *y[0], *y[1])
                if r % link == link - 1:
                    parts = [x for v in outs for x in _rows(v)][::-1]
                    lk = _running_sum(None, parts[:depth])
                    rs = [jnp.where(never, lk, x) for x in rs]

    def prep_x(src, k):
        ln = LN(k)
        for hf in range(2):
            for cc in range(8):
                xt = _unpk(tr(_unpk(gate(xio[8 * (1 - hf) + src, :, cc * L:(cc + 1) * L])))).astype(F32)
                xT[hf][k, cc * 128:(cc + 1) * 128, :] = xt
                ln.add(hf, xt)
        ln.finish(True, True)

    class Emit:
        def __init__(self):
            self.n = 0
            self.pend = []

        def later(self, lag, f):
            self.pend.append((self.n + lag, f))

        def tick(self, w=1):
            self.n += w
            due = [e for e in self.pend if e[0] <= self.n]
            self.pend = [e for e in self.pend if e[0] > self.n]
            for _, f in due:
                f()

        def flush(self):
            self.tick(1 << 20)

    def plan(em, steps, rhs, hk, tk, late6=False):
        units = [(n, u) for n, stp in enumerate(steps) for u in range(128 // stp[2])]
        hs = range(hk) if isinstance(hk, int) else hk
        head = [(n, u, q) for n, u in units if n in hs for q in (3, 1)]
        mid = []
        for n, u in units:
            qs = (3, 1, 4, 2, 0, 6, 5) if n < len(steps) - tk else (3, 1, 4, 0, 6)
            mid += [(n, u, q) for q in qs if n not in hs or q not in (3, 1)]
        tail = [(n, u, q) for n, u in units if n >= len(steps) - tk for q in (2, 5)]
        if late6:
            tail.sort(key=lambda e: -e[2])
        uses = {0: [((0, 0), 1), ((1, 1), 1)], 1: [((0, 1), 1), ((1, 1), -1)], 2: [((1, 0), 1), ((1, 1), 1)],
                3: [((0, 0), 1), ((0, 1), 1)], 4: [((0, 0), -1), ((1, 0), 1)], 5: [((1, 1), 1)], 6: [((0, 0), 1)]}
        need = {(0, 0): 4, (0, 1): 2, (1, 0): 2, (1, 1): 4}
        acc = {}

        def product(n, u, q):
            ref, st, sub, consumer = steps[n]
            r = (st * 128 + u * sub) // 2
            lhs = jnp.concatenate([_unpk(ref[q, c, r:r + sub // 2, :]) for c in range(4)], axis=1)
            m = _mm(lhs, _unpk(rhs(q)))
            for quad, sign in uses[q]:
                val, sg, cnt = acc.get((n, u, quad), (None, 1, 0))
                if val is None:
                    val, sg = m, sign
                elif sg == sign:
                    val = val + m
                else:
                    val, sg = (val - m, 1) if sg == 1 else (m - val, 1)
                acc[(n, u, quad)] = (val, sg, cnt + 1)
                if cnt + 1 == need[quad]:
                    consumer(quad[0], quad[1], u, val)
            em.tick(sub // 64)

        return [[(lambda e=e: product(*e)) for e in part] for part in (head, mid, tail)]

    def run(fs):
        for f in fs:
            f()

    def phase(em, steps, rhs, hk, tk):
        run(sum(plan(em, steps, rhs, hk, tk), []))

    def weave(tail, head, keep):
        out = tail[:keep]
        tail, head = tail[keep:], list(head)
        for f in tail:
            out += [head.pop(0), f] if head else [f]
        return out + head

    def x_rhs(k):
        return lambda q: u32(xr)[k, q]

    def o_rhs(q):
        return u32(orr)[q]

    def split(i):
        @pl.when((i >> 6) > 0)
        def _():
            zb[2 * D:2 * D + 8, :] = jnp.zeros((8, L), F32)

    def z_finish(t, z):
        zb[t * 128:(t + 1) * 128, :] = jnp.broadcast_to(jnp.sum(z, axis=1, keepdims=True), (128, L))

    def kv_finish(t, acc):
        r = lax.broadcasted_iota(jnp.int32, (64, 128), 0)
        c = lax.broadcasted_iota(jnp.int32, (64, 128), 1)
        kvm[t] = jnp.where((r >> 5) == (c & 1), acc, 0.0).astype(BF16)

    def pairs_of(bot, u, sub, val):
        return [(2 * bot + (u * sub) // 64 + w, val[w * 64:(w + 1) * 64, :]) for w in range(sub // 64)]

    def a_kv(em, lay, last):
        steps = []
        for ch in range(NCH):
            seen = {}

            def kcons(hf, bot, u, val, ch=ch, seen=seen):
                for pp, kp in pairs_of(bot, u, _cfg("sub_k"), val):
                    t = ch * PPC + pp
                    ep, en, sp, sn = _phi_parts(kp)
                    r = _recip(sp * sn)
                    rp = r * sn
                    rn = r * sp
                    phi = jnp.concatenate([e * rp for e in ep] + [e * rn for e in en], axis=0)
                    phis[hf][ch][pp * 128:(pp + 1) * 128, :] = phi.astype(BF16)
                    z = zacc[lay, t * 128:(t + 1) * 128, :] + phi
                    zacc[lay, t * 128:(t + 1) * 128, :] = z
                    seen[pp] = seen.get(pp, 0) + 1
                    if last and seen[pp] == 2 and CFG["zfin"] == 0:
                        z_finish(t, z)

            def mstep(ch=ch):
                for pp in range(PPC):
                    t = ch * PPC + pp
                    acc = kv_acc[lay, t]
                    for hf in range(2):
                        acc = acc + _mm_nt(_unpk(u32(vs[hf][ch])[pp * 32:(pp + 1) * 32, :]),
                                           _unpk(u32(phis[hf][ch])[pp * 64:(pp + 1) * 64, :]))
                    kv_acc[lay, t] = acc
                    if last:
                        kv_finish(t, acc)

            def vcons(hf, bot, u, val, ch=ch, seen=seen, mstep=mstep):
                sub = _cfg("sub_v")
                vs[hf][ch][bot * 128 + u * sub:bot * 128 + (u + 1) * sub, :] = val.astype(BF16)
                seen["v"] = seen.get("v", 0) + 1
                if seen["v"] == 4 * (128 // sub):
                    em.later(_cfg("lag_m") if ch < NCH - _cfg("hold") else 1 << 10, mstep)

            steps += [(u32(wkaT), ch, _cfg("sub_k"), kcons), (wvaT, ch, _cfg("sub_v"), vcons)]
        return steps

    def a_q(em, tk):
        steps = []
        for ch in range(NCH):
            seen = {0: 0, 1: 0}
            o = {}

            def num(hf, pp, ch=ch):
                return _mm(_unpk(u32(kvm)[ch * PPC + pp]), _unpk(u32(phis[hf][ch])[pp * 64:(pp + 1) * 64, :]))

            def nstep(hfs, ch=ch, o=o, num=num):
                for w in range(2):
                    for hf in hfs:
                        o[hf, w] = (num(hf, w), num(hf, 2 + w))
                    if 0 in hfs:
                        put_a(orr, ch * 128 + w * 64, *o[0, w])
                    if 1 in hfs:
                        put_b(orr, ch * 128 + w * 64, *o[0, w], *o[1, w])

            def qcons(hf, bot, u, val, ch=ch, seen=seen, nstep=nstep):
                for pp, qp in pairs_of(bot, u, _cfg("sub_q"), val):
                    t = ch * PPC + pp
                    ep, en, sp, sn = _phi_parts(qp)
                    zr = _rows(zb[t * 128:(t + 1) * 128, :])
                    dp = _fold2(jnp.add, [e * zz for e, zz in zip(ep, zr[:8])])
                    dn = _fold2(jnp.add, [e * zz for e, zz in zip(en, zr[8:])])
                    r = _recip(dp * sn + dn * sp + 1e-6 * (sp * sn))
                    rp = r * sn
                    rn = r * sp
                    phi = jnp.concatenate([e * rp for e in ep] + [e * rn for e in en], axis=0)
                    phis[hf][ch][pp * 128:(pp + 1) * 128, :] = phi.astype(BF16)
                    seen[hf] += 1
                    if seen[hf] == PPC:
                        if ch >= NCH - tk:
                            em.later(_cfg("lag_n"), lambda hf=hf: nstep((hf,)))
                        elif seen[1 - hf] == PPC:
                            em.later(_cfg("lag_n"), lambda: nstep((0, 1)))

            steps.append((u32(wqaT), ch, _cfg("sub_q"), qcons))
        return steps

    def out_proj(wo, k):
        ln = LN(k)
        seen = {0: 0, 1: 0}
        sub = _cfg("sub_o")
        steps = []
        for ch in range(NCH):
            def cons(hf, bot, u, val, ch=ch):
                r0 = ch * MC + bot * 128 + u * sub
                xt = xT[hf][k, r0:r0 + sub, :] + val
                xT[hf][k, r0:r0 + sub, :] = xt
                ln.add(hf, xt)
                seen[hf] += 1
                if seen[hf] == D // sub:
                    ln.finish(hf == 0, hf == 1)
            steps.append((wo, ch, sub, cons))
        return steps

    def b_kv(k):
        sub = _cfg("sub_b")
        steps = []
        for w, ref in ((wkbT, kb), (wvbT, vb)):
            for ch in range(NCH):
                def cons(hf, bot, u, val, ch=ch, ref=ref):
                    r0 = ch * MC + bot * 128 + u * sub
                    ref[WIN + 8 * (1 - hf) + k, r0:r0 + sub, :] = val
                    if hf == 0:
                        ref[k, r0:r0 + sub, :] = pltpu.roll(val, 2, 1)
                steps.append((w, ch, sub, cons))
        return steps

    def b_q(k):
        even = (lax.broadcasted_iota(jnp.int32, (8, L), 0) & 1) == 0
        first = lax.broadcasted_iota(jnp.int32, (8, L), 1) < 2
        cs = DH ** -0.5
        sub = _cfg("sub_qb")

        def softmax(lg, hf):
            if hf == 1:
                lg = [l if w == 0 else jnp.where(jnp.logical_and(first, k < w), -1e9 / cs, l)
                      for w, l in enumerate(lg)]
            mx = _tree(jnp.maximum, lg)
            ex = [jnp.exp2((l - mx) * (cs * LOG2E)) for l in lg]
            rs = _recip(_tree(jnp.add, ex))
            return [e * rs for e in ex]

        def pv(at, s, h, j):
            return _running_sum(None, [
                jnp.broadcast_to(at[w][s:s + 1, :], (DH, L)) * vb[WIN + j - w, h * DH:(h + 1) * DH, :]
                for w in range(WIN)])

        steps = []
        for G in range(4):
            lacc = {}
            seen = {}
            o = {}

            def cons(hf, bot, u, q, G=G, lacc=lacc, seen=seen, o=o):
                j = 8 * (1 - hf) + k
                acc = lacc.setdefault((hf, bot), [None] * WIN)
                for r in range(sub // 8):
                    r0 = G * 256 + bot * 128 + u * sub + r * 8
                    for w in range(WIN):
                        t = q[r * 8:r * 8 + 8, :] * kb[WIN + j - w, r0:r0 + 8, :]
                        acc[w] = t if acc[w] is None else acc[w] + t
                seen[hf, bot] = seen.get((hf, bot), 0) + 1
                if seen[hf, bot] < 128 // sub:
                    return
                both = seen.get((hf, 1 - bot), 0) == 128 // sub
                if G in _cfg("att4"):
                    at = softmax([x + pltpu.roll(x, 7, 0) for x in acc], hf)
                    for h4 in range(4):
                        o[hf, bot, h4] = pv(at, 2 * h4, G * 8 + 4 * bot + h4, j)
                elif both:
                    at = softmax([jnp.where(even, x + pltpu.roll(x, 7, 0), y + pltpu.roll(y, 1, 0))
                                  for x, y in zip(lacc[hf, 0], lacc[hf, 1])], hf)
                    for h4 in range(4):
                        for bb in range(2):
                            o[hf, bb, h4] = pv(at, 2 * h4 + bb, G * 8 + 4 * bb + h4, j)
                if both:
                    for h4 in range(4):
                        if hf == 0:
                            put_a(orr, G * 128 + h4 * DH, o[0, 0, h4], o[0, 1, h4])
                        else:
                            put_b(orr, G * 128 + h4 * DH, o[0, 0, h4], o[0, 1, h4], o[1, 0, h4], o[1, 1, h4])

            steps.append((wqbT, G, sub, cons))
        return steps

    def final_proj(k):
        steps = []
        for ch in range(NCH):
            def cons(hf, bot, u, val, ch=ch):
                cc = ch * GPC + bot
                y = (xT[hf][k, cc * 128:(cc + 1) * 128, :] + val).astype(BF16)
                if hf == 1 and cc >= 8 - ND:
                    ystage[k + 1, (cc - 8 + ND) * 128:(cc - 7 + ND) * 128, :] = y
                else:
                    xio[8 * (1 - hf) + k, :, cc * L:(cc + 1) * L] = tr(y)
            steps.append((wobT, ch, 128, cons))
        return steps

    def flush_out(k, slot):
        for u in range(ND):
            xio[slot, :, (8 - ND + u) * L:(9 - ND + u) * L] = tr(_unpk(u32(ystage)[k, u * 64:(u + 1) * 64, :]))

    def stage1():
        _Stage.cur = 0
        kv_acc[...] = jnp.zeros(kv_acc.shape, F32)
        zacc[...] = jnp.zeros(zacc.shape, F32)
        ystage[0] = jnp.zeros(ystage.shape[1:], BF16)
        cp_phi.wait()
        x_in(8).wait()
        x_in(0).wait()
        make_pmat(range(GPC))
        prep_x(0, 0)
        start_all(batch[1])

        em = Emit()
        steps = a_kv(em, 0, False)
        for ch in range(NCH if 0 in only else 0):
            wait_all(cp_k[ch])
            if ch == 0:
                fold(wkaT, 8, 0)
                phase(em, steps[0:1], x_rhs(0), 0, 0)
            wait_all(cp_v[ch])
            if ch == 0:
                cp_phi2.wait()
                make_pmat(range(GPC, 8))
            else:
                if ch == NCH - 1:
                    x_in(9).wait()
                    x_in(1).wait()
                fold(wkaT, 8, ch)
            for c in range(4):
                wprep(wvaT, wa_raw, 16, ch, c)
            em.flush()
            if ch == NCH - 1:
                side_begin(zacc[0, 0:8, :] < 0.0)
                prep_x(1, 1)
                side_begin(None)
            phase(em, steps[max(2 * ch, 1):2 * ch + 2], x_rhs(0), 0, 0)
        em.flush()

        def s1(i, c):
            _Stage.cur = 1

            @pl.when(i < 7)
            def _():
                x_in(9 + i).wait()
                x_in(1 + i).wait()

            for n in (2, 3):
                pl.when(i == n - 1)(lambda n=n: start_all(batch[n]))

            wait_all(w_set(i - 1))
            side_begin(jnp.full((8, L), i >> 6, jnp.int32) > 0)
            prep_x(jnp.minimum(i + 1, 7), i + 1)
            prep_set(i - 1)
            side_begin(None)
            em = Emit()
            phase(em, a_kv(em, 0, False), x_rhs(i), 0, 0)
            em.flush()
            return c

        if 1 in only:
            lax.fori_loop(1, 8, s1, 0)
        _Stage.cur = 0
        wait_all(w_set(7))
        wait_all(cp_late)
        for st in range(NCH):
            fold(wqaT, 0, st)
        prep_set(7)
        for t in range(16):
            z_finish(t, zacc[0, t * 128:(t + 1) * 128, :])
            kv_finish(t, kv_acc[0, t])

    def s2(i, c):
        _Stage.cur = 2
        hk, tk = _cfg("hk"), _cfg("tk")
        em = Emit()
        phase(em, a_q(em, tk), x_rhs(i), 0, tk)
        phase(em, out_proj(woaT, i), o_rhs, hk, tk)
        if CFG["side2"]:
            side_begin(jnp.full((8, L), i >> 6, jnp.int32) > 0)
        prep_late(i)
        side_begin(None)
        phase(em, b_kv(i), x_rhs(i), hk, 1)
        return c

    def s3(i, c):
        _Stage.cur = 3
        hk, tk = _cfg("hk"), _cfg("tk")
        em = Emit()
        pq = plan(em, b_q(i), x_rhs(i), 0, _cfg("tkq"), _cfg("late6"))
        po = plan(em, out_proj(wobT, i), o_rhs, _cfg("hko"), tk)
        run(pq[1] + weave(pq[2], po[0], _cfg("keep")))
        em.later(2 * _cfg("split_at"), lambda: split(i))
        run(po[1] + po[2])
        if CFG["split2"]:
            em.later(2 * CFG["split2"], lambda: split(i))
        phase(em, a_kv(em, 1, True), x_rhs(i), CFG["kvhead"], 0)
        em.flush()
        if CFG["zfin"] in (1, 2):
            la = 1 if CFG["zfin"] == 1 else 1 + (i >> 6)
            for t in range(16):
                z_finish(t, zacc[la, t * 128:(t + 1) * 128, :])
        return c

    def s5(i, c):
        _Stage.cur = 5
        em = Emit()
        pq = plan(em, b_q(i), x_rhs(i), 0, _cfg("tkq"), _cfg("late6"))
        po = plan(em, final_proj(i), o_rhs, _cfg("hko"), 1)
        flush_out(i, jnp.where(i > 0, i - 1, NBLK))
        run(pq[1] + weave(pq[2], po[0], _cfg("keep")) + po[1] + po[2])
        x_out(8 + i).start()
        x_out(i, 0, 8 - ND).start()

        @pl.when(i > 0)
        def _():
            x_out(i - 1, 8 - ND, 8, SEM_KV + i - 1).start()
        return c

    def layer_pair(l, c):
        pl.when(l == 0)(stage1)
        if 2 in only:
            lax.fori_loop(0, 8, s2, 0)

        @pl.when(l == 0)
        def _():
            if 3 in only:
                lax.fori_loop(0, 8, s3, 0)
                if CFG["zfin"] == 3:
                    for t in range(16):
                        z_finish(t, zacc[1, t * 128:(t + 1) * 128, :])

        @pl.when(l == 1)
        def _():
            if 5 in only:
                lax.fori_loop(0, 8, s5, 0)
            flush_out(8, 7)
            x_out(7, 8 - ND, 8, SEM_KV + 7).start()
        return c

    lax.fori_loop(0, 2, layer_pair, 0)

    for k in range(8):
        x_out(8 + k).wait()
        x_out(k, 0, 8 - ND).wait()
        x_out(k, 8 - ND, 8, SEM_KV + k).wait()


def _compiler_params():
    vmem = 120 * 1024 * 1024
    try:
        return pltpu.CompilerParams(vmem_limit_bytes=vmem, disable_semaphore_checks=True)
    except TypeError:
        return pltpu.CompilerParams(vmem_limit_bytes=vmem)


@jax.jit
def pallas_interleave_layers__linear_kernel_hedgehog__sliding_local_dilated__prompt_kernel(
    A_x: jax.Array,
    A_wqkv: jax.Array,
    A_w_phi: jax.Array,
    A_wo: jax.Array,
    B_x: jax.Array,
    B_wqkv: jax.Array,
    B_wo: jax.Array,
):
    del B_x
    x3 = A_x.reshape(S // 32, 32, D)
    wphi2 = A_w_phi.reshape(H * DH, DH)
    any_spec = pl.BlockSpec(memory_space=pl.ANY)
    scratch = [
        pltpu.VMEM((NBLK + 1, S // 32, D), U32),
        pltpu.VMEM((24, D, L), BF16),
        pltpu.VMEM((8, D, L), BF16),
        pltpu.VMEM((24, D, L), BF16),
        pltpu.VMEM((8, D, L), BF16),
        pltpu.VMEM((H * DH, DH), BF16),
        pltpu.VMEM((8, 128, 128), BF16),
        pltpu.VMEM((7, 4, D // 2, L), BF16),
        pltpu.VMEM((7, 4, D // 2, L), BF16),
        pltpu.VMEM((7, 4, D // 4, L), U32),
        pltpu.VMEM((7, 4, D // 4, L), U32),
        pltpu.VMEM((7, 4, D // 4 + 16, L), U32),
        pltpu.VMEM((7, 4, D // 4 + 16, L), U32),
        pltpu.VMEM((7, 4, D // 4, L), U32),
        pltpu.VMEM((7, 4, D // 4, L), U32),
        pltpu.VMEM((9, 7, D // 2, L), BF16),
        pltpu.VMEM((7, D // 2, L), BF16),
        pltpu.VMEM((WIN + NBLK, D, L), F32),
        pltpu.VMEM((WIN + NBLK, D, L), F32),
        pltpu.VMEM((2, 16, 64, 128), F32),
        pltpu.VMEM((16, 64, 128), BF16),
        pltpu.VMEM((2, 2 * D, L), F32),
        pltpu.VMEM((2 * D + 64, L), F32),
        pltpu.VMEM((9, ND * 128, L), BF16),
        pltpu.SemaphoreType.DMA((NSEM,)),
    ]
    scratch += [pltpu.VMEM((9, D, L), F32)] * 2
    scratch += [pltpu.VMEM((2 * MC, L), BF16)] * (2 * NCH)
    scratch += [pltpu.VMEM((MC, L), BF16)] * (2 * NCH)
    out = pl.pallas_call(
        _kernel,
        out_shape=jax.ShapeDtypeStruct((S // 32, 32, D), BF16),
        in_specs=[any_spec] * 6,
        out_specs=any_spec,
        scratch_shapes=scratch,
        compiler_params=_compiler_params(),
        name="hedgehog_dilated",
    )(x3, A_wqkv, wphi2, A_wo, B_wqkv, B_wo)
    return out.reshape(1, S, D)
```
